```python
import jax
import jax.numpy as jnp

def _softmax(x, axis=-1):
    return jax.nn.softmax(x, axis=axis)

def _gelu(x):
    return jax.nn.gelu(x, approximate=True)

def _silu(x):
    return jax.nn.silu(x)

def _sigmoid(x):
    return jax.nn.sigmoid(x)

def _layernorm(x, axis=-1, eps=1e-05):
    m = jnp.mean(x, axis=axis, keepdims=True)
    v = jnp.var(x, axis=axis, keepdims=True)
    return (x - m) / jnp.sqrt(v + eps)

def _scatter_add(tgt, idx, src, axis=0):
    return tgt.at[idx].add(src)

def _segment_sum(src, seg, n):
    return jax.ops.segment_sum(src, seg, n)

class _Rng:

    def __init__(self, key):
        self._k = key

    def _next(self):
        self._k, sub = jax.random.split(self._k)
        return sub

    def normal(self, shape):
        return jax.random.normal(self._next(), shape, dtype=jnp.bfloat16)

    def randint(self, lo, hi, shape):
        return jax.random.randint(self._next(), shape, lo, hi, dtype=jnp.int32)

    def uniform(self, shape, lo=0.0, hi=1.0):
        return jax.random.uniform(self._next(), shape, jnp.bfloat16, lo, hi)

    def permutation(self, n):
        return jax.random.permutation(self._next(), n)
kernel_name = 'standalone__conformer_family_conformer__speech'

def setup_inputs():
    _rng = _Rng(jax.random.key(int.from_bytes(__import__("os").urandom(4), "little")))
    _w = lambda a: (lambda t: t.astype(jnp.bfloat16) if jnp.issubdtype(t.dtype, jnp.floating) else t)(jnp.asarray(a))
    B, T, D, K = (2, 4000, 512, 15)
    F = 4 * D
    s = D ** (-0.5)
    sf = F ** (-0.5)
    return {'x': _w((lambda *s: _rng.normal(s) * 0.05)(B, T, D)), 'w_ff1_a': _w((lambda *s: _rng.normal(s) * 0.05)(D, F) * s), 'w_ff1_b': _w((lambda *s: _rng.normal(s) * 0.05)(F, D) * sf), 'w_q': _w((lambda *s: _rng.normal(s) * 0.05)(D, D) * s), 'w_k': _w((lambda *s: _rng.normal(s) * 0.05)(D, D) * s), 'w_v': _w((lambda *s: _rng.normal(s) * 0.05)(D, D) * s), 'w_o': _w((lambda *s: _rng.normal(s) * 0.05)(D, D) * s), 'w_pw1': _w((lambda *s: _rng.normal(s) * 0.05)(D, 2 * D) * s), 'dw': _w((lambda *s: _rng.normal(s) * 0.05)(K, D) * K ** (-0.5)), 'w_pw2': _w((lambda *s: _rng.normal(s) * 0.05)(D, D) * s), 'w_ff2_a': _w((lambda *s: _rng.normal(s) * 0.05)(D, F) * s), 'w_ff2_b': _w((lambda *s: _rng.normal(s) * 0.05)(F, D) * sf)}

def reference(x, w_ff1_a, w_ff1_b, w_q, w_k, w_v, w_o, w_pw1, dw, w_pw2, w_ff2_a, w_ff2_b):
    B, T, D = x.shape
    K = dw.shape[0]
    scale = D ** (-0.5)
    h = _layernorm(x, axis=-1)
    h = _silu(h @ w_ff1_a) @ w_ff1_b
    x1 = x + 0.5 * h
    h = _layernorm(x1, axis=-1)
    q = h @ w_q
    k = h @ w_k
    v = h @ w_v
    scores = jnp.einsum('btd,bsd->bts', q, k) * scale
    p = _softmax(scores, axis=-1)
    attn = jnp.einsum('bts,bsd->btd', p, v) @ w_o
    x2 = x1 + attn
    h = _layernorm(x2, axis=-1)
    h = h @ w_pw1
    a = h[..., :D].copy()
    b = h[..., D:].copy()
    h = a * _sigmoid(b)
    pad = K // 2
    hp = jnp.pad(h, ((0, 0), (pad, K - 1 - pad), (0, 0)))
    dc = jnp.zeros_like(h)
    for i in range(K):
        dc = dc + hp[:, i:i + T, :] * dw[i][None, None, :]
    flat = dc.reshape(-1, D)
    mu = flat.mean(0)
    var = ((flat - mu) ** 2).mean(0)
    dc = (dc - mu[None, None, :]) / jnp.sqrt(var[None, None, :] + 1e-05)
    h = _silu(dc) @ w_pw2
    x3 = x2 + h
    h = _layernorm(x3, axis=-1)
    h = _silu(h @ w_ff2_a) @ w_ff2_b
    x4 = x3 + 0.5 * h
    return _layernorm(x4, axis=-1)
```

```python
import functools
import math

import jax
import jax.numpy as jnp
from jax import lax
import jax.experimental.pallas as pl
import jax.experimental.pallas.tpu as pltpu

F32 = jnp.float32
BF16 = jnp.bfloat16

TMA = 400
TMB = 400
TMC = 400
FC = 512
HALO = 8
EPS = 1e-05


def _ln(x):
    m = jnp.mean(x, axis=-1, keepdims=True)
    xc = x - m
    v = jnp.mean(xc * xc, axis=-1, keepdims=True)
    return xc * lax.rsqrt(v + EPS)


def _silu(a):
    y = 0.5 * a
    return y + y * jnp.tanh(y)


def _dot(a, b):
    return jnp.dot(a, b, preferred_element_type=F32)


def _dot_nt(a, b):
    return lax.dot_general(a, b, (((1,), (1,)), ((), ())),
                           preferred_element_type=F32)


def _ffn(h, wa_ref, wb_ref):
    f = wa_ref.shape[1]
    acc = None
    for c in range(f // FC):
        a = _dot(h, wa_ref[:, c * FC:(c + 1) * FC])
        s = _silu(a).astype(BF16)
        p = _dot(s, wb_ref[c * FC:(c + 1) * FC, :])
        acc = p if acc is None else acc + p
    return acc


def _kernel(x_hbm, w1a_hbm, w1b_hbm, wq_hbm, wk_hbm, wv_hbm, wo_hbm,
            wp1_hbm, dw_hbm, wp2_hbm, w2a_hbm, w2b_hbm,
            out_hbm,
            xin, w1a, w1b, wq, wk, wv, wo, wp1, dw, wp2, w2a, w2b,
            mq, wvo, xs, hs, gs, dcs, st_mean, st_m2, bn, obuf,
            xsem, wsem, osem,
            *, B, T, D, K):
    N = B * T
    TP = hs.shape[1]
    NCB = D // 128
    nta, ntb, ntc = N // TMA, N // TMB, N // TMC
    tpb_a = T // TMA
    tpb_b = T // TMB

    def x_copy(i):
        r = pl.multiple_of(i * TMA, 16)
        return pltpu.make_async_copy(x_hbm.at[pl.ds(r, TMA), :],
                                     xin.at[pl.ds(r, TMA), :], xsem.at[i])

    def o_copy(i):
        r = pl.multiple_of(i * TMC, 16)
        return pltpu.make_async_copy(obuf.at[pl.ds(r, TMC), :],
                                     out_hbm.at[pl.ds(r, TMC), :], osem.at[i])

    w_pairs = [(w1a_hbm, w1a), (w1b_hbm, w1b), (wq_hbm, wq), (wk_hbm, wk),
               (wv_hbm, wv), (wo_hbm, wo), (wp1_hbm, wp1), (dw_hbm, dw),
               (wp2_hbm, wp2), (w2a_hbm, w2a), (w2b_hbm, w2b)]
    w_copies = [pltpu.make_async_copy(s, d, wsem.at[j])
                for j, (s, d) in enumerate(w_pairs)]

    x_copy(0).start()
    w_copies[0].start()
    w_copies[1].start()

    for b in range(B):
        hs[b, T:TP, :] = jnp.zeros((TP - T, D), BF16)
        for c in range(NCB):
            gs[b, c, 0:HALO, :] = jnp.zeros((HALO, 128), F32)
            gs[b, c, HALO + T:HALO + T + HALO, :] = jnp.zeros((HALO, 128), F32)

    w_copies[0].wait()
    w_copies[1].wait()
    for cp in w_copies[2:]:
        cp.start()

    def phase_a(i, carry):
        @pl.when(i + 1 < nta)
        def _():
            x_copy(i + 1).start()
        x_copy(i).wait()
        r = pl.multiple_of(i * TMA, 16)
        x = xin[pl.ds(r, TMA), :].astype(F32)
        x1 = x + 0.5 * _ffn(_ln(x).astype(BF16), w1a, w1b)
        xs[pl.ds(r, TMA), :] = x1
        b = i // tpb_a
        rb = pl.multiple_of((i % tpb_a) * TMA, 16)
        hs[b, pl.ds(rb, TMA), :] = _ln(x1).astype(BF16)
        return carry

    lax.fori_loop(0, nta, phase_a, 0)

    for cp in w_copies[2:]:
        cp.wait()

    qk_scale = (D ** -0.5) * math.log2(math.e)
    mq[...] = (_dot_nt(wq[...], wk[...]) * qk_scale).astype(BF16)
    wvo[...] = _dot(wv[...], wo[...]).astype(BF16)

    def conv_tile(p):
        pb = p // tpb_b
        prb = pl.multiple_of((p % tpb_b) * TMB, 8)
        pr = pl.multiple_of(p * TMB, 8)
        dwf = dw[...].astype(F32)
        for c in range(NCB):
            acc = None
            for k in range(K):
                off = HALO - K // 2 + k
                t = gs[pb, c, pl.ds(prb + off, TMB), :] * dwf[k:k + 1, c * 128:(c + 1) * 128]
                acc = t if acc is None else acc + t
            dcs[pl.ds(pr, TMB), c * 128:(c + 1) * 128] = acc
            a3 = acc.reshape(TMB // 8, 8, 128)
            mean = jnp.sum(a3, axis=0) * (8.0 / TMB)
            d = a3 - mean[None]
            st_mean[p, :, c * 128:(c + 1) * 128] = mean
            st_m2[p, :, c * 128:(c + 1) * 128] = jnp.sum(d * d, axis=0)

    def phase_b(i, carry):
        conv_tile(jnp.maximum(i - 2, 0))
        b = i // tpb_b
        rb = pl.multiple_of((i % tpb_b) * TMB, 16)
        r = pl.multiple_of(i * TMB, 16)
        h = hs[b, pl.ds(rb, TMB), :]
        q = _dot(h, mq[...]).astype(BF16)
        kv = hs[b]
        s = _dot_nt(q, kv)
        if TP != T:
            lo = TP - 128
            col = lax.broadcasted_iota(jnp.int32, (TMB, 128), 1) + lo
            s_last = jnp.where(col < T, s[:, lo:], -jnp.inf)
            s = jnp.concatenate([s[:, :lo], s_last], axis=1)
        m = jnp.max(s, axis=-1, keepdims=True)
        p = jnp.exp2(s - m)
        l = jnp.sum(p, axis=-1, keepdims=True)
        o = _dot(p.astype(BF16), kv)
        o = (o * (1.0 / l)).astype(BF16)
        x2 = xs[pl.ds(r, TMB), :] + _dot(o, wvo[...])
        xs[pl.ds(r, TMB), :] = x2
        u = _dot(_ln(x2).astype(BF16), wp1[...])
        g = u[:, :D] * (0.5 + 0.5 * jnp.tanh(0.5 * u[:, D:]))
        for c in range(NCB):
            gs[b, c, pl.ds(HALO + rb, TMB), :] = g[:, c * 128:(c + 1) * 128]
        return carry

    lax.fori_loop(0, ntb, phase_b, 0)
    conv_tile(ntb - 2)
    conv_tile(ntb - 1)

    means = st_mean[...].reshape(ntb * 8, D)
    mu = jnp.mean(means, axis=0, keepdims=True)
    dm = means - mu
    var = (jnp.sum(st_m2[...].reshape(ntb * 8, D), axis=0, keepdims=True)
           + (TMB // 8) * jnp.sum(dm * dm, axis=0, keepdims=True)) * (1.0 / N)
    rstd = lax.rsqrt(var + EPS)
    bn[0:1, :] = mu
    bn[1:2, :] = rstd

    def phase_c(i, carry):
        r = pl.multiple_of(i * TMC, 16)
        z = (dcs[pl.ds(r, TMC), :] - bn[0:1, :]) * bn[1:2, :]
        x3 = xs[pl.ds(r, TMC), :] + _dot(_silu(z).astype(BF16), wp2[...])
        x4 = x3 + 0.5 * _ffn(_ln(x3).astype(BF16), w2a, w2b)
        obuf[pl.ds(r, TMC), :] = _ln(x4).astype(BF16)
        o_copy(i).start()
        return carry

    lax.fori_loop(0, ntc, phase_c, 0)
    for i in range(ntc):
        o_copy(i).wait()


@jax.jit
def pallas_standalone__conformer_family_conformer__speech_kernel(
    x: jax.Array,
    w_ff1_a: jax.Array,
    w_ff1_b: jax.Array,
    w_q: jax.Array,
    w_k: jax.Array,
    w_v: jax.Array,
    w_o: jax.Array,
    w_pw1: jax.Array,
    dw: jax.Array,
    w_pw2: jax.Array,
    w_ff2_a: jax.Array,
    w_ff2_b: jax.Array,
):
    B, T, D = x.shape
    K = dw.shape[0]
    N = B * T
    TP = -(-T // 128) * 128
    weights = (w_ff1_a, w_ff1_b, w_q, w_k, w_v, w_o, w_pw1, dw, w_pw2,
               w_ff2_a, w_ff2_b)
    scratch = [pltpu.VMEM((N, D), BF16)]
    scratch += [pltpu.VMEM(w.shape, w.dtype) for w in weights]
    scratch += [
        pltpu.VMEM((D, D), BF16),
        pltpu.VMEM((D, D), BF16),
        pltpu.VMEM((N, D), F32),
        pltpu.VMEM((B, TP, D), BF16),
        pltpu.VMEM((B, D // 128, T + 2 * HALO, 128), F32),
        pltpu.VMEM((N, D), F32),
        pltpu.VMEM((N // TMB, 8, D), F32),
        pltpu.VMEM((N // TMB, 8, D), F32),
        pltpu.VMEM((8, D), F32),
        pltpu.VMEM((N, D), BF16),
        pltpu.SemaphoreType.DMA((N // TMA,)),
        pltpu.SemaphoreType.DMA((len(weights),)),
        pltpu.SemaphoreType.DMA((N // TMC,)),
    ]
    out = pl.pallas_call(
        functools.partial(_kernel, B=B, T=T, D=D, K=K),
        out_shape=jax.ShapeDtypeStruct((N, D), x.dtype),
        in_specs=[pl.BlockSpec(memory_space=pl.ANY)] * 12,
        out_specs=pl.BlockSpec(memory_space=pl.ANY),
        scratch_shapes=scratch,
        compiler_params=pltpu.CompilerParams(
            vmem_limit_bytes=120 * 1024 * 1024),
    )(x.reshape(N, D), *weights)
    return out.reshape(B, T, D)
```

```python
import functools
import math

import jax
import jax.numpy as jnp
from jax import lax
import jax.experimental.pallas as pl
import jax.experimental.pallas.tpu as pltpu

F32 = jnp.float32
BF16 = jnp.bfloat16

TM = 400
FC = 512
KC = 512
CR = 40
HALO = 8
EPS = 1e-05


def _ln(x):
    m = jnp.mean(x, axis=-1, keepdims=True)
    xc = x - m
    v = jnp.mean(xc * xc, axis=-1, keepdims=True)
    return xc * lax.rsqrt(v + EPS)


def _silu(a):
    y = 0.5 * a
    return y + y * jnp.tanh(y)


def _dot(a, b):
    return jnp.dot(a, b, preferred_element_type=F32)


def _dot_nt(a, b):
    return lax.dot_general(a, b, (((1,), (1,)), ((), ())),
                           preferred_element_type=F32)


def _ffn(h, wa_ref, wb_ref, fillers=()):
    f = wa_ref.shape[1]
    acc = None
    for c in range(f // FC):
        a = _dot(h, wa_ref[:, c * FC:(c + 1) * FC])
        s = _silu(a).astype(BF16)
        p = _dot(s, wb_ref[c * FC:(c + 1) * FC, :])
        acc = p if acc is None else acc + p
        if c < len(fillers):
            fillers[c]()
    return acc


def _kernel(x_hbm, w1a_hbm, w1b_hbm, wq_hbm, wk_hbm, wv_hbm, wo_hbm,
            wp1_hbm, dw_hbm, wp2_hbm, w2a_hbm, w2b_hbm,
            out_hbm,
            xin, w1a, w1b, wq, wk, wv, wo, wp1, dw, wp2, w2a, w2b,
            mq, wvo, xs, hs, gs, dcs, st_mean, st_m2, bn, obuf,
            lhs_a, lhs_b, dwb,
            xsem, wsem, osem,
            *, B, T, D, K):
    N = B * T
    TP = hs.shape[1]
    NCB = D // 128
    nt = N // TM
    tpb = T // TM

    def rows(i):
        return pl.ds(pl.multiple_of(i * TM, 16), TM)

    def brows(i, off=0):
        return i // tpb, pl.ds(pl.multiple_of((i % tpb) * TM, 16) + off, TM)

    def x_copy(i):
        return pltpu.make_async_copy(x_hbm.at[rows(i), :],
                                     xin.at[rows(i), :], xsem.at[i])

    def o_copy(i):
        return pltpu.make_async_copy(obuf.at[rows(i), :],
                                     out_hbm.at[rows(i), :], osem.at[i])

    w_pairs = [(w1a_hbm, w1a), (w1b_hbm, w1b), (wq_hbm, wq), (wk_hbm, wk),
               (wv_hbm, wv), (wo_hbm, wo), (wp1_hbm, wp1), (dw_hbm, dw),
               (wp2_hbm, wp2), (w2a_hbm, w2a), (w2b_hbm, w2b)]
    w_copies = [pltpu.make_async_copy(s, d, wsem.at[j])
                for j, (s, d) in enumerate(w_pairs)]

    x_copy(0).start()
    w_copies[0].start()
    w_copies[1].start()
    x_copy(1).start()

    for b in range(B):
        hs[b, T:TP, :] = jnp.zeros((TP - T, D), BF16)
        for c in range(NCB):
            gs[b, c, 0:HALO, :] = jnp.zeros((HALO, 128), F32)
            gs[b, c, HALO + T:HALO + T + HALO, :] = jnp.zeros((HALO, 128), F32)

    def ln_in(i):
        lhs_a[...] = _ln(xin[rows(i), :].astype(F32)).astype(BF16)

    def ln_out(i):
        b, rb = brows(i)
        hs[b, rb, :] = _ln(xs[rows(i), :]).astype(BF16)

    x_copy(0).wait()
    ln_in(0)
    w_copies[0].wait()
    w_copies[1].wait()
    for cp in w_copies[2:]:
        cp.start()

    def phase_a(i, carry):
        @pl.when(i + 2 < nt)
        def _():
            x_copy(i + 2).start()

        @pl.when(i + 1 < nt)
        def _():
            x_copy(i + 1).wait()
        h = lhs_a[...]
        f = _ffn(h, w1a, w1b,
                 fillers=(lambda: ln_out(jnp.maximum(i - 1, 0)),
                          lambda: ln_in(jnp.minimum(i + 1, nt - 1))))
        xs[rows(i), :] = xin[rows(i), :].astype(F32) + 0.5 * f
        return carry

    with jax.named_scope("phase_a"):
        lax.fori_loop(0, nt, phase_a, 0)
    ln_out(nt - 1)

    for cp in w_copies[2:]:
        cp.wait()

    qk_scale = (D ** -0.5) * math.log2(math.e)
    mq[...] = (_dot_nt(wq[...], wk[...]) * qk_scale).astype(BF16)
    wvo[...] = _dot(wv[...], wo[...]).astype(BF16)
    dwf = dw[...].astype(F32)
    for k in range(K):
        dwb[k] = jnp.broadcast_to(dwf[k:k + 1, :], (8, D))

    def q_cols(i, c):
        b, rb = brows(i)
        cs = slice(c * 128, (c + 1) * 128)
        lhs_a[:, cs] = _dot(hs[b, rb, :], mq[:, cs]).astype(BF16)

    for c in range(NCB):
        q_cols(0, c)

    def conv_cols(p, c):
        pb = p // tpb
        prb = pl.multiple_of((p % tpb) * TM, 8)
        pr = pl.multiple_of(p * TM, 8)
        cs = slice(c * 128, (c + 1) * 128)
        tot = None
        for r0 in range(0, TM, CR):
            acc = None
            for k in range(K):
                off = HALO - K // 2 + k + r0
                g = gs[pb, c, pl.ds(prb + off, CR), :].reshape(CR // 8, 8, 128)
                t = g * dwb[k, :, cs][None]
                acc = t if acc is None else acc + t
            dcs[pl.ds(pr + r0, CR), cs] = acc.reshape(CR, 128)
            part = jnp.sum(acc, axis=0)
            tot = part if tot is None else tot + part
        mean = tot * (8.0 / TM)
        d = dcs[pl.ds(pr, TM), cs].reshape(TM // 8, 8, 128) - mean[None]
        st_mean[p, :, cs] = mean
        st_m2[p, :, cs] = jnp.sum(d * d, axis=0)

    nkc = TP // KC

    def phase_b(i, carry):
        b, rb = brows(i)
        inext = jnp.minimum(i + 1, nt - 1)
        iconv = jnp.maximum(i - 2, 0)
        q = lhs_a[...]

        def scores(j):
            s = _dot_nt(q, hs[b, j * KC:(j + 1) * KC, :])
            if (j + 1) * KC > T:
                lo = KC - 128
                col = lax.broadcasted_iota(jnp.int32, (TM, 128), 1) + (j * KC + lo)
                s_last = jnp.where(col < T, s[:, lo:], -jnp.inf)
                s = jnp.concatenate([s[:, :lo], s_last], axis=1)
            return s

        m = l = acc = None
        s_next = scores(0)
        for j in range(nkc):
            s = s_next
            if j + 1 < nkc:
                s_next = scores(j + 1)
            mj = jnp.max(s, axis=-1, keepdims=True)
            m_new = mj if m is None else jnp.maximum(m, mj)
            p = jnp.exp2(s - m_new)
            ps = p[:, 0:128]
            for c in range(1, KC // 128):
                ps = ps + p[:, c * 128:(c + 1) * 128]
            pv = _dot(p.astype(BF16), hs[b, j * KC:(j + 1) * KC, :])
            if m is None:
                l, acc = ps, pv
            else:
                alpha = jnp.exp2(m - m_new)
                l = l * alpha + ps
                acc = acc * alpha + pv
            m = m_new
            if j % 2 == 1:
                conv_cols(iconv, j // 2)
        q_cols(inext, 0)
        o = (acc * (1.0 / jnp.sum(l, axis=-1, keepdims=True))).astype(BF16)
        x2 = xs[rows(i), :] + _dot(o, wvo[...])
        xs[rows(i), :] = x2
        q_cols(inext, 1)
        q_cols(inext, 2)
        hn = _ln(x2).astype(BF16)
        for c in range(NCB):
            ua = _dot(hn, wp1[:, c * 128:(c + 1) * 128])
            ub = _dot(hn, wp1[:, D + c * 128:D + (c + 1) * 128])
            g = ua * (0.5 + 0.5 * jnp.tanh(0.5 * ub))
            gs[b, c, pl.ds(pl.multiple_of((i % tpb) * TM, 8) + HALO, TM), :] = g
        q_cols(inext, 3)
        return carry

    with jax.named_scope("phase_b"):
        lax.fori_loop(0, nt, phase_b, 0)
    with jax.named_scope("conv_tail"):
        for p in (nt - 2, nt - 1):
            for c in range(NCB):
                conv_cols(p, c)

    means = st_mean[...].reshape(nt * 8, D)
    mu = jnp.mean(means, axis=0, keepdims=True)
    dm = means - mu
    var = (jnp.sum(st_m2[...].reshape(nt * 8, D), axis=0, keepdims=True)
           + (TM // 8) * jnp.sum(dm * dm, axis=0, keepdims=True)) * (1.0 / N)
    rstd = lax.rsqrt(var + EPS)
    bn[0:1, :] = mu
    bn[1:2, :] = rstd

    def bn_silu(i):
        z = (dcs[rows(i), :] - bn[0:1, :]) * bn[1:2, :]
        lhs_b[...] = _silu(z).astype(BF16)

    def pw2(i):
        return xs[rows(i), :] + _dot(lhs_b[...], wp2[...])

    def ln_final(i):
        obuf[rows(i), :] = _ln(xs[rows(i), :]).astype(BF16)

    bn_silu(0)
    x3 = pw2(0)
    dcs[rows(0), :] = x3
    lhs_a[...] = _ln(x3).astype(BF16)
    bn_silu(1)

    def phase_c(i, carry):
        @pl.when(i >= 2)
        def _():
            o_copy(i - 2).start()
        h = lhs_a[...]
        x3n = pw2(i + 1)
        dcs[rows(i + 1), :] = x3n

        def fill0():
            lhs_a[...] = _ln(x3n).astype(BF16)

        f = _ffn(h, w2a, w2b,
                 fillers=(fill0,
                          lambda: bn_silu(jnp.minimum(i + 2, nt)),
                          lambda: ln_final(jnp.maximum(i - 1, 0))))
        xs[rows(i), :] = dcs[rows(i), :] + 0.5 * f
        return carry

    with jax.named_scope("phase_c"):
        lax.fori_loop(0, nt, phase_c, 0)
    o_copy(nt - 2).start()
    ln_final(nt - 1)
    o_copy(nt - 1).start()
    for i in range(nt):
        o_copy(i).wait()


@jax.jit
def pallas_standalone__conformer_family_conformer__speech_kernel(
    x: jax.Array,
    w_ff1_a: jax.Array,
    w_ff1_b: jax.Array,
    w_q: jax.Array,
    w_k: jax.Array,
    w_v: jax.Array,
    w_o: jax.Array,
    w_pw1: jax.Array,
    dw: jax.Array,
    w_pw2: jax.Array,
    w_ff2_a: jax.Array,
    w_ff2_b: jax.Array,
):
    B, T, D = x.shape
    K = dw.shape[0]
    N = B * T
    TP = -(-T // KC) * KC
    weights = (w_ff1_a, w_ff1_b, w_q, w_k, w_v, w_o, w_pw1, dw, w_pw2,
               w_ff2_a, w_ff2_b)
    scratch = [pltpu.VMEM((N, D), BF16)]
    scratch += [pltpu.VMEM(w.shape, w.dtype) for w in weights]
    scratch += [
        pltpu.VMEM((D, D), BF16),
        pltpu.VMEM((D, D), BF16),
        pltpu.VMEM((N + TM, D), F32),
        pltpu.VMEM((B, TP, D), BF16),
        pltpu.VMEM((B, D // 128, T + 2 * HALO, 128), F32),
        pltpu.VMEM((N + TM, D), F32),
        pltpu.VMEM((N // TM, 8, D), F32),
        pltpu.VMEM((N // TM, 8, D), F32),
        pltpu.VMEM((8, D), F32),
        pltpu.VMEM((N, D), BF16),
        pltpu.VMEM((TM, D), BF16),
        pltpu.VMEM((TM, D), BF16),
        pltpu.VMEM((K, 8, D), F32),
        pltpu.SemaphoreType.DMA((N // TM,)),
        pltpu.SemaphoreType.DMA((len(weights),)),
        pltpu.SemaphoreType.DMA((N // TM,)),
    ]
    out = pl.pallas_call(
        functools.partial(_kernel, B=B, T=T, D=D, K=K),
        out_shape=jax.ShapeDtypeStruct((N, D), x.dtype),
        in_specs=[pl.BlockSpec(memory_space=pl.ANY)] * 12,
        out_specs=pl.BlockSpec(memory_space=pl.ANY),
        scratch_shapes=scratch,
        compiler_params=pltpu.CompilerParams(
            vmem_limit_bytes=120 * 1024 * 1024),
    )(x.reshape(N, D), *weights)
    return out.reshape(B, T, D)
```

```python
import functools
import math

import jax
import jax.numpy as jnp
from jax import lax
import jax.experimental.pallas as pl
import jax.experimental.pallas.tpu as pltpu

F32 = jnp.float32
BF16 = jnp.bfloat16

TM = 400
FC = 512
KC = 512
RB = 40
SB = 16
AB = 0
A_SLOTS = (1, 29)
B_SLOTS = (1, 61)
C_SLOTS = (4, 34)
SOFT = (0, 400)
PHASES = 'ABC'
MEM = 'fl'
ZR = 32
PU = 2
HALO = 8
EPS = 1e-05


def _ln(x, z=None):
    if z is None:
        m = jnp.mean(x, axis=-1, keepdims=True)
    else:
        t = z
        for c in range(x.shape[-1] // 128):
            t = t + x[:, c * 128:(c + 1) * 128]
        m = jnp.sum(t, axis=-1, keepdims=True) * (1.0 / x.shape[-1])
    xc = x - m
    v = jnp.mean(xc * xc, axis=-1, keepdims=True)
    return xc * lax.rsqrt(v + EPS)


def _silu(a):
    y = 0.5 * a
    return y + y * jnp.tanh(y)


def _dot(a, b):
    return jnp.dot(a, b, preferred_element_type=F32)


def _dot_nt(a, b):
    return lax.dot_general(a, b, (((1,), (1,)), ((), ())),
                           preferred_element_type=F32)


class _Anchor:
    def __init__(self, t, zero_v, zero_s):
        self.t, self.zero_v, self.zero_s = t, zero_v, zero_s

    def v(self):
        return pltpu.bitcast(
            pltpu.bitcast(self.t, jnp.uint32) & self.zero_v[0:8, :], F32)

    def s(self):
        return pltpu.bitcast(self.t, jnp.int32)[0, 0] & self.zero_s[0]


class _Sched:
    def __init__(self, zero_v, zero_s):
        self.zero_v, self.zero_s = zero_v, zero_s
        self.queue = []
        self.now = 0

    def add(self, items, t0, t1):
        assert t0 >= self.now
        n = len(items)
        self.queue += [(t0 + k * (t1 - t0) // n, it)
                       for k, it in enumerate(items)]
        self.queue.sort(key=lambda e: e[0])

    def anchor(self, t, r):
        return _Anchor(t[r:r + 8, :], self.zero_v, self.zero_s)

    def __call__(self, t):
        end = self.now + TM
        while self.queue and self.queue[0][0] < end:
            time, item = self.queue.pop(0)
            item(self.anchor(t, (time - self.now) // 8 * 8))
        self.now = end


def _rep(z, rows):
    return jnp.concatenate([z] * (rows // 8), axis=0)


def _ffn(h, wa_ref, wb_ref, sched):
    f = wa_ref.shape[1]
    d = wb_ref.shape[1]
    acc = [None] * (d // 128)
    for c in range(f // FC):
        ss = []
        for n in range(FC // 128):
            lo = c * FC + n * 128
            a = _dot(h, wa_ref[:, lo:lo + 128])
            ss.append(_silu(a))
            sched(a)
        s = jnp.concatenate(ss, axis=1).astype(BF16)
        for n in range(d // 128):
            p = _dot(s, wb_ref[c * FC:(c + 1) * FC, n * 128:(n + 1) * 128])
            acc[n] = p if acc[n] is None else acc[n] + p
            sched(p)
    return jnp.concatenate(acc, axis=1)


def _kernel(x_hbm, w1a_hbm, w1b_hbm, wq_hbm, wk_hbm, wv_hbm, wo_hbm,
            wp1_hbm, dw_hbm, wp2_hbm, w2a_hbm, w2b_hbm,
            out_hbm,
            xin, w1a, w1b, wq, wk, wv, wo, wp1, dw, wp2, w2a, w2b,
            mq, wvo, xs, hs, gs, dcs, st_mean, st_m2, bn, obuf,
            lhs_a, lhs_b, dwb, zero, zero_s, m_buf, l_buf, al_buf0, al_buf1,
            p_buf0, p_buf1,
            xsem, wsem, osem,
            *, B, T, D, K):
    N = B * T
    TP = hs.shape[1]
    NCB = D // 128
    nt = N // TM
    tpb = T // TM

    def rows(i, r0=0, n=TM):
        return pl.ds(pl.multiple_of(i * TM, 16) + r0, n)

    def brows(i, r0=0, n=TM):
        return i // tpb, pl.ds(pl.multiple_of((i % tpb) * TM, 16) + r0, n)

    def col(c):
        return slice(c * 128, (c + 1) * 128)

    def pieces(fn, i):
        return [functools.partial(fn, i, r0, RB) for r0 in range(0, TM, RB)]

    def interleave(*lists):
        return [it for group in zip(*lists) for it in group]

    def x_copy(i):
        return pltpu.make_async_copy(x_hbm.at[rows(i), :],
                                     xin.at[rows(i), :], xsem.at[i])

    def o_copy(i):
        return pltpu.make_async_copy(obuf.at[rows(i), :],
                                     out_hbm.at[rows(i), :], osem.at[i])

    w_pairs = [(w1a_hbm, w1a), (w1b_hbm, w1b), (wq_hbm, wq), (wk_hbm, wk),
               (wv_hbm, wv), (wo_hbm, wo), (wp1_hbm, wp1), (dw_hbm, dw),
               (wp2_hbm, wp2), (w2a_hbm, w2a), (w2b_hbm, w2b)]
    w_copies = [pltpu.make_async_copy(s, d, wsem.at[j])
                for j, (s, d) in enumerate(w_pairs)]

    x_copy(0).start()
    w_copies[0].start()
    w_copies[1].start()
    x_copy(1).start()

    zero[...] = jnp.zeros(zero.shape, jnp.uint32)
    zero_s[0] = 0
    for b in range(B):
        hs[b, T:TP, :] = jnp.zeros((TP - T, D), BF16)
    for c in range(NCB):
        gs[1, c, 0:HALO, :] = jnp.zeros((HALO, 128), F32)
        gs[nt, c, HALO + TM:, :] = jnp.zeros((HALO, 128), F32)

    def zrep(z, n):
        return None if z is None else _rep(z.v(), n)

    def ln_in(i, r0=0, n=TM, z=None):
        lhs_a[r0:r0 + n, :] = _ln(xin[rows(i, r0, n), :].astype(F32),
                                  zrep(z, n)).astype(BF16)

    def ln_out(i, r0=0, n=TM, z=None):
        b, rb = brows(i, r0, n)
        hs[b, rb, :] = _ln(xs[rows(i, r0, n), :], zrep(z, n)).astype(BF16)

    x_copy(0).wait()
    ln_in(0)
    w_copies[0].wait()
    w_copies[1].wait()
    for cp in w_copies[2:]:
        cp.start()

    def phase_a(i, carry):
        @pl.when(i + 2 < nt)
        def _():
            x_copy(i + 2).start()

        @pl.when(i + 1 < nt)
        def _():
            x_copy(i + 1).wait()
        h = lhs_a[...]
        items = interleave(pieces(ln_out, jnp.maximum(i - 1, 0)),
                           pieces(ln_in, jnp.minimum(i + 1, nt - 1)))
        sched = _Sched(zero, zero_s)
        sched.add(items, A_SLOTS[0] * TM, A_SLOTS[1] * TM)
        f = _ffn(h, w1a, w1b, sched)
        xs[rows(i), :] = xin[rows(i), :].astype(F32) + 0.5 * f
        return carry

    with jax.named_scope("phase_a"):
        if 'A' in PHASES:
            lax.fori_loop(0, nt, phase_a, 0)
        else:
            x_copy(1).wait()

    for cp in w_copies[2:]:
        cp.wait()

    qk_scale = (D ** -0.5) * math.log2(math.e)

    def q_cols(i, cs):
        b, rb = brows(i)
        lhs_a[:, cs] = _dot(hs[b, rb, :], mq[:, cs]).astype(BF16)

    def fold(u, carry):
        nr = TM // PU
        r0 = pl.multiple_of(u * nr, 8)
        sched = _Sched(zero, zero_s)
        sched.add([functools.partial(ln_out, nt - 1, r0 + r, RB)
                   for r in range(0, nr, RB)], 0, (2 * NCB // PU - 1) * TM)
        css = [pl.ds(pl.multiple_of((u * (NCB // PU) + c) * 128, 128), 128)
               for c in range(NCB // PU)]
        for cs in css:
            t = _dot_nt(wq[...], wk[cs, :])
            mq[:, cs] = (t * qk_scale).astype(BF16)
            sched(t)
        for cs in css:
            t = _dot(wv[...], wo[:, cs])
            wvo[:, cs] = t.astype(BF16)
            sched(t)
        for cs in css:
            q_cols(0, cs)
        return carry

    lax.fori_loop(0, PU, fold, 0)
    dwf = dw[...].astype(F32)
    for k in range(K):
        dwb[k] = jnp.broadcast_to(dwf[k:k + 1, :], (8, D))

    def conv_block(p, r0, c, z):
        cs = slice(c * 128, (c + 1) * 128)
        acc = None
        for k in range(K):
            off = HALO - K // 2 + k + r0
            w = dwb[k, :, cs]
            if z is not None:
                w = w + z
            t = gs[p + 1, c, off:off + 8, :] * w
            acc = t if acc is None else acc + t
        dcs[rows(p, r0, 8), cs] = acc
        return acc

    def conv_main(p):
        st = {}

        def item(r0, c, z=None):
            acc = conv_block(p, r0, c, None if z is None else z.v())
            if r0 == 0:
                st[c] = (acc, None, None)
                return
            shift, s1, s2 = st[c]
            d = acc - shift
            s1 = d if s1 is None else s1 + d
            s2 = d * d if s2 is None else s2 + d * d
            st[c] = (shift, s1, s2)
            if r0 + 16 == TM:
                dm = s1 * (1.0 / (TM // 8 - 1))
                st_mean[p, :, c * 128:(c + 1) * 128] = shift + dm
                st_m2[p, :, c * 128:(c + 1) * 128] = s2 - s1 * dm

        return [functools.partial(item, r0, c)
                for c in range(NCB) for r0 in range(0, TM - 8, 8)]

    def conv_edge(p):
        def item(c, z=None):
            conv_block(p, TM - 8, c, None if z is None else z.v())

        return [functools.partial(item, c) for c in range(NCB)]

    nkc = TP // KC

    def phase_b(i, carry):
        b, rb = brows(i)
        inext = jnp.minimum(i + 1, nt - 1)
        q = lhs_a[...]

        sched = _Sched(zero, zero_s)
        if 'n' not in PHASES:
            sched.add(conv_edge(jnp.maximum(i - 2, 0))
                      + conv_main(jnp.maximum(i - 1, 0)),
                      B_SLOTS[0] * TM, B_SLOTS[1] * TM)
        nsb = TM // SB
        dz = zero_s[0]
        p_buf, al_buf = (p_buf0, p_buf1), (al_buf0, al_buf1)

        def dyn(r0, n):
            return pl.ds(pl.multiple_of(dz + r0, 8), n)

        def scores(j):
            ss = []
            for n in range(KC // 128):
                lo = j * KC + n * 128
                s = _dot_nt(q, hs[b, lo:lo + 128, :])
                sched(s)
                if lo + 128 > T:
                    col = lax.broadcasted_iota(jnp.int32, (TM, 128), 1) + lo
                    s = jnp.where(col < T, s, -jnp.inf)
                ss.append(s)
            return ss

        m_v, l_v = [None] * nsb, [None] * nsb
        al_v = [[None] * nsb for _ in range(nkc)]
        p_v = [[None] * nsb for _ in range(nkc)]

        def soft(j, ss, k, z):
            rs = slice(k * SB, (k + 1) * SB)
            s = [t[rs, :] for t in ss]
            mj = functools.reduce(jnp.maximum, s[1:], s[0] + _rep(z.v(), SB))
            m_new = jnp.broadcast_to(jnp.max(mj, axis=-1, keepdims=True),
                                     (SB, 128))
            if j > 0:
                m_old = m_buf[dyn(k * SB, SB), :] if 'm' in MEM else m_v[k]
                m_new = jnp.maximum(m_old, m_new)
            p = [jnp.exp2(t - m_new) for t in s]
            ps = functools.reduce(jnp.add, p)
            if 'p' in MEM:
                pb = jnp.concatenate([t.astype(BF16) for t in p], axis=1)
                p_buf[j % 2][k * SB // 2:(k + 1) * SB // 2, :] = pltpu.bitcast(
                    pb, jnp.uint32)
            elif 'f' in MEM:
                p_v[j][k] = jnp.concatenate(p, axis=1)
            else:
                p_v[j][k] = jnp.concatenate(p, axis=1).astype(BF16)
            if j > 0:
                alpha = jnp.exp2(m_old - m_new)
                if 'a' in MEM:
                    al_buf[j % 2][rs, :] = alpha
                else:
                    al_v[j][k] = alpha
                l_old = l_buf[dyn(k * SB, SB), :] if 'l' in MEM else l_v[k]
                ps = l_old * alpha + ps
            if 'l' in MEM:
                l_buf[rs, :] = ps
            l_v[k] = ps
            if j + 1 < nkc and 'm' in MEM:
                m_buf[rs, :] = m_new
            m_v[k] = m_new

        def add_soft(j, ss, ndots):
            sched.add([functools.partial(soft, j, ss, k) for k in range(nsb)],
                      sched.now + SOFT[0], sched.now + ndots * TM - SOFT[1])

        acc = [None] * NCB
        nd = KC // 128
        add_soft(0, scores(0), nd)
        for j in range(nkc):
            if j + 1 < nkc:
                s_next = scores(j + 1)
            if j + 1 < nkc:
                add_soft(j + 1, s_next, NCB + (nd if j + 2 < nkc else 0))
            if 'p' not in MEM:
                p_all = jnp.concatenate(p_v[j], axis=0).astype(BF16)
            if j > 0 and 'a' not in MEM:
                al = jnp.concatenate(al_v[j], axis=0)
            for n in range(NCB):
                if 'p' in MEM:
                    p_all = pltpu.bitcast(p_buf[j % 2][dyn(0, TM // 2), :],
                                          BF16)
                pv = _dot(p_all, hs[b, j * KC:(j + 1) * KC,
                                    n * 128:(n + 1) * 128])
                sched(pv)
                if j == 0:
                    acc[n] = pv
                else:
                    if 'a' in MEM:
                        al = al_buf[j % 2][dyn(0, TM), :]
                    if AB:
                        zs = [_rep(sched.anchor(pv, r).v(), AB)
                              for r in range(0, TM, AB)]
                        acc[n] = (acc[n] * (al + jnp.concatenate(zs, axis=0))
                                  + pv)
                    else:
                        acc[n] = acc[n] * al + pv
        acc = jnp.concatenate(acc, axis=1)
        if 'l' in MEM:
            l = l_buf[dyn(0, TM), :]
        else:
            l = jnp.concatenate(l_v, axis=0)
        if 't' in PHASES:
            xs[rows(i), :] = acc
            return carry
        if 'q' not in PHASES:
            q_cols(inext, col(0))
        o = (acc * (1.0 / jnp.sum(l, axis=-1, keepdims=True))).astype(BF16)
        if 'o' in PHASES:
            x2 = xs[rows(i), :] + o.astype(F32)
        else:
            x2 = xs[rows(i), :] + _dot(o, wvo[...])
        xs[rows(i), :] = x2
        if 'q' not in PHASES:
            q_cols(inext, col(1))
            q_cols(inext, col(2))
        hn = _ln(x2).astype(BF16)
        for c in range(NCB):
            if 'w' in PHASES:
                g = hn[:, c * 128:(c + 1) * 128].astype(F32)
            else:
                ua = _dot(hn, wp1[:, c * 128:(c + 1) * 128])
                ub = _dot(hn, wp1[:, D + c * 128:D + (c + 1) * 128])
                g = ua * (0.5 + 0.5 * jnp.tanh(0.5 * ub))
            gs[i + 1, c, HALO:HALO + TM, :] = g
            gs[i, c, HALO + TM:, :] = jnp.where(i % tpb == 0, 0.0, g[:HALO])
            gs[i + 2, c, :HALO, :] = jnp.where(i % tpb == tpb - 1, 0.0,
                                               g[TM - HALO:])
        if 'q' not in PHASES:
            q_cols(inext, col(3))
        return carry

    with jax.named_scope("phase_b"):
        if 'B' in PHASES:
            lax.fori_loop(0, nt, phase_b, 0)
    with jax.named_scope("conv_tail"):
        for item in (conv_edge(nt - 2) + conv_edge(nt - 1)
                     + conv_main(nt - 1)):
            item()

    ng = TM // 8 - 1
    means = st_mean[...].reshape(nt * 8, D)
    edges = jnp.concatenate([dcs[(p + 1) * TM - 8:(p + 1) * TM, :]
                             for p in range(nt)], axis=0)
    mu = jnp.sum(ng * means + edges, axis=0, keepdims=True) * (1.0 / N)
    dm = means - mu
    de = edges - mu
    var = jnp.sum(st_m2[...].reshape(nt * 8, D) + ng * (dm * dm) + de * de,
                  axis=0, keepdims=True) * (1.0 / N)
    rstd = lax.rsqrt(var + EPS)
    bn[0] = jnp.broadcast_to(mu, (8, D))
    bn[1] = jnp.broadcast_to(rstd, (8, D))

    def bn_silu(i, r0=0, n=TM, z=None):
        mu = bn[0]
        if z is not None:
            mu = mu + jnp.concatenate([z.v()] * NCB, axis=1)
        d = dcs[rows(i, r0, n), :].reshape(n // 8, 8, D)
        y = ((d - mu[None]) * bn[1][None]).reshape(n, D)
        lhs_b[r0:r0 + n, :] = _silu(y).astype(BF16)

    def pw2(i, isrc, sched=None):
        lhs = lhs_b[...]
        for c in range(NCB):
            cs = slice(c * 128, (c + 1) * 128)
            t = _dot(lhs, wp2[:, cs])
            dcs[rows(i), cs] = xs[rows(isrc), cs] + t
            if sched is not None:
                sched(t)

    def ln_mid(i, r0=0, n=TM, z=None):
        lhs_a[r0:r0 + n, :] = _ln(dcs[rows(i, r0, n), :],
                                  zrep(z, n)).astype(BF16)

    def ln_final(i, r0=0, n=TM, z=None):
        obuf[rows(i, r0, n), :] = _ln(xs[rows(i, r0, n), :],
                                      zrep(z, n)).astype(BF16)

    bn_silu(0)
    pw2(0, 0)
    ln_mid(0)
    bn_silu(1)

    def phase_c(i, carry):
        @pl.when(i >= 2)
        def _():
            o_copy(i - 2).start()
        h = lhs_a[...]
        items = interleave(pieces(ln_final, jnp.maximum(i - 1, 0)),
                           pieces(bn_silu, jnp.minimum(i + 2, nt - 1)),
                           pieces(ln_mid, i + 1))
        sched = _Sched(zero, zero_s)
        sched.add(items, C_SLOTS[0] * TM, C_SLOTS[1] * TM)
        pw2(i + 1, jnp.minimum(i + 1, nt - 1), sched)
        f = _ffn(h, w2a, w2b, sched)
        xs[rows(i), :] = dcs[rows(i), :] + 0.5 * f
        return carry

    with jax.named_scope("phase_c"):
        if 'C' in PHASES:
            lax.fori_loop(0, nt, phase_c, 0)
        else:
            for i in range(nt - 2):
                o_copy(i).start()
    o_copy(nt - 2).start()
    ln_final(nt - 1)
    o_copy(nt - 1).start()
    for i in range(nt):
        o_copy(i).wait()


@jax.jit
def pallas_standalone__conformer_family_conformer__speech_kernel(
    x: jax.Array,
    w_ff1_a: jax.Array,
    w_ff1_b: jax.Array,
    w_q: jax.Array,
    w_k: jax.Array,
    w_v: jax.Array,
    w_o: jax.Array,
    w_pw1: jax.Array,
    dw: jax.Array,
    w_pw2: jax.Array,
    w_ff2_a: jax.Array,
    w_ff2_b: jax.Array,
):
    B, T, D = x.shape
    K = dw.shape[0]
    N = B * T
    TP = -(-T // KC) * KC
    weights = (w_ff1_a, w_ff1_b, w_q, w_k, w_v, w_o, w_pw1, dw, w_pw2,
               w_ff2_a, w_ff2_b)
    scratch = [pltpu.VMEM((N, D), BF16)]
    scratch += [pltpu.VMEM(w.shape, w.dtype) for w in weights]
    scratch += [
        pltpu.VMEM((D, D), BF16),
        pltpu.VMEM((D, D), BF16),
        pltpu.VMEM((N, D), F32),
        pltpu.VMEM((B, TP, D), BF16),
        pltpu.VMEM((N // TM + 2, D // 128, TM + 2 * HALO, 128), F32),
        pltpu.VMEM((N + TM, D), F32),
        pltpu.VMEM((N // TM, 8, D), F32),
        pltpu.VMEM((N // TM, 8, D), F32),
        pltpu.VMEM((2, 8, D), F32),
        pltpu.VMEM((N, D), BF16),
        pltpu.VMEM((TM, D), BF16),
        pltpu.VMEM((TM, D), BF16),
        pltpu.VMEM((K, 8, D), F32),
        pltpu.VMEM((ZR, 128), jnp.uint32),
        pltpu.SMEM((1,), jnp.int32),
        pltpu.VMEM((TM + 16, 128), F32),
        pltpu.VMEM((TM + 16, 128), F32),
        pltpu.VMEM((TM + 16, 128), F32),
        pltpu.VMEM((TM + 16, 128), F32),
        pltpu.VMEM((TM // 2, KC), jnp.uint32),
        pltpu.VMEM((TM // 2, KC), jnp.uint32),
        pltpu.SemaphoreType.DMA((N // TM,)),
        pltpu.SemaphoreType.DMA((len(weights),)),
        pltpu.SemaphoreType.DMA((N // TM,)),
    ]
    out = pl.pallas_call(
        functools.partial(_kernel, B=B, T=T, D=D, K=K),
        out_shape=jax.ShapeDtypeStruct((N, D), x.dtype),
        in_specs=[pl.BlockSpec(memory_space=pl.ANY)] * 12,
        out_specs=pl.BlockSpec(memory_space=pl.ANY),
        scratch_shapes=scratch,
        compiler_params=pltpu.CompilerParams(
            vmem_limit_bytes=120 * 1024 * 1024),
    )(x.reshape(N, D), *weights)
    return out.reshape(B, T, D)
```

```python
import functools
import math

import jax
import jax.numpy as jnp
from jax import lax
import jax.experimental.pallas as pl
import jax.experimental.pallas.tpu as pltpu

F32 = jnp.float32
BF16 = jnp.bfloat16

TM = 400
FC = 512
KC = 512
RB = 8
SB = 16
AB = 0
A_SLOTS = (1, 29)
B_SLOTS = (1, 60)
C_SLOTS = (6, 33)
SOFT = (0, 800)
PHASES = 'ABC'
MEM = 'pal'
ZR = 32
PU = 2
XW = 0
CT = 5
SW = None
WPAD = 128
QS = 4
BS = (80, 160, 240, 320)
PS = (320, 2)
WS = 1
FRB = 16
L0 = 3
LP = (0, 100, 3, 1)
OE = 0
EP = (0, 160, 288, 352, 400)
CS = (80, 160, 240, 320)
FS = (320, 2)
RC = (8, 8, 100)
RF = 8
F_END = 7
HALO = 8
EPS = 1e-05


def _ln(x, z=None):
    if z is None:
        m = jnp.mean(x, axis=-1, keepdims=True)
    else:
        t = z
        for c in range(x.shape[-1] // 128):
            t = t + x[:, c * 128:(c + 1) * 128]
        m = jnp.sum(t, axis=-1, keepdims=True) * (1.0 / x.shape[-1])
    xc = x - m
    v = jnp.mean(xc * xc, axis=-1, keepdims=True)
    return xc * lax.rsqrt(v + EPS)


def _silu(a):
    y = 0.5 * a
    return y + y * jnp.tanh(y)


def _dot(a, b):
    return jnp.dot(a, b, preferred_element_type=F32)


def _dot_nt(a, b):
    return lax.dot_general(a, b, (((1,), (1,)), ((), ())),
                           preferred_element_type=F32)


class _Anchor:
    def __init__(self, t, zero_v, zero_s):
        self.t, self.zero_v, self.zero_s = t, zero_v, zero_s

    def v(self):
        return pltpu.bitcast(
            pltpu.bitcast(self.t, jnp.uint32) & self.zero_v[0:8, :], F32)

    def s(self):
        return pltpu.bitcast(self.t, jnp.int32)[0, 0] & self.zero_s[0]


class _Sched:
    def __init__(self, zero_v, zero_s):
        self.zero_v, self.zero_s = zero_v, zero_s
        self.queue = []
        self.now = 0

    def add(self, items, t0, t1):
        assert t0 >= self.now
        n = len(items)
        self.queue += [(t0 + k * (t1 - t0) // n, it)
                       for k, it in enumerate(items)]
        self.queue.sort(key=lambda e: e[0])

    def anchor(self, t, r):
        return _Anchor(t[r:r + 8, :], self.zero_v, self.zero_s)

    def __call__(self, t):
        end = self.now + TM
        while self.queue and self.queue[0][0] < end:
            time, item = self.queue.pop(0)
            item(self.anchor(t, (time - self.now) // 8 * 8))
        self.now = end


def _rep(z, rows):
    return jnp.concatenate([z] * (rows // 8), axis=0)


def _ffn(h, wa_refs, wb_refs, sched, split=None):
    d = wb_refs[0].shape[1]
    acc = [None] * (d // 128)
    for c, (wa_ref, wb_ref) in enumerate(zip(wa_refs, wb_refs)):
        ss = []
        if c == 0 and split:
            r, nd = split
            top = [_dot(h[:r], wa_ref[:, n * 128:(n + 1) * 128])
                   for n in range(nd)]
            bot = [_dot(h[r:], wa_ref[:, n * 128:(n + 1) * 128])
                   for n in range(nd)]
            ss = [_silu(jnp.concatenate(tb, axis=0)) for tb in zip(top, bot)]
            sched.now += nd * TM
        for n in range(len(ss), FC // 128):
            a = _dot(h, wa_ref[:, n * 128:(n + 1) * 128])
            ss.append(_silu(a))
            sched(a)
        s = jnp.concatenate(ss, axis=1).astype(BF16)
        for n in range(d // 128):
            p = _dot(s, wb_ref[:, n * 128:(n + 1) * 128])
            acc[n] = p if acc[n] is None else acc[n] + p
            sched(p)
    return jnp.concatenate(acc, axis=1)


def _kernel(x_hbm, w1a_hbm, w1b_hbm, wq_hbm, wk_hbm, wv_hbm, wo_hbm,
            wp1_hbm, dw_hbm, wp2_hbm, w2a_hbm, w2b_hbm,
            out_hbm,
            xin, w1a, w1b, wq, wk, wv, wo, wp1, dw, wp2, w2a, w2b,
            mq, wvo, xs, hs, gs, dcs, st_mean, st_m2, bn, obuf,
            lhs_a, lhs_b, dwb, zero, zero_s, m_buf, l_buf, al_buf0, al_buf1,
            p_buf0, p_buf1,
            xsem, w1sem, wsem, osem,
            *, B, T, D, K):
    N = B * T
    TP = hs.shape[1]
    NCB = D // 128
    nt = N // TM
    tpb = T // TM

    def rows(i, r0=0, n=TM):
        return pl.ds(pl.multiple_of(i * TM, 16) + r0, n)

    def brows(i, r0=0, n=TM):
        return i // tpb, pl.ds(pl.multiple_of((i % tpb) * TM, 16) + r0, n)

    def col(c):
        if isinstance(c, int):
            return slice(c * 128, (c + 1) * 128)
        return pl.ds(pl.multiple_of(c * 128, 128), 128)

    def pieces(fn, i, rb=None):
        rb = rb or RB
        return [functools.partial(fn, i, r0, rb) for r0 in range(0, TM, rb)]

    def interleave(*lists):
        return [it for group in zip(*lists) for it in group]

    def x_copy(i):
        return pltpu.make_async_copy(x_hbm.at[rows(i), :],
                                     xin.at[rows(i), :], xsem.at[i])

    def o_copy(i):
        return pltpu.make_async_copy(obuf.at[rows(i), :],
                                     out_hbm.at[rows(i), :], osem.at[i])

    nfc = w1a.shape[0]

    def w1_copies(c):
        fs = pl.ds(pl.multiple_of(c * FC, FC), FC)
        return [pltpu.make_async_copy(w1a_hbm.at[:, fs], w1a.at[c],
                                      w1sem.at[0, c]),
                pltpu.make_async_copy(w1b_hbm.at[fs, :], w1b.at[c],
                                      w1sem.at[1, c])]

    w_pairs = [(wq_hbm, wq), (wk_hbm, wk),
               (wv_hbm, wv), (wo_hbm, wo), (wp1_hbm, wp1), (dw_hbm, dw),
               (wp2_hbm, wp2), (w2a_hbm, w2a), (w2b_hbm, w2b)]
    w_copies = [pltpu.make_async_copy(s, d.at[:, 0:s.shape[1]], wsem.at[j])
                for j, (s, d) in enumerate(w_pairs)]

    x_copy(0).start()
    for cp in w1_copies(0):
        cp.start()

    zero[...] = jnp.zeros(zero.shape, jnp.uint32)
    zero_s[0] = 0
    for b in range(B):
        hs[b, T:TP, :] = jnp.zeros((TP - T, D), BF16)
    for c in range(NCB):
        gs[1, c, 0:HALO, :] = jnp.zeros((HALO, 128), F32)
        gs[nt, c, HALO + TM:, :] = jnp.zeros((HALO, 128), F32)

    def zrep(z, n):
        return None if z is None else _rep(z.v(), n)

    def ln_in(i, r0=0, n=TM, z=None, dst=lhs_a):
        dst[pl.ds(r0, n), :] = _ln(xin[rows(i, r0, n), :].astype(F32),
                                   zrep(z, n)).astype(BF16)

    def ln_out(i, r0=0, n=TM, z=None):
        b, rb = brows(i, r0, n)
        hs[b, rb, :] = _ln(xs[rows(i, r0, n), :], zrep(z, n)).astype(BF16)

    x_copy(0).wait()
    ln_in(0, dst=lhs_b)
    xs[rows(0), :] = xin[rows(0), :].astype(F32)

    def rest_start():
        for j in range(3, nt):
            x_copy(j).start()
        for cp in w_copies:
            cp.start()

    def first_tile(c, carry):
        for cp in w1_copies(c):
            cp.wait()

        @pl.when(c == 1)
        def _():
            x_copy(1).wait()

        @pl.when(c + 1 < nfc)
        def _():
            for cp in w1_copies(c + 1):
                cp.start()

        @pl.when(c % 2 == 0)
        def _():
            x_copy(1 + c // 2).start()

        if WS == 2:
            pl.when(c == nfc - 1)(rest_start)

        n = -(-TM // (nfc - 1) // 16) * 16
        step = (TM - n) // (nfc - 2)
        assert step % 16 == 0 and step <= n
        r0 = pl.multiple_of(jnp.maximum(c - 1, 0) * step, 16)
        sched = _Sched(zero, zero_s)
        sched.add([functools.partial(ln_in, jnp.minimum(c, 1), r0 + r, FRB)
                   for r in range(0, n, FRB)], TM, F_END * TM)
        f = _ffn(lhs_b[...], [w1a.at[c]], [w1b.at[c]], sched)
        xs[rows(0), :] += 0.5 * f
        return carry

    lax.fori_loop(0, nfc, first_tile, 0)
    if WS != 2:
        rest_start()

    def phase_a(i, carry):
        if not XW:
            @pl.when(i + 1 < nt)
            def _():
                x_copy(i + 1).wait()
        h = lhs_a[...]
        items = interleave(pieces(ln_out, i - 1),
                           pieces(ln_in, jnp.minimum(i + 1, nt - 1)))
        sched = _Sched(zero, zero_s)
        sched.add(items, A_SLOTS[0] * TM, A_SLOTS[1] * TM)
        f = _ffn(h, [w1a.at[c] for c in range(nfc)],
                 [w1b.at[c] for c in range(nfc)], sched)
        xs[rows(i), :] = xin[rows(i), :].astype(F32) + 0.5 * f
        if XW:
            @pl.when(i + 2 < nt)
            def _():
                x_copy(i + 2).wait()
        return carry

    with jax.named_scope("phase_a"):
        if 'A' in PHASES:
            lax.fori_loop(1, nt, phase_a, 0)
        else:
            x_copy(1).wait()

    for cp in w_copies:
        cp.wait()

    qk_scale = (D ** -0.5) * math.log2(math.e)

    def q_cols(i, cs):
        b, rb = brows(i)
        lhs_a[:, cs] = _dot(hs[b, rb, :], mq[:, cs]).astype(BF16)

    def fold(u, carry):
        nr = TM // PU
        r0 = pl.multiple_of(u * nr, 8)
        sched = _Sched(zero, zero_s)
        assert nr % RF == 0
        sched.add([functools.partial(ln_out, nt - 1, r0 + r, RF)
                   for r in range(0, nr, RF)], 0, (2 * NCB // PU - 1) * TM)
        css = [pl.ds(pl.multiple_of((u * (NCB // PU) + c) * 128, 128), 128)
               for c in range(NCB // PU)]
        for cs in css:
            t = _dot_nt(wq[...], wk[cs, :])
            mq[:, cs] = (t * qk_scale).astype(BF16)
            sched(t)
        for cs in css:
            t = _dot(wv[...], wo[:, cs])
            wvo[:, cs] = t.astype(BF16)
            sched(t)
        for cs in css:
            if QS != 4:
                q_cols(0, cs)
        return carry

    lax.fori_loop(0, PU, fold, 0)
    dwf = dw[...].astype(F32)
    for k in range(K):
        dwb[k] = jnp.broadcast_to(dwf[k:k + 1, :], (8, D))

    def conv_block(p, r0, c, done, CT=CT, AT=K):
        cs = col(c)
        acc = [None]

        def item(k0, z=None):
            for k in range(k0, min(k0 + CT, K)):
                off = HALO - K // 2 + k + r0
                w = dwb[k, :, cs]
                if z is not None and k - k0 < AT:
                    w = w + z.v()
                t = gs[p + 1, c, off:off + 8, :] * w
                acc[0] = t if acc[0] is None else acc[0] + t
            if k0 + CT >= K:
                dcs[rows(p, r0, 8), cs] = acc[0]
                done(acc[0])

        return [functools.partial(item, k0) for k0 in range(0, K, CT)]

    def conv_main(p, cols=range(NCB), **kw):
        st = []

        def stats(r0, c, acc):
            if r0 == 0:
                st[:] = [acc, None, None]
                return
            shift, s1, s2 = st
            d = acc - shift
            s1 = d if s1 is None else s1 + d
            s2 = d * d if s2 is None else s2 + d * d
            st[:] = [shift, s1, s2]
            if r0 + 16 == TM:
                dm = s1 * (1.0 / (TM // 8 - 1))
                st_mean[p, :, col(c)] = shift + dm
                st_m2[p, :, col(c)] = s2 - s1 * dm

        return [it for c in cols for r0 in range(0, TM - 8, 8)
                for it in conv_block(p, r0, c,
                                     functools.partial(stats, r0, c), **kw)]

    def conv_edge(p, cols=range(NCB)):
        return [it for c in cols
                for it in conv_block(p, TM - 8, c, lambda acc: None)]

    nkc = TP // KC

    def phase_b(i, carry):
        b, rb = brows(i)
        inext = jnp.minimum(i + 1, nt - 1)
        sched = _Sched(zero, zero_s)
        sched.add(conv_edge(jnp.maximum(i - 2, 0))
                  + conv_main(jnp.maximum(i - 1, 0), range(L0, NCB)),
                  int(B_SLOTS[0] * TM), int(B_SLOTS[1] * TM))
        if QS == 4:
            qs = []
            for c in range(NCB):
                t = _dot(hs[b, rb, :], mq[:, col(c)])
                qs.append(t.astype(BF16))
                sched(t)
            q = jnp.concatenate(qs, axis=1)
        else:
            q = jnp.concatenate(
                [lhs_a[:, :D - 128],
                 _dot(hs[b, rb, :], mq[:, col(NCB - 1)]).astype(BF16)],
                axis=1)

        nsb = TM // SB
        dz = zero_s[0]
        p_buf, al_buf = (p_buf0, p_buf1), (al_buf0, al_buf1)

        def dyn(r0, n):
            return pl.ds(pl.multiple_of(dz + r0, 8), n)

        def scores(j):
            ss = []
            for n in range(KC // 128):
                lo = j * KC + n * 128
                s = _dot_nt(q, hs[b, lo:lo + 128, :])
                sched(s)
                if lo + 128 > T:
                    col = lax.broadcasted_iota(jnp.int32, (TM, 128), 1) + lo
                    s = jnp.where(col < T, s, -jnp.inf)
                ss.append(s)
            return ss

        m_v, l_v = [None] * nsb, [None] * nsb
        al_v = [[None] * nsb for _ in range(nkc)]
        p_v = [[None] * nsb for _ in range(nkc)]

        def soft(j, ss, k, z):
            rs = slice(k * SB, (k + 1) * SB)
            s = [t[rs, :] for t in ss]
            mj = functools.reduce(jnp.maximum, s[1:], s[0] + _rep(z.v(), SB))
            m_new = jnp.broadcast_to(jnp.max(mj, axis=-1, keepdims=True),
                                     (SB, 128))
            if j > 0:
                m_old = m_buf[dyn(k * SB, SB), :] if 'm' in MEM else m_v[k]
                m_new = jnp.maximum(m_old, m_new)
            p = [jnp.exp2(t - m_new) for t in s]
            ps = functools.reduce(jnp.add, p)
            if 'p' in MEM:
                pb = jnp.concatenate([t.astype(BF16) for t in p], axis=1)
                p_buf[j % 2][k * SB // 2:(k + 1) * SB // 2, :] = pltpu.bitcast(
                    pb, jnp.uint32)
            elif 'f' in MEM:
                p_v[j][k] = jnp.concatenate(p, axis=1)
            else:
                p_v[j][k] = jnp.concatenate(p, axis=1).astype(BF16)
            if j > 0:
                alpha = jnp.exp2(m_old - m_new)
                if 'a' in MEM:
                    al_buf[j % 2][rs, :] = alpha
                else:
                    al_v[j][k] = alpha
                l_old = l_buf[dyn(k * SB, SB), :] if 'l' in MEM else l_v[k]
                ps = l_old * alpha + ps
            if 'l' in MEM:
                l_buf[rs, :] = ps
            l_v[k] = ps
            if j + 1 < nkc and 'm' in MEM:
                m_buf[rs, :] = m_new
            m_v[k] = m_new

        def add_soft(j, ss, ndots):
            sched.add([functools.partial(soft, j, ss, k) for k in range(nsb)],
                      sched.now + SOFT[0], sched.now + ndots * TM - SOFT[1])

        def scores_soft(j):
            ss = scores(j)
            sched.add([functools.partial(soft, j, ss, k) for k in range(nsb)],
                      int(SW[j] * TM), int(SW[j + 1] * TM))

        acc = [None] * NCB
        nd = KC // 128
        if SW:
            scores_soft(0)
            scores_soft(1)
        else:
            add_soft(0, scores(0), nd)
        for j in range(nkc):
            if SW:
                if j + 2 < nkc:
                    scores_soft(j + 2)
            elif j + 1 < nkc:
                s_next = scores(j + 1)
                add_soft(j + 1, s_next, NCB + (nd if j + 2 < nkc else 0))
            if 'p' not in MEM:
                p_all = jnp.concatenate(p_v[j], axis=0).astype(BF16)
            if j > 0 and 'a' not in MEM:
                al = jnp.concatenate(al_v[j], axis=0)
            for n in range(NCB):
                if 'p' in MEM:
                    p_all = pltpu.bitcast(p_buf[j % 2][dyn(0, TM // 2), :],
                                          BF16)
                pv = _dot(p_all, hs[b, j * KC:(j + 1) * KC,
                                    n * 128:(n + 1) * 128])
                sched(pv)
                if j == 0:
                    acc[n] = pv
                else:
                    if 'a' in MEM:
                        al = al_buf[j % 2][dyn(0, TM), :]
                    if AB:
                        zs = [_rep(sched.anchor(pv, r).v(), AB)
                              for r in range(0, TM, AB)]
                        acc[n] = (acc[n] * (al + jnp.concatenate(zs, axis=0))
                                  + pv)
                    else:
                        acc[n] = acc[n] * al + pv
        acc = jnp.concatenate(acc, axis=1)
        if 'l' in MEM:
            l = l_buf[dyn(0, TM), :]
        else:
            l = jnp.concatenate(l_v, axis=0)
        if QS != 4:
            q_cols(inext, col(0))
        o = (acc * (1.0 / jnp.sum(l, axis=-1, keepdims=True))).astype(BF16)
        hh = []
        for r0, r1 in zip((0,) + BS, BS + (TM,)):
            x2 = jnp.concatenate(
                [xs[rows(i, r0, r1 - r0), col(c)]
                 + _dot(o[r0:r1], wvo[:, col(c)]) for c in range(NCB)], axis=1)
            xs[rows(i, r0, r1 - r0), :] = x2
            hh.append(_ln(x2).astype(BF16))
        if QS != 4:
            q_cols(inext, col(1))
            q_cols(inext, col(2))
        hn = jnp.concatenate(hh, axis=0)
        wcols = [slice(h * D + c * 128, h * D + (c + 1) * 128)
                 for c in range(NCB) for h in (1, 0)]
        r, nd = PS
        top = [_dot(hn[:r], wp1[:, cs]) for cs in wcols[:nd]]
        bot = [_dot(hn[r:], wp1[:, cs]) for cs in wcols[:nd]]
        u = [jnp.concatenate(tb, axis=0) for tb in zip(top, bot)]
        sched = _Sched(zero, zero_s)
        for c in range(NCB):
            while len(u) < 2 * c + 2:
                u.append(_dot(hn, wp1[:, wcols[len(u)]]))
                sched(u[-1])
            g = u[2 * c + 1] * (0.5 + 0.5 * jnp.tanh(0.5 * u[2 * c]))
            gs[i + 1, c, HALO:HALO + TM, :] = g
            gs[i, c, HALO + TM:, :] = jnp.where(i % tpb == 0, 0.0, g[:HALO])
            gs[i + 2, c, :HALO, :] = jnp.where(i % tpb == tpb - 1, 0.0,
                                               g[TM - HALO:])
            if c < L0:
                if LP:
                    sched.add(conv_main(i, [c], CT=LP[2], AT=LP[3]),
                              sched.now + LP[0],
                              sched.now + 2 * TM - LP[1])
                else:
                    for item in conv_main(i, [c]):
                        item()
        return carry

    with jax.named_scope("phase_b"):
        if 'B' in PHASES:
            lax.fori_loop(0, nt, phase_b, 0)
    def conv_tail(c, carry):
        for item in conv_main(nt - 1, [c]):
            item()
        return carry

    if L0 < NCB - 1:
        lax.fori_loop(L0, NCB, conv_tail, 0)
    else:
        conv_tail(NCB - 1, 0)
    for item in conv_edge(nt - 2) + conv_edge(nt - 1):
        item()

    ng = TM // 8 - 1
    means = st_mean[...].reshape(nt * 8, D)
    edges = jnp.concatenate([dcs[(p + 1) * TM - 8:(p + 1) * TM, :]
                             for p in range(nt)], axis=0)
    mu = jnp.sum(ng * means + edges, axis=0, keepdims=True) * (1.0 / N)
    dm = means - mu
    de = edges - mu
    var = jnp.sum(st_m2[...].reshape(nt * 8, D) + ng * (dm * dm) + de * de,
                  axis=0, keepdims=True) * (1.0 / N)
    rstd = lax.rsqrt(var + EPS)
    bn[0] = jnp.broadcast_to(mu, (8, D))
    bn[1] = jnp.broadcast_to(rstd, (8, D))

    def bn_silu(i, r0=0, n=TM, z=None):
        mu = bn[0]
        if z is not None:
            mu = mu + jnp.concatenate([z.v()] * NCB, axis=1)
        d = dcs[rows(i, r0, n), :].reshape(n // 8, 8, D)
        y = ((d - mu[None]) * bn[1][None]).reshape(n, D)
        lhs_b[r0:r0 + n, :] = _silu(y).astype(BF16)

    def pw2(i, isrc, sched=None):
        lhs = lhs_b[...]
        for c in range(NCB):
            cs = slice(c * 128, (c + 1) * 128)
            t = _dot(lhs, wp2[:, cs])
            dcs[rows(i), cs] = xs[rows(isrc), cs] + t
            if sched is not None:
                sched(t)

    def ln_mid(i, r0=0, n=TM, z=None):
        lhs_a[r0:r0 + n, :] = _ln(dcs[rows(i, r0, n), :],
                                  zrep(z, n)).astype(BF16)

    def ln_final(i, r0=0, n=TM, z=None):
        obuf[rows(i, r0, n), :] = _ln(xs[rows(i, r0, n), :],
                                      zrep(z, n)).astype(BF16)

    bn_silu(0)
    if not CS:
        pw2(0, 0)
        ln_mid(0)
        bn_silu(1)

    def phase_c(i, carry):
        def o_start(z):
            @pl.when(i >= 2 - OE)
            def _():
                o_copy(i - 2 + OE).start()

        sched = _Sched(zero, zero_s)
        if OE:
            sched.add([o_start], C_SLOTS[1] * TM, C_SLOTS[1] * TM)
        else:
            o_start(None)
        if CS:
            sched.add(pieces(ln_final, jnp.maximum(i - 1, 0), RC[0]),
                      C_SLOTS[0] * TM, C_SLOTS[1] * TM)
            sched.add(pieces(bn_silu, jnp.minimum(i + 1, nt - 1), RC[1]),
                      C_SLOTS[0] * TM + RC[2], C_SLOTS[1] * TM + RC[2])
            hh = []
            for r0, r1 in zip((0,) + CS, CS + (TM,)):
                lhs = lhs_b[r0:r1, :]
                x3 = jnp.concatenate(
                    [xs[rows(i, r0, r1 - r0), col(c)]
                     + _dot(lhs, wp2[:, col(c)]) for c in range(NCB)], axis=1)
                xs[rows(i, r0, r1 - r0), :] = x3
                hh.append(_ln(x3).astype(BF16))
            sched.now = NCB * TM
            h = jnp.concatenate(hh, axis=0)
        else:
            h = lhs_a[...]
            items = interleave(pieces(ln_final, jnp.maximum(i - 1, 0)),
                               pieces(bn_silu, jnp.minimum(i + 2, nt - 1)),
                               pieces(ln_mid, i + 1))
            sched.add(items, C_SLOTS[0] * TM, C_SLOTS[1] * TM)
            pw2(i + 1, jnp.minimum(i + 1, nt - 1), sched)
        f = _ffn(h, [w2a.at[:, c * FC:(c + 1) * FC] for c in range(nfc)],
                 [w2b.at[c * FC:(c + 1) * FC, :] for c in range(nfc)], sched,
                 FS)
        if CS:
            xs[rows(i), :] += 0.5 * f
        else:
            xs[rows(i), :] = dcs[rows(i), :] + 0.5 * f
        return carry

    with jax.named_scope("phase_c"):
        if 'C' in PHASES:
            lax.fori_loop(0, nt, phase_c, 0)
        else:
            for i in range(nt - 2):
                o_copy(i).start()
    if not OE:
        o_copy(nt - 2).start()
    last = []
    for k, (r0, r1) in enumerate(zip(EP[:-1], EP[1:])):
        ln_final(nt - 1, r0, r1 - r0)
        rs = rows(nt - 1, r0, r1 - r0)
        last.append(pltpu.make_async_copy(obuf.at[rs, :], out_hbm.at[rs, :],
                                          osem.at[nt - 1 + k]))
        last[-1].start()
    for i in range(nt - 1):
        o_copy(i).wait()
    for cp in last:
        cp.wait()


@jax.jit
def pallas_standalone__conformer_family_conformer__speech_kernel(
    x: jax.Array,
    w_ff1_a: jax.Array,
    w_ff1_b: jax.Array,
    w_q: jax.Array,
    w_k: jax.Array,
    w_v: jax.Array,
    w_o: jax.Array,
    w_pw1: jax.Array,
    dw: jax.Array,
    w_pw2: jax.Array,
    w_ff2_a: jax.Array,
    w_ff2_b: jax.Array,
):
    B, T, D = x.shape
    K = dw.shape[0]
    N = B * T
    TP = -(-T // KC) * KC
    weights = (w_ff1_a, w_ff1_b, w_q, w_k, w_v, w_o, w_pw1, dw, w_pw2,
               w_ff2_a, w_ff2_b)
    scratch = [pltpu.VMEM((N, D), BF16)]
    nfc = w_ff1_a.shape[1] // FC
    scratch += [pltpu.VMEM((nfc, D, FC), BF16), pltpu.VMEM((nfc, FC, D), BF16)]
    scratch += [pltpu.VMEM((w.shape[0], w.shape[1]
                            + (WPAD if w.shape[1] > D else 0)), w.dtype)
                for w in weights[2:]]
    scratch += [
        pltpu.VMEM((D, D), BF16),
        pltpu.VMEM((D, D), BF16),
        pltpu.VMEM((N, D), F32),
        pltpu.VMEM((B, TP, D), BF16),
        pltpu.VMEM((N // TM + 2, D // 128, TM + 2 * HALO, 128), F32),
        pltpu.VMEM((N + TM, D), F32),
        pltpu.VMEM((N // TM, 8, D), F32),
        pltpu.VMEM((N // TM, 8, D), F32),
        pltpu.VMEM((2, 8, D), F32),
        pltpu.VMEM((N, D), BF16),
        pltpu.VMEM((TM, D), BF16),
        pltpu.VMEM((TM, D), BF16),
        pltpu.VMEM((K, 8, D), F32),
        pltpu.VMEM((ZR, 128), jnp.uint32),
        pltpu.SMEM((1,), jnp.int32),
        pltpu.VMEM((TM + 16, 128), F32),
        pltpu.VMEM((TM + 16, 128), F32),
        pltpu.VMEM((TM + 16, 128), F32),
        pltpu.VMEM((TM + 16, 128), F32),
        pltpu.VMEM((TM // 2, KC), jnp.uint32),
        pltpu.VMEM((TM // 2, KC), jnp.uint32),
        pltpu.SemaphoreType.DMA((N // TM,)),
        pltpu.SemaphoreType.DMA((2, nfc)),
        pltpu.SemaphoreType.DMA((len(weights) - 2,)),
        pltpu.SemaphoreType.DMA((N // TM + len(EP),)),
    ]
    out = pl.pallas_call(
        functools.partial(_kernel, B=B, T=T, D=D, K=K),
        out_shape=jax.ShapeDtypeStruct((N, D), x.dtype),
        in_specs=[pl.BlockSpec(memory_space=pl.ANY)] * 12,
        out_specs=pl.BlockSpec(memory_space=pl.ANY),
        scratch_shapes=scratch,
        compiler_params=pltpu.CompilerParams(
            vmem_limit_bytes=120 * 1024 * 1024),
    )(x.reshape(N, D), *weights)
    return out.reshape(B, T, D)
```

```python
import functools
import math

import jax
import jax.numpy as jnp
from jax import lax
import jax.experimental.pallas as pl
import jax.experimental.pallas.tpu as pltpu

F32 = jnp.float32
BF16 = jnp.bfloat16

TM = 400
FC = 512
KC = 512
RB = 8
SB = 16
A_SLOTS = (1, 29)
B_SLOTS = (1, 60)
C_SLOTS = (6, 33)
SOFT = (0, 800)
F_END = 7
ZR = 32
PU = 2
CT = 5
WPAD = 128
BS = (80, 160, 240, 320)
PS = (320, 2)
FRB = 16
L0 = 3
LP = (0, 100, 3, 1)
EP = (0, 160, 288, 352, 400)
CS = (80, 160, 240, 320)
FS = (320, 2)
RC = (8, 8, 100)
RF = 8
HALO = 8
EPS = 1e-05


def _ln(x, z=None):
    if z is None:
        m = jnp.mean(x, axis=-1, keepdims=True)
    else:
        t = z
        for c in range(x.shape[-1] // 128):
            t = t + x[:, c * 128:(c + 1) * 128]
        m = jnp.sum(t, axis=-1, keepdims=True) * (1.0 / x.shape[-1])
    xc = x - m
    v = jnp.mean(xc * xc, axis=-1, keepdims=True)
    return xc * lax.rsqrt(v + EPS)


def _silu(a):
    y = 0.5 * a
    return y + y * jnp.tanh(y)


def _dot(a, b):
    return jnp.dot(a, b, preferred_element_type=F32)


def _dot_nt(a, b):
    return lax.dot_general(a, b, (((1,), (1,)), ((), ())),
                           preferred_element_type=F32)


class _Anchor:
    def __init__(self, t, zero_v):
        self.t, self.zero_v = t, zero_v

    def v(self):
        return pltpu.bitcast(
            pltpu.bitcast(self.t, jnp.uint32) & self.zero_v[0:8, :], F32)


class _Sched:
    def __init__(self, zero_v):
        self.zero_v = zero_v
        self.queue = []
        self.now = 0

    def add(self, items, t0, t1):
        assert t0 >= self.now
        n = len(items)
        self.queue += [(t0 + k * (t1 - t0) // n, it)
                       for k, it in enumerate(items)]
        self.queue.sort(key=lambda e: e[0])

    def __call__(self, t):
        end = self.now + TM
        while self.queue and self.queue[0][0] < end:
            time, item = self.queue.pop(0)
            r = (time - self.now) // 8 * 8
            item(_Anchor(t[r:r + 8, :], self.zero_v))
        self.now = end


def _rep(z, rows):
    return jnp.concatenate([z] * (rows // 8), axis=0)


def _ffn(h, wa_refs, wb_refs, sched, split=None):
    d = wb_refs[0].shape[1]
    acc = [None] * (d // 128)
    for c, (wa_ref, wb_ref) in enumerate(zip(wa_refs, wb_refs)):
        ss = []
        if c == 0 and split:
            r, nd = split
            top = [_dot(h[:r], wa_ref[:, n * 128:(n + 1) * 128])
                   for n in range(nd)]
            bot = [_dot(h[r:], wa_ref[:, n * 128:(n + 1) * 128])
                   for n in range(nd)]
            ss = [_silu(jnp.concatenate(tb, axis=0)) for tb in zip(top, bot)]
            sched.now += nd * TM
        for n in range(len(ss), FC // 128):
            a = _dot(h, wa_ref[:, n * 128:(n + 1) * 128])
            ss.append(_silu(a))
            sched(a)
        s = jnp.concatenate(ss, axis=1).astype(BF16)
        for n in range(d // 128):
            p = _dot(s, wb_ref[:, n * 128:(n + 1) * 128])
            acc[n] = p if acc[n] is None else acc[n] + p
            sched(p)
    return jnp.concatenate(acc, axis=1)


def _kernel(x_hbm, w1a_hbm, w1b_hbm, wq_hbm, wk_hbm, wv_hbm, wo_hbm,
            wp1_hbm, dw_hbm, wp2_hbm, w2a_hbm, w2b_hbm,
            out_hbm,
            xin, w1a, w1b, wq, wk, wv, wo, wp1, dw, wp2, w2a, w2b,
            mq, wvo, xs, hs, gs, dcs, st_mean, st_m2, bn, obuf,
            lhs_a, lhs_b, dwb, zero, zero_s, l_buf, al_buf0, al_buf1,
            p_buf0, p_buf1,
            xsem, w1sem, wsem, osem,
            *, B, T, D, K):
    N = B * T
    TP = hs.shape[1]
    NCB = D // 128
    nt = N // TM
    tpb = T // TM

    def rows(i, r0=0, n=TM):
        return pl.ds(pl.multiple_of(i * TM, 16) + r0, n)

    def brows(i, r0=0, n=TM):
        return i // tpb, pl.ds(pl.multiple_of((i % tpb) * TM, 16) + r0, n)

    def col(c):
        if isinstance(c, int):
            return slice(c * 128, (c + 1) * 128)
        return pl.ds(pl.multiple_of(c * 128, 128), 128)

    def pieces(fn, i, rb=None):
        rb = rb or RB
        return [functools.partial(fn, i, r0, rb) for r0 in range(0, TM, rb)]

    def interleave(*lists):
        return [it for group in zip(*lists) for it in group]

    def x_copy(i):
        return pltpu.make_async_copy(x_hbm.at[rows(i), :],
                                     xin.at[rows(i), :], xsem.at[i])

    def o_copy(i):
        return pltpu.make_async_copy(obuf.at[rows(i), :],
                                     out_hbm.at[rows(i), :], osem.at[i])

    nfc = w1a.shape[0]

    def w1_copies(c):
        fs = pl.ds(pl.multiple_of(c * FC, FC), FC)
        return [pltpu.make_async_copy(w1a_hbm.at[:, fs], w1a.at[c],
                                      w1sem.at[0, c]),
                pltpu.make_async_copy(w1b_hbm.at[fs, :], w1b.at[c],
                                      w1sem.at[1, c])]

    w_pairs = [(wq_hbm, wq), (wk_hbm, wk),
               (wv_hbm, wv), (wo_hbm, wo), (wp1_hbm, wp1), (dw_hbm, dw),
               (wp2_hbm, wp2), (w2a_hbm, w2a), (w2b_hbm, w2b)]
    w_copies = [pltpu.make_async_copy(s, d.at[:, 0:s.shape[1]], wsem.at[j])
                for j, (s, d) in enumerate(w_pairs)]

    x_copy(0).start()
    for cp in w1_copies(0):
        cp.start()

    zero[...] = jnp.zeros(zero.shape, jnp.uint32)
    zero_s[0] = 0
    for b in range(B):
        hs[b, T:TP, :] = jnp.zeros((TP - T, D), BF16)
    for c in range(NCB):
        gs[1, c, 0:HALO, :] = jnp.zeros((HALO, 128), F32)
        gs[nt, c, HALO + TM:, :] = jnp.zeros((HALO, 128), F32)

    def zrep(z, n):
        return None if z is None else _rep(z.v(), n)

    def ln_in(i, r0=0, n=TM, z=None, dst=lhs_a):
        dst[pl.ds(r0, n), :] = _ln(xin[rows(i, r0, n), :].astype(F32),
                                   zrep(z, n)).astype(BF16)

    def ln_out(i, r0=0, n=TM, z=None):
        b, rb = brows(i, r0, n)
        hs[b, rb, :] = _ln(xs[rows(i, r0, n), :], zrep(z, n)).astype(BF16)

    x_copy(0).wait()
    ln_in(0, dst=lhs_b)
    xs[rows(0), :] = xin[rows(0), :].astype(F32)

    def first_tile(c, carry):
        for cp in w1_copies(c):
            cp.wait()

        @pl.when(c == 1)
        def _():
            x_copy(1).wait()

        @pl.when(c + 1 < nfc)
        def _():
            for cp in w1_copies(c + 1):
                cp.start()

        @pl.when(c % 2 == 0)
        def _():
            x_copy(1 + c // 2).start()

        n = -(-TM // (nfc - 1) // 16) * 16
        step = (TM - n) // (nfc - 2)
        assert step % 16 == 0 and step <= n
        r0 = pl.multiple_of(jnp.maximum(c - 1, 0) * step, 16)
        sched = _Sched(zero)
        sched.add([functools.partial(ln_in, jnp.minimum(c, 1), r0 + r, FRB)
                   for r in range(0, n, FRB)], TM, F_END * TM)
        f = _ffn(lhs_b[...], [w1a.at[c]], [w1b.at[c]], sched)
        xs[rows(0), :] += 0.5 * f
        return carry

    lax.fori_loop(0, nfc, first_tile, 0)
    for j in range(3, nt):
        x_copy(j).start()
    for cp in w_copies:
        cp.start()

    def phase_a(i, carry):
        @pl.when(i + 1 < nt)
        def _():
            x_copy(i + 1).wait()

        h = lhs_a[...]
        items = interleave(pieces(ln_out, i - 1),
                           pieces(ln_in, jnp.minimum(i + 1, nt - 1)))
        sched = _Sched(zero)
        sched.add(items, A_SLOTS[0] * TM, A_SLOTS[1] * TM)
        f = _ffn(h, [w1a.at[c] for c in range(nfc)],
                 [w1b.at[c] for c in range(nfc)], sched)
        xs[rows(i), :] = xin[rows(i), :].astype(F32) + 0.5 * f
        return carry

    with jax.named_scope("phase_a"):
        lax.fori_loop(1, nt, phase_a, 0)

    for cp in w_copies:
        cp.wait()

    qk_scale = (D ** -0.5) * math.log2(math.e)

    def fold(u, carry):
        nr = TM // PU
        r0 = pl.multiple_of(u * nr, 8)
        sched = _Sched(zero)
        assert nr % RF == 0
        sched.add([functools.partial(ln_out, nt - 1, r0 + r, RF)
                   for r in range(0, nr, RF)], 0, (2 * NCB // PU - 1) * TM)
        css = [pl.ds(pl.multiple_of((u * (NCB // PU) + c) * 128, 128), 128)
               for c in range(NCB // PU)]
        for cs in css:
            t = _dot_nt(wq[...], wk[cs, :])
            mq[:, cs] = (t * qk_scale).astype(BF16)
            sched(t)
        for cs in css:
            t = _dot(wv[...], wo[:, cs])
            wvo[:, cs] = t.astype(BF16)
            sched(t)
        return carry

    lax.fori_loop(0, PU, fold, 0)
    dwf = dw[...].astype(F32)
    for k in range(K):
        dwb[k] = jnp.broadcast_to(dwf[k:k + 1, :], (8, D))

    def conv_block(p, r0, c, done, CT=CT, AT=K):
        cs = col(c)
        acc = [None]

        def item(k0, z=None):
            for k in range(k0, min(k0 + CT, K)):
                off = HALO - K // 2 + k + r0
                w = dwb[k, :, cs]
                if z is not None and k - k0 < AT:
                    w = w + z.v()
                t = gs[p + 1, c, off:off + 8, :] * w
                acc[0] = t if acc[0] is None else acc[0] + t
            if k0 + CT >= K:
                dcs[rows(p, r0, 8), cs] = acc[0]
                done(acc[0])

        return [functools.partial(item, k0) for k0 in range(0, K, CT)]

    def conv_main(p, cols=range(NCB), **kw):
        st = []

        def stats(r0, c, acc):
            if r0 == 0:
                st[:] = [acc, None, None]
                return
            shift, s1, s2 = st
            d = acc - shift
            s1 = d if s1 is None else s1 + d
            s2 = d * d if s2 is None else s2 + d * d
            st[:] = [shift, s1, s2]
            if r0 + 16 == TM:
                dm = s1 * (1.0 / (TM // 8 - 1))
                st_mean[p, :, col(c)] = shift + dm
                st_m2[p, :, col(c)] = s2 - s1 * dm

        return [it for c in cols for r0 in range(0, TM - 8, 8)
                for it in conv_block(p, r0, c,
                                     functools.partial(stats, r0, c), **kw)]

    def conv_edge(p, cols=range(NCB)):
        return [it for c in cols
                for it in conv_block(p, TM - 8, c, lambda acc: None)]

    nkc = TP // KC

    def phase_b(i, carry):
        b, rb = brows(i)
        sched = _Sched(zero)
        sched.add(conv_edge(jnp.maximum(i - 2, 0))
                  + conv_main(jnp.maximum(i - 1, 0), range(L0, NCB)),
                  int(B_SLOTS[0] * TM), int(B_SLOTS[1] * TM))
        qs = []
        for c in range(NCB):
            t = _dot(hs[b, rb, :], mq[:, col(c)])
            qs.append(t.astype(BF16))
            sched(t)
        q = jnp.concatenate(qs, axis=1)

        nsb = TM // SB
        dz = zero_s[0]
        p_buf, al_buf = (p_buf0, p_buf1), (al_buf0, al_buf1)

        def dyn(r0, n):
            return pl.ds(pl.multiple_of(dz + r0, 8), n)

        def scores(j):
            ss = []
            for n in range(KC // 128):
                lo = j * KC + n * 128
                s = _dot_nt(q, hs[b, lo:lo + 128, :])
                sched(s)
                if lo + 128 > T:
                    col = lax.broadcasted_iota(jnp.int32, (TM, 128), 1) + lo
                    s = jnp.where(col < T, s, -jnp.inf)
                ss.append(s)
            return ss

        m_v = [None] * nsb

        def soft(j, ss, k, z):
            rs = slice(k * SB, (k + 1) * SB)
            s = [t[rs, :] for t in ss]
            mj = functools.reduce(jnp.maximum, s[1:], s[0] + _rep(z.v(), SB))
            m_new = jnp.broadcast_to(jnp.max(mj, axis=-1, keepdims=True),
                                     (SB, 128))
            if j > 0:
                m_old = m_v[k]
                m_new = jnp.maximum(m_old, m_new)
            p = [jnp.exp2(t - m_new) for t in s]
            ps = functools.reduce(jnp.add, p)
            pb = jnp.concatenate([t.astype(BF16) for t in p], axis=1)
            p_buf[j % 2][k * SB // 2:(k + 1) * SB // 2, :] = pltpu.bitcast(
                pb, jnp.uint32)
            if j > 0:
                alpha = jnp.exp2(m_old - m_new)
                al_buf[j % 2][rs, :] = alpha
                ps = l_buf[dyn(k * SB, SB), :] * alpha + ps
            l_buf[rs, :] = ps
            m_v[k] = m_new

        def add_soft(j, ss, ndots):
            sched.add([functools.partial(soft, j, ss, k) for k in range(nsb)],
                      sched.now + SOFT[0], sched.now + ndots * TM - SOFT[1])

        acc = [None] * NCB
        nd = KC // 128
        add_soft(0, scores(0), nd)
        for j in range(nkc):
            if j + 1 < nkc:
                s_next = scores(j + 1)
                add_soft(j + 1, s_next, NCB + (nd if j + 2 < nkc else 0))
            for n in range(NCB):
                p_all = pltpu.bitcast(p_buf[j % 2][dyn(0, TM // 2), :], BF16)
                pv = _dot(p_all, hs[b, j * KC:(j + 1) * KC,
                                    n * 128:(n + 1) * 128])
                sched(pv)
                if j == 0:
                    acc[n] = pv
                else:
                    acc[n] = acc[n] * al_buf[j % 2][dyn(0, TM), :] + pv
        assert not sched.queue
        acc = jnp.concatenate(acc, axis=1)
        l = l_buf[dyn(0, TM), :]
        o = (acc * (1.0 / jnp.sum(l, axis=-1, keepdims=True))).astype(BF16)
        hh = []
        for r0, r1 in zip((0,) + BS, BS + (TM,)):
            x2 = jnp.concatenate(
                [xs[rows(i, r0, r1 - r0), col(c)]
                 + _dot(o[r0:r1], wvo[:, col(c)]) for c in range(NCB)], axis=1)
            xs[rows(i, r0, r1 - r0), :] = x2
            hh.append(_ln(x2).astype(BF16))
        hn = jnp.concatenate(hh, axis=0)
        wcols = [slice(h * D + c * 128, h * D + (c + 1) * 128)
                 for c in range(NCB) for h in (1, 0)]
        r, nd = PS
        top = [_dot(hn[:r], wp1[:, cs]) for cs in wcols[:nd]]
        bot = [_dot(hn[r:], wp1[:, cs]) for cs in wcols[:nd]]
        u = [jnp.concatenate(tb, axis=0) for tb in zip(top, bot)]
        sched = _Sched(zero)
        for c in range(NCB):
            while len(u) < 2 * c + 2:
                u.append(_dot(hn, wp1[:, wcols[len(u)]]))
                sched(u[-1])
            g = u[2 * c + 1] * (0.5 + 0.5 * jnp.tanh(0.5 * u[2 * c]))
            gs[i + 1, c, HALO:HALO + TM, :] = g
            gs[i, c, HALO + TM:, :] = jnp.where(i % tpb == 0, 0.0, g[:HALO])
            gs[i + 2, c, :HALO, :] = jnp.where(i % tpb == tpb - 1, 0.0,
                                               g[TM - HALO:])
            if c < L0:
                sched.add(conv_main(i, [c], CT=LP[2], AT=LP[3]),
                          sched.now + LP[0], sched.now + 2 * TM - LP[1])
        assert not sched.queue
        return carry

    with jax.named_scope("phase_b"):
        lax.fori_loop(0, nt, phase_b, 0)
    for item in (conv_main(nt - 1, range(L0, NCB)) + conv_edge(nt - 2)
                 + conv_edge(nt - 1)):
        item()

    ng = TM // 8 - 1
    means = st_mean[...].reshape(nt * 8, D)
    edges = jnp.concatenate([dcs[(p + 1) * TM - 8:(p + 1) * TM, :]
                             for p in range(nt)], axis=0)
    mu = jnp.sum(ng * means + edges, axis=0, keepdims=True) * (1.0 / N)
    dm = means - mu
    de = edges - mu
    var = jnp.sum(st_m2[...].reshape(nt * 8, D) + ng * (dm * dm) + de * de,
                  axis=0, keepdims=True) * (1.0 / N)
    rstd = lax.rsqrt(var + EPS)
    bn[0] = jnp.broadcast_to(mu, (8, D))
    bn[1] = jnp.broadcast_to(rstd, (8, D))

    def bn_silu(i, r0=0, n=TM, z=None):
        mu = bn[0]
        if z is not None:
            mu = mu + jnp.concatenate([z.v()] * NCB, axis=1)
        d = dcs[rows(i, r0, n), :].reshape(n // 8, 8, D)
        y = ((d - mu[None]) * bn[1][None]).reshape(n, D)
        lhs_b[r0:r0 + n, :] = _silu(y).astype(BF16)

    def ln_final(i, r0=0, n=TM, z=None):
        obuf[rows(i, r0, n), :] = _ln(xs[rows(i, r0, n), :],
                                      zrep(z, n)).astype(BF16)

    bn_silu(0)

    def phase_c(i, carry):
        @pl.when(i >= 2)
        def _():
            o_copy(i - 2).start()

        sched = _Sched(zero)
        sched.add(pieces(ln_final, jnp.maximum(i - 1, 0), RC[0]),
                  C_SLOTS[0] * TM, C_SLOTS[1] * TM)
        sched.add(pieces(bn_silu, jnp.minimum(i + 1, nt - 1), RC[1]),
                  C_SLOTS[0] * TM + RC[2], C_SLOTS[1] * TM + RC[2])
        hh = []
        for r0, r1 in zip((0,) + CS, CS + (TM,)):
            lhs = lhs_b[r0:r1, :]
            x3 = jnp.concatenate(
                [xs[rows(i, r0, r1 - r0), col(c)]
                 + _dot(lhs, wp2[:, col(c)]) for c in range(NCB)], axis=1)
            xs[rows(i, r0, r1 - r0), :] = x3
            hh.append(_ln(x3).astype(BF16))
        sched.now = NCB * TM
        h = jnp.concatenate(hh, axis=0)
        f = _ffn(h, [w2a.at[:, c * FC:(c + 1) * FC] for c in range(nfc)],
                 [w2b.at[c * FC:(c + 1) * FC, :] for c in range(nfc)], sched,
                 FS)
        assert not sched.queue
        xs[rows(i), :] += 0.5 * f
        return carry

    with jax.named_scope("phase_c"):
        lax.fori_loop(0, nt, phase_c, 0)
    o_copy(nt - 2).start()
    last = []
    for k, (r0, r1) in enumerate(zip(EP[:-1], EP[1:])):
        ln_final(nt - 1, r0, r1 - r0)
        rs = rows(nt - 1, r0, r1 - r0)
        last.append(pltpu.make_async_copy(obuf.at[rs, :], out_hbm.at[rs, :],
                                          osem.at[nt - 1 + k]))
        last[-1].start()
    for i in range(nt - 1):
        o_copy(i).wait()
    for cp in last:
        cp.wait()


@jax.jit
def pallas_standalone__conformer_family_conformer__speech_kernel(
    x: jax.Array,
    w_ff1_a: jax.Array,
    w_ff1_b: jax.Array,
    w_q: jax.Array,
    w_k: jax.Array,
    w_v: jax.Array,
    w_o: jax.Array,
    w_pw1: jax.Array,
    dw: jax.Array,
    w_pw2: jax.Array,
    w_ff2_a: jax.Array,
    w_ff2_b: jax.Array,
):
    B, T, D = x.shape
    K = dw.shape[0]
    N = B * T
    TP = -(-T // KC) * KC
    weights = (w_ff1_a, w_ff1_b, w_q, w_k, w_v, w_o, w_pw1, dw, w_pw2,
               w_ff2_a, w_ff2_b)
    scratch = [pltpu.VMEM((N, D), BF16)]
    nfc = w_ff1_a.shape[1] // FC
    scratch += [pltpu.VMEM((nfc, D, FC), BF16), pltpu.VMEM((nfc, FC, D), BF16)]
    scratch += [pltpu.VMEM((w.shape[0], w.shape[1]
                            + (WPAD if w.shape[1] > D else 0)), w.dtype)
                for w in weights[2:]]
    scratch += [
        pltpu.VMEM((D, D), BF16),
        pltpu.VMEM((D, D), BF16),
        pltpu.VMEM((N, D), F32),
        pltpu.VMEM((B, TP, D), BF16),
        pltpu.VMEM((N // TM + 2, D // 128, TM + 2 * HALO, 128), F32),
        pltpu.VMEM((N, D), F32),
        pltpu.VMEM((N // TM, 8, D), F32),
        pltpu.VMEM((N // TM, 8, D), F32),
        pltpu.VMEM((2, 8, D), F32),
        pltpu.VMEM((N, D), BF16),
        pltpu.VMEM((TM, D), BF16),
        pltpu.VMEM((TM, D), BF16),
        pltpu.VMEM((K, 8, D), F32),
        pltpu.VMEM((ZR, 128), jnp.uint32),
        pltpu.SMEM((1,), jnp.int32),
        pltpu.VMEM((TM + 16, 128), F32),
        pltpu.VMEM((TM + 16, 128), F32),
        pltpu.VMEM((TM + 16, 128), F32),
        pltpu.VMEM((TM // 2, KC), jnp.uint32),
        pltpu.VMEM((TM // 2, KC), jnp.uint32),
        pltpu.SemaphoreType.DMA((N // TM,)),
        pltpu.SemaphoreType.DMA((2, nfc)),
        pltpu.SemaphoreType.DMA((len(weights) - 2,)),
        pltpu.SemaphoreType.DMA((N // TM + len(EP),)),
    ]
    out = pl.pallas_call(
        functools.partial(_kernel, B=B, T=T, D=D, K=K),
        out_shape=jax.ShapeDtypeStruct((N, D), x.dtype),
        in_specs=[pl.BlockSpec(memory_space=pl.ANY)] * 12,
        out_specs=pl.BlockSpec(memory_space=pl.ANY),
        scratch_shapes=scratch,
        compiler_params=pltpu.CompilerParams(
            vmem_limit_bytes=120 * 1024 * 1024),
    )(x.reshape(N, D), *weights)
    return out.reshape(B, T, D)
```

```python
import functools
import math

import jax
import jax.numpy as jnp
from jax import lax
import jax.experimental.pallas as pl
import jax.experimental.pallas.tpu as pltpu

F32 = jnp.float32
BF16 = jnp.bfloat16

TM = 400
FC = 512
KC = 512
RB = 8
SB = 16
A_SLOTS = (1, 29)
B_SLOTS = (1, 60)
C_SLOTS = (6, 33)
SOFT = (0, 800)
F_END = 7
ZR = 32
PU = 2
CT = 5
WPAD = 128
BS = (80, 160, 240, 320)
PS = (320, 2)
FRB = 16
L0 = 3
LP = (0, 100, 3, 1)
EP = (0, 160, 288, 352, 400)
CS = (80, 160, 240, 320)
FS = (320, 2)
RC = (8, 8, 100)
RF = 8
RT = (0, 0)
TX = 1
HALO = 8
EPS = 1e-05


def _ln(x, z=None):
    if z is None:
        m = jnp.mean(x, axis=-1, keepdims=True)
    else:
        t = z
        for c in range(x.shape[-1] // 128):
            t = t + x[:, c * 128:(c + 1) * 128]
        m = jnp.sum(t, axis=-1, keepdims=True) * (1.0 / x.shape[-1])
    xc = x - m
    v = jnp.mean(xc * xc, axis=-1, keepdims=True)
    return xc * lax.rsqrt(v + EPS)


def _silu(a):
    y = 0.5 * a
    return y + y * jnp.tanh(y)


def _dot(a, b):
    return jnp.dot(a, b, preferred_element_type=F32)


def _dot_nt(a, b):
    return lax.dot_general(a, b, (((1,), (1,)), ((), ())),
                           preferred_element_type=F32)


class _Anchor:
    def __init__(self, t, zero_v):
        self.t, self.zero_v = t, zero_v

    def v(self):
        return pltpu.bitcast(
            pltpu.bitcast(self.t, jnp.uint32) & self.zero_v[0:8, :], F32)


class _Sched:
    def __init__(self, zero_v):
        self.zero_v = zero_v
        self.queue = []
        self.now = 0

    def add(self, items, t0, t1):
        assert t0 >= self.now
        n = len(items)
        self.queue += [(t0 + k * (t1 - t0) // n, it)
                       for k, it in enumerate(items)]
        self.queue.sort(key=lambda e: e[0])

    def __call__(self, t):
        end = self.now + TM
        while self.queue and self.queue[0][0] < end:
            time, item = self.queue.pop(0)
            r = (time - self.now) // 8 * 8
            item(_Anchor(t[r:r + 8, :], self.zero_v))
        self.now = end


def _rep(z, rows):
    return jnp.concatenate([z] * (rows // 8), axis=0)


def _ffn(h, wa_refs, wb_refs, sched, split=None):
    d = wb_refs[0].shape[1]
    acc = [None] * (d // 128)
    for c, (wa_ref, wb_ref) in enumerate(zip(wa_refs, wb_refs)):
        ss = []
        if c == 0 and split:
            r, nd = split
            top = [_dot(h[:r], wa_ref[:, n * 128:(n + 1) * 128])
                   for n in range(nd)]
            bot = [_dot(h[r:], wa_ref[:, n * 128:(n + 1) * 128])
                   for n in range(nd)]
            ss = [_silu(jnp.concatenate(tb, axis=0)) for tb in zip(top, bot)]
            sched.now += nd * TM
        for n in range(len(ss), FC // 128):
            a = _dot(h, wa_ref[:, n * 128:(n + 1) * 128])
            ss.append(_silu(a))
            sched(a)
        s = jnp.concatenate(ss, axis=1).astype(BF16)
        for n in range(d // 128):
            p = _dot(s, wb_ref[:, n * 128:(n + 1) * 128])
            acc[n] = p if acc[n] is None else acc[n] + p
            sched(p)
    return jnp.concatenate(acc, axis=1)


def _kernel(x_hbm, w1a_hbm, w1b_hbm, wq_hbm, wk_hbm, wv_hbm, wo_hbm,
            wp1_hbm, dw_hbm, wp2_hbm, w2a_hbm, w2b_hbm,
            out_hbm,
            xin, w1a, w1b, wq, wk, wv, wo, wp1, dw, wp2, w2a, w2b,
            mq, wvo, xs, hs, gs, dcs, st_mean, st_m2, bn, obuf,
            lhs_a, lhs_b, dwb, zero, zero_s, l_buf, al_buf0, al_buf1,
            p_buf0, p_buf1,
            xsem, w1sem, wsem, osem,
            *, B, T, D, K):
    N = B * T
    TP = hs.shape[1]
    NCB = D // 128
    nt = N // TM
    tpb = T // TM

    def rows(i, r0=0, n=TM):
        return pl.ds(pl.multiple_of(i * TM, 16) + r0, n)

    def brows(i, r0=0, n=TM):
        return i // tpb, pl.ds(pl.multiple_of((i % tpb) * TM, 16) + r0, n)

    def col(c):
        if isinstance(c, int):
            return slice(c * 128, (c + 1) * 128)
        return pl.ds(pl.multiple_of(c * 128, 128), 128)

    def pieces(fn, i, rb=None):
        rb = rb or RB
        return [functools.partial(fn, i, r0, rb) for r0 in range(0, TM, rb)]

    def interleave(*lists):
        return [it for group in zip(*lists) for it in group]

    def x_copy(i):
        return pltpu.make_async_copy(x_hbm.at[rows(i), :],
                                     xin.at[rows(i), :], xsem.at[i])

    def o_copy(i):
        return pltpu.make_async_copy(obuf.at[rows(i), :],
                                     out_hbm.at[rows(i), :], osem.at[i])

    nfc = w1a.shape[0]

    def w1_copies(c):
        fs = pl.ds(pl.multiple_of(c * FC, FC), FC)
        return [pltpu.make_async_copy(w1a_hbm.at[:, fs], w1a.at[c],
                                      w1sem.at[0, c]),
                pltpu.make_async_copy(w1b_hbm.at[fs, :], w1b.at[c],
                                      w1sem.at[1, c])]

    w_pairs = [(wq_hbm, wq), (wk_hbm, wk),
               (wv_hbm, wv), (wo_hbm, wo), (wp1_hbm, wp1), (dw_hbm, dw),
               (wp2_hbm, wp2), (w2a_hbm, w2a), (w2b_hbm, w2b)]
    w_copies = [pltpu.make_async_copy(s, d.at[:, 0:s.shape[1]], wsem.at[j])
                for j, (s, d) in enumerate(w_pairs)]

    x_copy(0).start()
    for cp in w1_copies(0):
        cp.start()

    zero[...] = jnp.zeros(zero.shape, jnp.uint32)
    zero_s[0] = 0
    for b in range(B):
        hs[b, T:TP, :] = jnp.zeros((TP - T, D), BF16)
    for c in range(NCB):
        gs[1, c, 0:HALO, :] = jnp.zeros((HALO, 128), F32)
        gs[nt, c, HALO + TM:, :] = jnp.zeros((HALO, 128), F32)

    def zrep(z, n):
        return None if z is None else _rep(z.v(), n)

    def ln_in(i, r0=0, n=TM, z=None, dst=lhs_a):
        dst[pl.ds(r0, n), :] = _ln(xin[rows(i, r0, n), :].astype(F32),
                                   zrep(z, n)).astype(BF16)

    def ln_out(i, r0=0, n=TM, z=None):
        b, rb = brows(i, r0, n)
        hs[b, rb, :] = _ln(xs[rows(i, r0, n), :], zrep(z, n)).astype(BF16)

    x_copy(0).wait()
    ln_in(0, dst=lhs_b)
    xs[rows(0), :] = xin[rows(0), :].astype(F32)

    def first_tile(c, carry):
        for cp in w1_copies(c):
            cp.wait()

        @pl.when(c == 1)
        def _():
            x_copy(1).wait()

        @pl.when(c + 1 < nfc)
        def _():
            for cp in w1_copies(c + 1):
                cp.start()

        @pl.when(c % 2 == 0)
        def _():
            x_copy(1 + c // 2).start()

        n = -(-TM // (nfc - 1) // 16) * 16
        step = (TM - n) // (nfc - 2)
        assert step % 16 == 0 and step <= n
        r0 = pl.multiple_of(jnp.maximum(c - 1, 0) * step, 16)
        sched = _Sched(zero)
        sched.add([functools.partial(ln_in, jnp.minimum(c, 1), r0 + r, FRB)
                   for r in range(0, n, FRB)], TM, F_END * TM)
        f = _ffn(lhs_b[...], [w1a.at[c]], [w1b.at[c]], sched)
        xs[rows(0), :] += 0.5 * f
        return carry

    lax.fori_loop(0, nfc, first_tile, 0)
    for j in range(3, nt):
        x_copy(j).start()
    for cp in w_copies:
        cp.start()

    def phase_a(i, carry):
        @pl.when(i + 1 < nt)
        def _():
            x_copy(i + 1).wait()

        h = lhs_a[...]
        items = interleave(pieces(ln_out, i - 1),
                           pieces(ln_in, jnp.minimum(i + 1, nt - 1)))
        sched = _Sched(zero)
        sched.add(items, A_SLOTS[0] * TM, A_SLOTS[1] * TM)
        f = _ffn(h, [w1a.at[c] for c in range(nfc)],
                 [w1b.at[c] for c in range(nfc)], sched)
        xs[rows(i), :] = xin[rows(i), :].astype(F32) + 0.5 * f
        return carry

    with jax.named_scope("phase_a"):
        lax.fori_loop(1, nt, phase_a, 0)

    for cp in w_copies:
        cp.wait()

    qk_scale = (D ** -0.5) * math.log2(math.e)

    def fold(u, carry):
        nr = TM // PU
        r0 = pl.multiple_of(u * nr, 8)
        sched = _Sched(zero)
        assert nr % RF == 0
        sched.add([functools.partial(ln_out, nt - 1, r0 + r, RF)
                   for r in range(0, nr, RF)], 0, (2 * NCB // PU - 1) * TM)
        css = [pl.ds(pl.multiple_of((u * (NCB // PU) + c) * 128, 128), 128)
               for c in range(NCB // PU)]
        for cs in css:
            t = _dot_nt(wq[...], wk[cs, :])
            mq[:, cs] = (t * qk_scale).astype(BF16)
            sched(t)
        for cs in css:
            t = _dot(wv[...], wo[:, cs])
            wvo[:, cs] = t.astype(BF16)
            sched(t)
        return carry

    lax.fori_loop(0, PU, fold, 0)
    dwf = dw[...].astype(F32)
    for k in range(K):
        dwb[k] = jnp.broadcast_to(dwf[k:k + 1, :], (8, D))

    def conv_block(p, r0, c, done, CT=CT, AT=K):
        cs = col(c)
        acc = [None]

        def item(k0, z=None):
            for k in range(k0, min(k0 + CT, K)):
                off = HALO - K // 2 + k + r0
                w = dwb[k, :, cs]
                if z is not None and k - k0 < AT:
                    w = w + z.v()
                t = gs[p + 1, c, off:off + 8, :] * w
                acc[0] = t if acc[0] is None else acc[0] + t
            if k0 + CT >= K:
                dcs[rows(p, r0, 8), cs] = acc[0]
                done(acc[0])

        return [functools.partial(item, k0) for k0 in range(0, K, CT)]

    def conv_main(p, cols=range(NCB), **kw):
        st = []

        def stats(r0, c, acc):
            if r0 == 0:
                st[:] = [acc, None, None]
                return
            shift, s1, s2 = st
            d = acc - shift
            s1 = d if s1 is None else s1 + d
            s2 = d * d if s2 is None else s2 + d * d
            st[:] = [shift, s1, s2]
            if r0 + 16 == TM:
                dm = s1 * (1.0 / (TM // 8 - 1))
                st_mean[p, :, col(c)] = shift + dm
                st_m2[p, :, col(c)] = s2 - s1 * dm

        return [it for c in cols for r0 in range(0, TM - 8, 8)
                for it in conv_block(p, r0, c,
                                     functools.partial(stats, r0, c), **kw)]

    def conv_edge(p, cols=range(NCB)):
        return [it for c in cols
                for it in conv_block(p, TM - 8, c, lambda acc: None)]

    nkc = TP // KC

    def phase_b(i, carry):
        b, rb = brows(i)
        sched = _Sched(zero)
        sched.add(conv_edge(jnp.maximum(i - 2, 0))
                  + conv_main(jnp.maximum(i - 1, 0), range(L0, NCB)),
                  int(B_SLOTS[0] * TM), int(B_SLOTS[1] * TM))
        qs = []
        for c in range(NCB):
            t = _dot(hs[b, rb, :], mq[:, col(c)])
            qs.append(t.astype(BF16))
            sched(t)
        q = jnp.concatenate(qs, axis=1)

        nsb = TM // SB
        dz = zero_s[0]
        p_buf, al_buf = (p_buf0, p_buf1), (al_buf0, al_buf1)

        def dyn(r0, n):
            return pl.ds(pl.multiple_of(dz + r0, 8), n)

        TK = T // 128 * 128
        srem = []

        def rem_scores(n):
            lo = min(n * 128, TM - 128)
            t = _dot_nt(hs[b, TK:T, :], q[lo:lo + 128])
            if TX == 1:
                t = jnp.concatenate(
                    [t, jnp.full((128 - (T - TK), 128), -jnp.inf, F32)], axis=0).T
            else:
                t = jnp.concatenate(
                    [t.T, jnp.full((128, 128 - (T - TK)), -jnp.inf, F32)], axis=1)
            srem.append(t[n * 128 - lo:])

        def scores(j):
            ss = []
            for n in range(KC // 128):
                lo = j * KC + n * 128
                if lo + 128 > T:
                    ss.append(jnp.concatenate(srem, axis=0))
                    continue
                s = _dot_nt(q, hs[b, lo:lo + 128, :])
                sched(s)
                ss.append(s)
                if j == RT[0]:
                    rem_scores(n)
            return ss

        m_v = [None] * nsb

        def soft(j, ss, k, z):
            rs = slice(k * SB, (k + 1) * SB)
            s = [t[rs, :] for t in ss]
            mj = functools.reduce(jnp.maximum, s[1:], s[0] + _rep(z.v(), SB))
            m_new = jnp.broadcast_to(jnp.max(mj, axis=-1, keepdims=True),
                                     (SB, 128))
            if j > 0:
                m_old = m_v[k]
                m_new = jnp.maximum(m_old, m_new)
            p = [jnp.exp2(t - m_new) for t in s]
            ps = functools.reduce(jnp.add, p)
            pb = jnp.concatenate([t.astype(BF16) for t in p], axis=1)
            p_buf[j % 2][k * SB // 2:(k + 1) * SB // 2, :] = pltpu.bitcast(
                pb, jnp.uint32)
            if j > 0:
                alpha = jnp.exp2(m_old - m_new)
                al_buf[j % 2][rs, :] = alpha
                ps = l_buf[dyn(k * SB, SB), :] * alpha + ps
            l_buf[rs, :] = ps
            m_v[k] = m_new

        def add_soft(j, ss, ndots):
            sched.add([functools.partial(soft, j, ss, k) for k in range(nsb)],
                      sched.now + SOFT[0], sched.now + ndots * TM - SOFT[1])

        acc = [None] * NCB
        nd = KC // 128
        add_soft(0, scores(0), nd)
        for j in range(nkc):
            if j + 1 < nkc:
                s_next = scores(j + 1)
                add_soft(j + 1, s_next, NCB + (nd if j + 2 < nkc else 0)
                         - (j + 3 == nkc))
            for n in range(NCB):
                p_all = pltpu.bitcast(p_buf[j % 2][dyn(0, TM // 2), :], BF16)
                pv = _dot(p_all, hs[b, j * KC:(j + 1) * KC,
                                    n * 128:(n + 1) * 128])
                sched(pv)
                if j == 0:
                    acc[n] = pv
                else:
                    acc[n] = acc[n] * al_buf[j % 2][dyn(0, TM), :] + pv
        assert not sched.queue
        acc = jnp.concatenate(acc, axis=1)
        l = l_buf[dyn(0, TM), :]
        o = (acc * (1.0 / jnp.sum(l, axis=-1, keepdims=True))).astype(BF16)
        hh = []
        for r0, r1 in zip((0,) + BS, BS + (TM,)):
            x2 = jnp.concatenate(
                [xs[rows(i, r0, r1 - r0), col(c)]
                 + _dot(o[r0:r1], wvo[:, col(c)]) for c in range(NCB)], axis=1)
            xs[rows(i, r0, r1 - r0), :] = x2
            hh.append(_ln(x2).astype(BF16))
        hn = jnp.concatenate(hh, axis=0)
        wcols = [slice(h * D + c * 128, h * D + (c + 1) * 128)
                 for c in range(NCB) for h in (1, 0)]
        r, nd = PS
        top = [_dot(hn[:r], wp1[:, cs]) for cs in wcols[:nd]]
        bot = [_dot(hn[r:], wp1[:, cs]) for cs in wcols[:nd]]
        u = [jnp.concatenate(tb, axis=0) for tb in zip(top, bot)]
        sched = _Sched(zero)
        for c in range(NCB):
            while len(u) < 2 * c + 2:
                u.append(_dot(hn, wp1[:, wcols[len(u)]]))
                sched(u[-1])
            g = u[2 * c + 1] * (0.5 + 0.5 * jnp.tanh(0.5 * u[2 * c]))
            gs[i + 1, c, HALO:HALO + TM, :] = g
            gs[i, c, HALO + TM:, :] = jnp.where(i % tpb == 0, 0.0, g[:HALO])
            gs[i + 2, c, :HALO, :] = jnp.where(i % tpb == tpb - 1, 0.0,
                                               g[TM - HALO:])
            if c < L0:
                sched.add(conv_main(i, [c], CT=LP[2], AT=LP[3]),
                          sched.now + LP[0], sched.now + 2 * TM - LP[1])
        assert not sched.queue
        return carry

    with jax.named_scope("phase_b"):
        lax.fori_loop(0, nt, phase_b, 0)
    for item in (conv_main(nt - 1, range(L0, NCB)) + conv_edge(nt - 2)
                 + conv_edge(nt - 1)):
        item()

    ng = TM // 8 - 1
    means = st_mean[...].reshape(nt * 8, D)
    edges = jnp.concatenate([dcs[(p + 1) * TM - 8:(p + 1) * TM, :]
                             for p in range(nt)], axis=0)
    mu = jnp.sum(ng * means + edges, axis=0, keepdims=True) * (1.0 / N)
    dm = means - mu
    de = edges - mu
    var = jnp.sum(st_m2[...].reshape(nt * 8, D) + ng * (dm * dm) + de * de,
                  axis=0, keepdims=True) * (1.0 / N)
    rstd = lax.rsqrt(var + EPS)
    bn[0] = jnp.broadcast_to(mu, (8, D))
    bn[1] = jnp.broadcast_to(rstd, (8, D))

    def bn_silu(i, r0=0, n=TM, z=None):
        mu = bn[0]
        if z is not None:
            mu = mu + jnp.concatenate([z.v()] * NCB, axis=1)
        d = dcs[rows(i, r0, n), :].reshape(n // 8, 8, D)
        y = ((d - mu[None]) * bn[1][None]).reshape(n, D)
        lhs_b[r0:r0 + n, :] = _silu(y).astype(BF16)

    def ln_final(i, r0=0, n=TM, z=None):
        obuf[rows(i, r0, n), :] = _ln(xs[rows(i, r0, n), :],
                                      zrep(z, n)).astype(BF16)

    bn_silu(0)

    def phase_c(i, carry):
        @pl.when(i >= 2)
        def _():
            o_copy(i - 2).start()

        sched = _Sched(zero)
        sched.add(pieces(ln_final, jnp.maximum(i - 1, 0), RC[0]),
                  C_SLOTS[0] * TM, C_SLOTS[1] * TM)
        sched.add(pieces(bn_silu, jnp.minimum(i + 1, nt - 1), RC[1]),
                  C_SLOTS[0] * TM + RC[2], C_SLOTS[1] * TM + RC[2])
        hh = []
        for r0, r1 in zip((0,) + CS, CS + (TM,)):
            lhs = lhs_b[r0:r1, :]
            x3 = jnp.concatenate(
                [xs[rows(i, r0, r1 - r0), col(c)]
                 + _dot(lhs, wp2[:, col(c)]) for c in range(NCB)], axis=1)
            xs[rows(i, r0, r1 - r0), :] = x3
            hh.append(_ln(x3).astype(BF16))
        sched.now = NCB * TM
        h = jnp.concatenate(hh, axis=0)
        f = _ffn(h, [w2a.at[:, c * FC:(c + 1) * FC] for c in range(nfc)],
                 [w2b.at[c * FC:(c + 1) * FC, :] for c in range(nfc)], sched,
                 FS)
        assert not sched.queue
        xs[rows(i), :] += 0.5 * f
        return carry

    with jax.named_scope("phase_c"):
        lax.fori_loop(0, nt, phase_c, 0)
    o_copy(nt - 2).start()
    last = []
    for k, (r0, r1) in enumerate(zip(EP[:-1], EP[1:])):
        ln_final(nt - 1, r0, r1 - r0)
        rs = rows(nt - 1, r0, r1 - r0)
        last.append(pltpu.make_async_copy(obuf.at[rs, :], out_hbm.at[rs, :],
                                          osem.at[nt - 1 + k]))
        last[-1].start()
    for i in range(nt - 1):
        o_copy(i).wait()
    for cp in last:
        cp.wait()


@jax.jit
def pallas_standalone__conformer_family_conformer__speech_kernel(
    x: jax.Array,
    w_ff1_a: jax.Array,
    w_ff1_b: jax.Array,
    w_q: jax.Array,
    w_k: jax.Array,
    w_v: jax.Array,
    w_o: jax.Array,
    w_pw1: jax.Array,
    dw: jax.Array,
    w_pw2: jax.Array,
    w_ff2_a: jax.Array,
    w_ff2_b: jax.Array,
):
    B, T, D = x.shape
    K = dw.shape[0]
    N = B * T
    TP = -(-T // KC) * KC
    weights = (w_ff1_a, w_ff1_b, w_q, w_k, w_v, w_o, w_pw1, dw, w_pw2,
               w_ff2_a, w_ff2_b)
    scratch = [pltpu.VMEM((N, D), BF16)]
    nfc = w_ff1_a.shape[1] // FC
    scratch += [pltpu.VMEM((nfc, D, FC), BF16), pltpu.VMEM((nfc, FC, D), BF16)]
    scratch += [pltpu.VMEM((w.shape[0], w.shape[1]
                            + (WPAD if w.shape[1] > D else 0)), w.dtype)
                for w in weights[2:]]
    scratch += [
        pltpu.VMEM((D, D), BF16),
        pltpu.VMEM((D, D), BF16),
        pltpu.VMEM((N, D), F32),
        pltpu.VMEM((B, TP, D), BF16),
        pltpu.VMEM((N // TM + 2, D // 128, TM + 2 * HALO, 128), F32),
        pltpu.VMEM((N, D), F32),
        pltpu.VMEM((N // TM, 8, D), F32),
        pltpu.VMEM((N // TM, 8, D), F32),
        pltpu.VMEM((2, 8, D), F32),
        pltpu.VMEM((N, D), BF16),
        pltpu.VMEM((TM, D), BF16),
        pltpu.VMEM((TM, D), BF16),
        pltpu.VMEM((K, 8, D), F32),
        pltpu.VMEM((ZR, 128), jnp.uint32),
        pltpu.SMEM((1,), jnp.int32),
        pltpu.VMEM((TM + 16, 128), F32),
        pltpu.VMEM((TM + 16, 128), F32),
        pltpu.VMEM((TM + 16, 128), F32),
        pltpu.VMEM((TM // 2, KC), jnp.uint32),
        pltpu.VMEM((TM // 2, KC), jnp.uint32),
        pltpu.SemaphoreType.DMA((N // TM,)),
        pltpu.SemaphoreType.DMA((2, nfc)),
        pltpu.SemaphoreType.DMA((len(weights) - 2,)),
        pltpu.SemaphoreType.DMA((N // TM + len(EP),)),
    ]
    out = pl.pallas_call(
        functools.partial(_kernel, B=B, T=T, D=D, K=K),
        out_shape=jax.ShapeDtypeStruct((N, D), x.dtype),
        in_specs=[pl.BlockSpec(memory_space=pl.ANY)] * 12,
        out_specs=pl.BlockSpec(memory_space=pl.ANY),
        scratch_shapes=scratch,
        compiler_params=pltpu.CompilerParams(
            vmem_limit_bytes=120 * 1024 * 1024),
    )(x.reshape(N, D), *weights)
    return out.reshape(B, T, D)
```

```python
import functools
import math

import jax
import jax.numpy as jnp
from jax import lax
import jax.experimental.pallas as pl
import jax.experimental.pallas.tpu as pltpu

F32 = jnp.float32
BF16 = jnp.bfloat16

TM = 400
FC = 512
KC = 512
RB = 8
SB = 16
A_SLOTS = (1, 29)
B_SLOTS = (1, 60)
C_SLOTS = (6, 33)
SOFT = (0, 800)
F_END = 7
ZR = 32
PU = 2
CT = 5
WPAD = 128
BS = (80, 160, 240, 320)
PS = (320, 2)
FRB = 16
L0 = 3
LP = (0, 100, 3, 1)
EP = (0, 160, 288, 352, 400)
CS = (80, 160, 240, 320)
FS = (320, 2)
RC = (8, 8, 100)
RF = 8
RT = 0
JR = 0
SHORT = 0
RK = 4
RW = (100, 700, 1200)
DBG = 0
HALO = 8
EPS = 1e-05


def _ln(x, z=None):
    if z is None:
        m = jnp.mean(x, axis=-1, keepdims=True)
    else:
        t = z
        for c in range(x.shape[-1] // 128):
            t = t + x[:, c * 128:(c + 1) * 128]
        m = jnp.sum(t, axis=-1, keepdims=True) * (1.0 / x.shape[-1])
    xc = x - m
    v = jnp.mean(xc * xc, axis=-1, keepdims=True)
    return xc * lax.rsqrt(v + EPS)


def _silu(a):
    y = 0.5 * a
    return y + y * jnp.tanh(y)


def _dot(a, b):
    return jnp.dot(a, b, preferred_element_type=F32)


def _dot_nt(a, b):
    return lax.dot_general(a, b, (((1,), (1,)), ((), ())),
                           preferred_element_type=F32)


class _Anchor:
    def __init__(self, t, zero_v):
        self.t, self.zero_v = t, zero_v

    def v(self):
        return pltpu.bitcast(
            pltpu.bitcast(self.t, jnp.uint32) & self.zero_v[0:8, :], F32)


class _Sched:
    def __init__(self, zero_v):
        self.zero_v = zero_v
        self.queue = []
        self.now = 0

    def add(self, items, t0, t1):
        assert t0 >= self.now
        n = len(items)
        self.queue += [(t0 + k * (t1 - t0) // n, it)
                       for k, it in enumerate(items)]
        self.queue.sort(key=lambda e: e[0])

    def __call__(self, t, dur=TM):
        end = self.now + dur
        while self.queue and self.queue[0][0] < end:
            time, item = self.queue.pop(0)
            r = (time - self.now) * TM // dur // 8 * 8
            item(_Anchor(t[r:r + 8, :], self.zero_v))
        self.now = end


def _rep(z, rows):
    return jnp.concatenate([z] * (rows // 8), axis=0)


def _ffn(h, wa_refs, wb_refs, sched, split=None):
    d = wb_refs[0].shape[1]
    acc = [None] * (d // 128)
    for c, (wa_ref, wb_ref) in enumerate(zip(wa_refs, wb_refs)):
        ss = []
        if c == 0 and split:
            r, nd = split
            top = [_dot(h[:r], wa_ref[:, n * 128:(n + 1) * 128])
                   for n in range(nd)]
            bot = [_dot(h[r:], wa_ref[:, n * 128:(n + 1) * 128])
                   for n in range(nd)]
            ss = [_silu(jnp.concatenate(tb, axis=0)) for tb in zip(top, bot)]
            sched.now += nd * TM
        for n in range(len(ss), FC // 128):
            a = _dot(h, wa_ref[:, n * 128:(n + 1) * 128])
            ss.append(_silu(a))
            sched(a)
        s = jnp.concatenate(ss, axis=1).astype(BF16)
        for n in range(d // 128):
            p = _dot(s, wb_ref[:, n * 128:(n + 1) * 128])
            acc[n] = p if acc[n] is None else acc[n] + p
            sched(p)
    return jnp.concatenate(acc, axis=1)


def _kernel(x_hbm, w1a_hbm, w1b_hbm, wq_hbm, wk_hbm, wv_hbm, wo_hbm,
            wp1_hbm, dw_hbm, wp2_hbm, w2a_hbm, w2b_hbm,
            out_hbm,
            xin, w1a, w1b, wq, wk, wv, wo, wp1, dw, wp2, w2a, w2b,
            mq, wvo, xs, hs, gs, dcs, st_mean, st_m2, bn, obuf,
            lhs_a, lhs_b, dwb, zero, zero_s, l_buf, al_buf0, al_buf1,
            p_buf0, p_buf1, hr, pr_buf, m0_buf, ra_buf, be_buf,
            xsem, w1sem, wsem, osem,
            *, B, T, D, K):
    N = B * T
    NR = T % 128
    NCB = D // 128
    nt = N // TM
    tpb = T // TM

    def rows(i, r0=0, n=TM):
        return pl.ds(pl.multiple_of(i * TM, 16) + r0, n)

    def brows(i, r0=0, n=TM):
        return i // tpb, pl.ds(pl.multiple_of((i % tpb) * TM, 16) + r0, n)

    def col(c):
        if isinstance(c, int):
            return slice(c * 128, (c + 1) * 128)
        return pl.ds(pl.multiple_of(c * 128, 128), 128)

    def pieces(fn, i, rb=None):
        rb = rb or RB
        return [functools.partial(fn, i, r0, rb) for r0 in range(0, TM, rb)]

    def interleave(*lists):
        return [it for group in zip(*lists) for it in group]

    def x_copy(i):
        return pltpu.make_async_copy(x_hbm.at[rows(i), :],
                                     xin.at[rows(i), :], xsem.at[i])

    def o_copy(i):
        return pltpu.make_async_copy(obuf.at[rows(i), :],
                                     out_hbm.at[rows(i), :], osem.at[i])

    nfc = w1a.shape[0]

    def w1_copies(c):
        fs = pl.ds(pl.multiple_of(c * FC, FC), FC)
        return [pltpu.make_async_copy(w1a_hbm.at[:, fs], w1a.at[c],
                                      w1sem.at[0, c]),
                pltpu.make_async_copy(w1b_hbm.at[fs, :], w1b.at[c],
                                      w1sem.at[1, c])]

    w_pairs = [(wq_hbm, wq), (wk_hbm, wk),
               (wv_hbm, wv), (wo_hbm, wo), (wp1_hbm, wp1), (dw_hbm, dw),
               (wp2_hbm, wp2), (w2a_hbm, w2a), (w2b_hbm, w2b)]
    w_copies = [pltpu.make_async_copy(s, d.at[:, 0:s.shape[1]], wsem.at[j])
                for j, (s, d) in enumerate(w_pairs)]

    x_copy(0).start()
    for cp in w1_copies(0):
        cp.start()

    zero[...] = jnp.zeros(zero.shape, jnp.uint32)
    zero_s[0] = 0
    for c in range(NCB):
        gs[1, c, 0:HALO, :] = jnp.zeros((HALO, 128), F32)
        gs[nt, c, HALO + TM:, :] = jnp.zeros((HALO, 128), F32)

    def zrep(z, n):
        return None if z is None else _rep(z.v(), n)

    def ln_in(i, r0=0, n=TM, z=None, dst=lhs_a):
        dst[pl.ds(r0, n), :] = _ln(xin[rows(i, r0, n), :].astype(F32),
                                   zrep(z, n)).astype(BF16)

    def ln_out(i, r0=0, n=TM, z=None):
        b, rb = brows(i, r0, n)
        hs[b, rb, :] = _ln(xs[rows(i, r0, n), :], zrep(z, n)).astype(BF16)

    x_copy(0).wait()
    ln_in(0, dst=lhs_b)
    xs[rows(0), :] = xin[rows(0), :].astype(F32)

    def first_tile(c, carry):
        for cp in w1_copies(c):
            cp.wait()

        @pl.when(c == 1)
        def _():
            x_copy(1).wait()

        @pl.when(c + 1 < nfc)
        def _():
            for cp in w1_copies(c + 1):
                cp.start()

        @pl.when(c % 2 == 0)
        def _():
            x_copy(1 + c // 2).start()

        n = -(-TM // (nfc - 1) // 16) * 16
        step = (TM - n) // (nfc - 2)
        assert step % 16 == 0 and step <= n
        r0 = pl.multiple_of(jnp.maximum(c - 1, 0) * step, 16)
        sched = _Sched(zero)
        sched.add([functools.partial(ln_in, jnp.minimum(c, 1), r0 + r, FRB)
                   for r in range(0, n, FRB)], TM, F_END * TM)
        f = _ffn(lhs_b[...], [w1a.at[c]], [w1b.at[c]], sched)
        xs[rows(0), :] += 0.5 * f
        return carry

    lax.fori_loop(0, nfc, first_tile, 0)
    for j in range(3, nt):
        x_copy(j).start()
    for cp in w_copies:
        cp.start()

    def phase_a(i, carry):
        @pl.when(i + 1 < nt)
        def _():
            x_copy(i + 1).wait()

        h = lhs_a[...]
        items = interleave(pieces(ln_out, i - 1),
                           pieces(ln_in, jnp.minimum(i + 1, nt - 1)))
        sched = _Sched(zero)
        sched.add(items, A_SLOTS[0] * TM, A_SLOTS[1] * TM)
        f = _ffn(h, [w1a.at[c] for c in range(nfc)],
                 [w1b.at[c] for c in range(nfc)], sched)
        xs[rows(i), :] = xin[rows(i), :].astype(F32) + 0.5 * f
        return carry

    with jax.named_scope("phase_a"):
        lax.fori_loop(1, nt, phase_a, 0)

    for cp in w_copies:
        cp.wait()

    qk_scale = (D ** -0.5) * math.log2(math.e)

    def fold(u, carry):
        nr = TM // PU
        r0 = pl.multiple_of(u * nr, 8)
        sched = _Sched(zero)
        assert nr % RF == 0
        sched.add([functools.partial(ln_out, nt - 1, r0 + r, RF)
                   for r in range(0, nr, RF)], 0, (2 * NCB // PU - 1) * TM)
        css = [pl.ds(pl.multiple_of((u * (NCB // PU) + c) * 128, 128), 128)
               for c in range(NCB // PU)]
        for cs in css:
            t = _dot_nt(wq[...], wk[cs, :])
            mq[:, cs] = (t * qk_scale).astype(BF16)
            sched(t)
        for cs in css:
            t = _dot(wv[...], wo[:, cs])
            wvo[:, cs] = t.astype(BF16)
            sched(t)
        return carry

    lax.fori_loop(0, PU, fold, 0)
    dwf = dw[...].astype(F32)
    for k in range(K):
        dwb[k] = jnp.broadcast_to(dwf[k:k + 1, :], (8, D))
    assert 128 % NR == 0 and NR & (NR - 1) == 0
    lane = lax.broadcasted_iota(jnp.int32, (NR, D), 1)
    for b in range(B):
        t = hs[b, :NR, :].astype(F32)
        for e in range(NR.bit_length() - 1):
            t = jnp.where((lane >> e) & 1 == 1,
                          pltpu.roll(t, NR - (1 << e), 0), t)
        hr[b] = t

    def conv_block(p, r0, c, done, CT=CT, AT=K):
        cs = col(c)
        acc = [None]

        def item(k0, z=None):
            for k in range(k0, min(k0 + CT, K)):
                off = HALO - K // 2 + k + r0
                w = dwb[k, :, cs]
                if z is not None and k - k0 < AT:
                    w = w + z.v()
                t = gs[p + 1, c, off:off + 8, :] * w
                acc[0] = t if acc[0] is None else acc[0] + t
            if k0 + CT >= K:
                dcs[rows(p, r0, 8), cs] = acc[0]
                done(acc[0])

        return [functools.partial(item, k0) for k0 in range(0, K, CT)]

    def conv_main(p, cols=range(NCB), **kw):
        st = []

        def stats(r0, c, acc):
            if r0 == 0:
                st[:] = [acc, None, None]
                return
            shift, s1, s2 = st
            d = acc - shift
            s1 = d if s1 is None else s1 + d
            s2 = d * d if s2 is None else s2 + d * d
            st[:] = [shift, s1, s2]
            if r0 + 16 == TM:
                dm = s1 * (1.0 / (TM // 8 - 1))
                st_mean[p, :, col(c)] = shift + dm
                st_m2[p, :, col(c)] = s2 - s1 * dm

        return [it for c in cols for r0 in range(0, TM - 8, 8)
                for it in conv_block(p, r0, c,
                                     functools.partial(stats, r0, c), **kw)]

    def conv_edge(p, cols=range(NCB)):
        return [it for c in cols
                for it in conv_block(p, TM - 8, c, lambda acc: None)]

    nkc = -(-(T - NR) // KC)
    nbl = [KC // 128] * nkc
    nbl[SHORT] -= (nkc * KC + NR - T) // 128
    kofs = [NR + 128 * sum(nbl[:j]) for j in range(nkc + 1)]

    def phase_b(i, carry):
        b, rb = brows(i)
        sched = _Sched(zero)
        sched.add(conv_edge(jnp.maximum(i - 2, 0))
                  + conv_main(jnp.maximum(i - 1, 0), range(L0, NCB)),
                  int(B_SLOTS[0] * TM), int(B_SLOTS[1] * TM))
        qs = []
        for c in range(NCB):
            t = _dot(hs[b, rb, :], mq[:, col(c)])
            qs.append(t.astype(BF16))
            sched(t)
        q = jnp.concatenate(qs, axis=1)

        nsb = TM // SB
        dz = zero_s[0]
        p_buf, al_buf = (p_buf0, p_buf1), (al_buf0, al_buf1)

        def dyn(r0, n):
            return pl.ds(pl.multiple_of(dz + r0, 8), n)

        srem = []

        def rem_scores():
            n = len(srem)
            lo = min(n * 128, TM - 128)
            t = _dot_nt(hs[b, :NR, :], q[lo:lo + 128])
            t = jnp.concatenate([t] * (128 // NR), axis=0).T
            srem.append(t[n * 128 - lo:])

        racc = [None]
        ties = []

        def rem_pv(r0, s0, z):
            src = pr_buf[dyn(r0, 8), :] + z.v()
            for s in range(s0, s0 + RK):
                r = pltpu.roll(src, s, 1) if s else src
                k = (NR - s) % NR
                t = [r * jnp.broadcast_to(hr[b, k:k + 1, col(n)], (8, 128))
                     for n in range(NCB)]
                racc[0] = t if s == 0 else [x + y for x, y in zip(racc[0], t)]
            if s0 + RK == NR:
                ra_buf[r0:r0 + 8, :] = jnp.concatenate(racc[0], axis=1)
                ties.append(racc[0][0])
                racc[0] = None

        rem = [functools.partial(rem_pv, r0, s0) for r0 in range(0, TM, 8)
               for s0 in range(0, NR, RK)]
        m_all = []

        def scores(j):
            ss = []
            for lo in range(kofs[j], kofs[j + 1], 128):
                ss.append(_dot_nt(q, hs[b, lo:lo + 128, :]))
                sched(ss[-1])
                if j == RT:
                    rem_scores()
            while j == RT and len(srem) * 128 < TM:
                rem_scores()
            if j == JR:
                ss.append(jnp.concatenate(srem, axis=0))
            mj = functools.reduce(jnp.maximum, ss)
            ts = ties + (racc[0] or [])[:1]
            if ts:
                z = _Anchor(functools.reduce(jnp.add, ts), zero).v()
                mj = jnp.concatenate([mj[:TM - 8], mj[TM - 8:] + z], axis=0)
                ties.clear()
            m = jnp.broadcast_to(jnp.max(mj, axis=-1, keepdims=True),
                                 (TM, 128))
            m_all.append(jnp.maximum(m_all[-1], m) if j else m)
            return ss

        def soft(j, ss, k, z):
            rs = slice(k * SB, (k + 1) * SB)
            m_new = m_all[j][rs, :] + _rep(z.v(), SB)
            p = [jnp.exp2(t[rs, :] - m_new) for t in ss]
            if j == JR:
                pr = p.pop()
                pr_buf[rs, :] = pr
                ps = functools.reduce(jnp.add, p, pr * (NR / 128))
            else:
                ps = functools.reduce(jnp.add, p)
            pb = jnp.concatenate([t.astype(BF16) for t in p], axis=1)
            p_buf[j % 2][k * SB // 2:(k + 1) * SB // 2,
                         :pb.shape[1]] = pltpu.bitcast(pb, jnp.uint32)
            if j > 0:
                alpha = jnp.exp2(m_all[j - 1][rs, :] - m_new)
                al_buf[j % 2][rs, :] = alpha
                ps = l_buf[dyn(k * SB, SB), :] * alpha + ps
            if j == nkc - 1:
                be_buf[rs, :] = jnp.exp2(m_all[JR][rs, :] - m_new)
            l_buf[rs, :] = ps

        def add_soft(j, ss, dur):
            sched.add([functools.partial(soft, j, ss, k) for k in range(nsb)],
                      sched.now + SOFT[0], sched.now + dur - SOFT[1])

        pvd = [nbl[j] * TM // NCB for j in range(nkc)]
        wins = [NCB * pvd[j] + nbl[j + 2] * TM - RW[1] - RW[0]
                for j in range(JR, nkc - 2)] + [RW[2]]
        cnt = [len(rem) * sum(wins[:k + 1]) // sum(wins)
               for k in range(len(wins))]

        acc = [None] * NCB
        add_soft(0, scores(0), nbl[1] * TM)
        for j in range(nkc):
            dur = pvd[j]
            if j + 1 < nkc:
                s_next = scores(j + 1)
                add_soft(j + 1, s_next, NCB * dur
                         + (nbl[j + 2] * TM if j + 2 < nkc else 0))
                if j >= JR and not DBG & 1:
                    k = j - JR
                    sched.add(rem[cnt[k - 1] if k else 0:cnt[k]],
                              sched.now + RW[0], sched.now + RW[0] + wins[k])
            for n in range(NCB):
                p_all = pltpu.bitcast(
                    p_buf[j % 2][dyn(0, TM // 2), :nbl[j] * 128], BF16)
                pv = _dot(p_all, hs[b, kofs[j]:kofs[j + 1], col(n)])
                sched(pv, dur)
                if j == 0:
                    acc[n] = pv
                    continue
                acc[n] = acc[n] * al_buf[j % 2][dyn(0, TM), :]
                if j == nkc - 1:
                    acc[n] += (ra_buf[dyn(0, TM), col(n)]
                               * be_buf[dyn(0, TM), :])
                acc[n] += pv
        assert not sched.queue
        acc = jnp.concatenate(acc, axis=1)
        l = l_buf[dyn(0, TM), :]
        o = (acc * (1.0 / jnp.sum(l, axis=-1, keepdims=True))).astype(BF16)
        hh = []
        for r0, r1 in zip((0,) + BS, BS + (TM,)):
            x2 = jnp.concatenate(
                [xs[rows(i, r0, r1 - r0), col(c)]
                 + _dot(o[r0:r1], wvo[:, col(c)]) for c in range(NCB)], axis=1)
            xs[rows(i, r0, r1 - r0), :] = x2
            hh.append(_ln(x2).astype(BF16))
        hn = jnp.concatenate(hh, axis=0)
        wcols = [slice(h * D + c * 128, h * D + (c + 1) * 128)
                 for c in range(NCB) for h in (1, 0)]
        r, nd = PS
        top = [_dot(hn[:r], wp1[:, cs]) for cs in wcols[:nd]]
        bot = [_dot(hn[r:], wp1[:, cs]) for cs in wcols[:nd]]
        u = [jnp.concatenate(tb, axis=0) for tb in zip(top, bot)]
        sched = _Sched(zero)
        for c in range(NCB):
            while len(u) < 2 * c + 2:
                u.append(_dot(hn, wp1[:, wcols[len(u)]]))
                sched(u[-1])
            g = u[2 * c + 1] * (0.5 + 0.5 * jnp.tanh(0.5 * u[2 * c]))
            gs[i + 1, c, HALO:HALO + TM, :] = g
            gs[i, c, HALO + TM:, :] = jnp.where(i % tpb == 0, 0.0, g[:HALO])
            gs[i + 2, c, :HALO, :] = jnp.where(i % tpb == tpb - 1, 0.0,
                                               g[TM - HALO:])
            if c < L0:
                sched.add(conv_main(i, [c], CT=LP[2], AT=LP[3]),
                          sched.now + LP[0], sched.now + 2 * TM - LP[1])
        assert not sched.queue
        return carry

    with jax.named_scope("phase_b"):
        lax.fori_loop(0, nt, phase_b, 0)
    for item in (conv_main(nt - 1, range(L0, NCB)) + conv_edge(nt - 2)
                 + conv_edge(nt - 1)):
        item()

    ng = TM // 8 - 1
    means = st_mean[...].reshape(nt * 8, D)
    edges = jnp.concatenate([dcs[(p + 1) * TM - 8:(p + 1) * TM, :]
                             for p in range(nt)], axis=0)
    mu = jnp.sum(ng * means + edges, axis=0, keepdims=True) * (1.0 / N)
    dm = means - mu
    de = edges - mu
    var = jnp.sum(st_m2[...].reshape(nt * 8, D) + ng * (dm * dm) + de * de,
                  axis=0, keepdims=True) * (1.0 / N)
    rstd = lax.rsqrt(var + EPS)
    bn[0] = jnp.broadcast_to(mu, (8, D))
    bn[1] = jnp.broadcast_to(rstd, (8, D))

    def bn_silu(i, r0=0, n=TM, z=None):
        mu = bn[0]
        if z is not None:
            mu = mu + jnp.concatenate([z.v()] * NCB, axis=1)
        d = dcs[rows(i, r0, n), :].reshape(n // 8, 8, D)
        y = ((d - mu[None]) * bn[1][None]).reshape(n, D)
        lhs_b[r0:r0 + n, :] = _silu(y).astype(BF16)

    def ln_final(i, r0=0, n=TM, z=None):
        obuf[rows(i, r0, n), :] = _ln(xs[rows(i, r0, n), :],
                                      zrep(z, n)).astype(BF16)

    bn_silu(0)

    def phase_c(i, carry):
        @pl.when(i >= 2)
        def _():
            o_copy(i - 2).start()

        sched = _Sched(zero)
        sched.add(pieces(ln_final, jnp.maximum(i - 1, 0), RC[0]),
                  C_SLOTS[0] * TM, C_SLOTS[1] * TM)
        sched.add(pieces(bn_silu, jnp.minimum(i + 1, nt - 1), RC[1]),
                  C_SLOTS[0] * TM + RC[2], C_SLOTS[1] * TM + RC[2])
        hh = []
        for r0, r1 in zip((0,) + CS, CS + (TM,)):
            lhs = lhs_b[r0:r1, :]
            x3 = jnp.concatenate(
                [xs[rows(i, r0, r1 - r0), col(c)]
                 + _dot(lhs, wp2[:, col(c)]) for c in range(NCB)], axis=1)
            xs[rows(i, r0, r1 - r0), :] = x3
            hh.append(_ln(x3).astype(BF16))
        sched.now = NCB * TM
        h = jnp.concatenate(hh, axis=0)
        f = _ffn(h, [w2a.at[:, c * FC:(c + 1) * FC] for c in range(nfc)],
                 [w2b.at[c * FC:(c + 1) * FC, :] for c in range(nfc)], sched,
                 FS)
        assert not sched.queue
        xs[rows(i), :] += 0.5 * f
        return carry

    with jax.named_scope("phase_c"):
        lax.fori_loop(0, nt, phase_c, 0)
    o_copy(nt - 2).start()
    last = []
    for k, (r0, r1) in enumerate(zip(EP[:-1], EP[1:])):
        ln_final(nt - 1, r0, r1 - r0)
        rs = rows(nt - 1, r0, r1 - r0)
        last.append(pltpu.make_async_copy(obuf.at[rs, :], out_hbm.at[rs, :],
                                          osem.at[nt - 1 + k]))
        last[-1].start()
    for i in range(nt - 1):
        o_copy(i).wait()
    for cp in last:
        cp.wait()


@jax.jit
def pallas_standalone__conformer_family_conformer__speech_kernel(
    x: jax.Array,
    w_ff1_a: jax.Array,
    w_ff1_b: jax.Array,
    w_q: jax.Array,
    w_k: jax.Array,
    w_v: jax.Array,
    w_o: jax.Array,
    w_pw1: jax.Array,
    dw: jax.Array,
    w_pw2: jax.Array,
    w_ff2_a: jax.Array,
    w_ff2_b: jax.Array,
):
    B, T, D = x.shape
    K = dw.shape[0]
    N = B * T
    NR = T % 128
    weights = (w_ff1_a, w_ff1_b, w_q, w_k, w_v, w_o, w_pw1, dw, w_pw2,
               w_ff2_a, w_ff2_b)
    scratch = [pltpu.VMEM((N, D), BF16)]
    nfc = w_ff1_a.shape[1] // FC
    scratch += [pltpu.VMEM((nfc, D, FC), BF16), pltpu.VMEM((nfc, FC, D), BF16)]
    scratch += [pltpu.VMEM((w.shape[0], w.shape[1]
                            + (WPAD if w.shape[1] > D else 0)), w.dtype)
                for w in weights[2:]]
    scratch += [
        pltpu.VMEM((D, D), BF16),
        pltpu.VMEM((D, D), BF16),
        pltpu.VMEM((N, D), F32),
        pltpu.VMEM((B, T, D), BF16),
        pltpu.VMEM((N // TM + 2, D // 128, TM + 2 * HALO, 128), F32),
        pltpu.VMEM((N, D), F32),
        pltpu.VMEM((N // TM, 8, D), F32),
        pltpu.VMEM((N // TM, 8, D), F32),
        pltpu.VMEM((2, 8, D), F32),
        pltpu.VMEM((N, D), BF16),
        pltpu.VMEM((TM, D), BF16),
        pltpu.VMEM((TM, D), BF16),
        pltpu.VMEM((K, 8, D), F32),
        pltpu.VMEM((ZR, 128), jnp.uint32),
        pltpu.SMEM((1,), jnp.int32),
        pltpu.VMEM((TM + 16, 128), F32),
        pltpu.VMEM((TM + 16, 128), F32),
        pltpu.VMEM((TM + 16, 128), F32),
        pltpu.VMEM((TM // 2, KC), jnp.uint32),
        pltpu.VMEM((TM // 2, KC), jnp.uint32),
        pltpu.VMEM((B, NR, D), F32),
        pltpu.VMEM((TM + 16, 128), F32),
        pltpu.VMEM((TM + 16, 128), F32),
        pltpu.VMEM((TM + 8, D), F32),
        pltpu.VMEM((TM + 16, 128), F32),
        pltpu.SemaphoreType.DMA((N // TM,)),
        pltpu.SemaphoreType.DMA((2, nfc)),
        pltpu.SemaphoreType.DMA((len(weights) - 2,)),
        pltpu.SemaphoreType.DMA((N // TM + len(EP),)),
    ]
    out = pl.pallas_call(
        functools.partial(_kernel, B=B, T=T, D=D, K=K),
        out_shape=jax.ShapeDtypeStruct((N, D), x.dtype),
        in_specs=[pl.BlockSpec(memory_space=pl.ANY)] * 12,
        out_specs=pl.BlockSpec(memory_space=pl.ANY),
        scratch_shapes=scratch,
        compiler_params=pltpu.CompilerParams(
            vmem_limit_bytes=120 * 1024 * 1024),
    )(x.reshape(N, D), *weights)
    return out.reshape(B, T, D)
```

```python
import functools
import math

import jax
import jax.numpy as jnp
from jax import lax
import jax.experimental.pallas as pl
import jax.experimental.pallas.tpu as pltpu

F32 = jnp.float32
BF16 = jnp.bfloat16

TM = 400
T0 = 320
TA = 320
TC = 320
FC = 512
KC = 512
IW = 5
O1 = (0, 1, 2, 3, 4, 5, 6)
O2 = (1, 3, 6, 0, 2, 4, 5)
FE = ((0, 2), (0, 4), (1, 2), (1, 4))
OQ = (0, 2, 3, 4, 6, 1, 5)
OS0 = (2, 4, 3, 1, 0, 5, 6)
OS = (0, 1, 2, 3, 4, 5, 6)
OP = (0, 1, 2, 3, 4, 5, 6)
OW = (2, 4, 3, 0, 6, 1, 5)
PO = tuple((h, k) for h in range(2) for k in OW)
FRB = 16
F_WIN = (0.1, 0.9)
RA = 8
RO = 8
A_WIN = (0.05, 0.8)
A_SKIP = (700, 1400)
RF = 8
B_SLOTS = (1, 53)
Q_SLOTS = (8, 50)
CT = 5
L0 = 2
LP = (0, 100, 3, 1)
S1 = 2
S2 = 1
SD = (0, 120, 100)
C_WIN = (0.29, 0.86)
C_SKIP = ((4200, 5100), (6450, 7350), (8700, 9600))
RC = (8, 100)
EP = (0, 128, 224, 288, 320)
ZR = 32
PR = 112
HALO = 8
EPS = 1e-05


def _ln(x, z=None):
    if z is None:
        m = jnp.mean(x, axis=-1, keepdims=True)
    else:
        t = z
        for c in range(x.shape[-1] // 128):
            t = t + x[:, c * 128:(c + 1) * 128]
        m = jnp.sum(t, axis=-1, keepdims=True) * (1.0 / x.shape[-1])
    xc = x - m
    v = jnp.mean(xc * xc, axis=-1, keepdims=True)
    return xc * lax.rsqrt(v + EPS)


def _silu(a):
    y = 0.5 * a
    return y + y * jnp.tanh(y)


def _dot(a, b):
    return jnp.dot(a, b, preferred_element_type=F32)


def _dot_nt(a, b):
    return lax.dot_general(a, b, (((1,), (1,)), ((), ())),
                           preferred_element_type=F32)


class _Anchor:
    def __init__(self, t, zero_v):
        self.t, self.zero_v = t, zero_v

    def v(self):
        return pltpu.bitcast(
            pltpu.bitcast(self.t, jnp.uint32) & self.zero_v[0:8, :], F32)


class _Sched:
    def __init__(self, zero_v):
        self.zero_v = zero_v
        self.queue = []
        self.now = 0

    def add(self, items, t0, t1, skip=()):
        assert t0 >= self.now
        ts = [t for t in range(t0, t1)
              if not any(a <= t < b for a, b in skip)]
        self.queue += [(ts[k * len(ts) // len(items)], it)
                       for k, it in enumerate(items)]
        self.queue.sort(key=lambda e: e[0])

    def __call__(self, t, dur=None):
        dur = dur or t.shape[0]
        end = self.now + dur
        while self.queue and self.queue[0][0] < end:
            time, item = self.queue.pop(0)
            r = (time - self.now) * t.shape[0] // dur // 8 * 8
            item(_Anchor(t[r:r + 8, :128], self.zero_v))
        self.now = end


def _rep(z, rows):
    return jnp.concatenate([z] * (rows // 8), axis=0)


def _ffn(h, wa_ref, wb_ref, sched):
    ss = []
    for n in range(wa_ref.shape[1] // 128):
        a = _dot(h, wa_ref[:, n * 128:(n + 1) * 128])
        ss.append(_silu(a))
        sched(a)
    s = jnp.concatenate(ss, axis=1).astype(BF16)
    acc = []
    for n in range(wb_ref.shape[1] // 128):
        acc.append(_dot(s, wb_ref[:, n * 128:(n + 1) * 128]))
        sched(acc[-1])
    return jnp.concatenate(acc, axis=1)


def _sa(a11, a12, a21, a22):
    return [a11 + a22, a21 + a22, a11, a22, a11 + a12, a21 - a11, a12 - a22]


def _sb(b11, b12, b21, b22):
    return [b11 + b22, b11, b12 - b22, b21 - b11, b22, b11 + b12, b21 + b22]


def _sc(m):
    return [m[0] + m[3] - m[4] + m[6], m[4] + m[2], m[3] + m[1],
            m[0] + m[2] - m[1] + m[5]]


def _lhs7(t, u):
    h = t.shape[1] // 2
    return [v.astype(BF16)
            for v in _sa(t[:, :h], t[:, h:], u[:, :h], u[:, h:])]


_TG = (((0, 1), (3, 1)), ((2, 1), (3, -1)), ((1, 1), (3, 1)), ((0, 1), (2, 1)),
       ((0, -1), (1, 1)), ((3, 1),), ((0, 1),))


def _quads(x, hm):
    h = x.shape[1] // 2
    t = x[:hm]
    if x.shape[0] > 2 * hm:
        t = jnp.concatenate([t, x[2 * hm:]], axis=0)
    return t[:, :h], t[:, h:], x[hm:, :h], x[hm:, h:]


def _sax(a11, a12, a21, a22, hm):
    return [a11[:hm] + a22[:hm], a21 + a22, a11, a22, a11 + a12,
            a21[:hm] - a11[:hm], a12[:hm] - a22[:hm]]


def _acc7(acc, k, m, hm):
    for a, sg in _TG[k]:
        t = m if a in (1, 2) else m[:hm]
        if acc[a] is None:
            acc[a] = t if sg > 0 else -t
        else:
            acc[a] = acc[a] + t if sg > 0 else acc[a] - t


def _join(acc, hm):
    rest = [acc[1][hm:]] if acc[1].shape[0] > hm else []
    return (jnp.concatenate([acc[0], acc[2]], axis=0),
            jnp.concatenate([acc[1][:hm], acc[3]] + rest, axis=0))


def _ffn7(h7, wa, wb, sched, early=()):
    acc = [None] * 7
    hm = h7[0].shape[0]
    u = [[None] * 4 for _ in wa]

    def first(c, k):
        t = _dot(h7[k], wa[c][k])
        _acc7(u[c], k, t, hm)
        sched(t)

    for c, k in early:
        first(c, k)
    for c, cb in enumerate(wb):
        for k in O1:
            if (c, k) not in early:
                first(c, k)
        s7 = [t.astype(BF16) for t in _sa(*[_silu(t) for t in u[c]])]
        for k in O2:
            p = _dot(s7[k], cb[k])
            acc[k] = p if acc[k] is None else acc[k] + p
            sched(p)
    c = _sc(acc)
    return jnp.concatenate(c[:2], axis=1), jnp.concatenate(c[2:], axis=1)


def _kernel(x_hbm, w1a_hbm, w1b_hbm, wq_hbm, wk_hbm, wv_hbm, wo_hbm,
            wp1_hbm, dw_hbm, wp2_hbm, w2a_hbm, w2b_hbm,
            out_hbm,
            xin, wblk, wq, wk, wv, wo, dw,
            mq, wvo, xs, hs, ks, gs, dcs, st_mean, st_m2, bn,
            lhs7, w17, w7, lhs_b, dwb, zero, zero_s, al_buf0, al_buf1,
            p_buf0, p_buf1, s_buf, hq7,
            xsem, w1sem, w2sem, wsem, osem,
            *, B, T, D, K):
    N = B * T
    obuf = xin
    KP = KC // 2
    nkc = -(-T // KC)
    TP = nkc * KP
    NCB = D // 128
    nt = N // TM
    tpb = T // TM

    def rows(i, r0=0, n=TM):
        return pl.ds(pl.multiple_of(i * TM, 16) + r0, n)

    def col(c):
        if isinstance(c, int):
            return slice(c * 128, (c + 1) * 128)
        return pl.ds(pl.multiple_of(c * 128, 128), 128)

    na = (N - T0) // TA
    H = D // 2

    def arows(i, r0=0, n=TA):
        return pl.ds(pl.multiple_of(T0 + (i - 1) * TA, 16) + r0, n)

    def x_copy(i):
        rs = pl.ds(0, T0) if isinstance(i, int) and i == 0 else arows(i)
        return pltpu.make_async_copy(x_hbm.at[rs, :], xin.at[rs, :],
                                     xsem.at[i])

    nc = N // TC

    def crows(i, r0=0, n=TC):
        return pl.ds(pl.multiple_of(i * TC, 16) + r0, n)

    def o_copy(i):
        return pltpu.make_async_copy(obuf.at[crows(i), :],
                                     out_hbm.at[crows(i), :], osem.at[i])

    nfc = w17.shape[1]
    P1, P2 = 4 * nfc, 4 * nfc + 2

    def w1_copies(c):
        fs = pl.ds(pl.multiple_of(c * FC, FC), FC)
        return [pltpu.make_async_copy(w1a_hbm.at[:, fs], wblk.at[c],
                                      w1sem.at[0, c]),
                pltpu.make_async_copy(w1b_hbm.at[fs, :], wblk.at[nfc + c],
                                      w1sem.at[1, c])]

    def w2_copies(c):
        fs = pl.ds(pl.multiple_of(c * FC, FC), FC)
        hs_ = pl.ds(pl.multiple_of(c // 2 * H, H), H)
        return [pltpu.make_async_copy(s, d, w2sem.at[j, c])
                for j, (s, d) in enumerate([
                    (w2a_hbm.at[:, fs], wblk.at[2 * nfc + c]),
                    (w2b_hbm.at[fs, :], wblk.at[3 * nfc + c]),
                    (wp1_hbm.at[:, pl.ds(pl.multiple_of(c * H, H), H)],
                     wblk.at[P1 + c % 2, :, hs_])])]

    assert nfc == 4
    w_pairs = [(wp2_hbm, wblk.at[P2]), (wq_hbm, wq), (wk_hbm, wk),
               (wv_hbm, wv), (wo_hbm, wo), (dw_hbm, dw)]
    w_copies = [pltpu.make_async_copy(s, d, wsem.at[j])
                for j, (s, d) in enumerate(w_pairs)]

    x_copy(0).start()
    for cp in w1_copies(0):
        cp.start()

    zero[...] = jnp.zeros(zero.shape, jnp.uint32)
    zero_s[0] = 0
    for c in range(NCB):
        gs[1, c, 0:HALO, :] = jnp.zeros((HALO, 128), F32)
        gs[nt, c, HALO + TM:, :] = jnp.zeros((HALO, 128), F32)
    for b in range(B):
        ks[:, b * TP + T // 2:(b + 1) * TP, :] = jnp.zeros(
            (7, TP - T // 2, H), BF16)

    def zrep(z, n):
        return None if z is None else _rep(z.v(), n)

    def ln_in(i, r0, n, z=None):
        t, u = [_ln(xin[arows(i, r + r0, n), :].astype(F32), zrep(z, n))
                for r in (0, TA // 2)]
        for k, v in enumerate(_lhs7(t, u)):
            lhs7[k, pl.ds(r0, n), :] = v

    def ln_out(base, r0, n, z=None):
        tu = []
        for r in (0, 16):
            rs = pl.ds(pl.multiple_of(base, 32) + r0 // 16 * 32 + r0 % 16 + r,
                       n)
            tu.append(_ln(xs[rs, :], zrep(z, n)))
            hs[rs, :] = tu[-1].astype(BF16)
        g = base // 32 + r0 // 16
        g += g // (T // 32) * ((TP - T // 2) // 16)
        ps = pl.ds(pl.multiple_of(g * 16, 16) + r0 % 16, n)
        for k, v in enumerate(_lhs7(*tu)):
            ks[k, ps, :] = v

    def prep(src, dst, r0, z=None):
        q = [src[pl.ds(r + r0, 16), c:c + H].astype(F32)
             for r in (0, H) for c in (0, H)]
        if z is not None:
            zz = jnp.concatenate([_rep(z.v(), 16)] * (H // 128), axis=1)
            q[0], q[3] = q[0] + zz, q[3] + zz
        for k, v in enumerate(_sb(*q)):
            dst[k, pl.ds(r0, 16), :] = v.astype(BF16)

    x_copy(0).wait()
    lhs_b[...] = _ln(xin[0:T0, :].astype(F32)).astype(BF16)
    xs[0:T0, :] = xin[0:T0, :].astype(F32)

    def first_tile(c, carry):
        for cp in w1_copies(c):
            cp.wait()

        @pl.when(c == 1)
        def _():
            x_copy(1).wait()

        @pl.when(c + 1 < nfc)
        def _():
            for cp in w1_copies(c + 1):
                cp.start()

        @pl.when(c % 2 == 0)
        def _():
            x_copy(1 + c // 2).start()

        n = -(-TA // 2 // (nfc - 1) // 16) * 16
        step = (TA // 2 - n) // (nfc - 2)
        assert step % 16 == 0 and step <= n
        r0 = pl.multiple_of(jnp.maximum(c - 1, 0) * step, 16)
        assert T0 == TA
        sched = _Sched(zero)
        dur = 2 * NCB * T0
        sched.add([functools.partial(ln_in, jnp.minimum(c, 1), r0 + r, FRB)
                   for r in range(0, n, FRB)],
                  int(F_WIN[0] * dur), int(F_WIN[1] * dur))
        sched.add([functools.partial(prep, wblk.at[j * nfc + c],
                                     w17.at[j, c], r)
                   for j in range(2) for r in range(0, H, 16)],
                  int(F_WIN[0] * dur), int(F_WIN[1] * dur))
        f = _ffn(lhs_b[...], wblk.at[c], wblk.at[nfc + c], sched)
        assert not sched.queue
        xs[0:T0, :] += 0.5 * f
        return carry

    lax.fori_loop(0, nfc, first_tile, 0)
    for j in range(3, na + 1):
        x_copy(j).start()
    for c in range(nfc):
        for cp in w2_copies(c):
            cp.start()
    for cp in w_copies:
        cp.start()

    def phase_a(i, carry):
        @pl.when(i < na)
        def _():
            x_copy(i + 1).wait()

        @pl.when((i >= IW) & (i < IW + nfc))
        def _():
            for cp in w2_copies(i - IW):
                cp.wait()

        @pl.when(i == IW)
        def _():
            w_copies[0].wait()

        h7 = [lhs7[k] for k in range(7)]
        sched = _Sched(zero)
        dur = 7 * nfc * TA
        win = (int(A_WIN[0] * dur), int(A_WIN[1] * dur),
               [(c * 7 * TA + A_SKIP[0], c * 7 * TA + A_SKIP[1])
                for c in range(nfc)])
        sched.add([functools.partial(ln_out, T0 + (i - 2) * TA, r, RO)
                   for r in range(0, TA // 2, RO)], *win)
        sched.add([functools.partial(ln_in, jnp.minimum(i + 1, na), r, RA)
                   for r in range(0, TA // 2, RA)], *win)
        rpb = H // 16
        total = w7.shape[0] * rpb
        ipi = -(-total // (na - IW + 1))
        items = []
        for k in range(ipi):
            n = jnp.minimum(jnp.maximum(i - IW, 0) * ipi + k, total - 1)
            src = n // rpb + jnp.where(i >= IW, 2 * nfc, 0)
            items.append(functools.partial(
                prep, wblk.at[src], w7.at[n // rpb],
                pl.multiple_of(n % rpb * 16, 16)))
        assert ipi <= rpb
        sched.add(items, *win)
        f = _ffn7(h7, [w17.at[0, c] for c in range(nfc)],
                  [w17.at[1, c] for c in range(nfc)], sched)
        assert not sched.queue
        xs[arows(i), :] = (xin[arows(i), :].astype(F32)
                           + 0.5 * jnp.concatenate(f, axis=0))
        return carry

    with jax.named_scope("phase_a"):
        lax.fori_loop(1, na + 1, phase_a, 0)

    for cp in w_copies[1:]:
        cp.wait()

    qk_scale = (D ** -0.5) * math.log2(math.e)

    HM = TM // 32 * 16

    def put7(dst, r0, cs, *p):
        if len(p) == 4:
            ops = enumerate(_sa(*p))
        else:
            ops = zip((1, 2, 3, 4), (p[0] + p[1], *p, p[0] + p[1]))
        for k, t in ops:
            dst[pl.ds(k * PR + r0 // 2, 8), cs] = pltpu.bitcast(
                t.astype(BF16), jnp.uint32)

    def get7(src, k, ds=pl.ds, nr=None):
        nr = nr or (TM - HM if 1 <= k <= 4 else HM)
        return pltpu.bitcast(src[ds(k * PR, nr // 2), :], BF16)

    def groups(r0):
        return (r0, HM + r0) if r0 < HM else (HM + r0,)

    def q_ops(i, r0, c, z):
        p = [hs[rows(i, r, 16), col(2 * h + c)].astype(F32)
             for r in groups(r0) for h in range(2)]
        p[0] = p[0] + _rep(z.v(), 16)
        p[-1] = p[-1] + _rep(z.v(), 16)
        put7(hq7, r0, col(c), *p)

    def q_items(i):
        return [functools.partial(q_ops, i, r0, c)
                for r0 in range(0, TM - HM, 16) for c in range(2)]

    def fold(u, carry):
        nr = TA // 2
        sched = _Sched(zero)
        sched.add([functools.partial(ln_out, N - TA + u * nr, r, RF)
                   for r in range(0, nr // 2, RF)], 0, 3 * D)
        sched.add(q_items(0), 0, 3 * D)
        css = [pl.ds(pl.multiple_of(u * 128, 128) + h * H, 128)
               for h in range(2)]
        for dst, scale in ((mq, qk_scale), (wvo, 1.0)):
            t = []
            for cs in css:
                t.append(_dot_nt(wq[...], wk[cs, :]) if dst is mq
                         else _dot(wv[...], wo[:, cs]))
                sched(t[-1])
            if dst is mq:
                t = [v * scale for v in t]
            for k, v in enumerate(
                    _sb(t[0][:H], t[1][:H], t[0][H:], t[1][H:])):
                dst[k, :, css[0]] = v.astype(BF16)
        return carry

    lax.fori_loop(0, 2, fold, 0)
    dwf = dw[...].astype(F32)
    for k in range(K):
        dwb[k] = jnp.broadcast_to(dwf[k:k + 1, :], (8, D))

    def conv_block(p, r0, c, done, CT=CT, AT=K):
        cs = col(c)
        acc = [None]

        def item(k0, z=None):
            for k in range(k0, min(k0 + CT, K)):
                off = HALO - K // 2 + k + r0
                w = dwb[k, :, cs]
                if z is not None and k - k0 < AT:
                    w = w + z.v()
                t = gs[p + 1, c, off:off + 8, :] * w
                acc[0] = t if acc[0] is None else acc[0] + t
            if k0 + CT >= K:
                dcs[rows(p, r0, 8), cs] = acc[0]
                done(acc[0])

        return [functools.partial(item, k0) for k0 in range(0, K, CT)]

    def conv_main(p, cols=range(NCB), **kw):
        st = []

        def stats(r0, c, acc):
            if r0 == 0:
                st[:] = [acc, None, None]
                return
            shift, s1, s2 = st
            d = acc - shift
            s1 = d if s1 is None else s1 + d
            s2 = d * d if s2 is None else s2 + d * d
            st[:] = [shift, s1, s2]
            if r0 + 16 == TM:
                dm = s1 * (1.0 / (TM // 8 - 1))
                st_mean[p, :, col(c)] = shift + dm
                st_m2[p, :, col(c)] = s2 - s1 * dm

        return [it for c in cols for r0 in range(0, TM - 8, 8)
                for it in conv_block(p, r0, c,
                                     functools.partial(stats, r0, c), **kw)]

    def conv_edge(p, cols=range(NCB)):
        return [it for c in cols
                for it in conv_block(p, TM - 8, c, lambda acc: None)]


    def phase_b(i, carry):
        b = i // tpb

        sched = _Sched(zero)
        sched.add(conv_edge(jnp.maximum(i - 2, 0))
                  + conv_main(jnp.maximum(i - 1, 0), range(L0, NCB)),
                  int(B_SLOTS[0] * TM), int(B_SLOTS[1] * TM))
        sched.add(q_items(jnp.minimum(i + 1, nt - 1)),
                  int(Q_SLOTS[0] * TM), int(Q_SLOTS[1] * TM))
        acc = [None] * 4
        for k in OQ:
            t = _dot(get7(hq7, k), mq[k])
            _acc7(acc, k, t, HM)
            sched(t)
        q11, q12, q21, q22 = _quads(
            jnp.concatenate(_join(acc, HM), axis=1), HM)
        q7 = [q11[:HM] - q22[:HM], q21 - q22, q11, q22, q12 - q11,
              q21[:HM] - q11[:HM], q12[:HM] - q22[:HM]]
        q7 = [t.astype(BF16) for t in q7]

        dz = zero_s[0]
        p_buf, al_buf = (p_buf0, p_buf1), (al_buf0, al_buf1)

        def dyn(r0, n):
            return pl.ds(pl.multiple_of(dz + r0, 8), n)

        nb = KP // 128

        def chunk(j):
            return pl.ds(pl.multiple_of(b * TP, KP) + j * KP, KP)

        def combine(m, j, c):
            if len(m) == 7:
                s = [m[0] + m[3] + m[4] + m[6], m[2] + m[4],
                     m[1] + m[3], m[1] - m[0] + m[2] + m[5]]
            else:
                s = [m[0] + m[2], m[1] + m[3]]
            nv = T // 2 - j * KP - c * 128
            if nv < 128:
                lane = lax.broadcasted_iota(jnp.int32, s[0].shape, 1)
                s = [jnp.where(lane < nv, t, -jnp.inf) for t in s]
            return s

        stat = {}

        def put(w, j, r, v):
            for r0 in range(0, v.shape[0], 16):
                stat[w, j, r + r0] = v[r0:r0 + 16]

        def get(w, j, r, n=16):
            return jnp.concatenate(
                [stat[w, j, r0] for r0 in range(r, r + n, 16)], axis=0)

        def scores(j):
            m = [None] * 7
            for k in OS if j else OS0:
                m[k] = _dot_nt(q7[k],
                               ks[(0, 2, 1, 4, 3, 5, 6)[k], chunk(j), :])
                sched(m[k])
            mx = None
            for c in range(nb):
                s = combine([t[:HM, col(c)] for t in m], j, c)
                e = combine([t[HM:, col(c)] for t in m[1:5]], j, c)
                for h in range(2):
                    t = jnp.concatenate([s[h], s[2 + h], e[h]], axis=0)
                    s_buf[:, col(h * nb + c)] = t
                    mx = t if mx is None else jnp.maximum(mx, t)
            mx = jnp.broadcast_to(jnp.max(mx, axis=-1, keepdims=True),
                                  mx.shape)
            if j:
                mx = jnp.maximum(mx, get(0, j - 1, 0, TM))
            put(0, j, 0, mx)

        part = {}

        def soft1(j, r, c0, z):
            rs = slice(r, r + 16)
            m = get(0, j, r) + _rep(z.v(), 16)
            l = functools.reduce(jnp.add, part.pop(r, []) + [
                jnp.exp2(s_buf[dyn(r, 16), col(c)] - m)
                for c in range(c0, c0 + S1)])
            if c0 + S1 < 2 * nb:
                part[r] = [l]
                return
            l = jnp.broadcast_to(jnp.sum(l, axis=-1, keepdims=True),
                                 (16, 128))
            if j:
                l += get(1, j - 1, r) * jnp.exp2(get(0, j - 1, r) - m)
            put(1, j, r, l)
            e = (pltpu.bitcast(l, jnp.int32) >> 23) - 127
            ref = m + e.astype(F32)
            put(2, j, r, ref)
            if j:
                al_buf[j % 2][rs, :] = jnp.exp2(get(2, j - 1, r) - ref)

        def soft2(j, r0, c0, z):
            ref = [get(2, j, r) + _rep(z.v(), 16) for r in groups(r0)]
            p = [jnp.concatenate(
                [jnp.exp2(s_buf[dyn(r, 16), col(h * nb + c)] - m)
                 for c in range(c0, c0 + S2)], axis=1)
                 for r, m in zip(groups(r0), ref) for h in range(2)]
            put7(p_buf[j % 2], r0, slice(c0 * 128, (c0 + S2) * 128), *p)

        def add_soft(j, dur):
            rbs = range(0, TM - HM, 16)
            u = (dur - sum(SD)) // (len(rbs) + 1)
            for n, r0 in enumerate(rbs):
                its = [[functools.partial(soft1, j, r, c)
                        for r in groups(r0) for c in range(0, 2 * nb, S1)],
                       [functools.partial(soft2, j, r0, c)
                        for c in range(0, nb, S2)]]
                for k, it in enumerate(its):
                    t0 = sched.now + SD[0] + n * u + k * (u + SD[1])
                    sched.add(it, t0, t0 + u)

        scd = 7 * HM + 4 * (TM - 2 * HM)

        scores(0)
        add_soft(0, scd)
        acc = [None] * 4
        for j in range(nkc):
            if j + 1 < nkc:
                scores(j + 1)
                add_soft(j + 1, scd * (2 if j + 2 < nkc else 1))
            fresh = [j > 0] * 4
            for k in OP if j + 1 < nkc else OQ:
                w = ks[(0, 2, 6, 5, 3, 4, 1)[k], chunk(j), :]
                m = _dot(get7(p_buf[j % 2], k, dyn), w)
                sched(m)
                for a, _ in _TG[k]:
                    if fresh[a]:
                        al = al_buf[j % 2][dyn(0, TM), :]
                        al = _quads(jnp.concatenate([al] * NCB, axis=1), HM)[a]
                        acc[a] = acc[a] * al[:acc[a].shape[0]]
                        fresh[a] = False
                _acc7(acc, k, m, HM)
        assert not sched.queue
        t = jnp.exp2(get(2, nkc - 1, 0, TM) - get(0, nkc - 1, 0, TM))
        t = t / get(1, nkc - 1, 0, TM)
        o = (jnp.concatenate(_join(acc, HM), axis=1)
             * jnp.concatenate([t] * NCB, axis=1))
        o7 = [t.astype(BF16) for t in _sax(*_quads(o, HM), HM)]
        acc = list(_quads(xs[rows(i), :], HM))
        acc = [acc[0][:HM], acc[1], acc[2], acc[3][:HM]]
        for k in OW:
            _acc7(acc, k, _dot(o7[k], wvo[k]), HM)
        x2 = jnp.concatenate(_join(acc, HM), axis=1)
        xs[rows(i), :] = x2
        h7 = [t.astype(BF16) for t in _sax(*_quads(_ln(x2), HM), HM)]
        sched = _Sched(zero)
        acc = [[None] * 4 for _ in range(2)]
        for n, (h, k) in enumerate(PO):
            t = _dot(h7[k], w7[2 * nfc + h, k])
            _acc7(acc[h], k, t, HM)
            sched(t)
            if any(e[0] == h for e in PO[n + 1:]):
                continue
            val, gate = _join(acc[h], HM)
            g2 = val * (0.5 + 0.5 * jnp.tanh(0.5 * gate))
            for c in (2 * h, 2 * h + 1):
                g = g2[:, col(c % 2)]
                gs[i + 1, c, HALO:HALO + TM, :] = g
                gs[i, c, HALO + TM:, :] = jnp.where(i % tpb == 0, 0.0,
                                                    g[:HALO])
                gs[i + 2, c, :HALO, :] = jnp.where(i % tpb == tpb - 1, 0.0,
                                                   g[TM - HALO:])
            if h == 0 and L0:
                rest = sum(h7[e[1]].shape[0] for e in PO[n + 1:])
                sched.add(conv_main(i, range(L0), CT=LP[2], AT=LP[3]),
                          sched.now + LP[0], sched.now + rest - LP[1])
        assert not sched.queue
        return carry

    with jax.named_scope("phase_b"):
        lax.fori_loop(0, nt, phase_b, 0)
    for item in (conv_main(nt - 1, range(L0, NCB)) + conv_edge(nt - 2)
                 + conv_edge(nt - 1)):
        item()

    ng = TM // 8 - 1
    means = st_mean[...].reshape(nt * 8, D)
    edges = jnp.concatenate([dcs[(p + 1) * TM - 8:(p + 1) * TM, :]
                             for p in range(nt)], axis=0)
    mu = jnp.sum(ng * means + edges, axis=0, keepdims=True) * (1.0 / N)
    dm = means - mu
    de = edges - mu
    var = jnp.sum(st_m2[...].reshape(nt * 8, D) + ng * (dm * dm) + de * de,
                  axis=0, keepdims=True) * (1.0 / N)
    rstd = lax.rsqrt(var + EPS)
    bn[0] = jnp.broadcast_to(mu, (8, D))
    bn[1] = jnp.broadcast_to(rstd, (8, D))

    def bn_silu(i, r0, c, z=None):
        p = []
        for r in (r0, TC // 2 + r0):
            for h in range(2):
                cs = col(2 * h + c)
                mu = bn[0, :, cs] if z is None else bn[0, :, cs] + z.v()
                y = dcs[crows(i, r, 16), cs] - _rep(mu, 16)
                p.append(_silu(y * _rep(bn[1, :, cs], 16)))
        put7(hq7, r0, col(c), *p)

    def bn_items(i):
        return [functools.partial(bn_silu, i, r0, c)
                for r0 in range(0, TC // 2, 16) for c in range(2)]

    def ln_final(i, r0=0, n=TC, z=None):
        obuf[crows(i, r0, n), :] = _ln(xs[crows(i, r0, n), :],
                                       zrep(z, n)).astype(BF16)

    for item in bn_items(0):
        item()

    def phase_c(i, carry):
        @pl.when(i >= 2)
        def _():
            o_copy(i - 2).start()

        sched = _Sched(zero)
        dur = 7 * (1 + 2 * nfc) * TC // 2
        t0, t1 = int(C_WIN[0] * dur), int(C_WIN[1] * dur)
        sched.add([functools.partial(ln_final, jnp.maximum(i - 1, 0), r, RC[0])
                   for r in range(0, TC, RC[0])], t0, t1, C_SKIP)
        sched.add(bn_items(jnp.minimum(i + 1, nc - 1)),
                  t0 + RC[1], t1 + RC[1], C_SKIP)
        acc = list(_quads(xs[crows(i), :], TC // 2))
        for k in OQ:
            t = _dot(get7(hq7, k, nr=TC // 2), w7[2 * nfc + 2, k])
            _acc7(acc, k, t, TC // 2)
            sched(t)
        x3 = jnp.concatenate(_join(acc, TC // 2), axis=1)
        xs[crows(i), :] = x3
        h = _ln(x3)
        f = _ffn7(_lhs7(h[:TC // 2], h[TC // 2:]),
                  [w7.at[c] for c in range(nfc)],
                  [w7.at[nfc + c] for c in range(nfc)], sched, FE)
        assert not sched.queue
        xs[crows(i), :] += 0.5 * jnp.concatenate(f, axis=0)
        return carry

    with jax.named_scope("phase_c"):
        lax.fori_loop(0, nc, phase_c, 0)
    o_copy(nc - 2).start()
    last = []
    for k, (r0, r1) in enumerate(zip(EP[:-1], EP[1:])):
        ln_final(nc - 1, r0, r1 - r0)
        rs = crows(nc - 1, r0, r1 - r0)
        last.append(pltpu.make_async_copy(obuf.at[rs, :], out_hbm.at[rs, :],
                                          osem.at[nc - 1 + k]))
        last[-1].start()
    for i in range(nc - 1):
        o_copy(i).wait()
    for cp in last:
        cp.wait()


@jax.jit
def pallas_standalone__conformer_family_conformer__speech_kernel(
    x: jax.Array,
    w_ff1_a: jax.Array,
    w_ff1_b: jax.Array,
    w_q: jax.Array,
    w_k: jax.Array,
    w_v: jax.Array,
    w_o: jax.Array,
    w_pw1: jax.Array,
    dw: jax.Array,
    w_pw2: jax.Array,
    w_ff2_a: jax.Array,
    w_ff2_b: jax.Array,
):
    B, T, D = x.shape
    K = dw.shape[0]
    N = B * T
    weights = (w_ff1_a, w_ff1_b, w_q, w_k, w_v, w_o, w_pw1, dw, w_pw2,
               w_ff2_a, w_ff2_b)
    scratch = [pltpu.VMEM((N, D), BF16)]
    nfc = w_ff1_a.shape[1] // FC
    scratch += [pltpu.VMEM((4 * nfc + 3, D, D), BF16)]
    scratch += [pltpu.VMEM(w.shape, w.dtype)
                for w in (w_q, w_k, w_v, w_o, dw)]
    scratch += [
        pltpu.VMEM((7, D // 2, D // 2), BF16),
        pltpu.VMEM((7, D // 2, D // 2), BF16),
        pltpu.VMEM((N, D), F32),
        pltpu.VMEM((N, D), BF16),
        pltpu.VMEM((7, B * -(-T // KC) * KC // 2, D // 2), BF16),
        pltpu.VMEM((N // TM + 2, D // 128, TM + 2 * HALO, 128), F32),
        pltpu.VMEM((N, D), F32),
        pltpu.VMEM((N // TM, 8, D), F32),
        pltpu.VMEM((N // TM, 8, D), F32),
        pltpu.VMEM((2, 8, D), F32),
        pltpu.VMEM((7, TA // 2, D // 2), BF16),
        pltpu.VMEM((2, nfc, 7, D // 2, D // 2), BF16),
        pltpu.VMEM((2 * nfc + 3, 7, D // 2, D // 2), BF16),
        pltpu.VMEM((T0, D), BF16),
        pltpu.VMEM((K, 8, D), F32),
        pltpu.VMEM((ZR, 128), jnp.uint32),
        pltpu.SMEM((1,), jnp.int32),
        pltpu.VMEM((TM + 16, 128), F32),
        pltpu.VMEM((TM + 16, 128), F32),
        pltpu.VMEM((7 * PR, KC // 2), jnp.uint32),
        pltpu.VMEM((7 * PR, KC // 2), jnp.uint32),
        pltpu.VMEM((TM, KC), F32),
        pltpu.VMEM((7 * PR, D // 2), jnp.uint32),
        pltpu.SemaphoreType.DMA(((N - T0) // TA + 1,)),
        pltpu.SemaphoreType.DMA((2, nfc)),
        pltpu.SemaphoreType.DMA((3, nfc)),
        pltpu.SemaphoreType.DMA((6,)),
        pltpu.SemaphoreType.DMA((N // TC + len(EP),)),
    ]
    out = pl.pallas_call(
        functools.partial(_kernel, B=B, T=T, D=D, K=K),
        out_shape=jax.ShapeDtypeStruct((N, D), x.dtype),
        in_specs=[pl.BlockSpec(memory_space=pl.ANY)] * 12,
        out_specs=pl.BlockSpec(memory_space=pl.ANY),
        scratch_shapes=scratch,
        compiler_params=pltpu.CompilerParams(
            vmem_limit_bytes=120 * 1024 * 1024),
    )(x.reshape(N, D), *weights)
    return out.reshape(B, T, D)
```

```python
import functools
import math

import jax
import jax.numpy as jnp
from jax import lax
import jax.experimental.pallas as pl
import jax.experimental.pallas.tpu as pltpu

F32 = jnp.float32
BF16 = jnp.bfloat16

TM = 400
T0 = 320
TA = 320
TC = 320
FC = 512
KC = 512
IW = 5
O1 = (0, 1, 2, 3, 4, 5, 6)
O2 = (1, 3, 6, 0, 2, 4, 5)
FE = ((0, 2), (0, 4), (1, 2), (1, 4))
OQ = (0, 2, 3, 4, 6, 1, 5)
OS0 = (2, 4, 3, 1, 0, 5, 6)
OS = (0, 1, 2, 3, 4, 5, 6)
OP = (0, 1, 2, 3, 4, 5, 6)
OW = (2, 4, 3, 0, 6, 1, 5)
PO = ((0, 2), (0, 4), (1, 2), (0, 3), (0, 0), (0, 6), (0, 1), (0, 5),
      (1, 4), (1, 3), (1, 0), (1, 6), (1, 1), (1, 5))
FRB = 16
F_WIN = (0.1, 0.9)
RA = 8
RO = 8
A_WIN = (0.05, 0.8)
A_SKIP = (700, 1400)
RF = 8
B_SLOTS = (1, 53)
Q_SLOTS = (8, 50)
CT = 5
L0 = 1
LP = (0, 100, 3, 1)
S1 = 2
S2 = 1
SD = (0, 140, 120)
LAG = 2
SW = tuple(1 + 1.75 * j for j in range(9))
C_WIN = (0.29, 0.86)
C_SKIP = ((4200, 5100), (6450, 7350), (8700, 9600))
RC = (8, 100)
EP = (0, 128, 224, 288, 320)
ZR = 32
PR = 112
HALO = 8
EPS = 1e-05


def _ln(x, z=None):
    if z is None:
        m = jnp.mean(x, axis=-1, keepdims=True)
    else:
        t = z
        for c in range(x.shape[-1] // 128):
            t = t + x[:, c * 128:(c + 1) * 128]
        m = jnp.sum(t, axis=-1, keepdims=True) * (1.0 / x.shape[-1])
    xc = x - m
    v = jnp.mean(xc * xc, axis=-1, keepdims=True)
    return xc * lax.rsqrt(v + EPS)


def _silu(a):
    y = 0.5 * a
    return y + y * jnp.tanh(y)


def _dot(a, b):
    return jnp.dot(a, b, preferred_element_type=F32)


def _dot_nt(a, b):
    return lax.dot_general(a, b, (((1,), (1,)), ((), ())),
                           preferred_element_type=F32)


class _Anchor:
    def __init__(self, t, zero_v):
        self.t, self.zero_v = t, zero_v

    def v(self):
        return pltpu.bitcast(
            pltpu.bitcast(self.t, jnp.uint32) & self.zero_v[0:8, :], F32)


class _Sched:
    def __init__(self, zero_v):
        self.zero_v = zero_v
        self.queue = []
        self.now = 0

    def add(self, items, t0, t1, skip=()):
        assert t0 >= self.now
        ts = [t for t in range(t0, t1)
              if not any(a <= t < b for a, b in skip)]
        self.queue += [(ts[k * len(ts) // len(items)], it)
                       for k, it in enumerate(items)]
        self.queue.sort(key=lambda e: e[0])

    def __call__(self, t, dur=None):
        dur = dur or t.shape[0]
        end = self.now + dur
        while self.queue and self.queue[0][0] < end:
            time, item = self.queue.pop(0)
            r = (time - self.now) * t.shape[0] // dur // 8 * 8
            item(_Anchor(t[r:r + 8, :128], self.zero_v))
        self.now = end


def _rep(z, rows):
    return jnp.concatenate([z] * (rows // 8), axis=0)


def _ffn(h, wa_ref, wb_ref, sched):
    ss = []
    for n in range(wa_ref.shape[1] // 128):
        a = _dot(h, wa_ref[:, n * 128:(n + 1) * 128])
        ss.append(_silu(a))
        sched(a)
    s = jnp.concatenate(ss, axis=1).astype(BF16)
    acc = []
    for n in range(wb_ref.shape[1] // 128):
        acc.append(_dot(s, wb_ref[:, n * 128:(n + 1) * 128]))
        sched(acc[-1])
    return jnp.concatenate(acc, axis=1)


def _sa(a11, a12, a21, a22):
    return [a11 + a22, a21 + a22, a11, a22, a11 + a12, a21 - a11, a12 - a22]


def _sb(b11, b12, b21, b22):
    return [b11 + b22, b11, b12 - b22, b21 - b11, b22, b11 + b12, b21 + b22]


def _sc(m):
    return [m[0] + m[3] - m[4] + m[6], m[4] + m[2], m[3] + m[1],
            m[0] + m[2] - m[1] + m[5]]


def _lhs7(t, u):
    h = t.shape[1] // 2
    return [v.astype(BF16)
            for v in _sa(t[:, :h], t[:, h:], u[:, :h], u[:, h:])]


_TG = (((0, 1), (3, 1)), ((2, 1), (3, -1)), ((1, 1), (3, 1)), ((0, 1), (2, 1)),
       ((0, -1), (1, 1)), ((3, 1),), ((0, 1),))


def _quads(x, hm):
    h = x.shape[1] // 2
    t = x[:hm]
    if x.shape[0] > 2 * hm:
        t = jnp.concatenate([t, x[2 * hm:]], axis=0)
    return t[:, :h], t[:, h:], x[hm:, :h], x[hm:, h:]


def _sax(a11, a12, a21, a22, hm):
    return [a11[:hm] + a22[:hm], a21 + a22, a11, a22, a11 + a12,
            a21[:hm] - a11[:hm], a12[:hm] - a22[:hm]]


def _acc7(acc, k, m, hm):
    for a, sg in _TG[k]:
        t = m if a in (1, 2) else m[:hm]
        if acc[a] is None:
            acc[a] = t if sg > 0 else -t
        else:
            acc[a] = acc[a] + t if sg > 0 else acc[a] - t


def _join(acc, hm):
    rest = [acc[1][hm:]] if acc[1].shape[0] > hm else []
    return (jnp.concatenate([acc[0], acc[2]], axis=0),
            jnp.concatenate([acc[1][:hm], acc[3]] + rest, axis=0))


def _ffn7(h7, wa, wb, sched, early=()):
    acc = [None] * 7
    hm = h7[0].shape[0]
    u = [[None] * 4 for _ in wa]

    def first(c, k):
        t = _dot(h7[k], wa[c][k])
        _acc7(u[c], k, t, hm)
        sched(t)

    for c, k in early:
        first(c, k)
    for c, cb in enumerate(wb):
        for k in O1:
            if (c, k) not in early:
                first(c, k)
        s7 = [t.astype(BF16) for t in _sa(*[_silu(t) for t in u[c]])]
        for k in O2:
            p = _dot(s7[k], cb[k])
            acc[k] = p if acc[k] is None else acc[k] + p
            sched(p)
    c = _sc(acc)
    return jnp.concatenate(c[:2], axis=1), jnp.concatenate(c[2:], axis=1)


def _kernel(x_hbm, w1a_hbm, w1b_hbm, wq_hbm, wk_hbm, wv_hbm, wo_hbm,
            wp1_hbm, dw_hbm, wp2_hbm, w2a_hbm, w2b_hbm,
            out_hbm,
            xin, wblk, wq, wk, wv, wo, dw,
            mq, wvo, xs, hs, ks, gs, dcs, st_mean, st_m2, bn,
            lhs7, w17, w7, lhs_b, dwb, zero, zero_s, al_buf0, al_buf1, al_buf2,
            p_buf0, p_buf1, p_buf2, s_buf0, s_buf1, hq7,
            xsem, w1sem, w2sem, wsem, osem,
            *, B, T, D, K):
    N = B * T
    obuf = xin
    KP = KC // 2
    nkc = -(-T // KC)
    TP = nkc * KP
    NCB = D // 128
    nt = N // TM
    tpb = T // TM

    def rows(i, r0=0, n=TM):
        return pl.ds(pl.multiple_of(i * TM, 16) + r0, n)

    def col(c):
        if isinstance(c, int):
            return slice(c * 128, (c + 1) * 128)
        return pl.ds(pl.multiple_of(c * 128, 128), 128)

    na = (N - T0) // TA
    H = D // 2

    def arows(i, r0=0, n=TA):
        return pl.ds(pl.multiple_of(T0 + (i - 1) * TA, 16) + r0, n)

    def x_copy(i):
        rs = pl.ds(0, T0) if isinstance(i, int) and i == 0 else arows(i)
        return pltpu.make_async_copy(x_hbm.at[rs, :], xin.at[rs, :],
                                     xsem.at[i])

    nc = N // TC

    def crows(i, r0=0, n=TC):
        return pl.ds(pl.multiple_of(i * TC, 16) + r0, n)

    def o_copy(i):
        return pltpu.make_async_copy(obuf.at[crows(i), :],
                                     out_hbm.at[crows(i), :], osem.at[i])

    nfc = w17.shape[1]
    P1, P2 = 4 * nfc, 4 * nfc + 2

    def w1_copies(c):
        fs = pl.ds(pl.multiple_of(c * FC, FC), FC)
        return [pltpu.make_async_copy(w1a_hbm.at[:, fs], wblk.at[c],
                                      w1sem.at[0, c]),
                pltpu.make_async_copy(w1b_hbm.at[fs, :], wblk.at[nfc + c],
                                      w1sem.at[1, c])]

    def w2_copies(c):
        fs = pl.ds(pl.multiple_of(c * FC, FC), FC)
        hs_ = pl.ds(pl.multiple_of(c // 2 * H, H), H)
        return [pltpu.make_async_copy(s, d, w2sem.at[j, c])
                for j, (s, d) in enumerate([
                    (w2a_hbm.at[:, fs], wblk.at[2 * nfc + c]),
                    (w2b_hbm.at[fs, :], wblk.at[3 * nfc + c]),
                    (wp1_hbm.at[:, pl.ds(pl.multiple_of(c * H, H), H)],
                     wblk.at[P1 + c % 2, :, hs_])])]

    assert nfc == 4
    w_pairs = [(wp2_hbm, wblk.at[P2]), (wq_hbm, wq), (wk_hbm, wk),
               (wv_hbm, wv), (wo_hbm, wo), (dw_hbm, dw)]
    w_copies = [pltpu.make_async_copy(s, d, wsem.at[j])
                for j, (s, d) in enumerate(w_pairs)]

    x_copy(0).start()
    for cp in w1_copies(0):
        cp.start()

    zero[...] = jnp.zeros(zero.shape, jnp.uint32)
    zero_s[0] = 0
    for c in range(NCB):
        gs[1, c, 0:HALO, :] = jnp.zeros((HALO, 128), F32)
        gs[nt, c, HALO + TM:, :] = jnp.zeros((HALO, 128), F32)
    for b in range(B):
        ks[:, b * TP + T // 2:(b + 1) * TP, :] = jnp.zeros(
            (7, TP - T // 2, H), BF16)

    def zrep(z, n):
        return None if z is None else _rep(z.v(), n)

    def ln_in(i, r0, n, z=None):
        t, u = [_ln(xin[arows(i, r + r0, n), :].astype(F32), zrep(z, n))
                for r in (0, TA // 2)]
        for k, v in enumerate(_lhs7(t, u)):
            lhs7[k, pl.ds(r0, n), :] = v

    def ln_out(base, r0, n, z=None):
        tu = []
        for r in (0, 16):
            rs = pl.ds(pl.multiple_of(base, 32) + r0 // 16 * 32 + r0 % 16 + r,
                       n)
            tu.append(_ln(xs[rs, :], zrep(z, n)))
            hs[rs, :] = tu[-1].astype(BF16)
        g = base // 32 + r0 // 16
        g += g // (T // 32) * ((TP - T // 2) // 16)
        ps = pl.ds(pl.multiple_of(g * 16, 16) + r0 % 16, n)
        for k, v in enumerate(_lhs7(*tu)):
            ks[k, ps, :] = v

    def prep(src, dst, r0, z=None):
        q = [src[pl.ds(r + r0, 16), c:c + H].astype(F32)
             for r in (0, H) for c in (0, H)]
        if z is not None:
            zz = jnp.concatenate([_rep(z.v(), 16)] * (H // 128), axis=1)
            q[0], q[3] = q[0] + zz, q[3] + zz
        for k, v in enumerate(_sb(*q)):
            dst[k, pl.ds(r0, 16), :] = v.astype(BF16)

    x_copy(0).wait()
    lhs_b[...] = _ln(xin[0:T0, :].astype(F32)).astype(BF16)
    xs[0:T0, :] = xin[0:T0, :].astype(F32)

    def first_tile(c, carry):
        for cp in w1_copies(c):
            cp.wait()

        @pl.when(c == 1)
        def _():
            x_copy(1).wait()

        @pl.when(c + 1 < nfc)
        def _():
            for cp in w1_copies(c + 1):
                cp.start()

        @pl.when(c % 2 == 0)
        def _():
            x_copy(1 + c // 2).start()

        n = -(-TA // 2 // (nfc - 1) // 16) * 16
        step = (TA // 2 - n) // (nfc - 2)
        assert step % 16 == 0 and step <= n
        r0 = pl.multiple_of(jnp.maximum(c - 1, 0) * step, 16)
        assert T0 == TA
        sched = _Sched(zero)
        dur = 2 * NCB * T0
        sched.add([functools.partial(ln_in, jnp.minimum(c, 1), r0 + r, FRB)
                   for r in range(0, n, FRB)],
                  int(F_WIN[0] * dur), int(F_WIN[1] * dur))
        sched.add([functools.partial(prep, wblk.at[j * nfc + c],
                                     w17.at[j, c], r)
                   for j in range(2) for r in range(0, H, 16)],
                  int(F_WIN[0] * dur), int(F_WIN[1] * dur))
        f = _ffn(lhs_b[...], wblk.at[c], wblk.at[nfc + c], sched)
        assert not sched.queue
        xs[0:T0, :] += 0.5 * f
        return carry

    lax.fori_loop(0, nfc, first_tile, 0)
    for j in range(3, na + 1):
        x_copy(j).start()
    for c in range(nfc):
        for cp in w2_copies(c):
            cp.start()
    for cp in w_copies:
        cp.start()

    def phase_a(i, carry):
        @pl.when(i < na)
        def _():
            x_copy(i + 1).wait()

        @pl.when((i >= IW) & (i < IW + nfc))
        def _():
            for cp in w2_copies(i - IW):
                cp.wait()

        @pl.when(i == IW)
        def _():
            w_copies[0].wait()

        h7 = [lhs7[k] for k in range(7)]
        sched = _Sched(zero)
        dur = 7 * nfc * TA
        win = (int(A_WIN[0] * dur), int(A_WIN[1] * dur),
               [(c * 7 * TA + A_SKIP[0], c * 7 * TA + A_SKIP[1])
                for c in range(nfc)])
        sched.add([functools.partial(ln_out, T0 + (i - 2) * TA, r, RO)
                   for r in range(0, TA // 2, RO)], *win)
        sched.add([functools.partial(ln_in, jnp.minimum(i + 1, na), r, RA)
                   for r in range(0, TA // 2, RA)], *win)
        rpb = H // 16
        total = w7.shape[0] * rpb
        ipi = -(-total // (na - IW + 1))
        items = []
        for k in range(ipi):
            n = jnp.minimum(jnp.maximum(i - IW, 0) * ipi + k, total - 1)
            src = n // rpb + jnp.where(i >= IW, 2 * nfc, 0)
            items.append(functools.partial(
                prep, wblk.at[src], w7.at[n // rpb],
                pl.multiple_of(n % rpb * 16, 16)))
        assert ipi <= rpb
        sched.add(items, *win)
        f = _ffn7(h7, [w17.at[0, c] for c in range(nfc)],
                  [w17.at[1, c] for c in range(nfc)], sched)
        assert not sched.queue
        xs[arows(i), :] = (xin[arows(i), :].astype(F32)
                           + 0.5 * jnp.concatenate(f, axis=0))
        return carry

    with jax.named_scope("phase_a"):
        lax.fori_loop(1, na + 1, phase_a, 0)

    for cp in w_copies[1:]:
        cp.wait()

    qk_scale = (D ** -0.5) * math.log2(math.e)

    HM = TM // 32 * 16

    def put7(dst, r0, cs, *p):
        if len(p) == 4:
            ops = enumerate(_sa(*p))
        else:
            ops = zip((1, 2, 3, 4), (p[0] + p[1], *p, p[0] + p[1]))
        for k, t in ops:
            dst[pl.ds(k * PR + r0 // 2, 8), cs] = pltpu.bitcast(
                t.astype(BF16), jnp.uint32)

    def get7(src, k, ds=pl.ds, nr=None):
        nr = nr or (TM - HM if 1 <= k <= 4 else HM)
        return pltpu.bitcast(src[ds(k * PR, nr // 2), :], BF16)

    def groups(r0):
        return (r0, HM + r0) if r0 < HM else (HM + r0,)

    def q_ops(i, r0, c, z):
        p = [hs[rows(i, r, 16), col(2 * h + c)].astype(F32)
             for r in groups(r0) for h in range(2)]
        p[0] = p[0] + _rep(z.v(), 16)
        p[-1] = p[-1] + _rep(z.v(), 16)
        put7(hq7, r0, col(c), *p)

    def q_items(i):
        return [functools.partial(q_ops, i, r0, c)
                for r0 in range(0, TM - HM, 16) for c in range(2)]

    def fold(u, carry):
        nr = TA // 2
        sched = _Sched(zero)
        sched.add([functools.partial(ln_out, N - TA + u * nr, r, RF)
                   for r in range(0, nr // 2, RF)], 0, 3 * D)
        sched.add(q_items(0), 0, 3 * D)
        css = [pl.ds(pl.multiple_of(u * 128, 128) + h * H, 128)
               for h in range(2)]
        for dst, scale in ((mq, qk_scale), (wvo, 1.0)):
            t = []
            for cs in css:
                t.append(_dot_nt(wq[...], wk[cs, :]) if dst is mq
                         else _dot(wv[...], wo[:, cs]))
                sched(t[-1])
            if dst is mq:
                t = [v * scale for v in t]
            for k, v in enumerate(
                    _sb(t[0][:H], t[1][:H], t[0][H:], t[1][H:])):
                dst[k, :, css[0]] = v.astype(BF16)
        return carry

    lax.fori_loop(0, 2, fold, 0)
    dwf = dw[...].astype(F32)
    for k in range(K):
        dwb[k] = jnp.broadcast_to(dwf[k:k + 1, :], (8, D))

    def conv_block(p, r0, c, done, CT=CT, AT=K):
        cs = col(c)
        acc = [None]

        def item(k0, z=None):
            for k in range(k0, min(k0 + CT, K)):
                off = HALO - K // 2 + k + r0
                w = dwb[k, :, cs]
                if z is not None and k - k0 < AT:
                    w = w + z.v()
                t = gs[p + 1, c, off:off + 8, :] * w
                acc[0] = t if acc[0] is None else acc[0] + t
            if k0 + CT >= K:
                dcs[rows(p, r0, 8), cs] = acc[0]
                done(acc[0])

        return [functools.partial(item, k0) for k0 in range(0, K, CT)]

    def conv_main(p, cols=range(NCB), **kw):
        st = []

        def stats(r0, c, acc):
            if r0 == 0:
                st[:] = [acc, None, None]
                return
            shift, s1, s2 = st
            d = acc - shift
            s1 = d if s1 is None else s1 + d
            s2 = d * d if s2 is None else s2 + d * d
            st[:] = [shift, s1, s2]
            if r0 + 16 == TM:
                dm = s1 * (1.0 / (TM // 8 - 1))
                st_mean[p, :, col(c)] = shift + dm
                st_m2[p, :, col(c)] = s2 - s1 * dm

        return [it for c in cols for r0 in range(0, TM - 8, 8)
                for it in conv_block(p, r0, c,
                                     functools.partial(stats, r0, c), **kw)]

    def conv_edge(p, cols=range(NCB)):
        return [it for c in cols
                for it in conv_block(p, TM - 8, c, lambda acc: None)]


    def phase_b(i, carry):
        b = i // tpb

        sched = _Sched(zero)
        sched.add(conv_edge(jnp.maximum(i - 2, 0))
                  + conv_main(jnp.maximum(i - 1, 0), range(L0, NCB)),
                  int(B_SLOTS[0] * TM), int(B_SLOTS[1] * TM))
        sched.add(q_items(jnp.minimum(i + 1, nt - 1)),
                  int(Q_SLOTS[0] * TM), int(Q_SLOTS[1] * TM))
        acc = [None] * 4
        for k in OQ:
            t = _dot(get7(hq7, k), mq[k])
            _acc7(acc, k, t, HM)
            sched(t)
        q11, q12, q21, q22 = _quads(
            jnp.concatenate(_join(acc, HM), axis=1), HM)
        q7 = [q11[:HM] - q22[:HM], q21 - q22, q11, q22, q12 - q11,
              q21[:HM] - q11[:HM], q12[:HM] - q22[:HM]]
        q7 = [t.astype(BF16) for t in q7]

        dz = zero_s[0]
        p_buf, al_buf = (p_buf0, p_buf1, p_buf2), (al_buf0, al_buf1, al_buf2)
        s_buf = (s_buf0, s_buf1)

        def dyn(r0, n):
            return pl.ds(pl.multiple_of(dz + r0, 8), n)

        nb = KP // 128

        def chunk(j):
            return pl.ds(pl.multiple_of(b * TP, KP) + j * KP, KP)

        def combine(m, j, c):
            if len(m) == 7:
                s = [m[0] + m[3] + m[4] + m[6], m[2] + m[4],
                     m[1] + m[3], m[1] - m[0] + m[2] + m[5]]
            else:
                s = [m[0] + m[2], m[1] + m[3]]
            nv = T // 2 - j * KP - c * 128
            if nv < 128:
                lane = lax.broadcasted_iota(jnp.int32, s[0].shape, 1)
                s = [jnp.where(lane < nv, t, -jnp.inf) for t in s]
            return s

        stat = {}

        def put(w, j, r, v):
            for r0 in range(0, v.shape[0], 16):
                stat[w, j, r + r0] = v[r0:r0 + 16]

        def get(w, j, r, n=16):
            return jnp.concatenate(
                [stat[w, j, r0] for r0 in range(r, r + n, 16)], axis=0)

        def scores(j):
            m = [None] * 7
            for k in OS if j else OS0:
                m[k] = _dot_nt(q7[k],
                               ks[(0, 2, 1, 4, 3, 5, 6)[k], chunk(j), :])
                sched(m[k])
            mx = None
            for c in range(nb):
                s = combine([t[:HM, col(c)] for t in m], j, c)
                e = combine([t[HM:, col(c)] for t in m[1:5]], j, c)
                for h in range(2):
                    t = jnp.concatenate([s[h], s[2 + h], e[h]], axis=0)
                    s_buf[j % 2][:, col(h * nb + c)] = t
                    mx = t if mx is None else jnp.maximum(mx, t)
            mx = jnp.broadcast_to(jnp.max(mx, axis=-1, keepdims=True),
                                  mx.shape)
            if j:
                mx = jnp.maximum(mx, get(0, j - 1, 0, TM))
            put(0, j, 0, mx)

        part = {}

        def soft1(j, r, c0, z):
            rs = slice(r, r + 16)
            m = get(0, j, r) + _rep(z.v(), 16)
            l = functools.reduce(jnp.add, part.pop((j, r), []) + [
                jnp.exp2(s_buf[j % 2][dyn(r, 16), col(c)] - m)
                for c in range(c0, c0 + S1)])
            if c0 + S1 < 2 * nb:
                part[j, r] = [l]
                return
            l = jnp.broadcast_to(jnp.sum(l, axis=-1, keepdims=True),
                                 (16, 128))
            if j:
                l += get(1, j - 1, r) * jnp.exp2(get(0, j - 1, r) - m)
            put(1, j, r, l)
            e = (pltpu.bitcast(l, jnp.int32) >> 23) - 127
            ref = m + e.astype(F32)
            put(2, j, r, ref)
            if j:
                al_buf[j % 3][rs, :] = jnp.exp2(get(2, j - 1, r) - ref)

        def soft2(j, r0, c0, z):
            ref = [get(2, j, r) + _rep(z.v(), 16) for r in groups(r0)]
            p = [jnp.concatenate(
                [jnp.exp2(s_buf[j % 2][dyn(r, 16), col(h * nb + c)] - m)
                 for c in range(c0, c0 + S2)], axis=1)
                 for r, m in zip(groups(r0), ref) for h in range(2)]
            put7(p_buf[j % 3], r0, slice(c0 * 128, (c0 + S2) * 128), *p)

        scd = 7 * HM + 4 * (TM - 2 * HM)
        start = sched.now

        def add_soft(j):
            rbs = range(0, TM - HM, 16)
            t0, t1 = (start + int(t * scd) for t in SW[j:j + 2])
            assert t1 <= start + min(2 * j + LAG + 1, nkc + j) * scd
            assert j < 3 or t0 >= start + min(2 * j + LAG - 4,
                                              nkc + j - 2) * scd
            assert (j + 2 >= nkc
                    or t1 <= start + max(2 * j + 5 - LAG, j + 3) * scd)
            u = (t1 - t0 - sum(SD)) // (len(rbs) + 1)
            for n, r0 in enumerate(rbs):
                its = [[functools.partial(soft1, j, r, c)
                        for r in groups(r0) for c in range(0, 2 * nb, S1)],
                       [functools.partial(soft2, j, r0, c)
                        for c in range(0, nb, S2)]]
                for k, it in enumerate(its):
                    t = t0 + SD[0] + n * u + k * (u + SD[1])
                    sched.add(it, t, t + u)

        for j in range(LAG):
            scores(j)
            add_soft(j)
        acc = [None] * 4
        for j in range(nkc):
            if j + LAG < nkc:
                scores(j + LAG)
                add_soft(j + LAG)
            fresh = [j > 0] * 4
            for k in OP if j + 1 < nkc else OQ:
                w = ks[(0, 2, 6, 5, 3, 4, 1)[k], chunk(j), :]
                m = _dot(get7(p_buf[j % 3], k, dyn), w)
                sched(m)
                for a, _ in _TG[k]:
                    if fresh[a]:
                        al = al_buf[j % 3][dyn(0, TM), :]
                        al = _quads(jnp.concatenate([al] * NCB, axis=1), HM)[a]
                        acc[a] = acc[a] * al[:acc[a].shape[0]]
                        fresh[a] = False
                _acc7(acc, k, m, HM)
        assert not sched.queue
        t = jnp.exp2(get(2, nkc - 1, 0, TM) - get(0, nkc - 1, 0, TM))
        t = t / get(1, nkc - 1, 0, TM)
        o = (jnp.concatenate(_join(acc, HM), axis=1)
             * jnp.concatenate([t] * NCB, axis=1))
        o7 = [t.astype(BF16) for t in _sax(*_quads(o, HM), HM)]
        acc = list(_quads(xs[rows(i), :], HM))
        acc = [acc[0][:HM], acc[1], acc[2], acc[3][:HM]]
        for k in OW:
            _acc7(acc, k, _dot(o7[k], wvo[k]), HM)
        x2 = jnp.concatenate(_join(acc, HM), axis=1)
        xs[rows(i), :] = x2
        h7 = [t.astype(BF16) for t in _sax(*_quads(_ln(x2), HM), HM)]
        sched = _Sched(zero)
        acc = [[None] * 4 for _ in range(2)]
        for n, (h, k) in enumerate(PO):
            t = _dot(h7[k], w7[2 * nfc + h, k])
            _acc7(acc[h], k, t, HM)
            sched(t)
            if any(e[0] == h for e in PO[n + 1:]):
                continue
            val, gate = _join(acc[h], HM)
            g2 = val * (0.5 + 0.5 * jnp.tanh(0.5 * gate))
            for c in (2 * h, 2 * h + 1):
                g = g2[:, col(c % 2)]
                gs[i + 1, c, HALO:HALO + TM, :] = g
                gs[i, c, HALO + TM:, :] = jnp.where(i % tpb == 0, 0.0,
                                                    g[:HALO])
                gs[i + 2, c, :HALO, :] = jnp.where(i % tpb == tpb - 1, 0.0,
                                                   g[TM - HALO:])
            if h == 0 and L0:
                rest = sum(h7[e[1]].shape[0] for e in PO[n + 1:])
                sched.add(conv_main(i, range(L0), CT=LP[2], AT=LP[3]),
                          sched.now + LP[0], sched.now + rest - LP[1])
        assert not sched.queue
        return carry

    with jax.named_scope("phase_b"):
        lax.fori_loop(0, nt, phase_b, 0)
    for item in (conv_main(nt - 1, range(L0, NCB)) + conv_edge(nt - 2)
                 + conv_edge(nt - 1)):
        item()

    ng = TM // 8 - 1
    means = st_mean[...].reshape(nt * 8, D)
    edges = jnp.concatenate([dcs[(p + 1) * TM - 8:(p + 1) * TM, :]
                             for p in range(nt)], axis=0)
    mu = jnp.sum(ng * means + edges, axis=0, keepdims=True) * (1.0 / N)
    dm = means - mu
    de = edges - mu
    var = jnp.sum(st_m2[...].reshape(nt * 8, D) + ng * (dm * dm) + de * de,
                  axis=0, keepdims=True) * (1.0 / N)
    rstd = lax.rsqrt(var + EPS)
    bn[0] = jnp.broadcast_to(mu, (8, D))
    bn[1] = jnp.broadcast_to(rstd, (8, D))

    def bn_silu(i, r0, c, z=None):
        p = []
        for r in (r0, TC // 2 + r0):
            for h in range(2):
                cs = col(2 * h + c)
                mu = bn[0, :, cs] if z is None else bn[0, :, cs] + z.v()
                y = dcs[crows(i, r, 16), cs] - _rep(mu, 16)
                p.append(_silu(y * _rep(bn[1, :, cs], 16)))
        put7(hq7, r0, col(c), *p)

    def bn_items(i):
        return [functools.partial(bn_silu, i, r0, c)
                for r0 in range(0, TC // 2, 16) for c in range(2)]

    def ln_final(i, r0=0, n=TC, z=None):
        obuf[crows(i, r0, n), :] = _ln(xs[crows(i, r0, n), :],
                                       zrep(z, n)).astype(BF16)

    for item in bn_items(0):
        item()

    def phase_c(i, carry):
        @pl.when(i >= 2)
        def _():
            o_copy(i - 2).start()

        sched = _Sched(zero)
        dur = 7 * (1 + 2 * nfc) * TC // 2
        t0, t1 = int(C_WIN[0] * dur), int(C_WIN[1] * dur)
        sched.add([functools.partial(ln_final, jnp.maximum(i - 1, 0), r, RC[0])
                   for r in range(0, TC, RC[0])], t0, t1, C_SKIP)
        sched.add(bn_items(jnp.minimum(i + 1, nc - 1)),
                  t0 + RC[1], t1 + RC[1], C_SKIP)
        acc = list(_quads(xs[crows(i), :], TC // 2))
        for k in OQ:
            t = _dot(get7(hq7, k, nr=TC // 2), w7[2 * nfc + 2, k])
            _acc7(acc, k, t, TC // 2)
            sched(t)
        x3 = jnp.concatenate(_join(acc, TC // 2), axis=1)
        xs[crows(i), :] = x3
        h = _ln(x3)
        f = _ffn7(_lhs7(h[:TC // 2], h[TC // 2:]),
                  [w7.at[c] for c in range(nfc)],
                  [w7.at[nfc + c] for c in range(nfc)], sched, FE)
        assert not sched.queue
        xs[crows(i), :] += 0.5 * jnp.concatenate(f, axis=0)
        return carry

    with jax.named_scope("phase_c"):
        lax.fori_loop(0, nc, phase_c, 0)
    o_copy(nc - 2).start()
    last = []
    for k, (r0, r1) in enumerate(zip(EP[:-1], EP[1:])):
        ln_final(nc - 1, r0, r1 - r0)
        rs = crows(nc - 1, r0, r1 - r0)
        last.append(pltpu.make_async_copy(obuf.at[rs, :], out_hbm.at[rs, :],
                                          osem.at[nc - 1 + k]))
        last[-1].start()
    for i in range(nc - 1):
        o_copy(i).wait()
    for cp in last:
        cp.wait()


@jax.jit
def pallas_standalone__conformer_family_conformer__speech_kernel(
    x: jax.Array,
    w_ff1_a: jax.Array,
    w_ff1_b: jax.Array,
    w_q: jax.Array,
    w_k: jax.Array,
    w_v: jax.Array,
    w_o: jax.Array,
    w_pw1: jax.Array,
    dw: jax.Array,
    w_pw2: jax.Array,
    w_ff2_a: jax.Array,
    w_ff2_b: jax.Array,
):
    B, T, D = x.shape
    K = dw.shape[0]
    N = B * T
    weights = (w_ff1_a, w_ff1_b, w_q, w_k, w_v, w_o, w_pw1, dw, w_pw2,
               w_ff2_a, w_ff2_b)
    scratch = [pltpu.VMEM((N, D), BF16)]
    nfc = w_ff1_a.shape[1] // FC
    scratch += [pltpu.VMEM((4 * nfc + 3, D, D), BF16)]
    scratch += [pltpu.VMEM(w.shape, w.dtype)
                for w in (w_q, w_k, w_v, w_o, dw)]
    scratch += [
        pltpu.VMEM((7, D // 2, D // 2), BF16),
        pltpu.VMEM((7, D // 2, D // 2), BF16),
        pltpu.VMEM((N, D), F32),
        pltpu.VMEM((N, D), BF16),
        pltpu.VMEM((7, B * -(-T // KC) * KC // 2, D // 2), BF16),
        pltpu.VMEM((N // TM + 2, D // 128, TM + 2 * HALO, 128), F32),
        pltpu.VMEM((N, D), F32),
        pltpu.VMEM((N // TM, 8, D), F32),
        pltpu.VMEM((N // TM, 8, D), F32),
        pltpu.VMEM((2, 8, D), F32),
        pltpu.VMEM((7, TA // 2, D // 2), BF16),
        pltpu.VMEM((2, nfc, 7, D // 2, D // 2), BF16),
        pltpu.VMEM((2 * nfc + 3, 7, D // 2, D // 2), BF16),
        pltpu.VMEM((T0, D), BF16),
        pltpu.VMEM((K, 8, D), F32),
        pltpu.VMEM((ZR, 128), jnp.uint32),
        pltpu.SMEM((1,), jnp.int32),
        pltpu.VMEM((TM + 16, 128), F32),
        pltpu.VMEM((TM + 16, 128), F32),
        pltpu.VMEM((TM + 16, 128), F32),
        pltpu.VMEM((7 * PR, KC // 2), jnp.uint32),
        pltpu.VMEM((7 * PR, KC // 2), jnp.uint32),
        pltpu.VMEM((7 * PR, KC // 2), jnp.uint32),
        pltpu.VMEM((TM, KC), F32),
        pltpu.VMEM((TM, KC), F32),
        pltpu.VMEM((7 * PR, D // 2), jnp.uint32),
        pltpu.SemaphoreType.DMA(((N - T0) // TA + 1,)),
        pltpu.SemaphoreType.DMA((2, nfc)),
        pltpu.SemaphoreType.DMA((3, nfc)),
        pltpu.SemaphoreType.DMA((6,)),
        pltpu.SemaphoreType.DMA((N // TC + len(EP),)),
    ]
    out = pl.pallas_call(
        functools.partial(_kernel, B=B, T=T, D=D, K=K),
        out_shape=jax.ShapeDtypeStruct((N, D), x.dtype),
        in_specs=[pl.BlockSpec(memory_space=pl.ANY)] * 12,
        out_specs=pl.BlockSpec(memory_space=pl.ANY),
        scratch_shapes=scratch,
        compiler_params=pltpu.CompilerParams(
            vmem_limit_bytes=124 * 1024 * 1024),
    )(x.reshape(N, D), *weights)
    return out.reshape(B, T, D)
```

```python
import functools
import math

import jax
import jax.numpy as jnp
from jax import lax
import jax.experimental.pallas as pl
import jax.experimental.pallas.tpu as pltpu

F32 = jnp.float32
BF16 = jnp.bfloat16

TM = 400
T0 = 320
TA = 480
TC = 320
FC = 512
KC = 512
IW = 3
O1 = (1, 3, 2, 4, 0, 5, 6)
O2 = (1, 3, 6, 0, 2, 4, 5)
FL = (1, 1)
FE = ((0, 2), (0, 4), (1, 2), (1, 4))
OQ = (0, 2, 3, 4, 6, 1, 5)
OS0 = (2, 4, 3, 1, 0, 5, 6)
OS = (0, 1, 2, 3, 4, 5, 6)
OP = (0, 1, 2, 3, 4, 5, 6)
OW = (2, 4, 3, 0, 6, 1, 5)
PO = ((0, 2), (0, 4), (1, 2), (0, 3), (0, 0), (0, 6), (0, 1), (0, 5),
      (1, 4), (1, 3), (1, 0), (1, 6), (1, 1), (1, 5))
FRB = 16
F_WIN = (0.1, 0.9)
RA = 8
RO = 8
A_WIN = (0.05, 0.8)
A_SKIP = (600, 1400)
RF = 8
FD = (0, 3200, 0, 3200)
B_SLOTS = (1, 53)
Q_SLOTS = (8, 50)
CT = 5
L0 = 1
LP = (0, 100, 3, 1)
S1 = 2
S2 = 1
SD = (0, 140, 120)
LAG = 2
SW = tuple(1 + 1.75 * j for j in range(9))
C_WIN = (0.25, 0.86)
C_SKIP = ((4200, 5100), (6450, 7350), (8700, 9600))
RC = (8, 100)
EP = (0, 128, 224, 288, 320)
ZR = 32
PR = 112
HALO = 8
EPS = 1e-05


def _ln(x, z=None):
    if z is None:
        m = jnp.mean(x, axis=-1, keepdims=True)
    else:
        t = z
        for c in range(x.shape[-1] // 128):
            t = t + x[:, c * 128:(c + 1) * 128]
        m = jnp.sum(t, axis=-1, keepdims=True) * (1.0 / x.shape[-1])
    xc = x - m
    v = jnp.mean(xc * xc, axis=-1, keepdims=True)
    return xc * lax.rsqrt(v + EPS)


def _silu(a):
    y = 0.5 * a
    return y + y * jnp.tanh(y)


def _dot(a, b):
    return jnp.dot(a, b, preferred_element_type=F32)


def _dot_nt(a, b):
    return lax.dot_general(a, b, (((1,), (1,)), ((), ())),
                           preferred_element_type=F32)


class _Anchor:
    def __init__(self, t, zero_v):
        self.t, self.zero_v = t, zero_v

    def v(self):
        return pltpu.bitcast(
            pltpu.bitcast(self.t, jnp.uint32) & self.zero_v[0:8, :], F32)


class _Sched:
    def __init__(self, zero_v):
        self.zero_v = zero_v
        self.queue = []
        self.now = 0

    def add(self, items, t0, t1, skip=()):
        assert t0 >= self.now
        ts = [t for t in range(t0, t1)
              if not any(a <= t < b for a, b in skip)]
        self.queue += [(ts[k * len(ts) // len(items)], it)
                       for k, it in enumerate(items)]
        self.queue.sort(key=lambda e: e[0])

    def __call__(self, t, dur=None):
        dur = dur or t.shape[0]
        end = self.now + dur
        while self.queue and self.queue[0][0] < end:
            time, item = self.queue.pop(0)
            r = (time - self.now) * t.shape[0] // dur // 8 * 8
            item(_Anchor(t[r:r + 8, :128], self.zero_v))
        self.now = end


def _rep(z, rows):
    return jnp.concatenate([z] * (rows // 8), axis=0)


def _ffn(h, wa_ref, wb_ref, sched):
    ss = []
    for n in range(wa_ref.shape[1] // 128):
        a = _dot(h, wa_ref[:, n * 128:(n + 1) * 128])
        ss.append(_silu(a))
        sched(a)
    s = jnp.concatenate(ss, axis=1).astype(BF16)
    acc = []
    for n in range(wb_ref.shape[1] // 128):
        acc.append(_dot(s, wb_ref[:, n * 128:(n + 1) * 128]))
        sched(acc[-1])
    return jnp.concatenate(acc, axis=1)


def _sa(a11, a12, a21, a22):
    return [a11 + a22, a21 + a22, a11, a22, a11 + a12, a21 - a11, a12 - a22]


def _sb(b11, b12, b21, b22):
    return [b11 + b22, b11, b12 - b22, b21 - b11, b22, b11 + b12, b21 + b22]


def _sc(m):
    return [m[0] + m[3] - m[4] + m[6], m[4] + m[2], m[3] + m[1],
            m[0] + m[2] - m[1] + m[5]]


def _lhs7(t, u):
    h = t.shape[1] // 2
    return [v.astype(BF16)
            for v in _sa(t[:, :h], t[:, h:], u[:, :h], u[:, h:])]


_SA = ((0, 1, 3), (2, 1, 3), (0, 0, 0), (3, 0, 3), (0, 1, 1), (2, -1, 0),
       (1, -1, 3))
_TG = (((0, 1), (3, 1)), ((2, 1), (3, -1)), ((1, 1), (3, 1)), ((0, 1), (2, 1)),
       ((0, -1), (1, 1)), ((3, 1),), ((0, 1),))


def _quads(x, hm):
    h = x.shape[1] // 2
    t = x[:hm]
    if x.shape[0] > 2 * hm:
        t = jnp.concatenate([t, x[2 * hm:]], axis=0)
    return t[:, :h], t[:, h:], x[hm:, :h], x[hm:, h:]


def _sax(a11, a12, a21, a22, hm):
    return [a11[:hm] + a22[:hm], a21 + a22, a11, a22, a11 + a12,
            a21[:hm] - a11[:hm], a12[:hm] - a22[:hm]]


def _acc7(acc, k, m, hm):
    for a, sg in _TG[k]:
        t = m if a in (1, 2) else m[:hm]
        if acc[a] is None:
            acc[a] = t if sg > 0 else -t
        else:
            acc[a] = acc[a] + t if sg > 0 else acc[a] - t


def _join(acc, hm):
    rest = [acc[1][hm:]] if acc[1].shape[0] > hm else []
    return (jnp.concatenate([acc[0], acc[2]], axis=0),
            jnp.concatenate([acc[1][:hm], acc[3]] + rest, axis=0))


def _ffn7(h7, wa, wb, sched, lag, early=()):
    acc = [None] * 7
    hm = h7[0].shape[0]
    u = [[None] * 4 for _ in wa]

    done = set()
    act = [[None] * 4 for _ in wa]
    s7 = [[None] * 7 for _ in wa]

    def run(cks):
        for c, k in cks:
            if (c, k) in done or c >= len(wa):
                continue
            done.add((c, k))
            t = _dot(h7[k], wa[c][k])
            _acc7(u[c], k, t, hm)
            sched(t)
            for a in range(4):
                if act[c][a] is None and all(
                        (c, n) in done for n in range(7)
                        if a in [e[0] for e in _TG[n]]):
                    act[c][a] = _silu(u[c][a])
            for n, (a, sg, b) in enumerate(_SA):
                if (s7[c][n] is None and act[c][a] is not None
                        and act[c][b] is not None):
                    v = act[c][a]
                    if sg:
                        v = v + act[c][b] if sg > 0 else v - act[c][b]
                    s7[c][n] = v.astype(BF16)

    run(early)
    for c, cb in enumerate(wb):
        run([(c, k) for k in O1] + [(c + 1, k) for k in O1[:lag]])
        for k in O2:
            p = _dot(s7[c][k], cb[k])
            acc[k] = p if acc[k] is None else acc[k] + p
            sched(p)
    c = _sc(acc)
    return jnp.concatenate(c[:2], axis=1), jnp.concatenate(c[2:], axis=1)


def _kernel(x_hbm, w1a_hbm, w1b_hbm, wq_hbm, wk_hbm, wv_hbm, wo_hbm,
            wp1_hbm, dw_hbm, wp2_hbm, w2a_hbm, w2b_hbm,
            out_hbm,
            xin, wblk, wq, wk, wv, wo, dw,
            mq, wvo, xs, hs, ks, gs, dcs, st_mean, st_m2, bn,
            lhs7, w17, w7, lhs_b, dwb, zero, zero_s, al_buf0, al_buf1, al_buf2,
            p_buf0, p_buf1, p_buf2, s_buf0, s_buf1, hq7,
            xsem, w1sem, w2sem, wsem, osem,
            *, B, T, D, K):
    N = B * T
    obuf = xin
    KP = KC // 2
    nkc = -(-T // KC)
    TP = nkc * KP
    NCB = D // 128
    nt = N // TM
    tpb = T // TM

    def rows(i, r0=0, n=TM):
        return pl.ds(pl.multiple_of(i * TM, 16) + r0, n)

    def col(c):
        if isinstance(c, int):
            return slice(c * 128, (c + 1) * 128)
        return pl.ds(pl.multiple_of(c * 128, 128), 128)

    na = (N - T0) // TA
    H = D // 2

    def arows(i, r0=0, n=TA):
        return pl.ds(pl.multiple_of(T0 + (i - 1) * TA, 16) + r0, n)

    def x_copy(i):
        rs = pl.ds(0, T0) if isinstance(i, int) and i == 0 else arows(i)
        return pltpu.make_async_copy(x_hbm.at[rs, :], xin.at[rs, :],
                                     xsem.at[i])

    nc = N // TC

    def crows(i, r0=0, n=TC):
        return pl.ds(pl.multiple_of(i * TC, 16) + r0, n)

    def o_copy(i):
        return pltpu.make_async_copy(obuf.at[crows(i), :],
                                     out_hbm.at[crows(i), :], osem.at[i])

    nfc = w17.shape[1]
    P1, P2 = 4 * nfc, 4 * nfc + 2

    def w1_copies(c):
        fs = pl.ds(pl.multiple_of(c * FC, FC), FC)
        return [pltpu.make_async_copy(w1a_hbm.at[:, fs], wblk.at[c],
                                      w1sem.at[0, c]),
                pltpu.make_async_copy(w1b_hbm.at[fs, :], wblk.at[nfc + c],
                                      w1sem.at[1, c])]

    def w2_copies(c):
        fs = pl.ds(pl.multiple_of(c * FC, FC), FC)
        hs_ = pl.ds(pl.multiple_of(c // 2 * H, H), H)
        return [pltpu.make_async_copy(s, d, w2sem.at[j, c])
                for j, (s, d) in enumerate([
                    (w2a_hbm.at[:, fs], wblk.at[2 * nfc + c]),
                    (w2b_hbm.at[fs, :], wblk.at[3 * nfc + c]),
                    (wp1_hbm.at[:, pl.ds(pl.multiple_of(c * H, H), H)],
                     wblk.at[P1 + c % 2, :, hs_])])]

    assert nfc == 4
    w_pairs = [(wp2_hbm, wblk.at[P2]), (wq_hbm, wq), (wk_hbm, wk),
               (wv_hbm, wv), (wo_hbm, wo), (dw_hbm, dw)]
    w_copies = [pltpu.make_async_copy(s, d, wsem.at[j])
                for j, (s, d) in enumerate(w_pairs)]

    x_copy(0).start()
    for cp in w1_copies(0):
        cp.start()

    zero[...] = jnp.zeros(zero.shape, jnp.uint32)
    zero_s[0] = 0
    for c in range(NCB):
        gs[1, c, 0:HALO, :] = jnp.zeros((HALO, 128), F32)
        gs[nt, c, HALO + TM:, :] = jnp.zeros((HALO, 128), F32)
    for b in range(B):
        ks[:, b * TP + T // 2:(b + 1) * TP, :] = jnp.zeros(
            (7, TP - T // 2, H), BF16)

    def zrep(z, n):
        return None if z is None else _rep(z.v(), n)

    def ln_in(base, half, r0, n, z=None):
        t, u = [_ln(xin[pl.ds(pl.multiple_of(r, 16) + r0, n), :].astype(F32),
                    zrep(z, n)) for r in (base, base + half)]
        for k, v in enumerate(_lhs7(t, u)):
            lhs7[k, pl.ds(r0, n), :] = v

    def ln_out(base, r0, n, z=None):
        tu = []
        for r in (0, 16):
            rs = pl.ds(pl.multiple_of(base, 32) + r0 // 16 * 32 + r0 % 16 + r,
                       n)
            tu.append(_ln(xs[rs, :], zrep(z, n)))
            hs[rs, :] = tu[-1].astype(BF16)
        g = base // 32 + r0 // 16
        g += g // (T // 32) * ((TP - T // 2) // 16)
        ps = pl.ds(pl.multiple_of(g * 16, 16) + r0 % 16, n)
        for k, v in enumerate(_lhs7(*tu)):
            ks[k, ps, :] = v

    def prep(src, dst, r0, z=None):
        q = [src[pl.ds(r + r0, 16), c:c + H].astype(F32)
             for r in (0, H) for c in (0, H)]
        if z is not None:
            zz = jnp.concatenate([_rep(z.v(), 16)] * (H // 128), axis=1)
            q[0], q[3] = q[0] + zz, q[3] + zz
        for k, v in enumerate(_sb(*q)):
            dst[k, pl.ds(r0, 16), :] = v.astype(BF16)

    x_copy(0).wait()
    lhs_b[...] = _ln(xin[0:T0, :].astype(F32)).astype(BF16)
    xs[0:T0, :] = xin[0:T0, :].astype(F32)

    def first_tile(c, carry):
        for cp in w1_copies(c):
            cp.wait()

        @pl.when(c == 1)
        def _():
            x_copy(1).wait()

        @pl.when(c + 1 < nfc)
        def _():
            for cp in w1_copies(c + 1):
                cp.start()

        @pl.when(c % 2 == 0)
        def _():
            x_copy(1 + c // 2).start()

        n = -(-TA // 2 // (nfc - 1) // 16) * 16
        step = (TA // 2 - n) // (nfc - 2)
        assert step % 16 == 0 and step <= n
        r0 = pl.multiple_of(jnp.maximum(c - 1, 0) * step, 16)
        assert n <= T0 // 2
        sched = _Sched(zero)
        dur = 2 * NCB * T0
        sched.add([functools.partial(ln_in, jnp.where(c > 0, T0, 0),
                                     jnp.where(c > 0, TA // 2, T0 // 2),
                                     r0 + r, FRB)
                   for r in range(0, n, FRB)],
                  int(F_WIN[0] * dur), int(F_WIN[1] * dur))
        sched.add([functools.partial(prep, wblk.at[j * nfc + c],
                                     w17.at[j, c], r)
                   for j in range(2) for r in range(0, H, 16)],
                  int(F_WIN[0] * dur), int(F_WIN[1] * dur))
        f = _ffn(lhs_b[...], wblk.at[c], wblk.at[nfc + c], sched)
        assert not sched.queue
        xs[0:T0, :] += 0.5 * f
        return carry

    lax.fori_loop(0, nfc, first_tile, 0)
    for j in range(3, na + 1):
        x_copy(j).start()
    for c in range(nfc):
        for cp in w2_copies(c):
            cp.start()
    for cp in w_copies:
        cp.start()

    def phase_a(i, carry):
        @pl.when(i < na)
        def _():
            x_copy(i + 1).wait()

        @pl.when((i >= IW) & (i < IW + nfc))
        def _():
            for cp in w2_copies(i - IW):
                cp.wait()

        @pl.when(i == IW)
        def _():
            w_copies[0].wait()

        h7 = [lhs7[k, :TA // 2, :] for k in range(7)]
        sched = _Sched(zero)
        dur = 7 * nfc * TA
        win = (int(A_WIN[0] * dur), int(A_WIN[1] * dur),
               [(c * 7 * TA + A_SKIP[0] * TA // 320,
                 c * 7 * TA + A_SKIP[1] * TA // 320)
                for c in range(nfc)])
        base = jnp.maximum(T0 + (i - 2) * TA, 0)
        sched.add([functools.partial(ln_out, base, r, RO)
                   for r in range(0, TA // 2, RO)], *win)
        base = T0 + jnp.minimum(i, na - 1) * TA
        sched.add([functools.partial(ln_in, base, TA // 2, r, RA)
                   for r in range(0, TA // 2, RA)], *win)
        rpb = H // 16
        total = w7.shape[0] * rpb
        ipi = -(-total // (na - IW + 1))
        items = []
        for k in range(ipi):
            n = jnp.minimum(jnp.maximum(i - IW, 0) * ipi + k, total - 1)
            src = n // rpb + jnp.where(i >= IW, 2 * nfc, 0)
            items.append(functools.partial(
                prep, wblk.at[src], w7.at[n // rpb],
                pl.multiple_of(n % rpb * 16, 16)))
        assert ipi <= rpb
        sched.add(items, *win)
        f = _ffn7(h7, [w17.at[0, c] for c in range(nfc)],
                  [w17.at[1, c] for c in range(nfc)], sched, FL[0])
        assert not sched.queue
        xs[arows(i), :] = (xin[arows(i), :].astype(F32)
                           + 0.5 * jnp.concatenate(f, axis=0))
        return carry

    with jax.named_scope("phase_a"):
        lax.fori_loop(1, na + 1, phase_a, 0)

    for cp in w_copies[1:]:
        cp.wait()

    qk_scale = (D ** -0.5) * math.log2(math.e)

    HM = TM // 32 * 16

    def put7(dst, r0, cs, *p):
        if len(p) == 4:
            ops = enumerate(_sa(*p))
        else:
            ops = zip((1, 2, 3, 4), (p[0] + p[1], *p, p[0] + p[1]))
        for k, t in ops:
            dst[pl.ds(k * PR + r0 // 2, 8), cs] = pltpu.bitcast(
                t.astype(BF16), jnp.uint32)

    def get7(src, k, ds=pl.ds, nr=None):
        nr = nr or (TM - HM if 1 <= k <= 4 else HM)
        return pltpu.bitcast(src[ds(k * PR, nr // 2), :], BF16)

    def groups(r0):
        return (r0, HM + r0) if r0 < HM else (HM + r0,)

    def q_ops(i, r0, c, z):
        p = [hs[rows(i, r, 16), col(2 * h + c)].astype(F32)
             for r in groups(r0) for h in range(2)]
        p[0] = p[0] + _rep(z.v(), 16)
        p[-1] = p[-1] + _rep(z.v(), 16)
        put7(hq7, r0, col(c), *p)

    def q_items(i):
        return [functools.partial(q_ops, i, r0, c)
                for r0 in range(0, TM - HM, 16) for c in range(2)]

    sched = _Sched(zero)
    sched.add([functools.partial(ln_out, N - TA, r, RF)
               for r in range(0, TA // 2, RF)], *FD[:2])
    sched.add(q_items(0), *FD[2:])
    for dst in (mq, wvo):
        for u in range(2):
            t = []
            for cs in (col(u), col(u + 2)):
                t.append(_dot_nt(wq[...], wk[cs, :]) if dst is mq
                         else _dot(wv[...], wo[:, cs]))
                sched(t[-1])
            if dst is mq:
                t = [v * qk_scale for v in t]
            for k, v in enumerate(
                    _sb(t[0][:H], t[1][:H], t[0][H:], t[1][H:])):
                dst[k, :, col(u)] = v.astype(BF16)
    assert not sched.queue
    dwf = dw[...].astype(F32)
    for k in range(K):
        dwb[k] = jnp.broadcast_to(dwf[k:k + 1, :], (8, D))

    def conv_block(p, r0, c, done, CT=CT, AT=K):
        cs = col(c)
        acc = [None]

        def item(k0, z=None):
            for k in range(k0, min(k0 + CT, K)):
                off = HALO - K // 2 + k + r0
                w = dwb[k, :, cs]
                if z is not None and k - k0 < AT:
                    w = w + z.v()
                t = gs[p + 1, c, off:off + 8, :] * w
                acc[0] = t if acc[0] is None else acc[0] + t
            if k0 + CT >= K:
                dcs[rows(p, r0, 8), cs] = acc[0]
                done(acc[0])

        return [functools.partial(item, k0) for k0 in range(0, K, CT)]

    def conv_main(p, cols=range(NCB), **kw):
        st = []

        def stats(r0, c, acc):
            if r0 == 0:
                st[:] = [acc, None, None]
                return
            shift, s1, s2 = st
            d = acc - shift
            s1 = d if s1 is None else s1 + d
            s2 = d * d if s2 is None else s2 + d * d
            st[:] = [shift, s1, s2]
            if r0 + 16 == TM:
                dm = s1 * (1.0 / (TM // 8 - 1))
                st_mean[p, :, col(c)] = shift + dm
                st_m2[p, :, col(c)] = s2 - s1 * dm

        return [it for c in cols for r0 in range(0, TM - 8, 8)
                for it in conv_block(p, r0, c,
                                     functools.partial(stats, r0, c), **kw)]

    def conv_edge(p, cols=range(NCB)):
        return [it for c in cols
                for it in conv_block(p, TM - 8, c, lambda acc: None)]


    def phase_b(i, carry):
        b = i // tpb

        sched = _Sched(zero)
        sched.add(conv_edge(jnp.maximum(i - 2, 0))
                  + conv_main(jnp.maximum(i - 1, 0), range(L0, NCB)),
                  int(B_SLOTS[0] * TM), int(B_SLOTS[1] * TM))
        sched.add(q_items(jnp.minimum(i + 1, nt - 1)),
                  int(Q_SLOTS[0] * TM), int(Q_SLOTS[1] * TM))
        acc = [None] * 4
        for k in OQ:
            t = _dot(get7(hq7, k), mq[k])
            _acc7(acc, k, t, HM)
            sched(t)
        q11, q12, q21, q22 = _quads(
            jnp.concatenate(_join(acc, HM), axis=1), HM)
        q7 = [q11[:HM] - q22[:HM], q21 - q22, q11, q22, q12 - q11,
              q21[:HM] - q11[:HM], q12[:HM] - q22[:HM]]
        q7 = [t.astype(BF16) for t in q7]

        dz = zero_s[0]
        p_buf, al_buf = (p_buf0, p_buf1, p_buf2), (al_buf0, al_buf1, al_buf2)
        s_buf = (s_buf0, s_buf1)

        def dyn(r0, n):
            return pl.ds(pl.multiple_of(dz + r0, 8), n)

        nb = KP // 128

        def chunk(j):
            return pl.ds(pl.multiple_of(b * TP, KP) + j * KP, KP)

        def combine(m, j, c):
            if len(m) == 7:
                s = [m[0] + m[3] + m[4] + m[6], m[2] + m[4],
                     m[1] + m[3], m[1] - m[0] + m[2] + m[5]]
            else:
                s = [m[0] + m[2], m[1] + m[3]]
            nv = T // 2 - j * KP - c * 128
            if nv < 128:
                lane = lax.broadcasted_iota(jnp.int32, s[0].shape, 1)
                s = [jnp.where(lane < nv, t, -jnp.inf) for t in s]
            return s

        stat = {}

        def put(w, j, r, v):
            for r0 in range(0, v.shape[0], 16):
                stat[w, j, r + r0] = v[r0:r0 + 16]

        def get(w, j, r, n=16):
            return jnp.concatenate(
                [stat[w, j, r0] for r0 in range(r, r + n, 16)], axis=0)

        def scores(j):
            m = [None] * 7
            for k in OS if j else OS0:
                m[k] = _dot_nt(q7[k],
                               ks[(0, 2, 1, 4, 3, 5, 6)[k], chunk(j), :])
                sched(m[k])
            mx = None
            for c in range(nb):
                s = combine([t[:HM, col(c)] for t in m], j, c)
                e = combine([t[HM:, col(c)] for t in m[1:5]], j, c)
                for h in range(2):
                    t = jnp.concatenate([s[h], s[2 + h], e[h]], axis=0)
                    s_buf[j % 2][:, col(h * nb + c)] = t
                    mx = t if mx is None else jnp.maximum(mx, t)
            mx = jnp.broadcast_to(jnp.max(mx, axis=-1, keepdims=True),
                                  mx.shape)
            if j:
                mx = jnp.maximum(mx, get(0, j - 1, 0, TM))
            put(0, j, 0, mx)

        part = {}

        def soft1(j, r, c0, z):
            rs = slice(r, r + 16)
            m = get(0, j, r) + _rep(z.v(), 16)
            l = functools.reduce(jnp.add, part.pop((j, r), []) + [
                jnp.exp2(s_buf[j % 2][dyn(r, 16), col(c)] - m)
                for c in range(c0, c0 + S1)])
            if c0 + S1 < 2 * nb:
                part[j, r] = [l]
                return
            l = jnp.broadcast_to(jnp.sum(l, axis=-1, keepdims=True),
                                 (16, 128))
            if j:
                l += get(1, j - 1, r) * jnp.exp2(get(0, j - 1, r) - m)
            put(1, j, r, l)
            e = (pltpu.bitcast(l, jnp.int32) >> 23) - 127
            ref = m + e.astype(F32)
            put(2, j, r, ref)
            if j:
                al_buf[j % 3][rs, :] = jnp.exp2(get(2, j - 1, r) - ref)

        def soft2(j, r0, c0, z):
            ref = [get(2, j, r) + _rep(z.v(), 16) for r in groups(r0)]
            p = [jnp.concatenate(
                [jnp.exp2(s_buf[j % 2][dyn(r, 16), col(h * nb + c)] - m)
                 for c in range(c0, c0 + S2)], axis=1)
                 for r, m in zip(groups(r0), ref) for h in range(2)]
            put7(p_buf[j % 3], r0, slice(c0 * 128, (c0 + S2) * 128), *p)

        scd = 7 * HM + 4 * (TM - 2 * HM)
        start = sched.now

        def add_soft(j):
            rbs = range(0, TM - HM, 16)
            t0, t1 = (start + int(t * scd) for t in SW[j:j + 2])
            assert t1 <= start + min(2 * j + LAG + 1, nkc + j) * scd
            assert j < 3 or t0 >= start + min(2 * j + LAG - 4,
                                              nkc + j - 2) * scd
            assert (j + 2 >= nkc
                    or t1 <= start + max(2 * j + 5 - LAG, j + 3) * scd)
            u = (t1 - t0 - sum(SD)) // (len(rbs) + 1)
            for n, r0 in enumerate(rbs):
                its = [[functools.partial(soft1, j, r, c)
                        for r in groups(r0) for c in range(0, 2 * nb, S1)],
                       [functools.partial(soft2, j, r0, c)
                        for c in range(0, nb, S2)]]
                for k, it in enumerate(its):
                    t = t0 + SD[0] + n * u + k * (u + SD[1])
                    sched.add(it, t, t + u)

        for j in range(LAG):
            scores(j)
            add_soft(j)
        acc = [None] * 4
        for j in range(nkc):
            if j + LAG < nkc:
                scores(j + LAG)
                add_soft(j + LAG)
            fresh = [j > 0] * 4
            for k in OP if j + 1 < nkc else OQ:
                w = ks[(0, 2, 6, 5, 3, 4, 1)[k], chunk(j), :]
                m = _dot(get7(p_buf[j % 3], k, dyn), w)
                sched(m)
                for a, _ in _TG[k]:
                    if fresh[a]:
                        al = al_buf[j % 3][dyn(0, TM), :]
                        al = _quads(jnp.concatenate([al] * NCB, axis=1), HM)[a]
                        acc[a] = acc[a] * al[:acc[a].shape[0]]
                        fresh[a] = False
                _acc7(acc, k, m, HM)
        assert not sched.queue
        t = jnp.exp2(get(2, nkc - 1, 0, TM) - get(0, nkc - 1, 0, TM))
        t = t / get(1, nkc - 1, 0, TM)
        o = (jnp.concatenate(_join(acc, HM), axis=1)
             * jnp.concatenate([t] * NCB, axis=1))
        o7 = [t.astype(BF16) for t in _sax(*_quads(o, HM), HM)]
        acc = list(_quads(xs[rows(i), :], HM))
        acc = [acc[0][:HM], acc[1], acc[2], acc[3][:HM]]
        for k in OW:
            _acc7(acc, k, _dot(o7[k], wvo[k]), HM)
        x2 = jnp.concatenate(_join(acc, HM), axis=1)
        xs[rows(i), :] = x2
        h7 = [t.astype(BF16) for t in _sax(*_quads(_ln(x2), HM), HM)]
        sched = _Sched(zero)
        acc = [[None] * 4 for _ in range(2)]
        for n, (h, k) in enumerate(PO):
            t = _dot(h7[k], w7[2 * nfc + h, k])
            _acc7(acc[h], k, t, HM)
            sched(t)
            if any(e[0] == h for e in PO[n + 1:]):
                continue
            val, gate = _join(acc[h], HM)
            g2 = val * (0.5 + 0.5 * jnp.tanh(0.5 * gate))
            for c in (2 * h, 2 * h + 1):
                g = g2[:, col(c % 2)]
                gs[i + 1, c, HALO:HALO + TM, :] = g
                gs[i, c, HALO + TM:, :] = jnp.where(
                    i % tpb == 0, 0.0, g[:HALO])
                gs[i + 2, c, :HALO, :] = jnp.where(
                    i % tpb == tpb - 1, 0.0, g[TM - HALO:])
            if h == 0 and L0:
                rest = sum(h7[e[1]].shape[0] for e in PO[n + 1:])
                sched.add(conv_main(i, range(L0), CT=LP[2], AT=LP[3]),
                          sched.now + LP[0], sched.now + rest - LP[1])
        assert not sched.queue
        return carry

    with jax.named_scope("phase_b"):
        lax.fori_loop(0, nt, phase_b, 0)
    for item in (conv_main(nt - 1, range(L0, NCB)) + conv_edge(nt - 2)
                 + conv_edge(nt - 1)):
        item()

    ng = TM // 8 - 1
    means = st_mean[...].reshape(nt * 8, D)
    edges = jnp.concatenate([dcs[(p + 1) * TM - 8:(p + 1) * TM, :]
                             for p in range(nt)], axis=0)
    mu = jnp.sum(ng * means + edges, axis=0, keepdims=True) * (1.0 / N)
    dm = means - mu
    de = edges - mu
    var = jnp.sum(st_m2[...].reshape(nt * 8, D) + ng * (dm * dm) + de * de,
                  axis=0, keepdims=True) * (1.0 / N)
    rstd = lax.rsqrt(var + EPS)
    bn[0] = jnp.broadcast_to(mu, (8, D))
    bn[1] = jnp.broadcast_to(rstd, (8, D))

    def bn_silu(i, r0, c, z=None):
        p = []
        for r in (r0, TC // 2 + r0):
            for h in range(2):
                cs = col(2 * h + c)
                mu = bn[0, :, cs] if z is None else bn[0, :, cs] + z.v()
                y = dcs[crows(i, r, 16), cs] - _rep(mu, 16)
                p.append(_silu(y * _rep(bn[1, :, cs], 16)))
        put7(hq7, r0, col(c), *p)

    def bn_items(i):
        return [functools.partial(bn_silu, i, r0, c)
                for r0 in range(0, TC // 2, 16) for c in range(2)]

    def ln_final(i, r0=0, n=TC, z=None):
        obuf[crows(i, r0, n), :] = _ln(xs[crows(i, r0, n), :],
                                       zrep(z, n)).astype(BF16)

    for item in bn_items(0):
        item()

    def phase_c(i, carry):
        @pl.when(i >= 2)
        def _():
            o_copy(i - 2).start()

        sched = _Sched(zero)
        dur = 7 * (1 + 2 * nfc) * TC // 2
        t0, t1 = int(C_WIN[0] * dur), int(C_WIN[1] * dur)
        sched.add([functools.partial(ln_final, jnp.maximum(i - 1, 0), r, RC[0])
                   for r in range(0, TC, RC[0])], t0, t1, C_SKIP)
        sched.add(bn_items(jnp.minimum(i + 1, nc - 1)),
                  t0 + RC[1], t1 + RC[1], C_SKIP)
        acc = list(_quads(xs[crows(i), :], TC // 2))
        for k in OQ:
            t = _dot(get7(hq7, k, nr=TC // 2), w7[2 * nfc + 2, k])
            _acc7(acc, k, t, TC // 2)
            sched(t)
        x3 = jnp.concatenate(_join(acc, TC // 2), axis=1)
        xs[crows(i), :] = x3
        h = _ln(x3)
        f = _ffn7(_lhs7(h[:TC // 2], h[TC // 2:]),
                  [w7.at[c] for c in range(nfc)],
                  [w7.at[nfc + c] for c in range(nfc)], sched, FL[1], FE)
        assert not sched.queue
        xs[crows(i), :] += 0.5 * jnp.concatenate(f, axis=0)
        return carry

    with jax.named_scope("phase_c"):
        lax.fori_loop(0, nc, phase_c, 0)
    o_copy(nc - 2).start()
    last = []
    for k, (r0, r1) in enumerate(zip(EP[:-1], EP[1:])):
        ln_final(nc - 1, r0, r1 - r0)
        rs = crows(nc - 1, r0, r1 - r0)
        last.append(pltpu.make_async_copy(obuf.at[rs, :], out_hbm.at[rs, :],
                                          osem.at[nc - 1 + k]))
        last[-1].start()
    for i in range(nc - 1):
        o_copy(i).wait()
    for cp in last:
        cp.wait()


@jax.jit
def pallas_standalone__conformer_family_conformer__speech_kernel(
    x: jax.Array,
    w_ff1_a: jax.Array,
    w_ff1_b: jax.Array,
    w_q: jax.Array,
    w_k: jax.Array,
    w_v: jax.Array,
    w_o: jax.Array,
    w_pw1: jax.Array,
    dw: jax.Array,
    w_pw2: jax.Array,
    w_ff2_a: jax.Array,
    w_ff2_b: jax.Array,
):
    B, T, D = x.shape
    K = dw.shape[0]
    N = B * T
    weights = (w_ff1_a, w_ff1_b, w_q, w_k, w_v, w_o, w_pw1, dw, w_pw2,
               w_ff2_a, w_ff2_b)
    scratch = [pltpu.VMEM((N, D), BF16)]
    nfc = w_ff1_a.shape[1] // FC
    scratch += [pltpu.VMEM((4 * nfc + 3, D, D), BF16)]
    scratch += [pltpu.VMEM(w.shape, w.dtype)
                for w in (w_q, w_k, w_v, w_o, dw)]
    scratch += [
        pltpu.VMEM((7, D // 2, D // 2), BF16),
        pltpu.VMEM((7, D // 2, D // 2), BF16),
        pltpu.VMEM((N, D), F32),
        pltpu.VMEM((N, D), BF16),
        pltpu.VMEM((7, B * -(-T // KC) * KC // 2, D // 2), BF16),
        pltpu.VMEM((N // TM + 2, D // 128, TM + 2 * HALO, 128), F32),
        pltpu.VMEM((N, D), F32),
        pltpu.VMEM((N // TM, 8, D), F32),
        pltpu.VMEM((N // TM, 8, D), F32),
        pltpu.VMEM((2, 8, D), F32),
        pltpu.VMEM((7, D // 2, D // 2), BF16),
        pltpu.VMEM((2, nfc, 7, D // 2, D // 2), BF16),
        pltpu.VMEM((2 * nfc + 3, 7, D // 2, D // 2), BF16),
        pltpu.VMEM((T0, D), BF16),
        pltpu.VMEM((K, 8, D), F32),
        pltpu.VMEM((ZR, 128), jnp.uint32),
        pltpu.SMEM((1,), jnp.int32),
        pltpu.VMEM((TM + 16, 128), F32),
        pltpu.VMEM((TM + 16, 128), F32),
        pltpu.VMEM((TM + 16, 128), F32),
        pltpu.VMEM((7 * PR, KC // 2), jnp.uint32),
        pltpu.VMEM((7 * PR, KC // 2), jnp.uint32),
        pltpu.VMEM((7 * PR, KC // 2), jnp.uint32),
        pltpu.VMEM((TM, KC), F32),
        pltpu.VMEM((TM, KC), F32),
        pltpu.VMEM((7 * PR, D // 2), jnp.uint32),
        pltpu.SemaphoreType.DMA(((N - T0) // TA + 1,)),
        pltpu.SemaphoreType.DMA((2, nfc)),
        pltpu.SemaphoreType.DMA((3, nfc)),
        pltpu.SemaphoreType.DMA((6,)),
        pltpu.SemaphoreType.DMA((N // TC + len(EP),)),
    ]
    out = pl.pallas_call(
        functools.partial(_kernel, B=B, T=T, D=D, K=K),
        out_shape=jax.ShapeDtypeStruct((N, D), x.dtype),
        in_specs=[pl.BlockSpec(memory_space=pl.ANY)] * 12,
        out_specs=pl.BlockSpec(memory_space=pl.ANY),
        scratch_shapes=scratch,
        compiler_params=pltpu.CompilerParams(
            vmem_limit_bytes=124 * 1024 * 1024),
    )(x.reshape(N, D), *weights)
    return out.reshape(B, T, D)
```

```python
import functools
import math

import jax
import jax.numpy as jnp
from jax import lax
import jax.experimental.pallas as pl
import jax.experimental.pallas.tpu as pltpu

F32 = jnp.float32
BF16 = jnp.bfloat16

TM = 400
T0 = 320
TA = 480
TC = 320
FC = 512
KC = 512
W1A = 1
XF = 0
IW = 3
FA = ((1, 3, 2, 4, 0, 5, 6), (1, 3, 6, 0, 2, 4, 5), 1)
FB = ((1, 3, 2, 4, 0, 5, 6), (1, 3, 6, 2, 4, 0, 5), 1,
      ((0, 2), (1, 2), (2, 2), (0, 4)))
OQ = (0, 2, 3, 4, 6, 1, 5)
OS0 = (2, 4, 3, 1, 0, 5, 6)
OS = (0, 1, 2, 3, 4, 5, 6)
OP = (0, 1, 2, 3, 4, 5, 6)
OW = (2, 4, 3, 0, 6, 1, 5)
PO = ((0, 2), (0, 4), (1, 2), (0, 3), (0, 0), (0, 6), (0, 1), (0, 5),
      (1, 4), (1, 3), (1, 0), (1, 6), (1, 1), (1, 5))
F_WIN = (0.1, 0.9)
A_WIN = (0.03, 0.81)
A_SKIP = (500, 1300)
FD = (0, 3200, 0, 3200)
B_SLOTS = (1, 53)
Q_SLOTS = (8, 50)
CT = 5
L0 = 1
LP = (0, 100, 3, 1)
S1 = 2
S2 = 1
SD = (0, 140, 120)
LAG = 2
SW = tuple(1 + 1.75 * j for j in range(9))
C_WIN = (0.21, 0.82)
C_SKIP = ((4050, 5050), (6290, 7290), (8530, 9530))
RC = (8, 100)
EP = (0, 128, 224, 288, 320)
ZR = 32
PR = 112
HALO = 8
EPS = 1e-05


def _ln(x, z=None):
    if z is None:
        m = jnp.mean(x, axis=-1, keepdims=True)
    else:
        t = z
        for c in range(x.shape[-1] // 128):
            t = t + x[:, c * 128:(c + 1) * 128]
        m = jnp.sum(t, axis=-1, keepdims=True) * (1.0 / x.shape[-1])
    xc = x - m
    v = jnp.mean(xc * xc, axis=-1, keepdims=True)
    return xc * lax.rsqrt(v + EPS)


def _silu(a):
    y = 0.5 * a
    return y + y * jnp.tanh(y)


def _dot(a, b):
    return jnp.dot(a, b, preferred_element_type=F32)


def _dot_nt(a, b):
    return lax.dot_general(a, b, (((1,), (1,)), ((), ())),
                           preferred_element_type=F32)


def _pk(v):
    return pltpu.bitcast(v.astype(BF16), jnp.uint32)


def _up(v):
    return pltpu.bitcast(v, BF16)


class _Anchor:
    def __init__(self, t, zero_v):
        self.t, self.zero_v = t, zero_v

    def v(self):
        return pltpu.bitcast(
            pltpu.bitcast(self.t, jnp.uint32) & self.zero_v[0:8, :], F32)


class _Sched:
    def __init__(self, zero_v):
        self.zero_v = zero_v
        self.queue = []
        self.now = 0

    def add(self, items, t0, t1, skip=()):
        assert t0 >= self.now
        ts = [t for t in range(t0, t1)
              if not any(a <= t < b for a, b in skip)]
        self.queue += [(ts[k * len(ts) // len(items)], it)
                       for k, it in enumerate(items)]
        self.queue.sort(key=lambda e: e[0])

    def __call__(self, t, dur=None):
        dur = dur or t.shape[0]
        end = self.now + dur
        while self.queue and self.queue[0][0] < end:
            time, item = self.queue.pop(0)
            r = (time - self.now) * t.shape[0] // dur // 8 * 8
            item(_Anchor(t[r:r + 8, :128], self.zero_v))
        self.now = end


def _rep(z, rows):
    return jnp.concatenate([z] * (rows // 8), axis=0)


def _ffn(h, wa_ref, wb_ref, sched):
    ss = []
    for n in range(wa_ref.shape[1] // 128):
        a = _dot(h, wa_ref[:, n * 128:(n + 1) * 128])
        ss.append(_silu(a))
        sched(a)
    s = jnp.concatenate(ss, axis=1).astype(BF16)
    acc = []
    for n in range(wb_ref.shape[1] // 128):
        acc.append(_dot(s, wb_ref[:, n * 128:(n + 1) * 128]))
        sched(acc[-1])
    return jnp.concatenate(acc, axis=1)


def _sa(a11, a12, a21, a22):
    return [a11 + a22, a21 + a22, a11, a22, a11 + a12, a21 - a11, a12 - a22]


def _sb(b11, b12, b21, b22):
    return [b11 + b22, b11, b12 - b22, b21 - b11, b22, b11 + b12, b21 + b22]


def _sc(m):
    return [m[0] + m[3] - m[4] + m[6], m[4] + m[2], m[3] + m[1],
            m[0] + m[2] - m[1] + m[5]]


def _lhs7(t, u):
    h = t.shape[1] // 2
    return [v.astype(BF16)
            for v in _sa(t[:, :h], t[:, h:], u[:, :h], u[:, h:])]


_SA = ((0, 1, 3), (2, 1, 3), (0, 0, 0), (3, 0, 3), (0, 1, 1), (2, -1, 0),
       (1, -1, 3))
_TG = (((0, 1), (3, 1)), ((2, 1), (3, -1)), ((1, 1), (3, 1)), ((0, 1), (2, 1)),
       ((0, -1), (1, 1)), ((3, 1),), ((0, 1),))


def _quads(x, hm):
    h = x.shape[1] // 2
    t = x[:hm]
    if x.shape[0] > 2 * hm:
        t = jnp.concatenate([t, x[2 * hm:]], axis=0)
    return t[:, :h], t[:, h:], x[hm:, :h], x[hm:, h:]


def _sax(a11, a12, a21, a22, hm):
    return [a11[:hm] + a22[:hm], a21 + a22, a11, a22, a11 + a12,
            a21[:hm] - a11[:hm], a12[:hm] - a22[:hm]]


def _acc7(acc, k, m, hm):
    for a, sg in _TG[k]:
        t = m if a in (1, 2) else m[:hm]
        if acc[a] is None:
            acc[a] = t if sg > 0 else -t
        else:
            acc[a] = acc[a] + t if sg > 0 else acc[a] - t


def _join(acc, hm):
    rest = [acc[1][hm:]] if acc[1].shape[0] > hm else []
    return (jnp.concatenate([acc[0], acc[2]], axis=0),
            jnp.concatenate([acc[1][:hm], acc[3]] + rest, axis=0))


def _ffn7(h7, wa, wb, sched, o1, o2, lag, early=()):
    acc = [None] * 7
    hm = h7[0].shape[0]
    u = [[None] * 4 for _ in wa]

    done = set()
    act = [[None] * 4 for _ in wa]
    s7 = [[None] * 7 for _ in wa]

    def run(cks):
        for c, k in cks:
            if (c, k) in done or c >= len(wa):
                continue
            done.add((c, k))
            t = _dot(h7[k], _up(wa[c][k]))
            _acc7(u[c], k, t, hm)
            sched(t)
            for a in range(4):
                if act[c][a] is None and all(
                        (c, n) in done for n in range(7)
                        if a in [e[0] for e in _TG[n]]):
                    act[c][a] = _silu(u[c][a])
            for n, (a, sg, b) in enumerate(_SA):
                if (s7[c][n] is None and act[c][a] is not None
                        and act[c][b] is not None):
                    v = act[c][a]
                    if sg:
                        v = v + act[c][b] if sg > 0 else v - act[c][b]
                    s7[c][n] = v.astype(BF16)

    run(early)
    for c, cb in enumerate(wb):
        run([(c, k) for k in o1] + [(c + 1, k) for k in o1[:lag]])
        for k in o2:
            p = _dot(s7[c][k], _up(cb[k]))
            acc[k] = p if acc[k] is None else acc[k] + p
            sched(p)
    c = _sc(acc)
    return jnp.concatenate(c[:2], axis=1), jnp.concatenate(c[2:], axis=1)


def _kernel(x_hbm, w1a_hbm, w1b_hbm, wq_hbm, wk_hbm, wv_hbm, wo_hbm,
            wp1_hbm, dw_hbm, wp2_hbm, w2a_hbm, w2b_hbm,
            out_hbm,
            xin, wblk, wq, wk, wv, wo, dw,
            mq, wvo, xs, hs, ks, gs, dcs, st_mean, st_m2, bn,
            lhs7, w17, w7, lhs_b, dwb, zero, zero_s, al_buf0, al_buf1, al_buf2,
            p_buf0, p_buf1, p_buf2, s_buf0, s_buf1, hq7,
            xsem, w1sem, w2sem, wsem, osem,
            *, B, T, D, K):
    N = B * T
    obuf = xin
    KP = KC // 2
    nkc = -(-T // KC)
    TP = nkc * KP
    NCB = D // 128
    nt = N // TM
    tpb = T // TM

    def rows(i, r0=0, n=TM):
        return pl.ds(pl.multiple_of(i * TM, 16) + r0, n)

    def col(c):
        if isinstance(c, int):
            return slice(c * 128, (c + 1) * 128)
        return pl.ds(pl.multiple_of(c * 128, 128), 128)

    na = (N - T0) // TA
    H = D // 2

    def arows(i, r0=0, n=TA):
        return pl.ds(pl.multiple_of(T0 + (i - 1) * TA, 16) + r0, n)

    def x_copy(i):
        rs = pl.ds(0, T0) if isinstance(i, int) and i == 0 else arows(i)
        return pltpu.make_async_copy(x_hbm.at[rs, :], xin.at[rs, :],
                                     xsem.at[i])

    nc = N // TC

    def crows(i, r0=0, n=TC):
        return pl.ds(pl.multiple_of(i * TC, 16) + r0, n)

    def o_copy(i):
        return pltpu.make_async_copy(obuf.at[crows(i), :],
                                     out_hbm.at[crows(i), :], osem.at[i])

    nfc = w17.shape[1]
    P1, P2 = 4 * nfc, 4 * nfc + 2

    def w1_copies(c):
        fs = pl.ds(pl.multiple_of(c * FC, FC), FC)
        return [pltpu.make_async_copy(w1a_hbm.at[:, fs], wblk.at[c],
                                      w1sem.at[0, c]),
                pltpu.make_async_copy(w1b_hbm.at[fs, :], wblk.at[nfc + c],
                                      w1sem.at[1, c])]

    def w2_copies(c):
        fs = pl.ds(pl.multiple_of(c * FC, FC), FC)
        hs_ = pl.ds(pl.multiple_of(c // 2 * H, H), H)
        return [pltpu.make_async_copy(s, d, w2sem.at[j, c])
                for j, (s, d) in enumerate([
                    (w2a_hbm.at[:, fs], wblk.at[2 * nfc + c]),
                    (w2b_hbm.at[fs, :], wblk.at[3 * nfc + c]),
                    (wp1_hbm.at[:, pl.ds(pl.multiple_of(c * H, H), H)],
                     wblk.at[P1 + c % 2, :, hs_])])]

    assert nfc == 4
    w_pairs = [(wp2_hbm, wblk.at[P2]), (wq_hbm, wq), (wk_hbm, wk),
               (wv_hbm, wv), (wo_hbm, wo), (dw_hbm, dw)]
    w_copies = [pltpu.make_async_copy(s, d, wsem.at[j])
                for j, (s, d) in enumerate(w_pairs)]

    x_copy(0).start()
    for cp in w1_copies(0):
        cp.start()

    zero[...] = jnp.zeros(zero.shape, jnp.uint32)
    zero_s[0] = 0
    for c in range(NCB):
        gs[1, c, 0:HALO, :] = jnp.zeros((HALO, 128), F32)
        gs[nt, c, HALO + TM:, :] = jnp.zeros((HALO, 128), F32)
    for b in range(B):
        ks[:, (b * TP + T // 2) // 2:(b + 1) * TP // 2, :] = jnp.zeros(
            (7, (TP - T // 2) // 2, H), jnp.uint32)

    def zrep(z, n):
        return None if z is None else _rep(z.v(), n)

    def pair_items(first, second, rows0):
        items = []
        for r0 in rows0:
            t = []
            items += [functools.partial(first, t, r0),
                      functools.partial(second, t, r0)]
        return items

    def ln_in(base, half, rows0):
        def first(t, r0, z, base=base):
            t.append(_ln(xin[pl.ds(pl.multiple_of(base, 16) + r0, 16), :]
                         .astype(F32), zrep(z, 16)))

        def second(t, r0, z):
            first(t, r0, z, base + half)
            r1 = r0 // 2 if isinstance(r0, int) else pl.multiple_of(r0 // 2, 8)
            for k, v in enumerate(_lhs7(*t)):
                lhs7[k, pl.ds(r1, 8), :] = _pk(v)

        return pair_items(first, second, rows0)

    def ln_out(base, rows0):
        def first(t, r0, z, off=0):
            rs = pl.ds(pl.multiple_of(base, 32) + 2 * r0 + off, 16)
            t.append(_ln(xs[rs, :], zrep(z, 16)))
            hs[rs, :] = t[-1].astype(BF16)

        def second(t, r0, z):
            first(t, r0, z, 16)
            g = base // 32 + r0 // 16
            g += g // (T // 32) * ((TP - T // 2) // 16)
            for k, v in enumerate(_lhs7(*t)):
                ks[k, pl.ds(pl.multiple_of(g * 8, 8), 8), :] = _pk(v)

        return pair_items(first, second, rows0)

    def prep(src, dst, r0, z=None):
        q = [src[pl.ds(r + r0, 16), c:c + H].astype(F32)
             for r in (0, H) for c in (0, H)]
        if z is not None:
            zz = jnp.concatenate([_rep(z.v(), 16)] * (H // 128), axis=1)
            q[0], q[3] = q[0] + zz, q[3] + zz
        r1 = r0 // 2 if isinstance(r0, int) else pl.multiple_of(r0 // 2, 8)
        for k, v in enumerate(_sb(*q)):
            dst[k, pl.ds(r1, 8), :] = _pk(v)

    x_copy(0).wait()
    if W1A == 2:
        for cp in w1_copies(1):
            cp.start()
    lhs_b[...] = _ln(xin[0:T0, :].astype(F32)).astype(BF16)
    xs[0:T0, :] = xin[0:T0, :].astype(F32)

    def first_tile(c, carry):
        for cp in w1_copies(c):
            cp.wait()

        @pl.when(c == 1)
        def _():
            x_copy(1).wait()

        if XF:
            @pl.when(c % 2 == 0)
            def _():
                x_copy(1 + c // 2).start()

        @pl.when(c + W1A < nfc)
        def _():
            for cp in w1_copies(c + W1A):
                cp.start()

        if not XF:
            @pl.when(c % 2 == 0)
            def _():
                x_copy(1 + c // 2).start()

        n = -(-TA // 2 // (nfc - 1) // 16) * 16
        step = (TA // 2 - n) // (nfc - 2)
        assert step % 16 == 0 and step <= n
        r0 = pl.multiple_of(jnp.maximum(c - 1, 0) * step, 16)
        assert n <= T0 // 2
        sched = _Sched(zero)
        dur = 2 * NCB * T0
        sched.add(ln_in(jnp.where(c > 0, T0, 0),
                        jnp.where(c > 0, TA // 2, T0 // 2),
                        [r0 + r for r in range(0, n, 16)]),
                  int(F_WIN[0] * dur), int(F_WIN[1] * dur))
        sched.add([functools.partial(prep, wblk.at[j * nfc + c],
                                     w17.at[j, c], r)
                   for j in range(2) for r in range(0, H, 16)],
                  int(F_WIN[0] * dur), int(F_WIN[1] * dur))
        f = _ffn(lhs_b[...], wblk.at[c], wblk.at[nfc + c], sched)
        assert not sched.queue
        xs[0:T0, :] += 0.5 * f
        return carry

    lax.fori_loop(0, nfc, first_tile, 0)
    for j in range(3, na + 1):
        x_copy(j).start()
    for c in range(nfc):
        for cp in w2_copies(c):
            cp.start()
    for cp in w_copies:
        cp.start()

    def phase_a(i, carry):
        @pl.when(i < na)
        def _():
            x_copy(i + 1).wait()

        @pl.when((i >= IW) & (i < IW + nfc))
        def _():
            for cp in w2_copies(i - IW):
                cp.wait()

        @pl.when(i == IW)
        def _():
            w_copies[0].wait()

        h7 = [_up(lhs7[k, :TA // 4, :]) for k in range(7)]
        sched = _Sched(zero)
        dur = 7 * nfc * TA
        win = (int(A_WIN[0] * dur), int(A_WIN[1] * dur),
               [(c * 7 * TA + A_SKIP[0] * TA // 320,
                 c * 7 * TA + A_SKIP[1] * TA // 320)
                for c in range(nfc)])
        base = jnp.maximum(T0 + (i - 2) * TA, 0)
        sched.add(ln_out(base, range(0, TA // 2, 16)), *win)
        base = T0 + jnp.minimum(i, na - 1) * TA
        sched.add(ln_in(base, TA // 2, range(0, TA // 2, 16)), *win)
        rpb = H // 16
        total = w7.shape[0] * rpb
        ipi = -(-total // (na - IW + 1))
        items = []
        for k in range(ipi):
            n = jnp.minimum(jnp.maximum(i - IW, 0) * ipi + k, total - 1)
            src = n // rpb + jnp.where(i >= IW, 2 * nfc, 0)
            items.append(functools.partial(
                prep, wblk.at[src], w7.at[n // rpb],
                pl.multiple_of(n % rpb * 16, 16)))
        assert ipi <= rpb
        sched.add(items, *win)
        f = _ffn7(h7, [w17.at[0, c] for c in range(nfc)],
                  [w17.at[1, c] for c in range(nfc)], sched, *FA)
        assert not sched.queue
        xs[arows(i), :] = (xin[arows(i), :].astype(F32)
                           + 0.5 * jnp.concatenate(f, axis=0))
        return carry

    with jax.named_scope("phase_a"):
        lax.fori_loop(1, na + 1, phase_a, 0)

    for cp in w_copies[1:]:
        cp.wait()

    qk_scale = (D ** -0.5) * math.log2(math.e)

    HM = TM // 32 * 16

    def put7(dst, r0, cs, *p):
        if len(p) == 4:
            ops = enumerate(_sa(*p))
        else:
            ops = zip((1, 2, 3, 4), (p[0] + p[1], *p, p[0] + p[1]))
        for k, t in ops:
            dst[pl.ds(k * PR + r0 // 2, 8), cs] = pltpu.bitcast(
                t.astype(BF16), jnp.uint32)

    def get7(src, k, ds=pl.ds, nr=None):
        nr = nr or (TM - HM if 1 <= k <= 4 else HM)
        return pltpu.bitcast(src[ds(k * PR, nr // 2), :], BF16)

    def groups(r0):
        return (r0, HM + r0) if r0 < HM else (HM + r0,)

    def q_ops(i, r0, c, z):
        p = [hs[rows(i, r, 16), col(2 * h + c)].astype(F32)
             for r in groups(r0) for h in range(2)]
        p[0] = p[0] + _rep(z.v(), 16)
        p[-1] = p[-1] + _rep(z.v(), 16)
        put7(hq7, r0, col(c), *p)

    def q_items(i):
        return [functools.partial(q_ops, i, r0, c)
                for r0 in range(0, TM - HM, 16) for c in range(2)]

    sched = _Sched(zero)
    sched.add(ln_out(N - TA, range(0, TA // 2, 16)), *FD[:2])
    sched.add(q_items(0), *FD[2:])
    for dst in (mq, wvo):
        for u in range(2):
            t = []
            for cs in (col(u), col(u + 2)):
                t.append(_dot_nt(wq[...], wk[cs, :]) if dst is mq
                         else _dot(wv[...], wo[:, cs]))
                sched(t[-1])
            if dst is mq:
                t = [v * qk_scale for v in t]
            for k, v in enumerate(
                    _sb(t[0][:H], t[1][:H], t[0][H:], t[1][H:])):
                dst[k, :, col(u)] = _pk(v)
    assert not sched.queue
    dwf = dw[...].astype(F32)
    for k in range(K):
        dwb[k] = jnp.broadcast_to(dwf[k:k + 1, :], (8, D))

    def conv_block(p, r0, c, done, CT=CT, AT=K):
        cs = col(c)
        acc = [None]

        def item(k0, z=None):
            for k in range(k0, min(k0 + CT, K)):
                off = HALO - K // 2 + k + r0
                w = dwb[k, :, cs]
                if z is not None and k - k0 < AT:
                    w = w + z.v()
                t = gs[p + 1, c, off:off + 8, :] * w
                acc[0] = t if acc[0] is None else acc[0] + t
            if k0 + CT >= K:
                dcs[rows(p, r0, 8), cs] = acc[0]
                done(acc[0])

        return [functools.partial(item, k0) for k0 in range(0, K, CT)]

    def conv_main(p, cols=range(NCB), **kw):
        st = []

        def stats(r0, c, acc):
            if r0 == 0:
                st[:] = [acc, None, None]
                return
            shift, s1, s2 = st
            d = acc - shift
            s1 = d if s1 is None else s1 + d
            s2 = d * d if s2 is None else s2 + d * d
            st[:] = [shift, s1, s2]
            if r0 + 16 == TM:
                dm = s1 * (1.0 / (TM // 8 - 1))
                st_mean[p, :, col(c)] = shift + dm
                st_m2[p, :, col(c)] = s2 - s1 * dm

        return [it for c in cols for r0 in range(0, TM - 8, 8)
                for it in conv_block(p, r0, c,
                                     functools.partial(stats, r0, c), **kw)]

    def conv_edge(p, cols=range(NCB)):
        return [it for c in cols
                for it in conv_block(p, TM - 8, c, lambda acc: None)]


    def phase_b(i, carry):
        b = i // tpb

        sched = _Sched(zero)
        sched.add(conv_edge(jnp.maximum(i - 2, 0))
                  + conv_main(jnp.maximum(i - 1, 0), range(L0, NCB)),
                  int(B_SLOTS[0] * TM), int(B_SLOTS[1] * TM))
        sched.add(q_items(jnp.minimum(i + 1, nt - 1)),
                  int(Q_SLOTS[0] * TM), int(Q_SLOTS[1] * TM))
        acc = [None] * 4
        for k in OQ:
            t = _dot(get7(hq7, k), _up(mq[k]))
            _acc7(acc, k, t, HM)
            sched(t)
        q11, q12, q21, q22 = _quads(
            jnp.concatenate(_join(acc, HM), axis=1), HM)
        q7 = [q11[:HM] - q22[:HM], q21 - q22, q11, q22, q12 - q11,
              q21[:HM] - q11[:HM], q12[:HM] - q22[:HM]]
        q7 = [t.astype(BF16) for t in q7]

        dz = zero_s[0]
        p_buf, al_buf = (p_buf0, p_buf1, p_buf2), (al_buf0, al_buf1, al_buf2)
        s_buf = (s_buf0, s_buf1)

        def dyn(r0, n):
            return pl.ds(pl.multiple_of(dz + r0, 8), n)

        nb = KP // 128

        def chunk(j):
            return pl.ds(pl.multiple_of(b * (TP // 2), KP // 2)
                         + j * KP // 2, KP // 2)

        def combine(m, j, c):
            if len(m) == 7:
                s = [m[0] + m[3] + m[4] + m[6], m[2] + m[4],
                     m[1] + m[3], m[1] - m[0] + m[2] + m[5]]
            else:
                s = [m[0] + m[2], m[1] + m[3]]
            nv = T // 2 - j * KP - c * 128
            if nv < 128:
                lane = lax.broadcasted_iota(jnp.int32, s[0].shape, 1)
                s = [jnp.where(lane < nv, t, -jnp.inf) for t in s]
            return s

        stat = {}

        def put(w, j, r, v):
            for r0 in range(0, v.shape[0], 16):
                stat[w, j, r + r0] = v[r0:r0 + 16]

        def get(w, j, r, n=16):
            return jnp.concatenate(
                [stat[w, j, r0] for r0 in range(r, r + n, 16)], axis=0)

        def scores(j):
            m = [None] * 7
            for k in OS if j else OS0:
                m[k] = _dot_nt(
                    q7[k], _up(ks[(0, 2, 1, 4, 3, 5, 6)[k], chunk(j), :]))
                sched(m[k])
            mx = None
            for c in range(nb):
                s = combine([t[:HM, col(c)] for t in m], j, c)
                e = combine([t[HM:, col(c)] for t in m[1:5]], j, c)
                for h in range(2):
                    t = jnp.concatenate([s[h], s[2 + h], e[h]], axis=0)
                    s_buf[j % 2][:, col(h * nb + c)] = t
                    mx = t if mx is None else jnp.maximum(mx, t)
            mx = jnp.broadcast_to(jnp.max(mx, axis=-1, keepdims=True),
                                  mx.shape)
            if j:
                mx = jnp.maximum(mx, get(0, j - 1, 0, TM))
            put(0, j, 0, mx)

        part = {}

        def soft1(j, r, c0, z):
            rs = slice(r, r + 16)
            m = get(0, j, r) + _rep(z.v(), 16)
            l = functools.reduce(jnp.add, part.pop((j, r), []) + [
                jnp.exp2(s_buf[j % 2][dyn(r, 16), col(c)] - m)
                for c in range(c0, c0 + S1)])
            if c0 + S1 < 2 * nb:
                part[j, r] = [l]
                return
            l = jnp.broadcast_to(jnp.sum(l, axis=-1, keepdims=True),
                                 (16, 128))
            if j:
                l += get(1, j - 1, r) * jnp.exp2(get(0, j - 1, r) - m)
            put(1, j, r, l)
            e = (pltpu.bitcast(l, jnp.int32) >> 23) - 127
            ref = m + e.astype(F32)
            put(2, j, r, ref)
            if j:
                al_buf[j % 3][rs, :] = jnp.exp2(get(2, j - 1, r) - ref)

        def soft2(j, r0, c0, z):
            ref = [get(2, j, r) + _rep(z.v(), 16) for r in groups(r0)]
            p = [jnp.concatenate(
                [jnp.exp2(s_buf[j % 2][dyn(r, 16), col(h * nb + c)] - m)
                 for c in range(c0, c0 + S2)], axis=1)
                 for r, m in zip(groups(r0), ref) for h in range(2)]
            put7(p_buf[j % 3], r0, slice(c0 * 128, (c0 + S2) * 128), *p)

        scd = 7 * HM + 4 * (TM - 2 * HM)
        start = sched.now

        def add_soft(j):
            rbs = range(0, TM - HM, 16)
            t0, t1 = (start + int(t * scd) for t in SW[j:j + 2])
            assert t1 <= start + min(2 * j + LAG + 1, nkc + j) * scd
            assert j < 3 or t0 >= start + min(2 * j + LAG - 4,
                                              nkc + j - 2) * scd
            assert (j + 2 >= nkc
                    or t1 <= start + max(2 * j + 5 - LAG, j + 3) * scd)
            u = (t1 - t0 - sum(SD)) // (len(rbs) + 1)
            for n, r0 in enumerate(rbs):
                its = [[functools.partial(soft1, j, r, c)
                        for r in groups(r0) for c in range(0, 2 * nb, S1)],
                       [functools.partial(soft2, j, r0, c)
                        for c in range(0, nb, S2)]]
                for k, it in enumerate(its):
                    t = t0 + SD[0] + n * u + k * (u + SD[1])
                    sched.add(it, t, t + u)

        for j in range(LAG):
            scores(j)
            add_soft(j)
        acc = [None] * 4
        for j in range(nkc):
            if j + LAG < nkc:
                scores(j + LAG)
                add_soft(j + LAG)
            fresh = [j > 0] * 4
            for k in OP if j + 1 < nkc else OQ:
                w = _up(ks[(0, 2, 6, 5, 3, 4, 1)[k], chunk(j), :])
                m = _dot(get7(p_buf[j % 3], k, dyn), w)
                sched(m)
                for a, _ in _TG[k]:
                    if fresh[a]:
                        al = al_buf[j % 3][dyn(0, TM), :]
                        al = _quads(jnp.concatenate([al] * NCB, axis=1), HM)[a]
                        acc[a] = acc[a] * al[:acc[a].shape[0]]
                        fresh[a] = False
                _acc7(acc, k, m, HM)
        assert not sched.queue
        t = jnp.exp2(get(2, nkc - 1, 0, TM) - get(0, nkc - 1, 0, TM))
        t = t / get(1, nkc - 1, 0, TM)
        o = (jnp.concatenate(_join(acc, HM), axis=1)
             * jnp.concatenate([t] * NCB, axis=1))
        o7 = [t.astype(BF16) for t in _sax(*_quads(o, HM), HM)]
        acc = list(_quads(xs[rows(i), :], HM))
        acc = [acc[0][:HM], acc[1], acc[2], acc[3][:HM]]
        for k in OW:
            _acc7(acc, k, _dot(o7[k], _up(wvo[k])), HM)
        x2 = jnp.concatenate(_join(acc, HM), axis=1)
        xs[rows(i), :] = x2
        h7 = [t.astype(BF16) for t in _sax(*_quads(_ln(x2), HM), HM)]
        sched = _Sched(zero)
        acc = [[None] * 4 for _ in range(2)]
        for n, (h, k) in enumerate(PO):
            t = _dot(h7[k], _up(w7[2 * nfc + h, k]))
            _acc7(acc[h], k, t, HM)
            sched(t)
            if any(e[0] == h for e in PO[n + 1:]):
                continue
            val, gate = _join(acc[h], HM)
            g2 = val * (0.5 + 0.5 * jnp.tanh(0.5 * gate))
            for c in (2 * h, 2 * h + 1):
                g = g2[:, col(c % 2)]
                gs[i + 1, c, HALO:HALO + TM, :] = g
                gs[i, c, HALO + TM:, :] = jnp.where(
                    i % tpb == 0, 0.0, g[:HALO])
                gs[i + 2, c, :HALO, :] = jnp.where(
                    i % tpb == tpb - 1, 0.0, g[TM - HALO:])
            if h == 0 and L0:
                rest = sum(h7[e[1]].shape[0] for e in PO[n + 1:])
                sched.add(conv_main(i, range(L0), CT=LP[2], AT=LP[3]),
                          sched.now + LP[0], sched.now + rest - LP[1])
        assert not sched.queue
        return carry

    with jax.named_scope("phase_b"):
        lax.fori_loop(0, nt, phase_b, 0)
    for item in (conv_main(nt - 1, range(L0, NCB)) + conv_edge(nt - 2)
                 + conv_edge(nt - 1)):
        item()

    ng = TM // 8 - 1
    means = st_mean[...].reshape(nt * 8, D)
    edges = jnp.concatenate([dcs[(p + 1) * TM - 8:(p + 1) * TM, :]
                             for p in range(nt)], axis=0)
    mu = jnp.sum(ng * means + edges, axis=0, keepdims=True) * (1.0 / N)
    dm = means - mu
    de = edges - mu
    var = jnp.sum(st_m2[...].reshape(nt * 8, D) + ng * (dm * dm) + de * de,
                  axis=0, keepdims=True) * (1.0 / N)
    rstd = lax.rsqrt(var + EPS)
    bn[0] = jnp.broadcast_to(mu, (8, D))
    bn[1] = jnp.broadcast_to(rstd, (8, D))

    def bn_silu(i, r0, c, z=None):
        p = []
        for r in (r0, TC // 2 + r0):
            for h in range(2):
                cs = col(2 * h + c)
                mu = bn[0, :, cs] if z is None else bn[0, :, cs] + z.v()
                y = dcs[crows(i, r, 16), cs] - _rep(mu, 16)
                p.append(_silu(y * _rep(bn[1, :, cs], 16)))
        put7(hq7, r0, col(c), *p)

    def bn_items(i):
        return [functools.partial(bn_silu, i, r0, c)
                for r0 in range(0, TC // 2, 16) for c in range(2)]

    def ln_final(i, r0=0, n=TC, z=None):
        obuf[crows(i, r0, n), :] = _ln(xs[crows(i, r0, n), :],
                                       zrep(z, n)).astype(BF16)

    for item in bn_items(0):
        item()

    def phase_c(i, carry):
        @pl.when(i >= 2)
        def _():
            o_copy(i - 2).start()

        sched = _Sched(zero)
        dur = 7 * (1 + 2 * nfc) * TC // 2
        t0, t1 = int(C_WIN[0] * dur), int(C_WIN[1] * dur)
        sched.add([functools.partial(ln_final, jnp.maximum(i - 1, 0), r, RC[0])
                   for r in range(0, TC, RC[0])], t0, t1, C_SKIP)
        sched.add(bn_items(jnp.minimum(i + 1, nc - 1)),
                  t0 + RC[1], t1 + RC[1], C_SKIP)
        acc = list(_quads(xs[crows(i), :], TC // 2))
        for k in OQ:
            t = _dot(get7(hq7, k, nr=TC // 2), _up(w7[2 * nfc + 2, k]))
            _acc7(acc, k, t, TC // 2)
            sched(t)
        x3 = jnp.concatenate(_join(acc, TC // 2), axis=1)
        xs[crows(i), :] = x3
        h = _ln(x3)
        f = _ffn7(_lhs7(h[:TC // 2], h[TC // 2:]),
                  [w7.at[c] for c in range(nfc)],
                  [w7.at[nfc + c] for c in range(nfc)], sched, *FB)
        assert not sched.queue
        xs[crows(i), :] += 0.5 * jnp.concatenate(f, axis=0)
        return carry

    with jax.named_scope("phase_c"):
        lax.fori_loop(0, nc, phase_c, 0)
    o_copy(nc - 2).start()
    last = []
    for k, (r0, r1) in enumerate(zip(EP[:-1], EP[1:])):
        ln_final(nc - 1, r0, r1 - r0)
        rs = crows(nc - 1, r0, r1 - r0)
        last.append(pltpu.make_async_copy(obuf.at[rs, :], out_hbm.at[rs, :],
                                          osem.at[nc - 1 + k]))
        last[-1].start()
    for i in range(nc - 1):
        o_copy(i).wait()
    for cp in last:
        cp.wait()


@jax.jit
def pallas_standalone__conformer_family_conformer__speech_kernel(
    x: jax.Array,
    w_ff1_a: jax.Array,
    w_ff1_b: jax.Array,
    w_q: jax.Array,
    w_k: jax.Array,
    w_v: jax.Array,
    w_o: jax.Array,
    w_pw1: jax.Array,
    dw: jax.Array,
    w_pw2: jax.Array,
    w_ff2_a: jax.Array,
    w_ff2_b: jax.Array,
):
    B, T, D = x.shape
    K = dw.shape[0]
    N = B * T
    weights = (w_ff1_a, w_ff1_b, w_q, w_k, w_v, w_o, w_pw1, dw, w_pw2,
               w_ff2_a, w_ff2_b)
    scratch = [pltpu.VMEM((N, D), BF16)]
    nfc = w_ff1_a.shape[1] // FC
    scratch += [pltpu.VMEM((4 * nfc + 3, D, D), BF16)]
    scratch += [pltpu.VMEM(w.shape, w.dtype)
                for w in (w_q, w_k, w_v, w_o, dw)]
    scratch += [
        pltpu.VMEM((7, D // 4, D // 2), jnp.uint32),
        pltpu.VMEM((7, D // 4, D // 2), jnp.uint32),
        pltpu.VMEM((N, D), F32),
        pltpu.VMEM((N, D), BF16),
        pltpu.VMEM((7, B * -(-T // KC) * KC // 4, D // 2), jnp.uint32),
        pltpu.VMEM((N // TM + 2, D // 128, TM + 2 * HALO, 128), F32),
        pltpu.VMEM((N, D), F32),
        pltpu.VMEM((N // TM, 8, D), F32),
        pltpu.VMEM((N // TM, 8, D), F32),
        pltpu.VMEM((2, 8, D), F32),
        pltpu.VMEM((7, D // 4, D // 2), jnp.uint32),
        pltpu.VMEM((2, nfc, 7, D // 4, D // 2), jnp.uint32),
        pltpu.VMEM((2 * nfc + 3, 7, D // 4, D // 2), jnp.uint32),
        pltpu.VMEM((T0, D), BF16),
        pltpu.VMEM((K, 8, D), F32),
        pltpu.VMEM((ZR, 128), jnp.uint32),
        pltpu.SMEM((1,), jnp.int32),
        pltpu.VMEM((TM + 16, 128), F32),
        pltpu.VMEM((TM + 16, 128), F32),
        pltpu.VMEM((TM + 16, 128), F32),
        pltpu.VMEM((7 * PR, KC // 2), jnp.uint32),
        pltpu.VMEM((7 * PR, KC // 2), jnp.uint32),
        pltpu.VMEM((7 * PR, KC // 2), jnp.uint32),
        pltpu.VMEM((TM, KC), F32),
        pltpu.VMEM((TM, KC), F32),
        pltpu.VMEM((7 * PR, D // 2), jnp.uint32),
        pltpu.SemaphoreType.DMA(((N - T0) // TA + 1,)),
        pltpu.SemaphoreType.DMA((2, nfc)),
        pltpu.SemaphoreType.DMA((3, nfc)),
        pltpu.SemaphoreType.DMA((6,)),
        pltpu.SemaphoreType.DMA((N // TC + len(EP),)),
    ]
    out = pl.pallas_call(
        functools.partial(_kernel, B=B, T=T, D=D, K=K),
        out_shape=jax.ShapeDtypeStruct((N, D), x.dtype),
        in_specs=[pl.BlockSpec(memory_space=pl.ANY)] * 12,
        out_specs=pl.BlockSpec(memory_space=pl.ANY),
        scratch_shapes=scratch,
        compiler_params=pltpu.CompilerParams(
            vmem_limit_bytes=124 * 1024 * 1024),
    )(x.reshape(N, D), *weights)
    return out.reshape(B, T, D)
```

```python
import functools
import math

import jax
import jax.numpy as jnp
from jax import lax
import jax.experimental.pallas as pl
import jax.experimental.pallas.tpu as pltpu

F32 = jnp.float32
BF16 = jnp.bfloat16

TM = 400
T0 = 320
TA = 480
TC = 320
FC = 512
KC = 512
W1A = 1
XF = 0
IW = 3
FA = ((1, 3, 2, 4, 0, 5, 6), (1, 3, 6, 0, 2, 4, 5), 1)
VL = 128
KO = 2
FB = (((2, 4, 3, 1, 0, 6, 5), (2, 4, 3, 1, 0, 6, 5)),
      ((1, 3, 6, 2, 4, 0, 5), (2, 4, 3, 1, 0, 6, 5)),
      ((0, 0, 49), (0, 1, 49), (0, 2, 14)) + ((1, 0, 4), (0, 2, 7)) * 5
      + ((1, 0, 3), (0, 3, 7)) * 7 + ((1, 0, 8), (1, 1, 49)))
P_WIN = (0.1, 0.8)
OQ = (0, 2, 3, 4, 6, 1, 5)
OS0 = (2, 4, 3, 1, 0, 5, 6)
OS = (0, 1, 2, 3, 4, 5, 6)
OP = (0, 1, 2, 3, 4, 5, 6)
OW = (2, 4, 3, 0, 6, 1, 5)
PO = ((0, 2), (0, 4), (1, 2), (0, 3), (0, 0), (0, 6), (0, 1), (0, 5),
      (1, 4), (1, 3), (1, 0), (1, 6), (1, 1), (1, 5))
F_WIN = (0.1, 0.9)
A_WIN = (0.03, 0.81)
A_SKIP = (500, 1300)
FD = (0, 3200, 0, 3200)
B_SLOTS = (1, 53)
Q_SLOTS = (8, 50)
CT = 5
L0 = 1
LP = (0, 100, 3, 1)
S1 = 2
S2 = 1
SD = (0, 140, 120)
LAG = 2
SW = tuple(1 + 1.75 * j for j in range(9))
C_WIN = (0.21, 0.82)
C_SKIP = ()
RC = (8, 100)
EP = (0, 128, 224, 288, 320)
ZR = 32
PR = 112
HALO = 8
EPS = 1e-05


def _ln(x, z=None):
    if z is None:
        m = jnp.mean(x, axis=-1, keepdims=True)
    else:
        t = z
        for c in range(x.shape[-1] // 128):
            t = t + x[:, c * 128:(c + 1) * 128]
        m = jnp.sum(t, axis=-1, keepdims=True) * (1.0 / x.shape[-1])
    xc = x - m
    v = jnp.mean(xc * xc, axis=-1, keepdims=True)
    return xc * lax.rsqrt(v + EPS)


def _silu(a):
    y = 0.5 * a
    return y + y * jnp.tanh(y)


def _dot(a, b):
    return jnp.dot(a, b, preferred_element_type=F32)


def _dot_nt(a, b):
    return lax.dot_general(a, b, (((1,), (1,)), ((), ())),
                           preferred_element_type=F32)


def _pk(v):
    return pltpu.bitcast(v.astype(BF16), jnp.uint32)


def _up(v):
    return pltpu.bitcast(v, BF16)


class _Anchor:
    def __init__(self, t, zero_v):
        self.t, self.zero_v = t, zero_v

    def v(self):
        return pltpu.bitcast(
            pltpu.bitcast(self.t, jnp.uint32) & self.zero_v[0:8, :], F32)


class _Sched:
    def __init__(self, zero_v):
        self.zero_v = zero_v
        self.queue = []
        self.now = 0

    def add(self, items, t0, t1, skip=()):
        assert t0 >= self.now
        ts = [t for t in range(t0, t1)
              if not any(a <= t < b for a, b in skip)]
        self.queue += [(ts[k * len(ts) // len(items)], it)
                       for k, it in enumerate(items)]
        self.queue.sort(key=lambda e: e[0])

    def __call__(self, t, dur=None):
        dur = dur or t.shape[0]
        end = self.now + dur
        while self.queue and self.queue[0][0] < end:
            time, item = self.queue.pop(0)
            r = (time - self.now) * t.shape[0] // dur // 8 * 8
            item(_Anchor(t[r:r + 8, :128], self.zero_v))
        self.now = end


def _rep(z, rows):
    return jnp.concatenate([z] * (rows // 8), axis=0)


def _ffn(h, wa_ref, wb_ref, sched):
    ss = []
    for n in range(wa_ref.shape[1] // 128):
        a = _dot(h, wa_ref[:, n * 128:(n + 1) * 128])
        ss.append(_silu(a))
        sched(a)
    s = jnp.concatenate(ss, axis=1).astype(BF16)
    acc = []
    for n in range(wb_ref.shape[1] // 128):
        acc.append(_dot(s, wb_ref[:, n * 128:(n + 1) * 128]))
        sched(acc[-1])
    return jnp.concatenate(acc, axis=1)


def _sa(a11, a12, a21, a22):
    return [a11 + a22, a21 + a22, a11, a22, a11 + a12, a21 - a11, a12 - a22]


def _sb(b11, b12, b21, b22):
    return [b11 + b22, b11, b12 - b22, b21 - b11, b22, b11 + b12, b21 + b22]


def _sc(m):
    return [m[0] + m[3] - m[4] + m[6], m[4] + m[2], m[3] + m[1],
            m[0] + m[2] - m[1] + m[5]]


def _lhs7(t, u):
    h = t.shape[1] // 2
    return [v.astype(BF16)
            for v in _sa(t[:, :h], t[:, h:], u[:, :h], u[:, h:])]


_SA = ((0, 1, 3), (2, 1, 3), (0, 0, 0), (3, 0, 3), (0, 1, 1), (2, -1, 0),
       (1, -1, 3))
_SB = ((0, 1, 3), (0, 0, 0), (1, -1, 3), (2, -1, 0), (3, 0, 3), (0, 1, 1),
       (2, 1, 3))
_TG = (((0, 1), (3, 1)), ((2, 1), (3, -1)), ((1, 1), (3, 1)), ((0, 1), (2, 1)),
       ((0, -1), (1, 1)), ((3, 1),), ((0, 1),))


def _quads(x, hm):
    h = x.shape[1] // 2
    t = x[:hm]
    if x.shape[0] > 2 * hm:
        t = jnp.concatenate([t, x[2 * hm:]], axis=0)
    return t[:, :h], t[:, h:], x[hm:, :h], x[hm:, h:]


def _sax(a11, a12, a21, a22, hm):
    return [a11[:hm] + a22[:hm], a21 + a22, a11, a22, a11 + a12,
            a21[:hm] - a11[:hm], a12[:hm] - a22[:hm]]


def _acc7(acc, k, m, hm):
    for a, sg in _TG[k]:
        t = m if a in (1, 2) else m[:hm]
        if acc[a] is None:
            acc[a] = t if sg > 0 else -t
        else:
            acc[a] = acc[a] + t if sg > 0 else acc[a] - t


def _join(acc, hm):
    rest = [acc[1][hm:]] if acc[1].shape[0] > hm else []
    return (jnp.concatenate([acc[0], acc[2]], axis=0),
            jnp.concatenate([acc[1][:hm], acc[3]] + rest, axis=0))


def _ffn7(h7, wa, wb, sched, o1, o2, lag, early=()):
    acc = [None] * 7
    hm = h7[0].shape[0]
    u = [[None] * 4 for _ in wa]

    done = set()
    act = [[None] * 4 for _ in wa]
    s7 = [[None] * 7 for _ in wa]

    def run(cks):
        for c, k in cks:
            if (c, k) in done or c >= len(wa):
                continue
            done.add((c, k))
            t = _dot(h7[k], _up(wa[c][k]))
            _acc7(u[c], k, t, hm)
            sched(t)
            for a in range(4):
                if act[c][a] is None and all(
                        (c, n) in done for n in range(7)
                        if a in [e[0] for e in _TG[n]]):
                    act[c][a] = _silu(u[c][a])
            for n, (a, sg, b) in enumerate(_SA):
                if (s7[c][n] is None and act[c][a] is not None
                        and act[c][b] is not None):
                    v = act[c][a]
                    if sg:
                        v = v + act[c][b] if sg > 0 else v - act[c][b]
                    s7[c][n] = v.astype(BF16)

    run(early)
    for c, cb in enumerate(wb):
        run([(c, k) for k in o1] + [(c + 1, k) for k in o1[:lag]])
        for k in o2:
            p = _dot(s7[c][k], _up(cb[k]))
            acc[k] = p if acc[k] is None else acc[k] + p
            sched(p)
    c = _sc(acc)
    return jnp.concatenate(c[:2], axis=1), jnp.concatenate(c[2:], axis=1)


def _q4(x):
    h, w = x.shape[0] // 2, x.shape[1] // 2
    return x[:h, :w], x[:h, w:], x[h:, :w], x[h:, w:]


def _twice(f, x):
    return [v for y in f(*_q4(x)) for v in f(*_q4(y))]


def _pm(a, sg, b):
    return a if not sg else a + b if sg > 0 else a - b


def _ffn49(h49, w, nfc, sched, oi, oo, plan):
    hm = h49[0].shape[0]
    src = [[n for n in range(7) if a in [e[0] for e in _TG[n]]]
           for a in range(4)]
    val = {}

    def add(key, sg, t):
        if key not in val:
            val[key] = t if sg > 0 else -t
        else:
            val[key] = _pm(val[key], sg, t)

    def collect(done, tag, k1, k2, t):
        done.add((k1, k2))
        for b, sg in _TG[k2]:
            add((tag, 'm', k1, b), sg, t)
            if all((k1, n) in done for n in src[b]):
                for a, sg1 in _TG[k1]:
                    add((tag, 'u', a, b), sg1, val[tag, 'm', k1, b])

    done = [set() for _ in range(nfc + 1)]

    def step_in(c, k1, k2):
        t = _dot(h49[7 * k1 + k2], w(7 * k1 + k2, c, 1))
        collect(done[c], c, k1, k2, t)
        sched(t, hm // 4)
        for a in range(4):
            for b in range(4):
                if (c, 'a', a, b) not in val and all(
                        (m, n) in done[c] for m in src[a] for n in src[b]):
                    val[c, 'a', a, b] = _silu(val[c, 'u', a, b])
        for n, (a, sg, a2) in enumerate(_SA):
            for b in range(4):
                if ((c, 'y', n, b) not in val and (c, 'a', a, b) in val
                        and (c, 'a', a2, b) in val):
                    val[c, 'y', n, b] = _pm(val[c, 'a', a, b], sg,
                                            val[c, 'a', a2, b])
            for m, (b, sg, b2) in enumerate(_SA):
                if ((c, 's', n, m) not in val and (c, 'y', n, b) in val
                        and (c, 'y', n, b2) in val):
                    val[c, 's', n, m] = _pm(val[c, 'y', n, b], sg,
                                            val[c, 'y', n, b2]).astype(BF16)

    def step_out(g, k1, k2):
        t = _dot(jnp.concatenate([val[c, 's', k1, k2] for c in
                                  range(g * KO, (g + 1) * KO)], axis=1),
                 w(7 * k1 + k2, nfc + g * KO, KO))
        sched(t, hm * KO // 4)
        add(('p', k1, k2), 1, t)
        if (g + 1) * KO == nfc:
            collect(done[-1], 'o', k1, k2, val['p', k1, k2])

    todo = {(d, c): [(k1, k2) for k1 in o[0] for k2 in o[1]]
            for d, o in enumerate((oi, oo)) for c in range(nfc)}
    for d, c, n in plan:
        for k1, k2 in todo[d, c][:n]:
            (step_out if d else step_in)(c, k1, k2)
        del todo[d, c][:n]
    return jnp.concatenate(
        [jnp.concatenate([val['o', 'u', a // 2 * 2 + b // 2, a % 2 * 2 + b % 2]
                          for b in range(4)], axis=1) for a in range(4)],
        axis=0)


def _kernel(x_hbm, w1a_hbm, w1b_hbm, wq_hbm, wk_hbm, wv_hbm, wo_hbm,
            wp1_hbm, dw_hbm, wp2_hbm, w2a_hbm, w2b_hbm,
            out_hbm,
            xin, wblk, wq, wk, wv, wo, dw,
            mq, wvo, xs, hs, ks, gs, dcs, st_mean, st_m2, bn,
            lhs7, w17, w7, w49, lhs_b, dwb, zero, zero_s,
            al_buf0, al_buf1, al_buf2,
            p_buf0, p_buf1, p_buf2, s_buf0, s_buf1, hq7,
            xsem, w1sem, w2sem, wsem, osem,
            *, B, T, D, K):
    N = B * T
    obuf = xin
    KP = KC // 2
    nkc = -(-T // KC)
    TP = nkc * KP
    NCB = D // 128
    nt = N // TM
    tpb = T // TM

    def rows(i, r0=0, n=TM):
        return pl.ds(pl.multiple_of(i * TM, 16) + r0, n)

    def col(c):
        if isinstance(c, int):
            return slice(c * 128, (c + 1) * 128)
        return pl.ds(pl.multiple_of(c * 128, 128), 128)

    na = (N - T0) // TA
    H = D // 2

    def arows(i, r0=0, n=TA):
        return pl.ds(pl.multiple_of(T0 + (i - 1) * TA, 16) + r0, n)

    def x_copy(i):
        rs = pl.ds(0, T0) if isinstance(i, int) and i == 0 else arows(i)
        return pltpu.make_async_copy(x_hbm.at[rs, :], xin.at[rs, :],
                                     xsem.at[i])

    nc = N // TC

    def crows(i, r0=0, n=TC):
        return pl.ds(pl.multiple_of(i * TC, 16) + r0, n)

    def o_copy(i):
        return pltpu.make_async_copy(obuf.at[crows(i), :],
                                     out_hbm.at[crows(i), :], osem.at[i])

    nfc = w17.shape[1]
    P1, P2 = 4 * nfc, 4 * nfc + 2

    def w1_copies(c):
        fs = pl.ds(pl.multiple_of(c * FC, FC), FC)
        return [pltpu.make_async_copy(w1a_hbm.at[:, fs], wblk.at[c],
                                      w1sem.at[0, c]),
                pltpu.make_async_copy(w1b_hbm.at[fs, :], wblk.at[nfc + c],
                                      w1sem.at[1, c])]

    def w2_copies(c):
        fs = pl.ds(pl.multiple_of(c * FC, FC), FC)
        hs_ = pl.ds(pl.multiple_of(c // 2 * H, H), H)
        return [pltpu.make_async_copy(s, d, w2sem.at[j, c])
                for j, (s, d) in enumerate([
                    (w2a_hbm.at[:, fs], wblk.at[2 * nfc + c]),
                    (w2b_hbm.at[fs, :], wblk.at[3 * nfc + c]),
                    (wp1_hbm.at[:, pl.ds(pl.multiple_of(c * H, H), H)],
                     wblk.at[P1 + c % 2, :, hs_])])]

    assert nfc == 4
    w_pairs = [(wp2_hbm, wblk.at[P2]), (wq_hbm, wq), (wk_hbm, wk),
               (wv_hbm, wv), (wo_hbm, wo), (dw_hbm, dw)]
    w_copies = [pltpu.make_async_copy(s, d, wsem.at[j])
                for j, (s, d) in enumerate(w_pairs)]

    x_copy(0).start()
    for cp in w1_copies(0):
        cp.start()

    zero[...] = jnp.zeros(zero.shape, jnp.uint32)
    zero_s[0] = 0
    for c in range(NCB):
        gs[1, c, 0:HALO, :] = jnp.zeros((HALO, 128), F32)
        gs[nt, c, HALO + TM:, :] = jnp.zeros((HALO, 128), F32)
    for b in range(B):
        ks[:, (b * TP + T // 2) // 2:(b + 1) * TP // 2, :] = jnp.zeros(
            (7, (TP - T // 2) // 2, H), jnp.uint32)

    def zrep(z, n):
        return None if z is None else _rep(z.v(), n)

    def pair_items(first, second, rows0):
        items = []
        for r0 in rows0:
            t = []
            items += [functools.partial(first, t, r0),
                      functools.partial(second, t, r0)]
        return items

    def ln_in(base, half, rows0):
        def first(t, r0, z, base=base):
            t.append(_ln(xin[pl.ds(pl.multiple_of(base, 16) + r0, 16), :]
                         .astype(F32), zrep(z, 16)))

        def second(t, r0, z):
            first(t, r0, z, base + half)
            r1 = r0 // 2 if isinstance(r0, int) else pl.multiple_of(r0 // 2, 8)
            for k, v in enumerate(_lhs7(*t)):
                lhs7[k, pl.ds(r1, 8), :] = _pk(v)

        return pair_items(first, second, rows0)

    def ln_out(base, rows0):
        def first(t, r0, z, off=0):
            rs = pl.ds(pl.multiple_of(base, 32) + 2 * r0 + off, 16)
            t.append(_ln(xs[rs, :], zrep(z, 16)))
            hs[rs, :] = t[-1].astype(BF16)

        def second(t, r0, z):
            first(t, r0, z, 16)
            g = base // 32 + r0 // 16
            g += g // (T // 32) * ((TP - T // 2) // 16)
            for k, v in enumerate(_lhs7(*t)):
                ks[k, pl.ds(pl.multiple_of(g * 8, 8), 8), :] = _pk(v)

        return pair_items(first, second, rows0)

    def prep(src, dst, r0, z=None):
        q = [src[pl.ds(r + r0, 16), c:c + H].astype(F32)
             for r in (0, H) for c in (0, H)]
        if z is not None:
            zz = jnp.concatenate([_rep(z.v(), 16)] * (H // 128), axis=1)
            q[0], q[3] = q[0] + zz, q[3] + zz
        r1 = r0 // 2 if isinstance(r0, int) else pl.multiple_of(r0 // 2, 8)
        for k, v in enumerate(_sb(*q)):
            dst[k, pl.ds(r1, 8), :] = _pk(v)

    def prep2(blk, n, k1, z):
        rpb = D // 64

        def quad(a):
            return jnp.concatenate(
                [wblk[blk + n // rpb,
                      pl.ds(pl.multiple_of(n % rpb * 16, 16) + r, 16),
                      a % 2 * H:(a % 2 + 1) * H].astype(F32)
                 for r in (a // 2 * H, a // 2 * H + H // 2)], axis=0)

        a, sg, b = _SB[k1]
        y = _pm(quad(a) + jnp.concatenate([_rep(z.v(), 32)] * 2, axis=1),
                sg, quad(b))
        for k, v in enumerate(_sb(*_q4(y))):
            w49[7 * k1 + k, pl.ds(pl.multiple_of(n * 8, 8), 8), :] = _pk(v)

    x_copy(0).wait()
    if W1A == 2:
        for cp in w1_copies(1):
            cp.start()
    lhs_b[...] = _ln(xin[0:T0, :].astype(F32)).astype(BF16)
    xs[0:T0, :] = xin[0:T0, :].astype(F32)

    def first_tile(c, carry):
        for cp in w1_copies(c):
            cp.wait()

        @pl.when(c == 1)
        def _():
            x_copy(1).wait()

        if XF:
            @pl.when(c % 2 == 0)
            def _():
                x_copy(1 + c // 2).start()

        @pl.when(c + W1A < nfc)
        def _():
            for cp in w1_copies(c + W1A):
                cp.start()

        if not XF:
            @pl.when(c % 2 == 0)
            def _():
                x_copy(1 + c // 2).start()

        n = -(-TA // 2 // (nfc - 1) // 16) * 16
        step = (TA // 2 - n) // (nfc - 2)
        assert step % 16 == 0 and step <= n
        r0 = pl.multiple_of(jnp.maximum(c - 1, 0) * step, 16)
        assert n <= T0 // 2
        sched = _Sched(zero)
        dur = 2 * NCB * T0
        sched.add(ln_in(jnp.where(c > 0, T0, 0),
                        jnp.where(c > 0, TA // 2, T0 // 2),
                        [r0 + r for r in range(0, n, 16)]),
                  int(F_WIN[0] * dur), int(F_WIN[1] * dur))
        sched.add([functools.partial(prep, wblk.at[j * nfc + c],
                                     w17.at[j, c], r)
                   for j in range(2) for r in range(0, H, 16)],
                  int(F_WIN[0] * dur), int(F_WIN[1] * dur))
        f = _ffn(lhs_b[...], wblk.at[c], wblk.at[nfc + c], sched)
        assert not sched.queue
        xs[0:T0, :] += 0.5 * f
        return carry

    lax.fori_loop(0, nfc, first_tile, 0)
    for j in range(3, na + 1):
        x_copy(j).start()
    for c in range(nfc):
        for cp in w2_copies(c):
            cp.start()
    for cp in w_copies:
        cp.start()

    def phase_a(i, carry):
        @pl.when(i < na)
        def _():
            x_copy(i + 1).wait()

        @pl.when((i >= IW) & (i < IW + nfc))
        def _():
            for cp in w2_copies(i - IW):
                cp.wait()

        @pl.when(i == IW)
        def _():
            w_copies[0].wait()

        h7 = [_up(lhs7[k, :TA // 4, :]) for k in range(7)]
        sched = _Sched(zero)
        dur = 7 * nfc * TA
        win = (int(A_WIN[0] * dur), int(A_WIN[1] * dur),
               [(c * 7 * TA + A_SKIP[0] * TA // 320,
                 c * 7 * TA + A_SKIP[1] * TA // 320)
                for c in range(nfc)])
        base = jnp.maximum(T0 + (i - 2) * TA, 0)
        sched.add(ln_out(base, range(0, TA // 2, 16)), *win)
        base = T0 + jnp.minimum(i, na - 1) * TA
        sched.add(ln_in(base, TA // 2, range(0, TA // 2, 16)), *win)
        rpb = H // 16
        total = w7.shape[0] * rpb
        ipi = -(-total // (na - IW + 1))
        items = []
        for k in range(ipi):
            n = jnp.minimum(jnp.maximum(i - IW, 0) * ipi + k, total - 1)
            src = n // rpb + jnp.where(i >= IW, P1, 0)
            items.append(functools.partial(
                prep, wblk.at[src], w7.at[n // rpb],
                pl.multiple_of(n % rpb * 16, 16)))
        assert ipi <= rpb
        sched.add(items, *win)
        total = w49.shape[1] // 8
        ipi = -(-total // (na - IW + 1))
        sched.add([functools.partial(
            prep2, jnp.where(i >= IW, 2 * nfc, 0),
            jnp.minimum(jnp.maximum(i - IW, 0) * ipi + k, total - 1), k1)
            for k in range(ipi) for k1 in range(7)],
            int(P_WIN[0] * dur), int(P_WIN[1] * dur), win[2])
        f = _ffn7(h7, [w17.at[0, c] for c in range(nfc)],
                  [w17.at[1, c] for c in range(nfc)], sched, *FA)
        assert not sched.queue
        xs[arows(i), :] = (xin[arows(i), :].astype(F32)
                           + 0.5 * jnp.concatenate(f, axis=0))
        return carry

    with jax.named_scope("phase_a"):
        lax.fori_loop(1, na + 1, phase_a, 0)

    for cp in w_copies[1:]:
        cp.wait()

    qk_scale = (D ** -0.5) * math.log2(math.e)

    HM = TM // 32 * 16

    def put7(dst, r0, cs, *p):
        if len(p) == 4:
            ops = enumerate(_sa(*p))
        else:
            ops = zip((1, 2, 3, 4), (p[0] + p[1], *p, p[0] + p[1]))
        for k, t in ops:
            dst[pl.ds(k * PR + r0 // 2, 8), cs] = pltpu.bitcast(
                t.astype(BF16), jnp.uint32)

    def get7(src, k, ds=pl.ds, nr=None):
        nr = nr or (TM - HM if 1 <= k <= 4 else HM)
        return pltpu.bitcast(src[ds(k * PR, nr // 2), :], BF16)

    def groups(r0):
        return (r0, HM + r0) if r0 < HM else (HM + r0,)

    def q_ops(i, r0, c, z):
        p = [hs[rows(i, r, 16), col(2 * h + c)].astype(F32)
             for r in groups(r0) for h in range(2)]
        p[0] = p[0] + _rep(z.v(), 16)
        p[-1] = p[-1] + _rep(z.v(), 16)
        put7(hq7, r0, col(c), *p)

    def q_items(i):
        return [functools.partial(q_ops, i, r0, c)
                for r0 in range(0, TM - HM, 16) for c in range(2)]

    sched = _Sched(zero)
    sched.add(ln_out(N - TA, range(0, TA // 2, 16)), *FD[:2])
    sched.add(q_items(0), *FD[2:])
    for dst in (mq, wvo):
        for u in range(2):
            t = []
            for cs in (col(u), col(u + 2)):
                t.append(_dot_nt(wq[...], wk[cs, :]) if dst is mq
                         else _dot(wv[...], wo[:, cs]))
                sched(t[-1])
            if dst is mq:
                t = [v * qk_scale for v in t]
            for k, v in enumerate(
                    _sb(t[0][:H], t[1][:H], t[0][H:], t[1][H:])):
                dst[k, :, col(u)] = _pk(v)
    assert not sched.queue
    dwf = dw[...].astype(F32)
    for k in range(K):
        dwb[k] = jnp.broadcast_to(dwf[k:k + 1, :], (8, D))

    def conv_block(p, r0, c, done, CT=CT, AT=K):
        cs = col(c)
        acc = [None]

        def item(k0, z=None):
            for k in range(k0, min(k0 + CT, K)):
                off = HALO - K // 2 + k + r0
                w = dwb[k, :, cs]
                if z is not None and k - k0 < AT:
                    w = w + z.v()
                t = gs[p + 1, c, off:off + 8, :] * w
                acc[0] = t if acc[0] is None else acc[0] + t
            if k0 + CT >= K:
                dcs[rows(p, r0, 8), cs] = acc[0]
                done(acc[0])

        return [functools.partial(item, k0) for k0 in range(0, K, CT)]

    def conv_main(p, cols=range(NCB), **kw):
        st = []

        def stats(r0, c, acc):
            if r0 == 0:
                st[:] = [acc, None, None]
                return
            shift, s1, s2 = st
            d = acc - shift
            s1 = d if s1 is None else s1 + d
            s2 = d * d if s2 is None else s2 + d * d
            st[:] = [shift, s1, s2]
            if r0 + 16 == TM:
                dm = s1 * (1.0 / (TM // 8 - 1))
                st_mean[p, :, col(c)] = shift + dm
                st_m2[p, :, col(c)] = s2 - s1 * dm

        return [it for c in cols for r0 in range(0, TM - 8, 8)
                for it in conv_block(p, r0, c,
                                     functools.partial(stats, r0, c), **kw)]

    def conv_edge(p, cols=range(NCB)):
        return [it for c in cols
                for it in conv_block(p, TM - 8, c, lambda acc: None)]


    def phase_b(i, carry):
        b = i // tpb

        sched = _Sched(zero)
        sched.add(conv_edge(jnp.maximum(i - 2, 0))
                  + conv_main(jnp.maximum(i - 1, 0), range(L0, NCB)),
                  int(B_SLOTS[0] * TM), int(B_SLOTS[1] * TM))
        sched.add(q_items(jnp.minimum(i + 1, nt - 1)),
                  int(Q_SLOTS[0] * TM), int(Q_SLOTS[1] * TM))
        acc = [None] * 4
        for k in OQ:
            t = _dot(get7(hq7, k), _up(mq[k]))
            _acc7(acc, k, t, HM)
            sched(t)
        q11, q12, q21, q22 = _quads(
            jnp.concatenate(_join(acc, HM), axis=1), HM)
        q7 = [q11[:HM] - q22[:HM], q21 - q22, q11, q22, q12 - q11,
              q21[:HM] - q11[:HM], q12[:HM] - q22[:HM]]
        q7 = [t.astype(BF16) for t in q7]

        dz = zero_s[0]
        p_buf, al_buf = (p_buf0, p_buf1, p_buf2), (al_buf0, al_buf1, al_buf2)
        s_buf = (s_buf0, s_buf1)

        def dyn(r0, n):
            return pl.ds(pl.multiple_of(dz + r0, 8), n)

        nb = KP // 128

        def chunk(j):
            return pl.ds(pl.multiple_of(b * (TP // 2), KP // 2)
                         + j * KP // 2, KP // 2)

        def combine(m, j, c):
            if len(m) == 7:
                s = [m[0] + m[3] + m[4] + m[6], m[2] + m[4],
                     m[1] + m[3], m[1] - m[0] + m[2] + m[5]]
            else:
                s = [m[0] + m[2], m[1] + m[3]]
            nv = T // 2 - j * KP - c * 128
            if nv < 128:
                lane = lax.broadcasted_iota(jnp.int32, s[0].shape, 1)
                s = [jnp.where(lane < nv, t, -jnp.inf) for t in s]
            return s

        stat = {}

        def put(w, j, r, v):
            for r0 in range(0, v.shape[0], 16):
                stat[w, j, r + r0] = v[r0:r0 + 16]

        def get(w, j, r, n=16):
            return jnp.concatenate(
                [stat[w, j, r0] for r0 in range(r, r + n, 16)], axis=0)

        def scores(j):
            m = [None] * 7
            for k in OS if j else OS0:
                m[k] = _dot_nt(
                    q7[k], _up(ks[(0, 2, 1, 4, 3, 5, 6)[k], chunk(j), :]))
                sched(m[k])
            mx = None
            for c in range(nb):
                s = combine([t[:HM, col(c)] for t in m], j, c)
                e = combine([t[HM:, col(c)] for t in m[1:5]], j, c)
                for h in range(2):
                    t = jnp.concatenate([s[h], s[2 + h], e[h]], axis=0)
                    s_buf[j % 2][:, col(h * nb + c)] = t
                    mx = t if mx is None else jnp.maximum(mx, t)
            mx = jnp.broadcast_to(jnp.max(mx, axis=-1, keepdims=True),
                                  mx.shape)
            if j:
                mx = jnp.maximum(mx, get(0, j - 1, 0, TM))
            put(0, j, 0, mx)

        part = {}

        def soft1(j, r, c0, z):
            rs = slice(r, r + 16)
            m = get(0, j, r) + _rep(z.v(), 16)
            l = functools.reduce(jnp.add, part.pop((j, r), []) + [
                jnp.exp2(s_buf[j % 2][dyn(r, 16), col(c)] - m)
                for c in range(c0, c0 + S1)])
            if c0 + S1 < 2 * nb:
                part[j, r] = [l]
                return
            l = jnp.broadcast_to(jnp.sum(l, axis=-1, keepdims=True),
                                 (16, 128))
            if j:
                l += get(1, j - 1, r) * jnp.exp2(get(0, j - 1, r) - m)
            put(1, j, r, l)
            e = (pltpu.bitcast(l, jnp.int32) >> 23) - 127
            ref = m + e.astype(F32)
            put(2, j, r, ref)
            if j:
                al_buf[j % 3][rs, :] = jnp.exp2(get(2, j - 1, r) - ref)

        def soft2(j, r0, c0, z):
            ref = [get(2, j, r) + _rep(z.v(), 16) for r in groups(r0)]
            p = [jnp.concatenate(
                [jnp.exp2(s_buf[j % 2][dyn(r, 16), col(h * nb + c)] - m)
                 for c in range(c0, c0 + S2)], axis=1)
                 for r, m in zip(groups(r0), ref) for h in range(2)]
            put7(p_buf[j % 3], r0, slice(c0 * 128, (c0 + S2) * 128), *p)

        scd = 7 * HM + 4 * (TM - 2 * HM)
        start = sched.now

        def add_soft(j):
            rbs = range(0, TM - HM, 16)
            t0, t1 = (start + int(t * scd) for t in SW[j:j + 2])
            assert t1 <= start + min(2 * j + LAG + 1, nkc + j) * scd
            assert j < 3 or t0 >= start + min(2 * j + LAG - 4,
                                              nkc + j - 2) * scd
            assert (j + 2 >= nkc
                    or t1 <= start + max(2 * j + 5 - LAG, j + 3) * scd)
            u = (t1 - t0 - sum(SD)) // (len(rbs) + 1)
            for n, r0 in enumerate(rbs):
                its = [[functools.partial(soft1, j, r, c)
                        for r in groups(r0) for c in range(0, 2 * nb, S1)],
                       [functools.partial(soft2, j, r0, c)
                        for c in range(0, nb, S2)]]
                for k, it in enumerate(its):
                    t = t0 + SD[0] + n * u + k * (u + SD[1])
                    sched.add(it, t, t + u)

        for j in range(LAG):
            scores(j)
            add_soft(j)
        acc = [None] * 4
        for j in range(nkc):
            if j + LAG < nkc:
                scores(j + LAG)
                add_soft(j + LAG)
            fresh = [j > 0] * 4
            for k in OP if j + 1 < nkc else OQ:
                w = _up(ks[(0, 2, 6, 5, 3, 4, 1)[k], chunk(j), :])
                m = _dot(get7(p_buf[j % 3], k, dyn), w)
                sched(m)
                for a, _ in _TG[k]:
                    if fresh[a]:
                        al = al_buf[j % 3][dyn(0, TM), :]
                        al = _quads(jnp.concatenate([al] * NCB, axis=1), HM)[a]
                        acc[a] = acc[a] * al[:acc[a].shape[0]]
                        fresh[a] = False
                _acc7(acc, k, m, HM)
        assert not sched.queue
        t = jnp.exp2(get(2, nkc - 1, 0, TM) - get(0, nkc - 1, 0, TM))
        t = t / get(1, nkc - 1, 0, TM)
        o = (jnp.concatenate(_join(acc, HM), axis=1)
             * jnp.concatenate([t] * NCB, axis=1))
        o7 = [t.astype(BF16) for t in _sax(*_quads(o, HM), HM)]
        acc = list(_quads(xs[rows(i), :], HM))
        acc = [acc[0][:HM], acc[1], acc[2], acc[3][:HM]]
        for k in OW:
            _acc7(acc, k, _dot(o7[k], _up(wvo[k])), HM)
        x2 = jnp.concatenate(_join(acc, HM), axis=1)
        xs[rows(i), :] = x2
        h7 = [t.astype(BF16) for t in _sax(*_quads(_ln(x2), HM), HM)]
        sched = _Sched(zero)
        acc = [[None] * 4 for _ in range(2)]
        for n, (h, k) in enumerate(PO):
            t = _dot(h7[k], _up(w7[h, k]))
            _acc7(acc[h], k, t, HM)
            sched(t)
            if any(e[0] == h for e in PO[n + 1:]):
                continue
            val, gate = _join(acc[h], HM)
            g2 = val * (0.5 + 0.5 * jnp.tanh(0.5 * gate))
            for c in (2 * h, 2 * h + 1):
                g = g2[:, col(c % 2)]
                gs[i + 1, c, HALO:HALO + TM, :] = g
                gs[i, c, HALO + TM:, :] = jnp.where(
                    i % tpb == 0, 0.0, g[:HALO])
                gs[i + 2, c, :HALO, :] = jnp.where(
                    i % tpb == tpb - 1, 0.0, g[TM - HALO:])
            if h == 0 and L0:
                rest = sum(h7[e[1]].shape[0] for e in PO[n + 1:])
                sched.add(conv_main(i, range(L0), CT=LP[2], AT=LP[3]),
                          sched.now + LP[0], sched.now + rest - LP[1])
        assert not sched.queue
        return carry

    with jax.named_scope("phase_b"):
        lax.fori_loop(0, nt, phase_b, 0)
    for item in (conv_main(nt - 1, range(L0, NCB)) + conv_edge(nt - 2)
                 + conv_edge(nt - 1)):
        item()

    ng = TM // 8 - 1
    means = st_mean[...].reshape(nt * 8, D)
    edges = jnp.concatenate([dcs[(p + 1) * TM - 8:(p + 1) * TM, :]
                             for p in range(nt)], axis=0)
    mu = jnp.sum(ng * means + edges, axis=0, keepdims=True) * (1.0 / N)
    dm = means - mu
    de = edges - mu
    var = jnp.sum(st_m2[...].reshape(nt * 8, D) + ng * (dm * dm) + de * de,
                  axis=0, keepdims=True) * (1.0 / N)
    rstd = lax.rsqrt(var + EPS)
    bn[0] = jnp.broadcast_to(mu, (8, D))
    bn[1] = jnp.broadcast_to(rstd, (8, D))

    def bn_silu(i, r0, c, z=None):
        p = []
        for r in (r0, TC // 2 + r0):
            for h in range(2):
                cs = col(2 * h + c)
                mu = bn[0, :, cs] if z is None else bn[0, :, cs] + z.v()
                y = dcs[crows(i, r, 16), cs] - _rep(mu, 16)
                p.append(_silu(y * _rep(bn[1, :, cs], 16)))
        put7(hq7, r0, col(c), *p)

    def bn_items(i):
        return [functools.partial(bn_silu, i, r0, c)
                for r0 in range(0, TC // 2, 16) for c in range(2)]

    def ln_final(i, r0=0, n=TC, z=None):
        obuf[crows(i, r0, n), :] = _ln(xs[crows(i, r0, n), :],
                                       zrep(z, n)).astype(BF16)

    for item in bn_items(0):
        item()

    def phase_c(i, carry):
        @pl.when(i >= 2)
        def _():
            o_copy(i - 2).start()

        sched = _Sched(zero)
        dur = (7 * 8 + 49 * 2 * nfc) * TC // 16
        t0, t1 = int(C_WIN[0] * dur), int(C_WIN[1] * dur)
        sched.add([functools.partial(ln_final, jnp.maximum(i - 1, 0), r, RC[0])
                   for r in range(0, TC, RC[0])], t0, t1, C_SKIP)
        sched.add(bn_items(jnp.minimum(i + 1, nc - 1)),
                  t0 + RC[1], t1 + RC[1], C_SKIP)
        acc = list(_quads(xs[crows(i), :], TC // 2))
        for k in OQ:
            t = _dot(get7(hq7, k, nr=TC // 2), _up(w7[2, k]))
            _acc7(acc, k, t, TC // 2)
            sched(t)
        x3 = jnp.concatenate(_join(acc, TC // 2), axis=1)
        xs[crows(i), :] = x3
        h = _ln(x3)
        f = _ffn49([v.astype(BF16) for v in _twice(_sa, h)],
                   lambda k, b, n: _up(w49[k, b * 64:(b + n) * 64, :]),
                   nfc, sched, *FB)
        assert not sched.queue
        xs[crows(i), :] += 0.5 * f
        return carry

    with jax.named_scope("phase_c"):
        lax.fori_loop(0, nc, phase_c, 0)
    o_copy(nc - 2).start()
    last = []
    for k, (r0, r1) in enumerate(zip(EP[:-1], EP[1:])):
        ln_final(nc - 1, r0, r1 - r0)
        rs = crows(nc - 1, r0, r1 - r0)
        last.append(pltpu.make_async_copy(obuf.at[rs, :], out_hbm.at[rs, :],
                                          osem.at[nc - 1 + k]))
        last[-1].start()
    for i in range(nc - 1):
        o_copy(i).wait()
    for cp in last:
        cp.wait()


@jax.jit
def pallas_standalone__conformer_family_conformer__speech_kernel(
    x: jax.Array,
    w_ff1_a: jax.Array,
    w_ff1_b: jax.Array,
    w_q: jax.Array,
    w_k: jax.Array,
    w_v: jax.Array,
    w_o: jax.Array,
    w_pw1: jax.Array,
    dw: jax.Array,
    w_pw2: jax.Array,
    w_ff2_a: jax.Array,
    w_ff2_b: jax.Array,
):
    B, T, D = x.shape
    K = dw.shape[0]
    N = B * T
    weights = (w_ff1_a, w_ff1_b, w_q, w_k, w_v, w_o, w_pw1, dw, w_pw2,
               w_ff2_a, w_ff2_b)
    scratch = [pltpu.VMEM((N, D), BF16)]
    nfc = w_ff1_a.shape[1] // FC
    scratch += [pltpu.VMEM((4 * nfc + 3, D, D), BF16)]
    scratch += [pltpu.VMEM(w.shape, w.dtype)
                for w in (w_q, w_k, w_v, w_o, dw)]
    scratch += [
        pltpu.VMEM((7, D // 4, D // 2), jnp.uint32),
        pltpu.VMEM((7, D // 4, D // 2), jnp.uint32),
        pltpu.VMEM((N, D), F32),
        pltpu.VMEM((N, D), BF16),
        pltpu.VMEM((7, B * -(-T // KC) * KC // 4, D // 2), jnp.uint32),
        pltpu.VMEM((N // TM + 2, D // 128, TM + 2 * HALO, 128), F32),
        pltpu.VMEM((N, D), F32),
        pltpu.VMEM((N // TM, 8, D), F32),
        pltpu.VMEM((N // TM, 8, D), F32),
        pltpu.VMEM((2, 8, D), F32),
        pltpu.VMEM((7, D // 4, D // 2), jnp.uint32),
        pltpu.VMEM((2, nfc, 7, D // 4, D // 2), jnp.uint32),
        pltpu.VMEM((3, 7, D // 4, D // 2), jnp.uint32),
        pltpu.VMEM((49, nfc * D // 4, D // 4), jnp.uint32),
        pltpu.VMEM((T0, D), BF16),
        pltpu.VMEM((K, 8, D), F32),
        pltpu.VMEM((ZR, 128), jnp.uint32),
        pltpu.SMEM((1,), jnp.int32),
        pltpu.VMEM((TM + 16, 128), F32),
        pltpu.VMEM((TM + 16, 128), F32),
        pltpu.VMEM((TM + 16, 128), F32),
        pltpu.VMEM((7 * PR, KC // 2), jnp.uint32),
        pltpu.VMEM((7 * PR, KC // 2), jnp.uint32),
        pltpu.VMEM((7 * PR, KC // 2), jnp.uint32),
        pltpu.VMEM((TM, KC), F32),
        pltpu.VMEM((TM, KC), F32),
        pltpu.VMEM((7 * PR, D // 2), jnp.uint32),
        pltpu.SemaphoreType.DMA(((N - T0) // TA + 1,)),
        pltpu.SemaphoreType.DMA((2, nfc)),
        pltpu.SemaphoreType.DMA((3, nfc)),
        pltpu.SemaphoreType.DMA((6,)),
        pltpu.SemaphoreType.DMA((N // TC + len(EP),)),
    ]
    out = pl.pallas_call(
        functools.partial(_kernel, B=B, T=T, D=D, K=K),
        out_shape=jax.ShapeDtypeStruct((N, D), x.dtype),
        in_specs=[pl.BlockSpec(memory_space=pl.ANY)] * 12,
        out_specs=pl.BlockSpec(memory_space=pl.ANY),
        scratch_shapes=scratch,
        compiler_params=pltpu.CompilerParams(
            vmem_limit_bytes=VL * 1024 * 1024),
    )(x.reshape(N, D), *weights)
    return out.reshape(B, T, D)
```

```python
import functools
import math

import jax
import jax.numpy as jnp
from jax import lax
import jax.experimental.pallas as pl
import jax.experimental.pallas.tpu as pltpu

F32 = jnp.float32
BF16 = jnp.bfloat16

TM = 400
T0 = 320
TA = 512
TC = 320
FC = 512
KC = 512
W1A = 1
XF = 0
IW = 3
VL = 127
SG = 1
O_WIN = (0.55, 0.95)
L_WIN = (0.02, 0.5)
FB = (((2, 4, 3, 1, 0, 6, 5), (2, 4, 3, 1, 0, 6, 5)),
      ((1, 3, 6, 2, 4, 0, 5), (2, 4, 3, 1, 0, 6, 5)),
      ((0, 0, 49), (0, 1, 49), (0, 2, 14)) + ((1, 0, 4), (0, 2, 7)) * 5
      + ((1, 0, 3), (0, 3, 7)) * 7 + ((1, 0, 8), (1, 1, 49)))
FA = FB[:2] + (((0, 0, 49), (0, 1, 49), (0, 2, 49), (0, 3, 49), (1, 0, 49),
                (1, 1, 49)),)
P_WIN = (0.55, 0.95)
OQ = (0, 2, 3, 4, 6, 1, 5)
OS0 = (2, 4, 3, 1, 0, 5, 6)
OS = (0, 1, 2, 3, 4, 5, 6)
OP = (0, 1, 2, 3, 4, 5, 6)
OW = (2, 4, 3, 0, 6, 1, 5)
PO = ((0, 2), (0, 4), (1, 2), (0, 3), (0, 0), (0, 6), (0, 1), (0, 5),
      (1, 4), (1, 3), (1, 0), (1, 6), (1, 1), (1, 5))
F_WIN = (0.1, 0.9, 0.55)
A_WIN = (0.02, 0.5)
A_SKIP = ()
FD = (0, 3200, 0, 3200)
B_SLOTS = (1, 53)
Q_SLOTS = (8, 50)
CT = 5
L0 = 1
LP = (0, 100, 3, 1)
S1 = 2
S2 = 1
SD = (0, 140, 120)
LAG = 2
SW = tuple(1 + 1.75 * j for j in range(9))
C_WIN = (0.21, 0.82)
C_SKIP = ()
RC = (8, 100)
EP = (0, 128, 224, 288, 320)
ZR = 32
PR = 112
HALO = 8
EPS = 1e-05


def _ln(x, z=None):
    if z is None:
        m = jnp.mean(x, axis=-1, keepdims=True)
    else:
        t = z
        for c in range(x.shape[-1] // 128):
            t = t + x[:, c * 128:(c + 1) * 128]
        m = jnp.sum(t, axis=-1, keepdims=True) * (1.0 / x.shape[-1])
    xc = x - m
    v = jnp.mean(xc * xc, axis=-1, keepdims=True)
    return xc * lax.rsqrt(v + EPS)


def _silu(a):
    y = 0.5 * a
    return y + y * jnp.tanh(y)


def _dot(a, b):
    return jnp.dot(a, b, preferred_element_type=F32)


def _dot_nt(a, b):
    return lax.dot_general(a, b, (((1,), (1,)), ((), ())),
                           preferred_element_type=F32)


def _pk(v):
    return pltpu.bitcast(v.astype(BF16), jnp.uint32)


def _up(v):
    return pltpu.bitcast(v, BF16)


class _Anchor:
    def __init__(self, t, zero_v):
        self.t, self.zero_v = t, zero_v

    def v(self):
        return pltpu.bitcast(
            pltpu.bitcast(self.t, jnp.uint32) & self.zero_v[0:8, :], F32)


class _Sched:
    def __init__(self, zero_v):
        self.zero_v = zero_v
        self.queue = []
        self.now = 0

    def add(self, items, t0, t1, skip=()):
        assert t0 >= self.now
        ts = [t for t in range(t0, t1)
              if not any(a <= t < b for a, b in skip)]
        self.queue += [(ts[k * len(ts) // len(items)], it)
                       for k, it in enumerate(items)]
        self.queue.sort(key=lambda e: e[0])

    def __call__(self, t, dur=None):
        dur = dur or t.shape[0]
        end = self.now + dur
        while self.queue and self.queue[0][0] < end:
            time, item = self.queue.pop(0)
            r = (time - self.now) * t.shape[0] // dur // 8 * 8
            item(_Anchor(t[r:r + 8, :128], self.zero_v))
        self.now = end


def _rep(z, rows):
    return jnp.concatenate([z] * (rows // 8), axis=0)


def _ffn(h, wa_ref, wb_ref, sched):
    ss = []
    for n in range(wa_ref.shape[1] // 128):
        a = _dot(h, wa_ref[:, n * 128:(n + 1) * 128])
        ss.append(_silu(a))
        sched(a)
    s = jnp.concatenate(ss, axis=1).astype(BF16)
    acc = []
    for n in range(wb_ref.shape[1] // 128):
        acc.append(_dot(s, wb_ref[:, n * 128:(n + 1) * 128]))
        sched(acc[-1])
    return jnp.concatenate(acc, axis=1)


def _sa(a11, a12, a21, a22):
    return [a11 + a22, a21 + a22, a11, a22, a11 + a12, a21 - a11, a12 - a22]


def _sb(b11, b12, b21, b22):
    return [b11 + b22, b11, b12 - b22, b21 - b11, b22, b11 + b12, b21 + b22]


def _sc(m):
    return [m[0] + m[3] - m[4] + m[6], m[4] + m[2], m[3] + m[1],
            m[0] + m[2] - m[1] + m[5]]


def _lhs7(t, u):
    h = t.shape[1] // 2
    return [v.astype(BF16)
            for v in _sa(t[:, :h], t[:, h:], u[:, :h], u[:, h:])]


_SA = ((0, 1, 3), (2, 1, 3), (0, 0, 0), (3, 0, 3), (0, 1, 1), (2, -1, 0),
       (1, -1, 3))
_SB = ((0, 1, 3), (0, 0, 0), (1, -1, 3), (2, -1, 0), (3, 0, 3), (0, 1, 1),
       (2, 1, 3))
_TG = (((0, 1), (3, 1)), ((2, 1), (3, -1)), ((1, 1), (3, 1)), ((0, 1), (2, 1)),
       ((0, -1), (1, 1)), ((3, 1),), ((0, 1),))


def _quads(x, hm):
    h = x.shape[1] // 2
    t = x[:hm]
    if x.shape[0] > 2 * hm:
        t = jnp.concatenate([t, x[2 * hm:]], axis=0)
    return t[:, :h], t[:, h:], x[hm:, :h], x[hm:, h:]


def _sax(a11, a12, a21, a22, hm):
    return [a11[:hm] + a22[:hm], a21 + a22, a11, a22, a11 + a12,
            a21[:hm] - a11[:hm], a12[:hm] - a22[:hm]]


def _acc7(acc, k, m, hm):
    for a, sg in _TG[k]:
        t = m if a in (1, 2) else m[:hm]
        if acc[a] is None:
            acc[a] = t if sg > 0 else -t
        else:
            acc[a] = acc[a] + t if sg > 0 else acc[a] - t


def _join(acc, hm):
    rest = [acc[1][hm:]] if acc[1].shape[0] > hm else []
    return (jnp.concatenate([acc[0], acc[2]], axis=0),
            jnp.concatenate([acc[1][:hm], acc[3]] + rest, axis=0))


def _ffn7(h7, wa, wb, sched, o1, o2, lag, early=()):
    acc = [None] * 7
    hm = h7[0].shape[0]
    u = [[None] * 4 for _ in wa]

    done = set()
    act = [[None] * 4 for _ in wa]
    s7 = [[None] * 7 for _ in wa]

    def run(cks):
        for c, k in cks:
            if (c, k) in done or c >= len(wa):
                continue
            done.add((c, k))
            t = _dot(h7[k], _up(wa[c][k]))
            _acc7(u[c], k, t, hm)
            sched(t)
            for a in range(4):
                if act[c][a] is None and all(
                        (c, n) in done for n in range(7)
                        if a in [e[0] for e in _TG[n]]):
                    act[c][a] = _silu(u[c][a])
            for n, (a, sg, b) in enumerate(_SA):
                if (s7[c][n] is None and act[c][a] is not None
                        and act[c][b] is not None):
                    v = act[c][a]
                    if sg:
                        v = v + act[c][b] if sg > 0 else v - act[c][b]
                    s7[c][n] = v.astype(BF16)

    run(early)
    for c, cb in enumerate(wb):
        run([(c, k) for k in o1] + [(c + 1, k) for k in o1[:lag]])
        for k in o2:
            p = _dot(s7[c][k], _up(cb[k]))
            acc[k] = p if acc[k] is None else acc[k] + p
            sched(p)
    c = _sc(acc)
    return jnp.concatenate(c[:2], axis=1), jnp.concatenate(c[2:], axis=1)


def _q4(x):
    h, w = x.shape[0] // 2, x.shape[1] // 2
    return x[:h, :w], x[:h, w:], x[h:, :w], x[h:, w:]


def _twice(f, x):
    return [v for y in f(*_q4(x)) for v in f(*_q4(y))]


def _pm(a, sg, b):
    return a if not sg else a + b if sg > 0 else a - b


def _ops2(load, put, tab, f, k1, z):
    def quad(a):
        return [load(a // 2 * 2 + j // 2, a % 2 * 2 + j % 2) for j in range(4)]

    a, sg, b = tab[k1]
    y = [_pm(u + _rep(z.v(), 16), sg, v) for u, v in zip(quad(a), quad(b))]
    for k2, v in enumerate(f(*y)):
        put(7 * k1 + k2, v)


def _ffn49(h49, hm, w, nfc, sched, oi, oo, plan, KO=2):
    src = [[n for n in range(7) if a in [e[0] for e in _TG[n]]]
           for a in range(4)]
    val = {}

    def add(key, sg, t):
        if key not in val:
            val[key] = t if sg > 0 else -t
        else:
            val[key] = _pm(val[key], sg, t)

    def collect(done, tag, k1, k2, t):
        done.add((k1, k2))
        for b, sg in _TG[k2]:
            add((tag, 'm', k1, b), sg, t)
            if all((k1, n) in done for n in src[b]):
                for a, sg1 in _TG[k1]:
                    add((tag, 'u', a, b), sg1, val[tag, 'm', k1, b])

    done = [set() for _ in range(nfc + 1)]

    def step_in(c, k1, k2):
        t = _dot(h49(7 * k1 + k2), w(7 * k1 + k2, c, 1))
        collect(done[c], c, k1, k2, t)
        sched(t, hm // 4)
        for a in range(4):
            for b in range(4):
                if (c, 'a', a, b) not in val and all(
                        (m, n) in done[c] for m in src[a] for n in src[b]):
                    val[c, 'a', a, b] = _silu(val[c, 'u', a, b])
        g = c // SG
        cs = range(g * SG, (g + 1) * SG)
        for n, (a, sg, a2) in enumerate(_SA):
            for b in range(4):
                if (g, 'y', n, b) not in val and all(
                        (e, 'a', q, b) in val for e in cs for q in (a, a2)):
                    val[g, 'y', n, b] = jnp.concatenate(
                        [_pm(val[e, 'a', a, b], sg, val[e, 'a', a2, b])
                         for e in cs], axis=1)
            for m, (b, sg, b2) in enumerate(_SA):
                if ((g, 's', n, m) not in val and (g, 'y', n, b) in val
                        and (g, 'y', n, b2) in val):
                    val[g, 's', n, m] = _pm(val[g, 'y', n, b], sg,
                                            val[g, 'y', n, b2]).astype(BF16)

    def step_out(g, k1, k2):
        t = _dot(jnp.concatenate(
            [val[e, 's', k1, k2]
             for e in range(g * KO // SG, (g + 1) * KO // SG)], axis=1),
            w(7 * k1 + k2, nfc + g * KO, KO))
        sched(t, hm * KO // 4)
        add(('p', k1, k2), 1, t)
        if (g + 1) * KO == nfc:
            collect(done[-1], 'o', k1, k2, val['p', k1, k2])

    todo = {(d, c): [(k1, k2) for k1 in o[0] for k2 in o[1]]
            for d, o in enumerate((oi, oo)) for c in range(nfc)}
    for d, c, n in plan:
        for k1, k2 in todo[d, c][:n]:
            (step_out if d else step_in)(c, k1, k2)
        del todo[d, c][:n]
    return jnp.concatenate(
        [jnp.concatenate([val['o', 'u', a // 2 * 2 + b // 2, a % 2 * 2 + b % 2]
                          for b in range(4)], axis=1) for a in range(4)],
        axis=0)


def _kernel(x_hbm, w1a_hbm, w1b_hbm, wq_hbm, wk_hbm, wv_hbm, wo_hbm,
            wp1_hbm, dw_hbm, wp2_hbm, w2a_hbm, w2b_hbm,
            out_hbm,
            xin, wblk, wq, wk, wv, wo, dw,
            mq, wvo, xs, hs, ks, gs, dcs, st_mean, st_m2, bn,
            lhs49, w7, w49, lhs_b, dwb, zero, zero_s,
            al_buf0, al_buf1, al_buf2,
            p_buf0, p_buf1, p_buf2, s_buf0, s_buf1, hq7,
            xsem, w1sem, w2sem, wsem, osem,
            *, B, T, D, K):
    N = B * T
    obuf = xin
    KP = KC // 2
    nkc = -(-T // KC)
    TP = nkc * KP
    NCB = D // 128
    nt = N // TM
    tpb = T // TM

    def rows(i, r0=0, n=TM):
        return pl.ds(pl.multiple_of(i * TM, 16) + r0, n)

    def col(c):
        if isinstance(c, int):
            return slice(c * 128, (c + 1) * 128)
        return pl.ds(pl.multiple_of(c * 128, 128), 128)

    na = (N - T0) // TA
    H = D // 2
    QA = TA // 4
    s_buf = (s_buf0, s_buf1)

    def arows(i, r0=0, n=TA):
        return pl.ds(pl.multiple_of(T0 + (i - 1) * TA, 16) + r0, n)

    def x_copy(i):
        rs = pl.ds(0, T0) if isinstance(i, int) and i == 0 else arows(i)
        return pltpu.make_async_copy(x_hbm.at[rs, :], xin.at[rs, :],
                                     xsem.at[i])

    nc = N // TC

    def crows(i, r0=0, n=TC):
        return pl.ds(pl.multiple_of(i * TC, 16) + r0, n)

    def o_copy(i):
        return pltpu.make_async_copy(obuf.at[crows(i), :],
                                     out_hbm.at[crows(i), :], osem.at[i])

    nfc = w49.shape[1] // (D // 4)
    P1, P2 = 4 * nfc, 4 * nfc + 2

    def w1_copies(c):
        fs = pl.ds(pl.multiple_of(c * FC, FC), FC)
        return [pltpu.make_async_copy(w1a_hbm.at[:, fs], wblk.at[c],
                                      w1sem.at[0, c]),
                pltpu.make_async_copy(w1b_hbm.at[fs, :], wblk.at[nfc + c],
                                      w1sem.at[1, c])]

    def w2_copies(c):
        fs = pl.ds(pl.multiple_of(c * FC, FC), FC)
        hs_ = pl.ds(pl.multiple_of(c // 2 * H, H), H)
        return [pltpu.make_async_copy(s, d, w2sem.at[j, c])
                for j, (s, d) in enumerate([
                    (w2a_hbm.at[:, fs], wblk.at[2 * nfc + c]),
                    (w2b_hbm.at[fs, :], wblk.at[3 * nfc + c]),
                    (wp1_hbm.at[:, pl.ds(pl.multiple_of(c * H, H), H)],
                     wblk.at[P1 + c % 2, :, hs_])])]

    assert nfc == 4
    w_pairs = [(wp2_hbm, wblk.at[P2]), (wq_hbm, wq), (wk_hbm, wk),
               (wv_hbm, wv), (wo_hbm, wo), (dw_hbm, dw)]
    w_copies = [pltpu.make_async_copy(s, d, wsem.at[j])
                for j, (s, d) in enumerate(w_pairs)]

    x_copy(0).start()
    for cp in w1_copies(0):
        cp.start()

    zero[...] = jnp.zeros(zero.shape, jnp.uint32)
    zero_s[0] = 0
    for c in range(NCB):
        gs[1, c, 0:HALO, :] = jnp.zeros((HALO, 128), F32)
        gs[nt, c, HALO + TM:, :] = jnp.zeros((HALO, 128), F32)
    for b in range(B):
        ks[:, (b * TP + T // 2) // 2:(b + 1) * TP // 2, :] = jnp.zeros(
            (7, (TP - T // 2) // 2, H), jnp.uint32)

    def zrep(z, n):
        return None if z is None else _rep(z.v(), n)

    def pair_items(first, second, rows0):
        items = []
        for r0 in rows0:
            t = []
            items += [functools.partial(first, t, r0),
                      functools.partial(second, t, r0)]
        return items

    def ln_in(base, quarter, rows0):
        zs = zero_s[0]

        def ln(r0, j, z):
            s_buf[j // 2][pl.ds(j % 2 * QA + r0, 16), :] = _ln(
                xin[pl.ds(pl.multiple_of(base + j * quarter, 16) + r0, 16), :]
                .astype(F32), zrep(z, 16))

        def ops(r0, k1):
            def load(j, c):
                return s_buf[j // 2][pl.ds(
                    pl.multiple_of(zs + r0, 16) + j % 2 * QA, 16), col(c)]

            def put(k, v):
                lhs49.at[k // 2][pl.ds(pl.multiple_of(r0 // 2, 8), 8),
                                 col(k % 2)] = _pk(v)

            return functools.partial(_ops2, load, put, _SA, _sa, k1)

        return ([functools.partial(ln, r0, j)
                 for r0 in rows0 for j in range(4)],
                [ops(r0, k1) for r0 in rows0 for k1 in range(7)])

    def ln_out(base, rows0):
        def first(t, r0, z, off=0):
            rs = pl.ds(pl.multiple_of(base, 32) + 2 * r0 + off, 16)
            t.append(_ln(xs[rs, :], zrep(z, 16)))
            hs[rs, :] = t[-1].astype(BF16)

        def second(t, r0, z):
            first(t, r0, z, 16)
            g = base // 32 + r0 // 16
            g += g // (T // 32) * ((TP - T // 2) // 16)
            for k, v in enumerate(_lhs7(*t)):
                ks.at[k][pl.ds(pl.multiple_of(g * 8, 8), 8), :] = _pk(v)

        return pair_items(first, second, rows0)

    def prep(src, dst, r0, z=None):
        q = [src[pl.ds(r + r0, 16), c:c + H].astype(F32)
             for r in (0, H) for c in (0, H)]
        if z is not None:
            zz = jnp.concatenate([_rep(z.v(), 16)] * (H // 128), axis=1)
            q[0], q[3] = q[0] + zz, q[3] + zz
        r1 = r0 // 2 if isinstance(r0, int) else pl.multiple_of(r0 // 2, 8)
        for k, v in enumerate(_sb(*q)):
            dst.at[k][pl.ds(r1, 8), :] = _pk(v)

    Q = D // 4

    def prep2(ff, blk, n, k1):
        rpb = Q // 16

        def load(r, c):
            return wblk[blk + n // rpb, pl.ds(pl.multiple_of(
                n % rpb * 16, 16) + r * Q, 16), col(c)].astype(F32)

        def put(k, v):
            rs = pl.multiple_of(n * 8, 8)
            if ff:
                w49.at[k // 2][pl.ds(rs, 8), col(k % 2)] = _pk(v)
            else:
                dcs[pl.ds(rs + k // NCB * D, 8), col(k % NCB)] = (
                    pltpu.bitcast(v.astype(BF16), F32))

        return functools.partial(_ops2, load, put, _SB, _sb, k1)

    x_copy(0).wait()
    if W1A == 2:
        for cp in w1_copies(1):
            cp.start()
    lhs_b[...] = _ln(xin[0:T0, :].astype(F32)).astype(BF16)
    xs[0:T0, :] = xin[0:T0, :].astype(F32)

    def first_tile(c, carry):
        for cp in w1_copies(c):
            cp.wait()

        @pl.when(c == 1)
        def _():
            x_copy(1).wait()

        if XF:
            @pl.when(c % 2 == 0)
            def _():
                x_copy(1 + c // 2).start()

        @pl.when(c + W1A < nfc)
        def _():
            for cp in w1_copies(c + W1A):
                cp.start()

        if not XF:
            @pl.when(c % 2 == 0)
            def _():
                x_copy(1 + c // 2).start()

        n = -(-QA // (nfc - 1) // 16) * 16
        r0 = pl.multiple_of(jnp.clip((c - 1) * n, 0, QA - n), 16)
        assert n <= T0 // 4
        sched = _Sched(zero)
        dur = 2 * NCB * T0
        items = ln_in(jnp.where(c > 0, T0, 0), jnp.where(c > 0, QA, T0 // 4),
                      [r0 + r for r in range(0, n, 16)])
        sched.add(items[0], int(F_WIN[0] * dur), int(F_WIN[2] * dur))
        sched.add(items[1], int(F_WIN[2] * dur), int(F_WIN[1] * dur))
        sched.add([prep2(0, 0, (j * nfc + c) * (Q // 16) + r, k1)
                   for j in range(2) for r in range(Q // 16)
                   for k1 in range(7)],
                  int(F_WIN[0] * dur), int(F_WIN[1] * dur))
        f = _ffn(lhs_b[...], wblk.at[c], wblk.at[nfc + c], sched)
        assert not sched.queue
        xs[0:T0, :] += 0.5 * f
        return carry

    lax.fori_loop(0, nfc, first_tile, 0)
    for j in range(3, na + 1):
        x_copy(j).start()
    for c in range(nfc):
        for cp in w2_copies(c):
            cp.start()
    for cp in w_copies:
        cp.start()

    def phase_a(i, carry):
        @pl.when(i < na)
        def _():
            x_copy(i + 1).wait()

        @pl.when((i >= IW) & (i < IW + nfc))
        def _():
            for cp in w2_copies(i - IW):
                cp.wait()

        @pl.when(i == IW)
        def _():
            w_copies[0].wait()

        sched = _Sched(zero)
        dur = 49 * 2 * nfc * TA // 16
        win = (int(A_WIN[0] * dur), int(A_WIN[1] * dur), A_SKIP)
        base = jnp.maximum(T0 + (i - 2) * TA, 0)
        sched.add(ln_out(base, range(0, TA // 2, 16)),
                  int(L_WIN[0] * dur), int(L_WIN[1] * dur), A_SKIP)
        base = T0 + jnp.minimum(i, na - 1) * TA
        items = ln_in(base, QA, range(0, QA, 16))
        sched.add(items[0], *win)
        sched.add(items[1], int(O_WIN[0] * dur), int(O_WIN[1] * dur))
        rpb = H // 16
        total = w7.shape[0] * rpb
        ipi = -(-total // (na - IW + 1))
        items = []
        for k in range(ipi):
            n = jnp.minimum(jnp.maximum(i - IW, 0) * ipi + k, total - 1)
            blk = (n // rpb + 2) % 3
            items.append(functools.partial(
                prep, wblk.at[blk + jnp.where(i >= IW, P1, 0)], w7.at[blk],
                pl.multiple_of(n % rpb * 16, 16)))
        assert ipi * (nfc - 1) <= rpb
        sched.add(items, int(P_WIN[0] * dur), int(P_WIN[1] * dur))
        total = w49.shape[1] // 8
        ipi = -(-total // (na - IW + 1))
        assert ipi <= Q // 16
        sched.add([prep2(
            1, jnp.where(i >= IW, 2 * nfc, 0),
            jnp.minimum(jnp.maximum(i - IW, 0) * ipi + k, total - 1), k1)
            for k in range(ipi) for k1 in range(7)],
            int(P_WIN[0] * dur), int(P_WIN[1] * dur), win[2])

        def h49(k):
            assert sched.now <= int(O_WIN[0] * dur) and A_WIN[1] <= O_WIN[0]
            return _up(lhs49[k // 2, :, col(k % 2)])

        f = _ffn49(
            h49, QA,
            lambda k, b, n: pltpu.bitcast(
                dcs[pl.ds(k // NCB * D + b * 64, n * 64), col(k % NCB)], BF16),
            nfc, sched, *FA)
        assert not sched.queue
        xs[arows(i), :] = xin[arows(i), :].astype(F32) + 0.5 * f
        return carry

    with jax.named_scope("phase_a"):
        lax.fori_loop(1, na + 1, phase_a, 0)

    for cp in w_copies[1:]:
        cp.wait()

    qk_scale = (D ** -0.5) * math.log2(math.e)

    HM = TM // 32 * 16

    def put7(dst, r0, cs, *p):
        if len(p) == 4:
            ops = enumerate(_sa(*p))
        else:
            ops = zip((1, 2, 3, 4), (p[0] + p[1], *p, p[0] + p[1]))
        for k, t in ops:
            dst[pl.ds(k * PR + r0 // 2, 8), cs] = pltpu.bitcast(
                t.astype(BF16), jnp.uint32)

    def get7(src, k, ds=pl.ds, nr=None):
        nr = nr or (TM - HM if 1 <= k <= 4 else HM)
        return pltpu.bitcast(src[ds(k * PR, nr // 2), :], BF16)

    def groups(r0):
        return (r0, HM + r0) if r0 < HM else (HM + r0,)

    def q_ops(i, r0, c, z):
        p = [hs[rows(i, r, 16), col(2 * h + c)].astype(F32)
             for r in groups(r0) for h in range(2)]
        p[0] = p[0] + _rep(z.v(), 16)
        p[-1] = p[-1] + _rep(z.v(), 16)
        put7(hq7, r0, col(c), *p)

    def q_items(i):
        return [functools.partial(q_ops, i, r0, c)
                for r0 in range(0, TM - HM, 16) for c in range(2)]

    sched = _Sched(zero)
    sched.add(ln_out(N - TA, range(0, TA // 2, 16)), *FD[:2])
    sched.add(q_items(0), *FD[2:])
    for dst in (mq, wvo):
        for u in range(2):
            t = []
            for cs in (col(u), col(u + 2)):
                t.append(_dot_nt(wq[...], wk[cs, :]) if dst is mq
                         else _dot(wv[...], wo[:, cs]))
                sched(t[-1])
            if dst is mq:
                t = [v * qk_scale for v in t]
            for k, v in enumerate(
                    _sb(t[0][:H], t[1][:H], t[0][H:], t[1][H:])):
                dst[k, :, col(u)] = _pk(v)
    assert not sched.queue
    dwf = dw[...].astype(F32)
    for k in range(K):
        dwb[k] = jnp.broadcast_to(dwf[k:k + 1, :], (8, D))

    def conv_block(p, r0, c, done, CT=CT, AT=K):
        cs = col(c)
        acc = [None]

        def item(k0, z=None):
            for k in range(k0, min(k0 + CT, K)):
                off = HALO - K // 2 + k + r0
                w = dwb[k, :, cs]
                if z is not None and k - k0 < AT:
                    w = w + z.v()
                t = gs[p + 1, c, off:off + 8, :] * w
                acc[0] = t if acc[0] is None else acc[0] + t
            if k0 + CT >= K:
                dcs[rows(p, r0, 8), cs] = acc[0]
                done(acc[0])

        return [functools.partial(item, k0) for k0 in range(0, K, CT)]

    def conv_main(p, cols=range(NCB), **kw):
        st = []

        def stats(r0, c, acc):
            if r0 == 0:
                st[:] = [acc, None, None]
                return
            shift, s1, s2 = st
            d = acc - shift
            s1 = d if s1 is None else s1 + d
            s2 = d * d if s2 is None else s2 + d * d
            st[:] = [shift, s1, s2]
            if r0 + 16 == TM:
                dm = s1 * (1.0 / (TM // 8 - 1))
                st_mean[p, :, col(c)] = shift + dm
                st_m2[p, :, col(c)] = s2 - s1 * dm

        return [it for c in cols for r0 in range(0, TM - 8, 8)
                for it in conv_block(p, r0, c,
                                     functools.partial(stats, r0, c), **kw)]

    def conv_edge(p, cols=range(NCB)):
        return [it for c in cols
                for it in conv_block(p, TM - 8, c, lambda acc: None)]


    def phase_b(i, carry):
        b = i // tpb

        sched = _Sched(zero)
        sched.add(conv_edge(jnp.maximum(i - 2, 0))
                  + conv_main(jnp.maximum(i - 1, 0), range(L0, NCB)),
                  int(B_SLOTS[0] * TM), int(B_SLOTS[1] * TM))
        sched.add(q_items(jnp.minimum(i + 1, nt - 1)),
                  int(Q_SLOTS[0] * TM), int(Q_SLOTS[1] * TM))
        acc = [None] * 4
        for k in OQ:
            t = _dot(get7(hq7, k), _up(mq[k]))
            _acc7(acc, k, t, HM)
            sched(t)
        q11, q12, q21, q22 = _quads(
            jnp.concatenate(_join(acc, HM), axis=1), HM)
        q7 = [q11[:HM] - q22[:HM], q21 - q22, q11, q22, q12 - q11,
              q21[:HM] - q11[:HM], q12[:HM] - q22[:HM]]
        q7 = [t.astype(BF16) for t in q7]

        dz = zero_s[0]
        p_buf, al_buf = (p_buf0, p_buf1, p_buf2), (al_buf0, al_buf1, al_buf2)
        s_buf = (s_buf0, s_buf1)

        def dyn(r0, n):
            return pl.ds(pl.multiple_of(dz + r0, 8), n)

        nb = KP // 128

        def chunk(j):
            return pl.ds(pl.multiple_of(b * (TP // 2), KP // 2)
                         + j * KP // 2, KP // 2)

        def combine(m, j, c):
            if len(m) == 7:
                s = [m[0] + m[3] + m[4] + m[6], m[2] + m[4],
                     m[1] + m[3], m[1] - m[0] + m[2] + m[5]]
            else:
                s = [m[0] + m[2], m[1] + m[3]]
            nv = T // 2 - j * KP - c * 128
            if nv < 128:
                lane = lax.broadcasted_iota(jnp.int32, s[0].shape, 1)
                s = [jnp.where(lane < nv, t, -jnp.inf) for t in s]
            return s

        stat = {}

        def put(w, j, r, v):
            for r0 in range(0, v.shape[0], 16):
                stat[w, j, r + r0] = v[r0:r0 + 16]

        def get(w, j, r, n=16):
            return jnp.concatenate(
                [stat[w, j, r0] for r0 in range(r, r + n, 16)], axis=0)

        def scores(j):
            m = [None] * 7
            for k in OS if j else OS0:
                m[k] = _dot_nt(
                    q7[k], _up(ks[(0, 2, 1, 4, 3, 5, 6)[k], chunk(j), :]))
                sched(m[k])
            mx = None
            for c in range(nb):
                s = combine([t[:HM, col(c)] for t in m], j, c)
                e = combine([t[HM:, col(c)] for t in m[1:5]], j, c)
                for h in range(2):
                    t = jnp.concatenate([s[h], s[2 + h], e[h]], axis=0)
                    s_buf[j % 2][:, col(h * nb + c)] = t
                    mx = t if mx is None else jnp.maximum(mx, t)
            mx = jnp.broadcast_to(jnp.max(mx, axis=-1, keepdims=True),
                                  mx.shape)
            if j:
                mx = jnp.maximum(mx, get(0, j - 1, 0, TM))
            put(0, j, 0, mx)

        part = {}

        def soft1(j, r, c0, z):
            rs = slice(r, r + 16)
            m = get(0, j, r) + _rep(z.v(), 16)
            l = functools.reduce(jnp.add, part.pop((j, r), []) + [
                jnp.exp2(s_buf[j % 2][dyn(r, 16), col(c)] - m)
                for c in range(c0, c0 + S1)])
            if c0 + S1 < 2 * nb:
                part[j, r] = [l]
                return
            l = jnp.broadcast_to(jnp.sum(l, axis=-1, keepdims=True),
                                 (16, 128))
            if j:
                l += get(1, j - 1, r) * jnp.exp2(get(0, j - 1, r) - m)
            put(1, j, r, l)
            e = (pltpu.bitcast(l, jnp.int32) >> 23) - 127
            ref = m + e.astype(F32)
            put(2, j, r, ref)
            if j:
                al_buf[j % 3][rs, :] = jnp.exp2(get(2, j - 1, r) - ref)

        def soft2(j, r0, c0, z):
            ref = [get(2, j, r) + _rep(z.v(), 16) for r in groups(r0)]
            p = [jnp.concatenate(
                [jnp.exp2(s_buf[j % 2][dyn(r, 16), col(h * nb + c)] - m)
                 for c in range(c0, c0 + S2)], axis=1)
                 for r, m in zip(groups(r0), ref) for h in range(2)]
            put7(p_buf[j % 3], r0, slice(c0 * 128, (c0 + S2) * 128), *p)

        scd = 7 * HM + 4 * (TM - 2 * HM)
        start = sched.now

        def add_soft(j):
            rbs = range(0, TM - HM, 16)
            t0, t1 = (start + int(t * scd) for t in SW[j:j + 2])
            assert t1 <= start + min(2 * j + LAG + 1, nkc + j) * scd
            assert j < 3 or t0 >= start + min(2 * j + LAG - 4,
                                              nkc + j - 2) * scd
            assert (j + 2 >= nkc
                    or t1 <= start + max(2 * j + 5 - LAG, j + 3) * scd)
            u = (t1 - t0 - sum(SD)) // (len(rbs) + 1)
            for n, r0 in enumerate(rbs):
                its = [[functools.partial(soft1, j, r, c)
                        for r in groups(r0) for c in range(0, 2 * nb, S1)],
                       [functools.partial(soft2, j, r0, c)
                        for c in range(0, nb, S2)]]
                for k, it in enumerate(its):
                    t = t0 + SD[0] + n * u + k * (u + SD[1])
                    sched.add(it, t, t + u)

        for j in range(LAG):
            scores(j)
            add_soft(j)
        acc = [None] * 4
        for j in range(nkc):
            if j + LAG < nkc:
                scores(j + LAG)
                add_soft(j + LAG)
            fresh = [j > 0] * 4
            for k in OP if j + 1 < nkc else OQ:
                w = _up(ks[(0, 2, 6, 5, 3, 4, 1)[k], chunk(j), :])
                m = _dot(get7(p_buf[j % 3], k, dyn), w)
                sched(m)
                for a, _ in _TG[k]:
                    if fresh[a]:
                        al = al_buf[j % 3][dyn(0, TM), :]
                        al = _quads(jnp.concatenate([al] * NCB, axis=1), HM)[a]
                        acc[a] = acc[a] * al[:acc[a].shape[0]]
                        fresh[a] = False
                _acc7(acc, k, m, HM)
        assert not sched.queue
        t = jnp.exp2(get(2, nkc - 1, 0, TM) - get(0, nkc - 1, 0, TM))
        t = t / get(1, nkc - 1, 0, TM)
        o = (jnp.concatenate(_join(acc, HM), axis=1)
             * jnp.concatenate([t] * NCB, axis=1))
        o7 = [t.astype(BF16) for t in _sax(*_quads(o, HM), HM)]
        acc = list(_quads(xs[rows(i), :], HM))
        acc = [acc[0][:HM], acc[1], acc[2], acc[3][:HM]]
        for k in OW:
            _acc7(acc, k, _dot(o7[k], _up(wvo[k])), HM)
        x2 = jnp.concatenate(_join(acc, HM), axis=1)
        xs[rows(i), :] = x2
        h7 = [t.astype(BF16) for t in _sax(*_quads(_ln(x2), HM), HM)]
        sched = _Sched(zero)
        acc = [[None] * 4 for _ in range(2)]
        for n, (h, k) in enumerate(PO):
            t = _dot(h7[k], _up(w7[h, k]))
            _acc7(acc[h], k, t, HM)
            sched(t)
            if any(e[0] == h for e in PO[n + 1:]):
                continue
            val, gate = _join(acc[h], HM)
            g2 = val * (0.5 + 0.5 * jnp.tanh(0.5 * gate))
            for c in (2 * h, 2 * h + 1):
                g = g2[:, col(c % 2)]
                gs[i + 1, c, HALO:HALO + TM, :] = g
                gs[i, c, HALO + TM:, :] = jnp.where(
                    i % tpb == 0, 0.0, g[:HALO])
                gs[i + 2, c, :HALO, :] = jnp.where(
                    i % tpb == tpb - 1, 0.0, g[TM - HALO:])
            if h == 0 and L0:
                rest = sum(h7[e[1]].shape[0] for e in PO[n + 1:])
                sched.add(conv_main(i, range(L0), CT=LP[2], AT=LP[3]),
                          sched.now + LP[0], sched.now + rest - LP[1])
        assert not sched.queue
        return carry

    with jax.named_scope("phase_b"):
        lax.fori_loop(0, nt, phase_b, 0)
    for item in (conv_main(nt - 1, range(L0, NCB)) + conv_edge(nt - 2)
                 + conv_edge(nt - 1)):
        item()

    ng = TM // 8 - 1
    means = st_mean[...].reshape(nt * 8, D)
    edges = jnp.concatenate([dcs[(p + 1) * TM - 8:(p + 1) * TM, :]
                             for p in range(nt)], axis=0)
    mu = jnp.sum(ng * means + edges, axis=0, keepdims=True) * (1.0 / N)
    dm = means - mu
    de = edges - mu
    var = jnp.sum(st_m2[...].reshape(nt * 8, D) + ng * (dm * dm) + de * de,
                  axis=0, keepdims=True) * (1.0 / N)
    rstd = lax.rsqrt(var + EPS)
    bn[0] = jnp.broadcast_to(mu, (8, D))
    bn[1] = jnp.broadcast_to(rstd, (8, D))

    def bn_silu(i, r0, c, z=None):
        p = []
        for r in (r0, TC // 2 + r0):
            for h in range(2):
                cs = col(2 * h + c)
                mu = bn[0, :, cs] if z is None else bn[0, :, cs] + z.v()
                y = dcs[crows(i, r, 16), cs] - _rep(mu, 16)
                p.append(_silu(y * _rep(bn[1, :, cs], 16)))
        put7(hq7, r0, col(c), *p)

    def bn_items(i):
        return [functools.partial(bn_silu, i, r0, c)
                for r0 in range(0, TC // 2, 16) for c in range(2)]

    def ln_final(i, r0=0, n=TC, z=None):
        obuf[crows(i, r0, n), :] = _ln(xs[crows(i, r0, n), :],
                                       zrep(z, n)).astype(BF16)

    for item in bn_items(0):
        item()

    def phase_c(i, carry):
        @pl.when(i >= 2)
        def _():
            o_copy(i - 2).start()

        sched = _Sched(zero)
        dur = (7 * 8 + 49 * 2 * nfc) * TC // 16
        t0, t1 = int(C_WIN[0] * dur), int(C_WIN[1] * dur)
        sched.add([functools.partial(ln_final, jnp.maximum(i - 1, 0), r, RC[0])
                   for r in range(0, TC, RC[0])], t0, t1, C_SKIP)
        sched.add(bn_items(jnp.minimum(i + 1, nc - 1)),
                  t0 + RC[1], t1 + RC[1], C_SKIP)
        acc = list(_quads(xs[crows(i), :], TC // 2))
        for k in OQ:
            t = _dot(get7(hq7, k, nr=TC // 2), _up(w7[2, k]))
            _acc7(acc, k, t, TC // 2)
            sched(t)
        x3 = jnp.concatenate(_join(acc, TC // 2), axis=1)
        xs[crows(i), :] = x3
        h = _ln(x3)
        h49 = [v.astype(BF16) for v in _twice(_sa, h)]
        f = _ffn49(h49.__getitem__, TC // 4,
                   lambda k, b, n: _up(
                       w49[k // 2, b * 64:(b + n) * 64, col(k % 2)]),
                   nfc, sched, *FB)
        assert not sched.queue
        xs[crows(i), :] += 0.5 * f
        return carry

    with jax.named_scope("phase_c"):
        lax.fori_loop(0, nc, phase_c, 0)
    o_copy(nc - 2).start()
    last = []
    for k, (r0, r1) in enumerate(zip(EP[:-1], EP[1:])):
        ln_final(nc - 1, r0, r1 - r0)
        rs = crows(nc - 1, r0, r1 - r0)
        last.append(pltpu.make_async_copy(obuf.at[rs, :], out_hbm.at[rs, :],
                                          osem.at[nc - 1 + k]))
        last[-1].start()
    for i in range(nc - 1):
        o_copy(i).wait()
    for cp in last:
        cp.wait()


@jax.jit
def pallas_standalone__conformer_family_conformer__speech_kernel(
    x: jax.Array,
    w_ff1_a: jax.Array,
    w_ff1_b: jax.Array,
    w_q: jax.Array,
    w_k: jax.Array,
    w_v: jax.Array,
    w_o: jax.Array,
    w_pw1: jax.Array,
    dw: jax.Array,
    w_pw2: jax.Array,
    w_ff2_a: jax.Array,
    w_ff2_b: jax.Array,
):
    B, T, D = x.shape
    K = dw.shape[0]
    N = B * T
    weights = (w_ff1_a, w_ff1_b, w_q, w_k, w_v, w_o, w_pw1, dw, w_pw2,
               w_ff2_a, w_ff2_b)
    scratch = [pltpu.VMEM((N, D), BF16)]
    nfc = w_ff1_a.shape[1] // FC
    scratch += [pltpu.VMEM((4 * nfc + 3, D, D), BF16)]
    scratch += [pltpu.VMEM(w.shape, w.dtype)
                for w in (w_q, w_k, w_v, w_o, dw)]
    scratch += [
        pltpu.VMEM((7, D // 4, D // 2), jnp.uint32),
        pltpu.VMEM((7, D // 4, D // 2), jnp.uint32),
        pltpu.VMEM((N, D), F32),
        pltpu.VMEM((N, D), BF16),
        pltpu.VMEM((7, B * -(-T // KC) * KC // 4, D // 2), jnp.uint32),
        pltpu.VMEM((N // TM + 2, D // 128, TM + 2 * HALO, 128), F32),
        pltpu.VMEM((N, D), F32),
        pltpu.VMEM((N // TM, 8, D), F32),
        pltpu.VMEM((N // TM, 8, D), F32),
        pltpu.VMEM((2, 8, D), F32),
        pltpu.VMEM((25, TA // 8, D // 2), jnp.uint32),
        pltpu.VMEM((3, 7, D // 4, D // 2), jnp.uint32),
        pltpu.VMEM((25, nfc * D // 4, D // 2), jnp.uint32),
        pltpu.VMEM((T0, D), BF16),
        pltpu.VMEM((K, 8, D), F32),
        pltpu.VMEM((ZR, 128), jnp.uint32),
        pltpu.SMEM((1,), jnp.int32),
        pltpu.VMEM((TM + 16, 128), F32),
        pltpu.VMEM((TM + 16, 128), F32),
        pltpu.VMEM((TM + 16, 128), F32),
        pltpu.VMEM((7 * PR, KC // 2), jnp.uint32),
        pltpu.VMEM((7 * PR, KC // 2), jnp.uint32),
        pltpu.VMEM((7 * PR, KC // 2), jnp.uint32),
        pltpu.VMEM((TM, KC), F32),
        pltpu.VMEM((TM, KC), F32),
        pltpu.VMEM((7 * PR, D // 2), jnp.uint32),
        pltpu.SemaphoreType.DMA(((N - T0) // TA + 1,)),
        pltpu.SemaphoreType.DMA((2, nfc)),
        pltpu.SemaphoreType.DMA((3, nfc)),
        pltpu.SemaphoreType.DMA((6,)),
        pltpu.SemaphoreType.DMA((N // TC + len(EP),)),
    ]
    out = pl.pallas_call(
        functools.partial(_kernel, B=B, T=T, D=D, K=K),
        out_shape=jax.ShapeDtypeStruct((N, D), x.dtype),
        in_specs=[pl.BlockSpec(memory_space=pl.ANY)] * 12,
        out_specs=pl.BlockSpec(memory_space=pl.ANY),
        scratch_shapes=scratch,
        compiler_params=pltpu.CompilerParams(
            vmem_limit_bytes=VL * 1024 * 1024),
    )(x.reshape(N, D), *weights)
    return out.reshape(B, T, D)
```

```python
import functools
import math

import jax
import jax.numpy as jnp
from jax import lax
import jax.experimental.pallas as pl
import jax.experimental.pallas.tpu as pltpu

F32 = jnp.float32
BF16 = jnp.bfloat16

TM = 400
T0 = 320
TA = 512
TC = 320
FC = 512
KC = 512
W1A = 1
XF = 0
IW = 3
VL = 128
GC = (42, 60, 16)
KO = 2
O_WIN = (0.51, 0.85)
L_WIN = (0.02, 0.5)
PL = ((0, 0, 49), (0, 1, 49), (0, 2, 49), (0, 3, 49), (1, 0, 49), (1, 1, 49))
FA = (((2, 4, 3, 1, 0, 6, 5), (2, 4, 3, 1, 0, 6, 5)),
      ((1, 3, 6, 2, 4, 0, 5), (2, 4, 3, 1, 0, 6, 5)), PL)
FB = (((2, 4, 3, 1, 0, 6, 5), (2, 4, 3, 1, 0, 6, 5)),
      ((2, 4, 5, 3, 1, 6, 0), (2, 4, 3, 1, 0, 6, 5)),
      PL[:4] + ((1, 0, 35), (2, 0, 0), (1, 0, 14), (1, 1, 49)))
P_WIN = (0.52, 0.92)
OQ = (0, 2, 3, 4, 6, 1, 5)
OS0 = (2, 4, 3, 1, 0, 5, 6)
OS = (0, 1, 2, 3, 4, 5, 6)
OP = (0, 1, 2, 3, 4, 5, 6)
OW = (2, 4, 3, 0, 6, 1, 5)
PO = ((0, 2), (0, 4), (1, 2), (0, 3), (0, 0), (0, 6), (0, 1), (0, 5),
      (1, 4), (1, 3), (1, 0), (1, 6), (1, 1), (1, 5))
F_WIN = (0.02, 0.95, 0.5)
A_WIN = (0.02, 0.5)
A_SKIP = ()
FD = (0, 3200, 0, 3200)
B_SLOTS = (1, 53)
Q_SLOTS = (8, 50)
CT = 5
L0 = 1
LP = (0, 100, 3, 1)
S1 = 2
S2 = 1
SD = (0, 140, 120)
LAG = 2
SW = tuple(1 + 1.75 * j for j in range(9))
C_WIN = (0.02, 0.5, 0.3, 0.58)
M_WIN = (100, 1300, 2350)
RC = 8
EP = (0, 128, 224, 288, 320)
ZR = 32
PR = 112
HALO = 8
EPS = 1e-05


def _ln(x, z=None):
    if z is None:
        m = jnp.mean(x, axis=-1, keepdims=True)
    else:
        t = z
        for c in range(x.shape[-1] // 128):
            t = t + x[:, c * 128:(c + 1) * 128]
        m = jnp.sum(t, axis=-1, keepdims=True) * (1.0 / x.shape[-1])
    xc = x - m
    v = jnp.mean(xc * xc, axis=-1, keepdims=True)
    return xc * lax.rsqrt(v + EPS)


def _silu(a):
    y = 0.5 * a
    return y + y * jnp.tanh(y)


def _dot(a, b):
    return jnp.dot(a, b, preferred_element_type=F32)


def _dot_nt(a, b):
    return lax.dot_general(a, b, (((1,), (1,)), ((), ())),
                           preferred_element_type=F32)


def _pk(v):
    return pltpu.bitcast(v.astype(BF16), jnp.uint32)


def _up(v):
    return pltpu.bitcast(v, BF16)


class _Anchor:
    def __init__(self, t, zero_v):
        self.t, self.zero_v = t, zero_v

    def v(self):
        return pltpu.bitcast(
            pltpu.bitcast(self.t, jnp.uint32) & self.zero_v[0:8, :], F32)


class _Sched:
    def __init__(self, zero_v):
        self.zero_v = zero_v
        self.queue = []
        self.now = 0

    def add(self, items, t0, t1, skip=()):
        assert t0 >= self.now
        ts = [t for t in range(t0, t1)
              if not any(a <= t < b for a, b in skip)]
        self.queue += [(ts[k * len(ts) // len(items)], it)
                       for k, it in enumerate(items)]
        self.queue.sort(key=lambda e: e[0])

    def __call__(self, t, dur=None):
        dur = dur or t.shape[0]
        end = self.now + dur
        while self.queue and self.queue[0][0] < end:
            time, item = self.queue.pop(0)
            r = (time - self.now) * t.shape[0] // dur // 8 * 8
            item(_Anchor(t[r:r + 8, :128], self.zero_v))
        self.now = end
        self.last = t

    def force(self, items):
        for e in [e for e in self.queue if e[1] in items]:
            self.queue.remove(e)
            e[1](_Anchor(self.last[-8:, :128], self.zero_v))


def _rep(z, rows):
    return jnp.concatenate([z] * (rows // 8), axis=0)


def _ffn(h, wa_ref, wb_ref, sched):
    ss = []
    for n in range(wa_ref.shape[1] // 128):
        a = _dot(h, wa_ref[:, n * 128:(n + 1) * 128])
        ss.append(_silu(a))
        sched(a)
    s = jnp.concatenate(ss, axis=1).astype(BF16)
    acc = []
    for n in range(wb_ref.shape[1] // 128):
        acc.append(_dot(s, wb_ref[:, n * 128:(n + 1) * 128]))
        sched(acc[-1])
    return jnp.concatenate(acc, axis=1)


def _sa(a11, a12, a21, a22):
    return [a11 + a22, a21 + a22, a11, a22, a11 + a12, a21 - a11, a12 - a22]


def _sb(b11, b12, b21, b22):
    return [b11 + b22, b11, b12 - b22, b21 - b11, b22, b11 + b12, b21 + b22]


def _sc(m):
    return [m[0] + m[3] - m[4] + m[6], m[4] + m[2], m[3] + m[1],
            m[0] + m[2] - m[1] + m[5]]


def _lhs7(t, u):
    h = t.shape[1] // 2
    return [v.astype(BF16)
            for v in _sa(t[:, :h], t[:, h:], u[:, :h], u[:, h:])]


_SA = ((0, 1, 3), (2, 1, 3), (0, 0, 0), (3, 0, 3), (0, 1, 1), (2, -1, 0),
       (1, -1, 3))
_SB = ((0, 1, 3), (0, 0, 0), (1, -1, 3), (2, -1, 0), (3, 0, 3), (0, 1, 1),
       (2, 1, 3))
_TG = (((0, 1), (3, 1)), ((2, 1), (3, -1)), ((1, 1), (3, 1)), ((0, 1), (2, 1)),
       ((0, -1), (1, 1)), ((3, 1),), ((0, 1),))


def _quads(x, hm):
    h = x.shape[1] // 2
    t = x[:hm]
    if x.shape[0] > 2 * hm:
        t = jnp.concatenate([t, x[2 * hm:]], axis=0)
    return t[:, :h], t[:, h:], x[hm:, :h], x[hm:, h:]


def _sax(a11, a12, a21, a22, hm):
    return [a11[:hm] + a22[:hm], a21 + a22, a11, a22, a11 + a12,
            a21[:hm] - a11[:hm], a12[:hm] - a22[:hm]]


def _acc7(acc, k, m, hm):
    for a, sg in _TG[k]:
        t = m if a in (1, 2) else m[:hm]
        if acc[a] is None:
            acc[a] = t if sg > 0 else -t
        else:
            acc[a] = acc[a] + t if sg > 0 else acc[a] - t


def _join(acc, hm):
    rest = [acc[1][hm:]] if acc[1].shape[0] > hm else []
    return (jnp.concatenate([acc[0], acc[2]], axis=0),
            jnp.concatenate([acc[1][:hm], acc[3]] + rest, axis=0))


def _ffn7(h7, wa, wb, sched, o1, o2, lag, early=()):
    acc = [None] * 7
    hm = h7[0].shape[0]
    u = [[None] * 4 for _ in wa]

    done = set()
    act = [[None] * 4 for _ in wa]
    s7 = [[None] * 7 for _ in wa]

    def run(cks):
        for c, k in cks:
            if (c, k) in done or c >= len(wa):
                continue
            done.add((c, k))
            t = _dot(h7[k], _up(wa[c][k]))
            _acc7(u[c], k, t, hm)
            sched(t)
            for a in range(4):
                if act[c][a] is None and all(
                        (c, n) in done for n in range(7)
                        if a in [e[0] for e in _TG[n]]):
                    act[c][a] = _silu(u[c][a])
            for n, (a, sg, b) in enumerate(_SA):
                if (s7[c][n] is None and act[c][a] is not None
                        and act[c][b] is not None):
                    v = act[c][a]
                    if sg:
                        v = v + act[c][b] if sg > 0 else v - act[c][b]
                    s7[c][n] = v.astype(BF16)

    run(early)
    for c, cb in enumerate(wb):
        run([(c, k) for k in o1] + [(c + 1, k) for k in o1[:lag]])
        for k in o2:
            p = _dot(s7[c][k], _up(cb[k]))
            acc[k] = p if acc[k] is None else acc[k] + p
            sched(p)
    c = _sc(acc)
    return jnp.concatenate(c[:2], axis=1), jnp.concatenate(c[2:], axis=1)


def _q4(x):
    h, w = x.shape[0] // 2, x.shape[1] // 2
    return x[:h, :w], x[:h, w:], x[h:, :w], x[h:, w:]


def _twice(f, x):
    return [v for y in f(*_q4(x)) for v in f(*_q4(y))]


def _pm(a, sg, b):
    return a if not sg else a + b if sg > 0 else a - b


def _ops2(load, put, tab, f, k1, z):
    def quad(a):
        return [load(a // 2 * 2 + j // 2, a % 2 * 2 + j % 2) for j in range(4)]

    a, sg, b = tab[k1]
    y = [_pm(u + _rep(z.v(), 16), sg, v) for u, v in zip(quad(a), quad(b))]
    for k2, v in enumerate(f(*y)):
        put(7 * k1 + k2, v)


def _ffn49(h49, hm, w, nfc, sched, oi, oo, plan, sb=None, gap=None,
           mid=None):
    src = [[n for n in range(7) if a in [e[0] for e in _TG[n]]]
           for a in range(4)]
    val = {}

    def add(key, sg, t):
        if key not in val:
            val[key] = t if sg > 0 else -t
        else:
            val[key] = _pm(val[key], sg, t)

    def collect(done, tag, k1, k2, t):
        done.add((k1, k2))
        for b, sg in _TG[k2]:
            add((tag, 'm', k1, b), sg, t)
            if all((k1, n) in done for n in src[b]):
                for a, sg1 in _TG[k1]:
                    add((tag, 'u', a, b), sg1, val[tag, 'm', k1, b])

    done = [set() for _ in range(nfc + 1)]

    pend, free = {}, [0]

    def ops(c, n, r, z):
        a, sg, a2 = _SA[n]
        rs = slice(r, r + gap[2])
        y = [_pm(val[c, 'a', a, b][rs] + _rep(z.v(), gap[2]), sg,
                 val[c, 'a', a2, b][rs]) for b in range(4)]
        for m, v in enumerate(_sa(*y)):
            sb.at[n][pl.ds(((c // KO * 7 + m) * hm + r) // 2, gap[2] // 2),
                     pl.ds(c % KO * 128, 128)] = _pk(v)

    def step_in(c, k1, k2):
        t = _dot(h49(7 * k1 + k2), w(7 * k1 + k2, c, 1))
        collect(done[c], c, k1, k2, t)
        sched(t, hm // 4)
        for a in range(4):
            for b in range(4):
                if (c, 'a', a, b) not in val and all(
                        (m, n) in done[c] for m in src[a] for n in src[b]):
                    val[c, 'a', a, b] = _silu(val[c, 'u', a, b])
        for n in oo[0] * (sb is not None):
            if (c, n) not in pend and all(
                    (c, 'a', a, b) in val
                    for a in _SA[n][::2] for b in range(4)):
                pend[c, n] = [functools.partial(ops, c, n, r)
                              for r in range(0, hm, gap[2])]
                for e in pend[c, n]:
                    free[0] = max(free[0] + gap[0], sched.now + gap[1])
                    sched.add([e], free[0], free[0] + 1)
        for n, (a, sg, a2) in enumerate(_SA * (sb is None)):
            for b in range(4):
                if ((c, 'y', n, b) not in val and (c, 'a', a, b) in val
                        and (c, 'a', a2, b) in val):
                    val[c, 'y', n, b] = _pm(val[c, 'a', a, b], sg,
                                            val[c, 'a', a2, b])
            for m, (b, sg, b2) in enumerate(_SA):
                if ((c, 's', n, m) not in val and (c, 'y', n, b) in val
                        and (c, 'y', n, b2) in val):
                    val[c, 's', n, m] = _pm(val[c, 'y', n, b], sg,
                                            val[c, 'y', n, b2]).astype(BF16)

    def step_out(g, k1, k2):
        cs = range(g * KO, (g + 1) * KO)
        if sb is None:
            v = jnp.concatenate([val[c, 's', k1, k2] for c in cs], axis=1)
        else:
            sched.force([e for c in cs for e in pend[c, k1]])
            v = _up(sb[k1, pl.ds((g * 7 + k2) * hm // 2, hm // 2), :])
        t = _dot(v, w(7 * k1 + k2, nfc + g * KO, KO))
        sched(t, hm * KO // 4)
        add(('p', k1, k2), 1, t)
        if (g + 1) * KO == nfc:
            collect(done[-1], 'o', k1, k2, val['p', k1, k2])

    todo = {(d, c): [(k1, k2) for k1 in o[0] for k2 in o[1]]
            for d, o in enumerate((oi, oo)) for c in range(nfc)}
    for d, c, n in plan:
        if d == 2:
            mid()
            continue
        for k1, k2 in todo[d, c][:n]:
            (step_out if d else step_in)(c, k1, k2)
        del todo[d, c][:n]
    return jnp.concatenate(
        [jnp.concatenate([val['o', 'u', a // 2 * 2 + b // 2, a % 2 * 2 + b % 2]
                          for b in range(4)], axis=1) for a in range(4)],
        axis=0)


def _kernel(x_hbm, w1a_hbm, w1b_hbm, wq_hbm, wk_hbm, wv_hbm, wo_hbm,
            wp1_hbm, dw_hbm, wp2_hbm, w2a_hbm, w2b_hbm,
            out_hbm,
            xin, wblk, wq, wk, wv, wo, dw,
            mq, wvo, xs, hs, ks, gs, dcs, st_mean, st_m2, bn,
            lhs49, w7, w49, lhs_b, dwb, zero, zero_s,
            al_buf0, al_buf1, al_buf2,
            p_buf0, p_buf1, p_buf2, s_buf0, s_buf1, hq7,
            xsem, w1sem, w2sem, wsem, osem,
            *, B, T, D, K):
    N = B * T
    obuf = xin
    KP = KC // 2
    nkc = -(-T // KC)
    TP = nkc * KP
    NCB = D // 128
    nt = N // TM
    tpb = T // TM

    def rows(i, r0=0, n=TM):
        return pl.ds(pl.multiple_of(i * TM, 16) + r0, n)

    def col(c):
        if isinstance(c, int):
            return slice(c * 128, (c + 1) * 128)
        return pl.ds(pl.multiple_of(c * 128, 128), 128)

    na = (N - T0) // TA
    H = D // 2
    QA = TA // 4
    s_buf = (s_buf0, s_buf1)

    def arows(i, r0=0, n=TA):
        return pl.ds(pl.multiple_of(T0 + (i - 1) * TA, 16) + r0, n)

    def x_copy(i):
        rs = pl.ds(0, T0) if isinstance(i, int) and i == 0 else arows(i)
        return pltpu.make_async_copy(x_hbm.at[rs, :], xin.at[rs, :],
                                     xsem.at[i])

    nc = N // TC

    def crows(i, r0=0, n=TC):
        return pl.ds(pl.multiple_of(i * TC, 16) + r0, n)

    def o_copy(i):
        return pltpu.make_async_copy(obuf.at[crows(i), :],
                                     out_hbm.at[crows(i), :], osem.at[i])

    nfc = w49.shape[1] // (D // 4)
    P1, P2 = 4 * nfc, 4 * nfc + 2

    def w1_copies(c):
        fs = pl.ds(pl.multiple_of(c * FC, FC), FC)
        return [pltpu.make_async_copy(w1a_hbm.at[:, fs], wblk.at[c],
                                      w1sem.at[0, c]),
                pltpu.make_async_copy(w1b_hbm.at[fs, :], wblk.at[nfc + c],
                                      w1sem.at[1, c])]

    def w2_copies(c):
        fs = pl.ds(pl.multiple_of(c * FC, FC), FC)
        hs_ = pl.ds(pl.multiple_of(c // 2 * H, H), H)
        return [pltpu.make_async_copy(s, d, w2sem.at[j, c])
                for j, (s, d) in enumerate([
                    (w2a_hbm.at[:, fs], wblk.at[2 * nfc + c]),
                    (w2b_hbm.at[fs, :], wblk.at[3 * nfc + c]),
                    (wp1_hbm.at[:, pl.ds(pl.multiple_of(c * H, H), H)],
                     wblk.at[P1 + c % 2, :, hs_])])]

    assert nfc == 4
    w_pairs = [(wp2_hbm, wblk.at[P2]), (wq_hbm, wq), (wk_hbm, wk),
               (wv_hbm, wv), (wo_hbm, wo), (dw_hbm, dw)]
    w_copies = [pltpu.make_async_copy(s, d, wsem.at[j])
                for j, (s, d) in enumerate(w_pairs)]

    x_copy(0).start()
    for cp in w1_copies(0):
        cp.start()

    zero[...] = jnp.zeros(zero.shape, jnp.uint32)
    zero_s[0] = 0
    for c in range(NCB):
        gs[1, c, 0:HALO, :] = jnp.zeros((HALO, 128), F32)
        gs[nt, c, HALO + TM:, :] = jnp.zeros((HALO, 128), F32)
    for b in range(B):
        ks[:, (b * TP + T // 2) // 2:(b + 1) * TP // 2, :] = jnp.zeros(
            (7, (TP - T // 2) // 2, H), jnp.uint32)

    def zrep(z, n):
        return None if z is None else _rep(z.v(), n)

    def pair_items(first, second, rows0):
        items = []
        for r0 in rows0:
            t = []
            items += [functools.partial(first, t, r0),
                      functools.partial(second, t, r0)]
        return items

    def ln_in(src, base, quarter, rows0):
        zs = zero_s[0]

        def ln(r0, j, z):
            s_buf[j // 2][pl.ds(j % 2 * QA + r0, 16), :] = _ln(
                src[pl.ds(pl.multiple_of(base + j * quarter, 16) + r0, 16), :]
                .astype(F32), zrep(z, 16))

        def ops(r0, k1):
            def load(j, c):
                return s_buf[j // 2][pl.ds(
                    pl.multiple_of(zs + r0, 16) + j % 2 * QA, 16), col(c)]

            def put(k, v):
                lhs49.at[k // 2][pl.ds(pl.multiple_of(r0 // 2, 8), 8),
                                 col(k % 2)] = _pk(v)

            return functools.partial(_ops2, load, put, _SA, _sa, k1)

        return ([functools.partial(ln, r0, j)
                 for r0 in rows0 for j in range(4)],
                [ops(r0, k1) for r0 in rows0 for k1 in range(7)])

    def ln_out(base, rows0):
        def first(t, r0, z, off=0):
            rs = pl.ds(pl.multiple_of(base, 32) + 2 * r0 + off, 16)
            t.append(_ln(xs[rs, :], zrep(z, 16)))
            hs[rs, :] = t[-1].astype(BF16)

        def second(t, r0, z):
            first(t, r0, z, 16)
            g = base // 32 + r0 // 16
            g += g // (T // 32) * ((TP - T // 2) // 16)
            for k, v in enumerate(_lhs7(*t)):
                ks.at[k][pl.ds(pl.multiple_of(g * 8, 8), 8), :] = _pk(v)

        return pair_items(first, second, rows0)

    def prep(src, dst, r0, z=None):
        q = [src[pl.ds(r + r0, 16), c:c + H].astype(F32)
             for r in (0, H) for c in (0, H)]
        if z is not None:
            zz = jnp.concatenate([_rep(z.v(), 16)] * (H // 128), axis=1)
            q[0], q[3] = q[0] + zz, q[3] + zz
        r1 = r0 // 2 if isinstance(r0, int) else pl.multiple_of(r0 // 2, 8)
        for k, v in enumerate(_sb(*q)):
            dst.at[k][pl.ds(r1, 8), :] = _pk(v)

    Q = D // 4

    def prep2(ff, blk, n, k1):
        rpb = Q // 16

        def load(r, c):
            return wblk[blk + n // rpb, pl.ds(pl.multiple_of(
                n % rpb * 16, 16) + r * Q, 16), col(c)].astype(F32)

        def put(k, v):
            rs = pl.multiple_of(n * 8, 8)
            if ff:
                w49.at[k // 2][pl.ds(rs, 8), col(k % 2)] = _pk(v)
            else:
                dcs[pl.ds(rs + k // NCB * D, 8), col(k % NCB)] = (
                    pltpu.bitcast(v.astype(BF16), F32))

        return functools.partial(_ops2, load, put, _SB, _sb, k1)

    x_copy(0).wait()
    if W1A == 2:
        for cp in w1_copies(1):
            cp.start()
    lhs_b[...] = _ln(xin[0:T0, :].astype(F32)).astype(BF16)
    xs[0:T0, :] = xin[0:T0, :].astype(F32)

    def first_tile(c, carry):
        for cp in w1_copies(c):
            cp.wait()

        @pl.when(c == 1)
        def _():
            x_copy(1).wait()

        if XF:
            @pl.when(c % 2 == 0)
            def _():
                x_copy(1 + c // 2).start()

        @pl.when(c + W1A < nfc)
        def _():
            for cp in w1_copies(c + W1A):
                cp.start()

        if not XF:
            @pl.when(c % 2 == 0)
            def _():
                x_copy(1 + c // 2).start()

        n = -(-QA // (nfc - 1) // 16) * 16
        r0 = pl.multiple_of(jnp.clip((c - 1) * n, 0, QA - n), 16)
        assert n <= T0 // 4
        sched = _Sched(zero)
        dur = 2 * NCB * T0
        items = ln_in(xin, jnp.where(c > 0, T0, 0),
                      jnp.where(c > 0, QA, T0 // 4),
                      [r0 + r for r in range(0, n, 16)])
        sched.add(items[0], int(F_WIN[0] * dur), int(F_WIN[2] * dur))
        sched.add(items[1], int(F_WIN[2] * dur), int(F_WIN[1] * dur))
        sched.add([prep2(0, 0, (j * nfc + c) * (Q // 16) + r, k1)
                   for j in range(2) for r in range(Q // 16)
                   for k1 in range(7)],
                  int(F_WIN[0] * dur), int(F_WIN[1] * dur))
        f = _ffn(lhs_b[...], wblk.at[c], wblk.at[nfc + c], sched)
        assert not sched.queue
        xs[0:T0, :] += 0.5 * f
        return carry

    lax.fori_loop(0, nfc, first_tile, 0)
    for j in range(3, na + 1):
        x_copy(j).start()
    for c in range(nfc):
        for cp in w2_copies(c):
            cp.start()
    for cp in w_copies:
        cp.start()

    def phase_a(i, carry):
        @pl.when(i < na)
        def _():
            x_copy(i + 1).wait()

        @pl.when((i >= IW) & (i < IW + nfc))
        def _():
            for cp in w2_copies(i - IW):
                cp.wait()

        @pl.when(i == IW)
        def _():
            w_copies[0].wait()

        sched = _Sched(zero)
        dur = 49 * 2 * nfc * TA // 16
        win = (int(A_WIN[0] * dur), int(A_WIN[1] * dur), A_SKIP)
        base = jnp.maximum(T0 + (i - 2) * TA, 0)
        sched.add(ln_out(base, range(0, TA // 2, 16)),
                  int(L_WIN[0] * dur), int(L_WIN[1] * dur), A_SKIP)
        base = T0 + jnp.minimum(i, na - 1) * TA
        items = ln_in(xin, base, QA, range(0, QA, 16))
        sched.add(items[0], *win)
        sched.add(items[1], int(O_WIN[0] * dur), int(O_WIN[1] * dur))
        rpb = H // 16
        total = w7.shape[0] * rpb
        ipi = -(-total // (na - IW + 1))
        items = []
        for k in range(ipi):
            n = jnp.minimum(jnp.maximum(i - IW, 0) * ipi + k, total - 1)
            blk = (n // rpb + 2) % 3
            items.append(functools.partial(
                prep, wblk.at[blk + jnp.where(i >= IW, P1, 0)], w7.at[blk],
                pl.multiple_of(n % rpb * 16, 16)))
        assert ipi * (nfc - 1) <= rpb
        sched.add(items, int(P_WIN[0] * dur), int(P_WIN[1] * dur))
        total = w49.shape[1] // 8
        ipi = -(-total // (na - IW + 1))
        assert ipi <= Q // 16
        sched.add([prep2(
            1, jnp.where(i >= IW, 2 * nfc, 0),
            jnp.minimum(jnp.maximum(i - IW, 0) * ipi + k, total - 1), k1)
            for k in range(ipi) for k1 in range(7)],
            int(P_WIN[0] * dur), int(P_WIN[1] * dur), win[2])

        def h49(k):
            assert sched.now <= int(O_WIN[0] * dur) and A_WIN[1] <= O_WIN[0]
            return _up(lhs49[k // 2, :, col(k % 2)])

        f = _ffn49(
            h49, QA,
            lambda k, b, n: pltpu.bitcast(
                dcs[pl.ds(k // NCB * D + b * 64, n * 64), col(k % NCB)], BF16),
            nfc, sched, *FA)
        assert not sched.queue
        xs[arows(i), :] = xin[arows(i), :].astype(F32) + 0.5 * f
        return carry

    with jax.named_scope("phase_a"):
        lax.fori_loop(1, na + 1, phase_a, 0)

    for cp in w_copies[1:]:
        cp.wait()

    qk_scale = (D ** -0.5) * math.log2(math.e)

    HM = TM // 32 * 16

    def put7(dst, r0, cs, *p):
        if len(p) == 4:
            ops = enumerate(_sa(*p))
        else:
            ops = zip((1, 2, 3, 4), (p[0] + p[1], *p, p[0] + p[1]))
        for k, t in ops:
            dst[pl.ds(k * PR + r0 // 2, 8), cs] = pltpu.bitcast(
                t.astype(BF16), jnp.uint32)

    def get7(src, k, ds=pl.ds, nr=None):
        nr = nr or (TM - HM if 1 <= k <= 4 else HM)
        return pltpu.bitcast(src[ds(k * PR, nr // 2), :], BF16)

    def groups(r0):
        return (r0, HM + r0) if r0 < HM else (HM + r0,)

    def q_ops(i, r0, c, z):
        p = [hs[rows(i, r, 16), col(2 * h + c)].astype(F32)
             for r in groups(r0) for h in range(2)]
        p[0] = p[0] + _rep(z.v(), 16)
        p[-1] = p[-1] + _rep(z.v(), 16)
        put7(hq7, r0, col(c), *p)

    def q_items(i):
        return [functools.partial(q_ops, i, r0, c)
                for r0 in range(0, TM - HM, 16) for c in range(2)]

    sched = _Sched(zero)
    sched.add(ln_out(N - TA, range(0, TA // 2, 16)), *FD[:2])
    sched.add(q_items(0), *FD[2:])
    for dst in (mq, wvo):
        for u in range(2):
            t = []
            for cs in (col(u), col(u + 2)):
                t.append(_dot_nt(wq[...], wk[cs, :]) if dst is mq
                         else _dot(wv[...], wo[:, cs]))
                sched(t[-1])
            if dst is mq:
                t = [v * qk_scale for v in t]
            for k, v in enumerate(
                    _sb(t[0][:H], t[1][:H], t[0][H:], t[1][H:])):
                dst[k, :, col(u)] = _pk(v)
    assert not sched.queue
    dwf = dw[...].astype(F32)
    for k in range(K):
        dwb[k] = jnp.broadcast_to(dwf[k:k + 1, :], (8, D))

    def conv_block(p, r0, c, done, CT=CT, AT=K):
        cs = col(c)
        acc = [None]

        def item(k0, z=None):
            for k in range(k0, min(k0 + CT, K)):
                off = HALO - K // 2 + k + r0
                w = dwb[k, :, cs]
                if z is not None and k - k0 < AT:
                    w = w + z.v()
                t = gs[p + 1, c, off:off + 8, :] * w
                acc[0] = t if acc[0] is None else acc[0] + t
            if k0 + CT >= K:
                dcs[rows(p, r0, 8), cs] = acc[0]
                done(acc[0])

        return [functools.partial(item, k0) for k0 in range(0, K, CT)]

    def conv_main(p, cols=range(NCB), **kw):
        st = []

        def stats(r0, c, acc):
            if r0 == 0:
                st[:] = [acc, None, None]
                return
            shift, s1, s2 = st
            d = acc - shift
            s1 = d if s1 is None else s1 + d
            s2 = d * d if s2 is None else s2 + d * d
            st[:] = [shift, s1, s2]
            if r0 + 16 == TM:
                dm = s1 * (1.0 / (TM // 8 - 1))
                st_mean[p, :, col(c)] = shift + dm
                st_m2[p, :, col(c)] = s2 - s1 * dm

        return [it for c in cols for r0 in range(0, TM - 8, 8)
                for it in conv_block(p, r0, c,
                                     functools.partial(stats, r0, c), **kw)]

    def conv_edge(p, cols=range(NCB)):
        return [it for c in cols
                for it in conv_block(p, TM - 8, c, lambda acc: None)]


    def phase_b(i, carry):
        b = i // tpb

        sched = _Sched(zero)
        sched.add(conv_edge(jnp.maximum(i - 2, 0))
                  + conv_main(jnp.maximum(i - 1, 0), range(L0, NCB)),
                  int(B_SLOTS[0] * TM), int(B_SLOTS[1] * TM))
        sched.add(q_items(jnp.minimum(i + 1, nt - 1)),
                  int(Q_SLOTS[0] * TM), int(Q_SLOTS[1] * TM))
        acc = [None] * 4
        for k in OQ:
            t = _dot(get7(hq7, k), _up(mq[k]))
            _acc7(acc, k, t, HM)
            sched(t)
        q11, q12, q21, q22 = _quads(
            jnp.concatenate(_join(acc, HM), axis=1), HM)
        q7 = [q11[:HM] - q22[:HM], q21 - q22, q11, q22, q12 - q11,
              q21[:HM] - q11[:HM], q12[:HM] - q22[:HM]]
        q7 = [t.astype(BF16) for t in q7]

        dz = zero_s[0]
        p_buf, al_buf = (p_buf0, p_buf1, p_buf2), (al_buf0, al_buf1, al_buf2)
        s_buf = (s_buf0, s_buf1)

        def dyn(r0, n):
            return pl.ds(pl.multiple_of(dz + r0, 8), n)

        nb = KP // 128

        def chunk(j):
            return pl.ds(pl.multiple_of(b * (TP // 2), KP // 2)
                         + j * KP // 2, KP // 2)

        def combine(m, j, c):
            if len(m) == 7:
                s = [m[0] + m[3] + m[4] + m[6], m[2] + m[4],
                     m[1] + m[3], m[1] - m[0] + m[2] + m[5]]
            else:
                s = [m[0] + m[2], m[1] + m[3]]
            nv = T // 2 - j * KP - c * 128
            if nv < 128:
                lane = lax.broadcasted_iota(jnp.int32, s[0].shape, 1)
                s = [jnp.where(lane < nv, t, -jnp.inf) for t in s]
            return s

        stat = {}

        def put(w, j, r, v):
            for r0 in range(0, v.shape[0], 16):
                stat[w, j, r + r0] = v[r0:r0 + 16]

        def get(w, j, r, n=16):
            return jnp.concatenate(
                [stat[w, j, r0] for r0 in range(r, r + n, 16)], axis=0)

        def scores(j):
            m = [None] * 7
            for k in OS if j else OS0:
                m[k] = _dot_nt(
                    q7[k], _up(ks[(0, 2, 1, 4, 3, 5, 6)[k], chunk(j), :]))
                sched(m[k])
            mx = None
            for c in range(nb):
                s = combine([t[:HM, col(c)] for t in m], j, c)
                e = combine([t[HM:, col(c)] for t in m[1:5]], j, c)
                for h in range(2):
                    t = jnp.concatenate([s[h], s[2 + h], e[h]], axis=0)
                    s_buf[j % 2][:, col(h * nb + c)] = t
                    mx = t if mx is None else jnp.maximum(mx, t)
            mx = jnp.broadcast_to(jnp.max(mx, axis=-1, keepdims=True),
                                  mx.shape)
            if j:
                mx = jnp.maximum(mx, get(0, j - 1, 0, TM))
            put(0, j, 0, mx)

        part = {}

        def soft1(j, r, c0, z):
            rs = slice(r, r + 16)
            m = get(0, j, r) + _rep(z.v(), 16)
            l = functools.reduce(jnp.add, part.pop((j, r), []) + [
                jnp.exp2(s_buf[j % 2][dyn(r, 16), col(c)] - m)
                for c in range(c0, c0 + S1)])
            if c0 + S1 < 2 * nb:
                part[j, r] = [l]
                return
            l = jnp.broadcast_to(jnp.sum(l, axis=-1, keepdims=True),
                                 (16, 128))
            if j:
                l += get(1, j - 1, r) * jnp.exp2(get(0, j - 1, r) - m)
            put(1, j, r, l)
            e = (pltpu.bitcast(l, jnp.int32) >> 23) - 127
            ref = m + e.astype(F32)
            put(2, j, r, ref)
            if j:
                al_buf[j % 3][rs, :] = jnp.exp2(get(2, j - 1, r) - ref)

        def soft2(j, r0, c0, z):
            ref = [get(2, j, r) + _rep(z.v(), 16) for r in groups(r0)]
            p = [jnp.concatenate(
                [jnp.exp2(s_buf[j % 2][dyn(r, 16), col(h * nb + c)] - m)
                 for c in range(c0, c0 + S2)], axis=1)
                 for r, m in zip(groups(r0), ref) for h in range(2)]
            put7(p_buf[j % 3], r0, slice(c0 * 128, (c0 + S2) * 128), *p)

        scd = 7 * HM + 4 * (TM - 2 * HM)
        start = sched.now

        def add_soft(j):
            rbs = range(0, TM - HM, 16)
            t0, t1 = (start + int(t * scd) for t in SW[j:j + 2])
            assert t1 <= start + min(2 * j + LAG + 1, nkc + j) * scd
            assert j < 3 or t0 >= start + min(2 * j + LAG - 4,
                                              nkc + j - 2) * scd
            assert (j + 2 >= nkc
                    or t1 <= start + max(2 * j + 5 - LAG, j + 3) * scd)
            u = (t1 - t0 - sum(SD)) // (len(rbs) + 1)
            for n, r0 in enumerate(rbs):
                its = [[functools.partial(soft1, j, r, c)
                        for r in groups(r0) for c in range(0, 2 * nb, S1)],
                       [functools.partial(soft2, j, r0, c)
                        for c in range(0, nb, S2)]]
                for k, it in enumerate(its):
                    t = t0 + SD[0] + n * u + k * (u + SD[1])
                    sched.add(it, t, t + u)

        for j in range(LAG):
            scores(j)
            add_soft(j)
        acc = [None] * 4
        for j in range(nkc):
            if j + LAG < nkc:
                scores(j + LAG)
                add_soft(j + LAG)
            fresh = [j > 0] * 4
            for k in OP if j + 1 < nkc else OQ:
                w = _up(ks[(0, 2, 6, 5, 3, 4, 1)[k], chunk(j), :])
                m = _dot(get7(p_buf[j % 3], k, dyn), w)
                sched(m)
                for a, _ in _TG[k]:
                    if fresh[a]:
                        al = al_buf[j % 3][dyn(0, TM), :]
                        al = _quads(jnp.concatenate([al] * NCB, axis=1), HM)[a]
                        acc[a] = acc[a] * al[:acc[a].shape[0]]
                        fresh[a] = False
                _acc7(acc, k, m, HM)
        assert not sched.queue
        t = jnp.exp2(get(2, nkc - 1, 0, TM) - get(0, nkc - 1, 0, TM))
        t = t / get(1, nkc - 1, 0, TM)
        o = (jnp.concatenate(_join(acc, HM), axis=1)
             * jnp.concatenate([t] * NCB, axis=1))
        o7 = [t.astype(BF16) for t in _sax(*_quads(o, HM), HM)]
        acc = list(_quads(xs[rows(i), :], HM))
        acc = [acc[0][:HM], acc[1], acc[2], acc[3][:HM]]
        for k in OW:
            _acc7(acc, k, _dot(o7[k], _up(wvo[k])), HM)
        x2 = jnp.concatenate(_join(acc, HM), axis=1)
        xs[rows(i), :] = x2
        h7 = [t.astype(BF16) for t in _sax(*_quads(_ln(x2), HM), HM)]
        sched = _Sched(zero)
        acc = [[None] * 4 for _ in range(2)]
        for n, (h, k) in enumerate(PO):
            t = _dot(h7[k], _up(w7[h, k]))
            _acc7(acc[h], k, t, HM)
            sched(t)
            if any(e[0] == h for e in PO[n + 1:]):
                continue
            val, gate = _join(acc[h], HM)
            g2 = val * (0.5 + 0.5 * jnp.tanh(0.5 * gate))
            for c in (2 * h, 2 * h + 1):
                g = g2[:, col(c % 2)]
                gs[i + 1, c, HALO:HALO + TM, :] = g
                gs[i, c, HALO + TM:, :] = jnp.where(
                    i % tpb == 0, 0.0, g[:HALO])
                gs[i + 2, c, :HALO, :] = jnp.where(
                    i % tpb == tpb - 1, 0.0, g[TM - HALO:])
            if h == 0 and L0:
                rest = sum(h7[e[1]].shape[0] for e in PO[n + 1:])
                sched.add(conv_main(i, range(L0), CT=LP[2], AT=LP[3]),
                          sched.now + LP[0], sched.now + rest - LP[1])
        assert not sched.queue
        return carry

    with jax.named_scope("phase_b"):
        lax.fori_loop(0, nt, phase_b, 0)
    for item in (conv_main(nt - 1, range(L0, NCB)) + conv_edge(nt - 2)
                 + conv_edge(nt - 1)):
        item()

    ng = TM // 8 - 1
    means = st_mean[...].reshape(nt * 8, D)
    edges = jnp.concatenate([dcs[(p + 1) * TM - 8:(p + 1) * TM, :]
                             for p in range(nt)], axis=0)
    mu = jnp.sum(ng * means + edges, axis=0, keepdims=True) * (1.0 / N)
    dm = means - mu
    de = edges - mu
    var = jnp.sum(st_m2[...].reshape(nt * 8, D) + ng * (dm * dm) + de * de,
                  axis=0, keepdims=True) * (1.0 / N)
    rstd = lax.rsqrt(var + EPS)
    bn[0] = jnp.broadcast_to(mu, (8, D))
    bn[1] = jnp.broadcast_to(rstd, (8, D))

    def bn_silu(i, r0, c, z=None):
        p = []
        for r in (r0, TC // 2 + r0):
            for h in range(2):
                cs = col(2 * h + c)
                mu = bn[0, :, cs] if z is None else bn[0, :, cs] + z.v()
                y = dcs[crows(i, r, 16), cs] - _rep(mu, 16)
                p.append(_silu(y * _rep(bn[1, :, cs], 16)))
        put7(hq7, r0, col(c), *p)

    def bn_items(i):
        return [functools.partial(bn_silu, i, r0, c)
                for r0 in range(0, TC // 2, 16) for c in range(2)]

    def ln_final(i, r0=0, n=TC, z=None):
        obuf[crows(i, r0, n), :] = _ln(xs[crows(i, r0, n), :],
                                       zrep(z, n)).astype(BF16)

    for item in bn_items(0):
        item()

    QC = TC // 4

    def pw2(src, dst, sched, win):
        acc = list(_quads(xs[crows(src), :], TC // 2))
        for k in OQ:
            t = _dot(get7(hq7, k, nr=TC // 2), _up(w7[2, k]))
            _acc7(acc, k, t, TC // 2)
            sched(t)
        xs[crows(dst), :] = jnp.concatenate(_join(acc, TC // 2), axis=1)
        for items, t0, t1 in zip(
                ln_in(xs, dst * TC, QC, range(0, QC, 16)), win, win[1:]):
            sched.add(items, sched.now + t0, sched.now + t1)

    sched = _Sched(zero)
    pw2(0, 0, sched, (0, 1, 2))
    sched.force([e[1] for e in sched.queue])

    def phase_c(i, carry):
        @pl.when(i >= 2)
        def _():
            o_copy(i - 2).start()

        sched = _Sched(zero)
        dur = (7 * 8 + 49 * 2 * nfc) * TC // 16
        sched.add([functools.partial(ln_final, jnp.maximum(i - 1, 0), r, RC)
                   for r in range(0, TC, RC)],
                  int(C_WIN[0] * dur), int(C_WIN[1] * dur))
        nxt = jnp.minimum(i + 1, nc - 1)
        items = bn_items(nxt)
        sched.add(items, int(C_WIN[2] * dur), int(C_WIN[3] * dur))
        done = []

        def mid():
            sched.force(items)
            done.append(1)
            pw2(nxt, jnp.where(i + 1 < nc, i + 1, 0), sched, M_WIN)

        def h49(k):
            assert not done
            return _up(lhs49[k // 2, :QC // 2, col(k % 2)])

        f = _ffn49(h49, QC, lambda k, b, n: _up(
            w49[k // 2, b * 64:(b + n) * 64, col(k % 2)]),
            nfc, sched, *FB, ks, GC, mid)
        assert not sched.queue
        xs[crows(i), :] += 0.5 * f
        return carry

    with jax.named_scope("phase_c"):
        lax.fori_loop(0, nc, phase_c, 0)
    o_copy(nc - 2).start()
    last = []
    for k, (r0, r1) in enumerate(zip(EP[:-1], EP[1:])):
        ln_final(nc - 1, r0, r1 - r0)
        rs = crows(nc - 1, r0, r1 - r0)
        last.append(pltpu.make_async_copy(obuf.at[rs, :], out_hbm.at[rs, :],
                                          osem.at[nc - 1 + k]))
        last[-1].start()
    for i in range(nc - 1):
        o_copy(i).wait()
    for cp in last:
        cp.wait()


@jax.jit
def pallas_standalone__conformer_family_conformer__speech_kernel(
    x: jax.Array,
    w_ff1_a: jax.Array,
    w_ff1_b: jax.Array,
    w_q: jax.Array,
    w_k: jax.Array,
    w_v: jax.Array,
    w_o: jax.Array,
    w_pw1: jax.Array,
    dw: jax.Array,
    w_pw2: jax.Array,
    w_ff2_a: jax.Array,
    w_ff2_b: jax.Array,
):
    B, T, D = x.shape
    K = dw.shape[0]
    N = B * T
    weights = (w_ff1_a, w_ff1_b, w_q, w_k, w_v, w_o, w_pw1, dw, w_pw2,
               w_ff2_a, w_ff2_b)
    scratch = [pltpu.VMEM((N, D), BF16)]
    nfc = w_ff1_a.shape[1] // FC
    scratch += [pltpu.VMEM((4 * nfc + 3, D, D), BF16)]
    scratch += [pltpu.VMEM(w.shape, w.dtype)
                for w in (w_q, w_k, w_v, w_o, dw)]
    scratch += [
        pltpu.VMEM((7, D // 4, D // 2), jnp.uint32),
        pltpu.VMEM((7, D // 4, D // 2), jnp.uint32),
        pltpu.VMEM((N, D), F32),
        pltpu.VMEM((N, D), BF16),
        pltpu.VMEM((7, B * -(-T // KC) * KC // 4, D // 2), jnp.uint32),
        pltpu.VMEM((N // TM + 2, D // 128, TM + 2 * HALO, 128), F32),
        pltpu.VMEM((N, D), F32),
        pltpu.VMEM((N // TM, 8, D), F32),
        pltpu.VMEM((N // TM, 8, D), F32),
        pltpu.VMEM((2, 8, D), F32),
        pltpu.VMEM((25, TA // 8, D // 2), jnp.uint32),
        pltpu.VMEM((3, 7, D // 4, D // 2), jnp.uint32),
        pltpu.VMEM((25, nfc * D // 4, D // 2), jnp.uint32),
        pltpu.VMEM((T0, D), BF16),
        pltpu.VMEM((K, 8, D), F32),
        pltpu.VMEM((ZR, 128), jnp.uint32),
        pltpu.SMEM((1,), jnp.int32),
        pltpu.VMEM((TM + 16, 128), F32),
        pltpu.VMEM((TM + 16, 128), F32),
        pltpu.VMEM((TM + 16, 128), F32),
        pltpu.VMEM((7 * PR, KC // 2), jnp.uint32),
        pltpu.VMEM((7 * PR, KC // 2), jnp.uint32),
        pltpu.VMEM((7 * PR, KC // 2), jnp.uint32),
        pltpu.VMEM((TM, KC), F32),
        pltpu.VMEM((TM, KC), F32),
        pltpu.VMEM((7 * PR, D // 2), jnp.uint32),
        pltpu.SemaphoreType.DMA(((N - T0) // TA + 1,)),
        pltpu.SemaphoreType.DMA((2, nfc)),
        pltpu.SemaphoreType.DMA((3, nfc)),
        pltpu.SemaphoreType.DMA((6,)),
        pltpu.SemaphoreType.DMA((N // TC + len(EP),)),
    ]
    out = pl.pallas_call(
        functools.partial(_kernel, B=B, T=T, D=D, K=K),
        out_shape=jax.ShapeDtypeStruct((N, D), x.dtype),
        in_specs=[pl.BlockSpec(memory_space=pl.ANY)] * 12,
        out_specs=pl.BlockSpec(memory_space=pl.ANY),
        scratch_shapes=scratch,
        compiler_params=pltpu.CompilerParams(
            vmem_limit_bytes=VL * 1024 * 1024),
    )(x.reshape(N, D), *weights)
    return out.reshape(B, T, D)
```

```python
import functools
import math

import jax
import jax.numpy as jnp
from jax import lax
import jax.experimental.pallas as pl
import jax.experimental.pallas.tpu as pltpu

F32 = jnp.float32
BF16 = jnp.bfloat16

TM = 400
T0 = 320
TA = 512
TC = 320
FC = 512
KC = 512
W1A = 1
XF = 0
IW = 3
VL = 128
GA = (42, 60, 16)
GC = (42, 90, 16)
KO = 2
O_WIN = (0.75, 0.97)
L_WIN = (0.0, 0.12)
PL = ((0, 0, 49), (0, 1, 49), (0, 2, 49), (0, 3, 49), (1, 0, 49), (1, 1, 49))
FA = (((2, 4, 3, 1, 0, 6, 5), (2, 4, 3, 1, 0, 6, 5)),
      ((2, 4, 5, 3, 1, 6, 0), (2, 4, 3, 1, 0, 6, 5)), PL)
FB = (((2, 4, 3, 1, 0, 6, 5), (2, 4, 3, 1, 0, 6, 5)),
      ((2, 4, 5, 3, 1, 6, 0), (2, 4, 3, 1, 0, 6, 5)),
      PL[:4] + ((1, 0, 35), (2, 0, 0), (1, 0, 14), (1, 1, 49)))
P_WIN = (0.5, 0.97)
OQ = (0, 2, 3, 4, 6, 1, 5)
OS0 = (2, 4, 3, 1, 0, 5, 6)
OS = (0, 1, 2, 3, 4, 5, 6)
OP = (0, 1, 2, 3, 4, 5, 6)
OW = (2, 4, 3, 0, 6, 1, 5)
PO = ((0, 2), (0, 4), (1, 2), (0, 3), (0, 0), (0, 6), (0, 1), (0, 5),
      (1, 4), (1, 3), (1, 0), (1, 6), (1, 1), (1, 5))
F_WIN = (0.02, 0.95, 0.5)
A_WIN = (0.5, 0.75)
FD = (0, 3200, 0, 3200)
B_SLOTS = (1, 53)
Q_SLOTS = (8, 50)
CT = 5
L0 = 1
LP = (0, 100, 3, 1)
S1 = 2
S2 = 1
SD = (0, 140, 120)
LAG = 2
SW = tuple(1 + 1.75 * j for j in range(9))
C_WIN = (0.02, 0.5, 0.3, 0.58)
M_WIN = (60, 1200, 2400)
RC = 8
EP = (0, 128, 224, 288, 320)
ZR = 32
PR = 112
HALO = 8
EPS = 1e-05


def _ln(x, z=None):
    if z is None:
        m = jnp.mean(x, axis=-1, keepdims=True)
    else:
        t = z
        for c in range(x.shape[-1] // 128):
            t = t + x[:, c * 128:(c + 1) * 128]
        m = jnp.sum(t, axis=-1, keepdims=True) * (1.0 / x.shape[-1])
    xc = x - m
    v = jnp.mean(xc * xc, axis=-1, keepdims=True)
    return xc * lax.rsqrt(v + EPS)


def _silu(a):
    y = 0.5 * a
    return y + y * jnp.tanh(y)


def _dot(a, b):
    return jnp.dot(a, b, preferred_element_type=F32)


def _dot_nt(a, b):
    return lax.dot_general(a, b, (((1,), (1,)), ((), ())),
                           preferred_element_type=F32)


def _pk(v):
    return pltpu.bitcast(v.astype(BF16), jnp.uint32)


def _up(v):
    return pltpu.bitcast(v, BF16)


class _Anchor:
    def __init__(self, t, zero_v):
        self.t, self.zero_v = t, zero_v

    def v(self):
        return pltpu.bitcast(
            pltpu.bitcast(self.t, jnp.uint32) & self.zero_v[0:8, :], F32)


class _Sched:
    def __init__(self, zero_v):
        self.zero_v = zero_v
        self.queue = []
        self.now = 0

    def add(self, items, t0, t1, skip=()):
        assert t0 >= self.now
        ts = [t for t in range(t0, t1)
              if not any(a <= t < b for a, b in skip)]
        self.queue += [(ts[k * len(ts) // len(items)], it)
                       for k, it in enumerate(items)]
        self.queue.sort(key=lambda e: e[0])

    def __call__(self, t, dur=None):
        dur = dur or t.shape[0]
        end = self.now + dur
        while self.queue and self.queue[0][0] < end:
            time, item = self.queue.pop(0)
            r = (time - self.now) * t.shape[0] // dur // 8 * 8
            item(_Anchor(t[r:r + 8, :128], self.zero_v))
        self.now = end
        self.last = t

    def force(self, items):
        for e in [e for e in self.queue if e[1] in items]:
            self.queue.remove(e)
            e[1](_Anchor(self.last[-8:, :128], self.zero_v))


def _rep(z, rows):
    return jnp.concatenate([z] * (rows // 8), axis=0)


def _ffn(h, wa_ref, wb_ref, sched):
    ss = []
    for n in range(wa_ref.shape[1] // 128):
        a = _dot(h, wa_ref[:, n * 128:(n + 1) * 128])
        ss.append(_silu(a))
        sched(a)
    s = jnp.concatenate(ss, axis=1).astype(BF16)
    acc = []
    for n in range(wb_ref.shape[1] // 128):
        acc.append(_dot(s, wb_ref[:, n * 128:(n + 1) * 128]))
        sched(acc[-1])
    return jnp.concatenate(acc, axis=1)


def _sa(a11, a12, a21, a22):
    return [a11 + a22, a21 + a22, a11, a22, a11 + a12, a21 - a11, a12 - a22]


def _sb(b11, b12, b21, b22):
    return [b11 + b22, b11, b12 - b22, b21 - b11, b22, b11 + b12, b21 + b22]


def _sc(m):
    return [m[0] + m[3] - m[4] + m[6], m[4] + m[2], m[3] + m[1],
            m[0] + m[2] - m[1] + m[5]]


def _lhs7(t, u):
    h = t.shape[1] // 2
    return [v.astype(BF16)
            for v in _sa(t[:, :h], t[:, h:], u[:, :h], u[:, h:])]


_SA = ((0, 1, 3), (2, 1, 3), (0, 0, 0), (3, 0, 3), (0, 1, 1), (2, -1, 0),
       (1, -1, 3))
_SB = ((0, 1, 3), (0, 0, 0), (1, -1, 3), (2, -1, 0), (3, 0, 3), (0, 1, 1),
       (2, 1, 3))
_TG = (((0, 1), (3, 1)), ((2, 1), (3, -1)), ((1, 1), (3, 1)), ((0, 1), (2, 1)),
       ((0, -1), (1, 1)), ((3, 1),), ((0, 1),))


def _quads(x, hm):
    h = x.shape[1] // 2
    t = x[:hm]
    if x.shape[0] > 2 * hm:
        t = jnp.concatenate([t, x[2 * hm:]], axis=0)
    return t[:, :h], t[:, h:], x[hm:, :h], x[hm:, h:]


def _sax(a11, a12, a21, a22, hm):
    return [a11[:hm] + a22[:hm], a21 + a22, a11, a22, a11 + a12,
            a21[:hm] - a11[:hm], a12[:hm] - a22[:hm]]


def _acc7(acc, k, m, hm):
    for a, sg in _TG[k]:
        t = m if a in (1, 2) else m[:hm]
        if acc[a] is None:
            acc[a] = t if sg > 0 else -t
        else:
            acc[a] = acc[a] + t if sg > 0 else acc[a] - t


def _join(acc, hm):
    rest = [acc[1][hm:]] if acc[1].shape[0] > hm else []
    return (jnp.concatenate([acc[0], acc[2]], axis=0),
            jnp.concatenate([acc[1][:hm], acc[3]] + rest, axis=0))


def _ffn7(h7, wa, wb, sched, o1, o2, lag, early=()):
    acc = [None] * 7
    hm = h7[0].shape[0]
    u = [[None] * 4 for _ in wa]

    done = set()
    act = [[None] * 4 for _ in wa]
    s7 = [[None] * 7 for _ in wa]

    def run(cks):
        for c, k in cks:
            if (c, k) in done or c >= len(wa):
                continue
            done.add((c, k))
            t = _dot(h7[k], _up(wa[c][k]))
            _acc7(u[c], k, t, hm)
            sched(t)
            for a in range(4):
                if act[c][a] is None and all(
                        (c, n) in done for n in range(7)
                        if a in [e[0] for e in _TG[n]]):
                    act[c][a] = _silu(u[c][a])
            for n, (a, sg, b) in enumerate(_SA):
                if (s7[c][n] is None and act[c][a] is not None
                        and act[c][b] is not None):
                    v = act[c][a]
                    if sg:
                        v = v + act[c][b] if sg > 0 else v - act[c][b]
                    s7[c][n] = v.astype(BF16)

    run(early)
    for c, cb in enumerate(wb):
        run([(c, k) for k in o1] + [(c + 1, k) for k in o1[:lag]])
        for k in o2:
            p = _dot(s7[c][k], _up(cb[k]))
            acc[k] = p if acc[k] is None else acc[k] + p
            sched(p)
    c = _sc(acc)
    return jnp.concatenate(c[:2], axis=1), jnp.concatenate(c[2:], axis=1)


def _q4(x):
    h, w = x.shape[0] // 2, x.shape[1] // 2
    return x[:h, :w], x[:h, w:], x[h:, :w], x[h:, w:]


def _twice(f, x):
    return [v for y in f(*_q4(x)) for v in f(*_q4(y))]


def _pm(a, sg, b):
    return a if not sg else a + b if sg > 0 else a - b


def _ops2(load, put, tab, f, k1, z):
    def quad(a):
        return [load(a // 2 * 2 + j // 2, a % 2 * 2 + j % 2) for j in range(4)]

    a, sg, b = tab[k1]
    y = [_pm(u + _rep(z.v(), 16), sg, v) for u, v in zip(quad(a), quad(b))]
    for k2, v in enumerate(f(*y)):
        put(7 * k1 + k2, v)


def _ffn49(h49, hm, w, nfc, sched, oi, oo, plan, sb=None, gap=None,
           mid=None):
    src = [[n for n in range(7) if a in [e[0] for e in _TG[n]]]
           for a in range(4)]
    val = {}

    def add(key, sg, t):
        if key not in val:
            val[key] = t if sg > 0 else -t
        else:
            val[key] = _pm(val[key], sg, t)

    def collect(done, tag, k1, k2, t):
        done.add((k1, k2))
        for b, sg in _TG[k2]:
            add((tag, 'm', k1, b), sg, t)
            if all((k1, n) in done for n in src[b]):
                for a, sg1 in _TG[k1]:
                    add((tag, 'u', a, b), sg1, val[tag, 'm', k1, b])

    done = [set() for _ in range(nfc + 1)]

    pend, free = {}, [0]

    def ops(c, n, r, z):
        a, sg, a2 = _SA[n]
        rs = slice(r, r + gap[2])
        y = [_pm(val[c, 'a', a, b][rs] + _rep(z.v(), gap[2]), sg,
                 val[c, 'a', a2, b][rs]) for b in range(4)]
        for m, v in enumerate(_sa(*y)):
            sb.at[n][pl.ds(((c // KO * 7 + m) * hm + r) // 2, gap[2] // 2),
                     pl.ds(c % KO * 128, 128)] = _pk(v)

    def step_in(c, k1, k2):
        t = _dot(h49(7 * k1 + k2), w(7 * k1 + k2, c, 1))
        collect(done[c], c, k1, k2, t)
        sched(t, hm // 4)
        for a in range(4):
            for b in range(4):
                if (c, 'a', a, b) not in val and all(
                        (m, n) in done[c] for m in src[a] for n in src[b]):
                    val[c, 'a', a, b] = _silu(val[c, 'u', a, b])
        for n in oo[0] * (sb is not None):
            if (c, n) not in pend and all(
                    (c, 'a', a, b) in val
                    for a in _SA[n][::2] for b in range(4)):
                pend[c, n] = [functools.partial(ops, c, n, r)
                              for r in range(0, hm, gap[2])]
                for e in pend[c, n]:
                    free[0] = max(free[0] + gap[0], sched.now + gap[1])
                    sched.add([e], free[0], free[0] + 1)
        for n, (a, sg, a2) in enumerate(_SA * (sb is None)):
            for b in range(4):
                if ((c, 'y', n, b) not in val and (c, 'a', a, b) in val
                        and (c, 'a', a2, b) in val):
                    val[c, 'y', n, b] = _pm(val[c, 'a', a, b], sg,
                                            val[c, 'a', a2, b])
            for m, (b, sg, b2) in enumerate(_SA):
                if ((c, 's', n, m) not in val and (c, 'y', n, b) in val
                        and (c, 'y', n, b2) in val):
                    val[c, 's', n, m] = _pm(val[c, 'y', n, b], sg,
                                            val[c, 'y', n, b2]).astype(BF16)

    def step_out(g, k1, k2):
        cs = range(g * KO, (g + 1) * KO)
        if sb is None:
            v = jnp.concatenate([val[c, 's', k1, k2] for c in cs], axis=1)
        else:
            sched.force([e for c in cs for e in pend[c, k1]])
            v = _up(sb[k1, pl.ds((g * 7 + k2) * hm // 2, hm // 2), :])
        t = _dot(v, w(7 * k1 + k2, nfc + g * KO, KO))
        sched(t, hm * KO // 4)
        add(('p', k1, k2), 1, t)
        if (g + 1) * KO == nfc:
            collect(done[-1], 'o', k1, k2, val['p', k1, k2])

    todo = {(d, c): [(k1, k2) for k1 in o[0] for k2 in o[1]]
            for d, o in enumerate((oi, oo)) for c in range(nfc)}
    for d, c, n in plan:
        if d == 2:
            mid()
            continue
        for k1, k2 in todo[d, c][:n]:
            (step_out if d else step_in)(c, k1, k2)
        del todo[d, c][:n]
    return jnp.concatenate(
        [jnp.concatenate([val['o', 'u', a // 2 * 2 + b // 2, a % 2 * 2 + b % 2]
                          for b in range(4)], axis=1) for a in range(4)],
        axis=0)


def _kernel(x_hbm, w1a_hbm, w1b_hbm, wq_hbm, wk_hbm, wv_hbm, wo_hbm,
            wp1_hbm, dw_hbm, wp2_hbm, w2a_hbm, w2b_hbm,
            out_hbm,
            xin, wblk, wq, wk, wv, wo, dw,
            mq, wvo, xs, hs, ks, gs, dcs, st_mean, st_m2, bn,
            lhs49, sb, w7, w49, lhs_b, dwb, zero, zero_s,
            al_buf0, al_buf1, al_buf2,
            p_buf0, p_buf1, p_buf2, s_buf0, s_buf1, hq7,
            xsem, w1sem, w2sem, wsem, osem,
            *, B, T, D, K):
    N = B * T
    obuf = xin
    KP = KC // 2
    nkc = -(-T // KC)
    TP = nkc * KP
    NCB = D // 128
    nt = N // TM
    tpb = T // TM

    def rows(i, r0=0, n=TM):
        return pl.ds(pl.multiple_of(i * TM, 16) + r0, n)

    def col(c):
        if isinstance(c, int):
            return slice(c * 128, (c + 1) * 128)
        return pl.ds(pl.multiple_of(c * 128, 128), 128)

    na = (N - T0) // TA
    H = D // 2
    QA = TA // 4
    s_buf = (s_buf0, s_buf1)

    def arows(i, r0=0, n=TA):
        return pl.ds(pl.multiple_of(T0 + (i - 1) * TA, 16) + r0, n)

    def x_copy(i):
        rs = pl.ds(0, T0) if isinstance(i, int) and i == 0 else arows(i)
        return pltpu.make_async_copy(x_hbm.at[rs, :], xin.at[rs, :],
                                     xsem.at[i])

    nc = N // TC

    def crows(i, r0=0, n=TC):
        return pl.ds(pl.multiple_of(i * TC, 16) + r0, n)

    def o_copy(i):
        return pltpu.make_async_copy(obuf.at[crows(i), :],
                                     out_hbm.at[crows(i), :], osem.at[i])

    nfc = w49.shape[1] // (D // 4)
    P1, P2 = 4 * nfc, 4 * nfc + 2

    def w1_copies(c):
        fs = pl.ds(pl.multiple_of(c * FC, FC), FC)
        return [pltpu.make_async_copy(w1a_hbm.at[:, fs], wblk.at[c],
                                      w1sem.at[0, c]),
                pltpu.make_async_copy(w1b_hbm.at[fs, :], wblk.at[nfc + c],
                                      w1sem.at[1, c])]

    def w2_copies(c):
        fs = pl.ds(pl.multiple_of(c * FC, FC), FC)
        hs_ = pl.ds(pl.multiple_of(c // 2 * H, H), H)
        return [pltpu.make_async_copy(s, d, w2sem.at[j, c])
                for j, (s, d) in enumerate([
                    (w2a_hbm.at[:, fs], wblk.at[2 * nfc + c]),
                    (w2b_hbm.at[fs, :], wblk.at[3 * nfc + c]),
                    (wp1_hbm.at[:, pl.ds(pl.multiple_of(c * H, H), H)],
                     wblk.at[P1 + c % 2, :, hs_])])]

    assert nfc == 4
    w_pairs = [(wp2_hbm, wblk.at[P2]), (wq_hbm, wq), (wk_hbm, wk),
               (wv_hbm, wv), (wo_hbm, wo), (dw_hbm, dw)]
    w_copies = [pltpu.make_async_copy(s, d, wsem.at[j])
                for j, (s, d) in enumerate(w_pairs)]

    x_copy(0).start()
    for cp in w1_copies(0):
        cp.start()

    zero[...] = jnp.zeros(zero.shape, jnp.uint32)
    zero_s[0] = 0
    for c in range(NCB):
        gs[1, c, 0:HALO, :] = jnp.zeros((HALO, 128), F32)
        gs[nt, c, HALO + TM:, :] = jnp.zeros((HALO, 128), F32)
    for b in range(B):
        ks[:, (b * TP + T // 2) // 2:(b + 1) * TP // 2, :] = jnp.zeros(
            (7, (TP - T // 2) // 2, H), jnp.uint32)

    def zrep(z, n):
        return None if z is None else _rep(z.v(), n)

    def pair_items(first, second, rows0):
        items = []
        for r0 in rows0:
            t = []
            items += [functools.partial(first, t, r0),
                      functools.partial(second, t, r0)]
        return items

    def ln_in(src, base, quarter, rows0):
        zs = zero_s[0]

        def ln(r0, j, z):
            s_buf[j // 2][pl.ds(j % 2 * QA + r0, 16), :] = _ln(
                src[pl.ds(pl.multiple_of(base + j * quarter, 16) + r0, 16), :]
                .astype(F32), zrep(z, 16))

        def ops(r0, k1):
            def load(j, c):
                return s_buf[j // 2][pl.ds(
                    pl.multiple_of(zs + r0, 16) + j % 2 * QA, 16), col(c)]

            def put(k, v):
                lhs49.at[k // 2][pl.ds(pl.multiple_of(r0 // 2, 8), 8),
                                 col(k % 2)] = _pk(v)

            return functools.partial(_ops2, load, put, _SA, _sa, k1)

        return ([functools.partial(ln, r0, j)
                 for r0 in rows0 for j in range(4)],
                [ops(r0, k1) for r0 in rows0 for k1 in range(7)])

    def ln_out(base, rows0):
        def first(t, r0, z, off=0):
            rs = pl.ds(pl.multiple_of(base, 32) + 2 * r0 + off, 16)
            t.append(_ln(xs[rs, :], zrep(z, 16)))
            hs[rs, :] = t[-1].astype(BF16)

        def second(t, r0, z):
            first(t, r0, z, 16)
            g = base // 32 + r0 // 16
            g += g // (T // 32) * ((TP - T // 2) // 16)
            for k, v in enumerate(_lhs7(*t)):
                ks.at[k][pl.ds(pl.multiple_of(g * 8, 8), 8), :] = _pk(v)

        return pair_items(first, second, rows0)

    def prep(src, dst, r0, z=None):
        q = [src[pl.ds(r + r0, 16), c:c + H].astype(F32)
             for r in (0, H) for c in (0, H)]
        if z is not None:
            zz = jnp.concatenate([_rep(z.v(), 16)] * (H // 128), axis=1)
            q[0], q[3] = q[0] + zz, q[3] + zz
        r1 = r0 // 2 if isinstance(r0, int) else pl.multiple_of(r0 // 2, 8)
        for k, v in enumerate(_sb(*q)):
            dst.at[k][pl.ds(r1, 8), :] = _pk(v)

    Q = D // 4

    def prep2(ff, blk, n, k1):
        rpb = Q // 16

        def load(r, c):
            return wblk[blk + n // rpb, pl.ds(pl.multiple_of(
                n % rpb * 16, 16) + r * Q, 16), col(c)].astype(F32)

        def put(k, v):
            rs = pl.multiple_of(n * 8, 8)
            if ff:
                w49.at[k // 2][pl.ds(rs, 8), col(k % 2)] = _pk(v)
            else:
                dcs[pl.ds(rs + k // NCB * D, 8), col(k % NCB)] = (
                    pltpu.bitcast(v.astype(BF16), F32))

        return functools.partial(_ops2, load, put, _SB, _sb, k1)

    x_copy(0).wait()
    if W1A == 2:
        for cp in w1_copies(1):
            cp.start()
    lhs_b[...] = _ln(xin[0:T0, :].astype(F32)).astype(BF16)
    xs[0:T0, :] = xin[0:T0, :].astype(F32)

    def first_tile(c, carry):
        for cp in w1_copies(c):
            cp.wait()

        @pl.when(c == 1)
        def _():
            x_copy(1).wait()

        if XF:
            @pl.when(c % 2 == 0)
            def _():
                x_copy(1 + c // 2).start()

        @pl.when(c + W1A < nfc)
        def _():
            for cp in w1_copies(c + W1A):
                cp.start()

        if not XF:
            @pl.when(c % 2 == 0)
            def _():
                x_copy(1 + c // 2).start()

        n = -(-QA // (nfc - 1) // 16) * 16
        r0 = pl.multiple_of(jnp.clip((c - 1) * n, 0, QA - n), 16)
        assert n <= T0 // 4
        sched = _Sched(zero)
        dur = 2 * NCB * T0
        items = ln_in(xin, jnp.where(c > 0, T0, 0),
                      jnp.where(c > 0, QA, T0 // 4),
                      [r0 + r for r in range(0, n, 16)])
        sched.add(items[0], int(F_WIN[0] * dur), int(F_WIN[2] * dur))
        sched.add(items[1], int(F_WIN[2] * dur), int(F_WIN[1] * dur))
        sched.add([prep2(0, 0, (j * nfc + c) * (Q // 16) + r, k1)
                   for j in range(2) for r in range(Q // 16)
                   for k1 in range(7)],
                  int(F_WIN[0] * dur), int(F_WIN[1] * dur))
        f = _ffn(lhs_b[...], wblk.at[c], wblk.at[nfc + c], sched)
        assert not sched.queue
        xs[0:T0, :] += 0.5 * f
        return carry

    lax.fori_loop(0, nfc, first_tile, 0)
    for j in range(3, na + 1):
        x_copy(j).start()
    for c in range(nfc):
        for cp in w2_copies(c):
            cp.start()
    for cp in w_copies:
        cp.start()

    def phase_a(i, carry):
        @pl.when(i < na)
        def _():
            x_copy(i + 1).wait()

        @pl.when((i >= IW) & (i < IW + nfc))
        def _():
            for cp in w2_copies(i - IW):
                cp.wait()

        @pl.when(i == IW)
        def _():
            w_copies[0].wait()

        sched = _Sched(zero)
        dur = 49 * 2 * nfc * TA // 16
        base = jnp.maximum(T0 + (i - 2) * TA, 0)
        sched.add(ln_out(base, range(0, TA // 2, 16)),
                  int(L_WIN[0] * dur), int(L_WIN[1] * dur))
        base = T0 + jnp.minimum(i, na - 1) * TA
        items = ln_in(xin, base, QA, range(0, QA, 16))
        sched.add(items[0], int(A_WIN[0] * dur), int(A_WIN[1] * dur))
        sched.add(items[1], int(O_WIN[0] * dur), int(O_WIN[1] * dur))
        rpb = H // 16
        total = w7.shape[0] * rpb
        ipi = -(-total // (na - IW + 1))
        items = []
        for k in range(ipi):
            n = jnp.minimum(jnp.maximum(i - IW, 0) * ipi + k, total - 1)
            blk = (n // rpb + 2) % 3
            items.append(functools.partial(
                prep, wblk.at[blk + jnp.where(i >= IW, P1, 0)], w7.at[blk],
                pl.multiple_of(n % rpb * 16, 16)))
        assert ipi * (nfc - 1) <= rpb
        sched.add(items, int(P_WIN[0] * dur), int(P_WIN[1] * dur))
        total = w49.shape[1] // 8
        ipi = -(-total // (na - IW + 1))
        assert ipi <= Q // 16
        sched.add([prep2(
            1, jnp.where(i >= IW, 2 * nfc, 0),
            jnp.minimum(jnp.maximum(i - IW, 0) * ipi + k, total - 1), k1)
            for k in range(ipi) for k1 in range(7)],
            int(P_WIN[0] * dur), int(P_WIN[1] * dur))

        def h49(k):
            assert sched.now <= int(O_WIN[0] * dur) and A_WIN[1] <= O_WIN[0]
            return _up(lhs49[k // 2, :, col(k % 2)])

        f = _ffn49(
            h49, QA,
            lambda k, b, n: pltpu.bitcast(
                dcs[pl.ds(k // NCB * D + b * 64, n * 64), col(k % NCB)], BF16),
            nfc, sched, *FA, sb, GA)
        assert not sched.queue
        xs[arows(i), :] = xin[arows(i), :].astype(F32) + 0.5 * f
        return carry

    with jax.named_scope("phase_a"):
        lax.fori_loop(1, na + 1, phase_a, 0)

    for cp in w_copies[1:]:
        cp.wait()

    qk_scale = (D ** -0.5) * math.log2(math.e)

    HM = TM // 32 * 16

    def put7(dst, r0, cs, *p):
        if len(p) == 4:
            ops = enumerate(_sa(*p))
        else:
            ops = zip((1, 2, 3, 4), (p[0] + p[1], *p, p[0] + p[1]))
        for k, t in ops:
            dst[pl.ds(k * PR + r0 // 2, 8), cs] = pltpu.bitcast(
                t.astype(BF16), jnp.uint32)

    def get7(src, k, ds=pl.ds, nr=None):
        nr = nr or (TM - HM if 1 <= k <= 4 else HM)
        return pltpu.bitcast(src[ds(k * PR, nr // 2), :], BF16)

    def groups(r0):
        return (r0, HM + r0) if r0 < HM else (HM + r0,)

    def q_ops(i, r0, c, z):
        p = [hs[rows(i, r, 16), col(2 * h + c)].astype(F32)
             for r in groups(r0) for h in range(2)]
        p[0] = p[0] + _rep(z.v(), 16)
        p[-1] = p[-1] + _rep(z.v(), 16)
        put7(hq7, r0, col(c), *p)

    def q_items(i):
        return [functools.partial(q_ops, i, r0, c)
                for r0 in range(0, TM - HM, 16) for c in range(2)]

    sched = _Sched(zero)
    sched.add(ln_out(N - TA, range(0, TA // 2, 16)), *FD[:2])
    sched.add(q_items(0), *FD[2:])
    for dst in (mq, wvo):
        for u in range(2):
            t = []
            for cs in (col(u), col(u + 2)):
                t.append(_dot_nt(wq[...], wk[cs, :]) if dst is mq
                         else _dot(wv[...], wo[:, cs]))
                sched(t[-1])
            if dst is mq:
                t = [v * qk_scale for v in t]
            for k, v in enumerate(
                    _sb(t[0][:H], t[1][:H], t[0][H:], t[1][H:])):
                dst[k, :, col(u)] = _pk(v)
    assert not sched.queue
    dwf = dw[...].astype(F32)
    for k in range(K):
        dwb[k] = jnp.broadcast_to(dwf[k:k + 1, :], (8, D))

    def conv_block(p, r0, c, done, CT=CT, AT=K):
        cs = col(c)
        acc = [None]

        def item(k0, z=None):
            for k in range(k0, min(k0 + CT, K)):
                off = HALO - K // 2 + k + r0
                w = dwb[k, :, cs]
                if z is not None and k - k0 < AT:
                    w = w + z.v()
                t = gs[p + 1, c, off:off + 8, :] * w
                acc[0] = t if acc[0] is None else acc[0] + t
            if k0 + CT >= K:
                dcs[rows(p, r0, 8), cs] = acc[0]
                done(acc[0])

        return [functools.partial(item, k0) for k0 in range(0, K, CT)]

    def conv_main(p, cols=range(NCB), **kw):
        st = []

        def stats(r0, c, acc):
            if r0 == 0:
                st[:] = [acc, None, None]
                return
            shift, s1, s2 = st
            d = acc - shift
            s1 = d if s1 is None else s1 + d
            s2 = d * d if s2 is None else s2 + d * d
            st[:] = [shift, s1, s2]
            if r0 + 16 == TM:
                dm = s1 * (1.0 / (TM // 8 - 1))
                st_mean[p, :, col(c)] = shift + dm
                st_m2[p, :, col(c)] = s2 - s1 * dm

        return [it for c in cols for r0 in range(0, TM - 8, 8)
                for it in conv_block(p, r0, c,
                                     functools.partial(stats, r0, c), **kw)]

    def conv_edge(p, cols=range(NCB)):
        return [it for c in cols
                for it in conv_block(p, TM - 8, c, lambda acc: None)]


    def phase_b(i, carry):
        b = i // tpb

        sched = _Sched(zero)
        sched.add(conv_edge(jnp.maximum(i - 2, 0))
                  + conv_main(jnp.maximum(i - 1, 0), range(L0, NCB)),
                  int(B_SLOTS[0] * TM), int(B_SLOTS[1] * TM))
        sched.add(q_items(jnp.minimum(i + 1, nt - 1)),
                  int(Q_SLOTS[0] * TM), int(Q_SLOTS[1] * TM))
        acc = [None] * 4
        for k in OQ:
            t = _dot(get7(hq7, k), _up(mq[k]))
            _acc7(acc, k, t, HM)
            sched(t)
        q11, q12, q21, q22 = _quads(
            jnp.concatenate(_join(acc, HM), axis=1), HM)
        q7 = [q11[:HM] - q22[:HM], q21 - q22, q11, q22, q12 - q11,
              q21[:HM] - q11[:HM], q12[:HM] - q22[:HM]]
        q7 = [t.astype(BF16) for t in q7]

        dz = zero_s[0]
        p_buf, al_buf = (p_buf0, p_buf1, p_buf2), (al_buf0, al_buf1, al_buf2)
        s_buf = (s_buf0, s_buf1)

        def dyn(r0, n):
            return pl.ds(pl.multiple_of(dz + r0, 8), n)

        nb = KP // 128

        def chunk(j):
            return pl.ds(pl.multiple_of(b * (TP // 2), KP // 2)
                         + j * KP // 2, KP // 2)

        def combine(m, j, c):
            if len(m) == 7:
                s = [m[0] + m[3] + m[4] + m[6], m[2] + m[4],
                     m[1] + m[3], m[1] - m[0] + m[2] + m[5]]
            else:
                s = [m[0] + m[2], m[1] + m[3]]
            nv = T // 2 - j * KP - c * 128
            if nv < 128:
                lane = lax.broadcasted_iota(jnp.int32, s[0].shape, 1)
                s = [jnp.where(lane < nv, t, -jnp.inf) for t in s]
            return s

        stat = {}

        def put(w, j, r, v):
            for r0 in range(0, v.shape[0], 16):
                stat[w, j, r + r0] = v[r0:r0 + 16]

        def get(w, j, r, n=16):
            return jnp.concatenate(
                [stat[w, j, r0] for r0 in range(r, r + n, 16)], axis=0)

        def scores(j):
            m = [None] * 7
            for k in OS if j else OS0:
                m[k] = _dot_nt(
                    q7[k], _up(ks[(0, 2, 1, 4, 3, 5, 6)[k], chunk(j), :]))
                sched(m[k])
            mx = None
            for c in range(nb):
                s = combine([t[:HM, col(c)] for t in m], j, c)
                e = combine([t[HM:, col(c)] for t in m[1:5]], j, c)
                for h in range(2):
                    t = jnp.concatenate([s[h], s[2 + h], e[h]], axis=0)
                    s_buf[j % 2][:, col(h * nb + c)] = t
                    mx = t if mx is None else jnp.maximum(mx, t)
            mx = jnp.broadcast_to(jnp.max(mx, axis=-1, keepdims=True),
                                  mx.shape)
            if j:
                mx = jnp.maximum(mx, get(0, j - 1, 0, TM))
            put(0, j, 0, mx)

        part = {}

        def soft1(j, r, c0, z):
            rs = slice(r, r + 16)
            m = get(0, j, r) + _rep(z.v(), 16)
            l = functools.reduce(jnp.add, part.pop((j, r), []) + [
                jnp.exp2(s_buf[j % 2][dyn(r, 16), col(c)] - m)
                for c in range(c0, c0 + S1)])
            if c0 + S1 < 2 * nb:
                part[j, r] = [l]
                return
            l = jnp.broadcast_to(jnp.sum(l, axis=-1, keepdims=True),
                                 (16, 128))
            if j:
                l += get(1, j - 1, r) * jnp.exp2(get(0, j - 1, r) - m)
            put(1, j, r, l)
            e = (pltpu.bitcast(l, jnp.int32) >> 23) - 127
            ref = m + e.astype(F32)
            put(2, j, r, ref)
            if j:
                al_buf[j % 3][rs, :] = jnp.exp2(get(2, j - 1, r) - ref)

        def soft2(j, r0, c0, z):
            ref = [get(2, j, r) + _rep(z.v(), 16) for r in groups(r0)]
            p = [jnp.concatenate(
                [jnp.exp2(s_buf[j % 2][dyn(r, 16), col(h * nb + c)] - m)
                 for c in range(c0, c0 + S2)], axis=1)
                 for r, m in zip(groups(r0), ref) for h in range(2)]
            put7(p_buf[j % 3], r0, slice(c0 * 128, (c0 + S2) * 128), *p)

        scd = 7 * HM + 4 * (TM - 2 * HM)
        start = sched.now

        def add_soft(j):
            rbs = range(0, TM - HM, 16)
            t0, t1 = (start + int(t * scd) for t in SW[j:j + 2])
            assert t1 <= start + min(2 * j + LAG + 1, nkc + j) * scd
            assert j < 3 or t0 >= start + min(2 * j + LAG - 4,
                                              nkc + j - 2) * scd
            assert (j + 2 >= nkc
                    or t1 <= start + max(2 * j + 5 - LAG, j + 3) * scd)
            u = (t1 - t0 - sum(SD)) // (len(rbs) + 1)
            for n, r0 in enumerate(rbs):
                its = [[functools.partial(soft1, j, r, c)
                        for r in groups(r0) for c in range(0, 2 * nb, S1)],
                       [functools.partial(soft2, j, r0, c)
                        for c in range(0, nb, S2)]]
                for k, it in enumerate(its):
                    t = t0 + SD[0] + n * u + k * (u + SD[1])
                    sched.add(it, t, t + u)

        for j in range(LAG):
            scores(j)
            add_soft(j)
        acc = [None] * 4
        for j in range(nkc):
            if j + LAG < nkc:
                scores(j + LAG)
                add_soft(j + LAG)
            fresh = [j > 0] * 4
            for k in OP if j + 1 < nkc else OQ:
                w = _up(ks[(0, 2, 6, 5, 3, 4, 1)[k], chunk(j), :])
                m = _dot(get7(p_buf[j % 3], k, dyn), w)
                sched(m)
                for a, _ in _TG[k]:
                    if fresh[a]:
                        al = al_buf[j % 3][dyn(0, TM), :]
                        al = _quads(jnp.concatenate([al] * NCB, axis=1), HM)[a]
                        acc[a] = acc[a] * al[:acc[a].shape[0]]
                        fresh[a] = False
                _acc7(acc, k, m, HM)
        assert not sched.queue
        t = jnp.exp2(get(2, nkc - 1, 0, TM) - get(0, nkc - 1, 0, TM))
        t = t / get(1, nkc - 1, 0, TM)
        o = (jnp.concatenate(_join(acc, HM), axis=1)
             * jnp.concatenate([t] * NCB, axis=1))
        o7 = [t.astype(BF16) for t in _sax(*_quads(o, HM), HM)]
        acc = list(_quads(xs[rows(i), :], HM))
        acc = [acc[0][:HM], acc[1], acc[2], acc[3][:HM]]
        for k in OW:
            _acc7(acc, k, _dot(o7[k], _up(wvo[k])), HM)
        x2 = jnp.concatenate(_join(acc, HM), axis=1)
        xs[rows(i), :] = x2
        h7 = [t.astype(BF16) for t in _sax(*_quads(_ln(x2), HM), HM)]
        sched = _Sched(zero)
        acc = [[None] * 4 for _ in range(2)]
        for n, (h, k) in enumerate(PO):
            t = _dot(h7[k], _up(w7[h, k]))
            _acc7(acc[h], k, t, HM)
            sched(t)
            if any(e[0] == h for e in PO[n + 1:]):
                continue
            val, gate = _join(acc[h], HM)
            g2 = val * (0.5 + 0.5 * jnp.tanh(0.5 * gate))
            for c in (2 * h, 2 * h + 1):
                g = g2[:, col(c % 2)]
                gs[i + 1, c, HALO:HALO + TM, :] = g
                gs[i, c, HALO + TM:, :] = jnp.where(
                    i % tpb == 0, 0.0, g[:HALO])
                gs[i + 2, c, :HALO, :] = jnp.where(
                    i % tpb == tpb - 1, 0.0, g[TM - HALO:])
            if h == 0 and L0:
                rest = sum(h7[e[1]].shape[0] for e in PO[n + 1:])
                sched.add(conv_main(i, range(L0), CT=LP[2], AT=LP[3]),
                          sched.now + LP[0], sched.now + rest - LP[1])
        assert not sched.queue
        return carry

    with jax.named_scope("phase_b"):
        lax.fori_loop(0, nt, phase_b, 0)
    for item in (conv_main(nt - 1, range(L0, NCB)) + conv_edge(nt - 2)
                 + conv_edge(nt - 1)):
        item()

    ng = TM // 8 - 1
    means = st_mean[...].reshape(nt * 8, D)
    edges = jnp.concatenate([dcs[(p + 1) * TM - 8:(p + 1) * TM, :]
                             for p in range(nt)], axis=0)
    mu = jnp.sum(ng * means + edges, axis=0, keepdims=True) * (1.0 / N)
    dm = means - mu
    de = edges - mu
    var = jnp.sum(st_m2[...].reshape(nt * 8, D) + ng * (dm * dm) + de * de,
                  axis=0, keepdims=True) * (1.0 / N)
    rstd = lax.rsqrt(var + EPS)
    bn[0] = jnp.broadcast_to(mu, (8, D))
    bn[1] = jnp.broadcast_to(rstd, (8, D))

    def bn_silu(i, r0, c, z=None):
        p = []
        for r in (r0, TC // 2 + r0):
            for h in range(2):
                cs = col(2 * h + c)
                mu = bn[0, :, cs] if z is None else bn[0, :, cs] + z.v()
                y = dcs[crows(i, r, 16), cs] - _rep(mu, 16)
                p.append(_silu(y * _rep(bn[1, :, cs], 16)))
        put7(hq7, r0, col(c), *p)

    def bn_items(i):
        return [functools.partial(bn_silu, i, r0, c)
                for r0 in range(0, TC // 2, 16) for c in range(2)]

    def ln_final(i, r0=0, n=TC, z=None):
        obuf[crows(i, r0, n), :] = _ln(xs[crows(i, r0, n), :],
                                       zrep(z, n)).astype(BF16)

    for item in bn_items(0):
        item()

    QC = TC // 4

    def pw2(src, dst, sched, win):
        acc = list(_quads(xs[crows(src), :], TC // 2))
        for k in OQ:
            t = _dot(get7(hq7, k, nr=TC // 2), _up(w7[2, k]))
            _acc7(acc, k, t, TC // 2)
            sched(t)
        xs[crows(dst), :] = jnp.concatenate(_join(acc, TC // 2), axis=1)
        for items, t0, t1 in zip(
                ln_in(xs, dst * TC, QC, range(0, QC, 16)), win, win[1:]):
            sched.add(items, sched.now + t0, sched.now + t1)

    sched = _Sched(zero)
    pw2(0, 0, sched, (0, 1, 2))
    sched.force([e[1] for e in sched.queue])

    def phase_c(i, carry):
        @pl.when(i >= 2)
        def _():
            o_copy(i - 2).start()

        sched = _Sched(zero)
        dur = (7 * 8 + 49 * 2 * nfc) * TC // 16
        sched.add([functools.partial(ln_final, jnp.maximum(i - 1, 0), r, RC)
                   for r in range(0, TC, RC)],
                  int(C_WIN[0] * dur), int(C_WIN[1] * dur))
        nxt = jnp.minimum(i + 1, nc - 1)
        items = bn_items(nxt)
        sched.add(items, int(C_WIN[2] * dur), int(C_WIN[3] * dur))
        done = []

        def mid():
            sched.force(items)
            done.append(1)
            pw2(nxt, jnp.where(i + 1 < nc, i + 1, 0), sched, M_WIN)

        def h49(k):
            assert not done
            return _up(lhs49[k // 2, :QC // 2, col(k % 2)])

        f = _ffn49(h49, QC, lambda k, b, n: _up(
            w49[k // 2, b * 64:(b + n) * 64, col(k % 2)]),
            nfc, sched, *FB, sb, GC, mid)
        assert not sched.queue
        xs[crows(i), :] += 0.5 * f
        return carry

    with jax.named_scope("phase_c"):
        lax.fori_loop(0, nc, phase_c, 0)
    o_copy(nc - 2).start()
    last = []
    for k, (r0, r1) in enumerate(zip(EP[:-1], EP[1:])):
        ln_final(nc - 1, r0, r1 - r0)
        rs = crows(nc - 1, r0, r1 - r0)
        last.append(pltpu.make_async_copy(obuf.at[rs, :], out_hbm.at[rs, :],
                                          osem.at[nc - 1 + k]))
        last[-1].start()
    for i in range(nc - 1):
        o_copy(i).wait()
    for cp in last:
        cp.wait()


@jax.jit
def pallas_standalone__conformer_family_conformer__speech_kernel(
    x: jax.Array,
    w_ff1_a: jax.Array,
    w_ff1_b: jax.Array,
    w_q: jax.Array,
    w_k: jax.Array,
    w_v: jax.Array,
    w_o: jax.Array,
    w_pw1: jax.Array,
    dw: jax.Array,
    w_pw2: jax.Array,
    w_ff2_a: jax.Array,
    w_ff2_b: jax.Array,
):
    B, T, D = x.shape
    K = dw.shape[0]
    N = B * T
    weights = (w_ff1_a, w_ff1_b, w_q, w_k, w_v, w_o, w_pw1, dw, w_pw2,
               w_ff2_a, w_ff2_b)
    scratch = [pltpu.VMEM((N, D), BF16)]
    nfc = w_ff1_a.shape[1] // FC
    scratch += [pltpu.VMEM((4 * nfc + 3, D, D), BF16)]
    scratch += [pltpu.VMEM(w.shape, w.dtype)
                for w in (w_q, w_k, w_v, w_o, dw)]
    scratch += [
        pltpu.VMEM((7, D // 4, D // 2), jnp.uint32),
        pltpu.VMEM((7, D // 4, D // 2), jnp.uint32),
        pltpu.VMEM((N, D), F32),
        pltpu.VMEM((N, D), BF16),
        pltpu.VMEM((7, B * -(-T // KC) * KC // 4, D // 2), jnp.uint32),
        pltpu.VMEM((N // TM + 2, D // 128, TM + 2 * HALO, 128), F32),
        pltpu.VMEM((N, D), F32),
        pltpu.VMEM((N // TM, 8, D), F32),
        pltpu.VMEM((N // TM, 8, D), F32),
        pltpu.VMEM((2, 8, D), F32),
        pltpu.VMEM((25, TA // 8, D // 2), jnp.uint32),
        pltpu.VMEM((7, 14 * TA // 8, D // 2), jnp.uint32),
        pltpu.VMEM((3, 7, D // 4, D // 2), jnp.uint32),
        pltpu.VMEM((25, nfc * D // 4, D // 2), jnp.uint32),
        pltpu.VMEM((T0, D), BF16),
        pltpu.VMEM((K, 8, D), F32),
        pltpu.VMEM((ZR, 128), jnp.uint32),
        pltpu.SMEM((1,), jnp.int32),
        pltpu.VMEM((TM + 16, 128), F32),
        pltpu.VMEM((TM + 16, 128), F32),
        pltpu.VMEM((TM + 16, 128), F32),
        pltpu.VMEM((7 * PR, KC // 2), jnp.uint32),
        pltpu.VMEM((7 * PR, KC // 2), jnp.uint32),
        pltpu.VMEM((7 * PR, KC // 2), jnp.uint32),
        pltpu.VMEM((TM, KC), F32),
        pltpu.VMEM((TM, KC), F32),
        pltpu.VMEM((7 * PR, D // 2), jnp.uint32),
        pltpu.SemaphoreType.DMA(((N - T0) // TA + 1,)),
        pltpu.SemaphoreType.DMA((2, nfc)),
        pltpu.SemaphoreType.DMA((3, nfc)),
        pltpu.SemaphoreType.DMA((6,)),
        pltpu.SemaphoreType.DMA((N // TC + len(EP),)),
    ]
    out = pl.pallas_call(
        functools.partial(_kernel, B=B, T=T, D=D, K=K),
        out_shape=jax.ShapeDtypeStruct((N, D), x.dtype),
        in_specs=[pl.BlockSpec(memory_space=pl.ANY)] * 12,
        out_specs=pl.BlockSpec(memory_space=pl.ANY),
        scratch_shapes=scratch,
        compiler_params=pltpu.CompilerParams(
            vmem_limit_bytes=VL * 1024 * 1024),
    )(x.reshape(N, D), *weights)
    return out.reshape(B, T, D)
```

```python
import functools
import math

import jax
import jax.numpy as jnp
from jax import lax
import jax.experimental.pallas as pl
import jax.experimental.pallas.tpu as pltpu

F32 = jnp.float32
BF16 = jnp.bfloat16

TM = 400
T0 = 320
TA = 512
TC = 320
FC = 512
KC = 512
IW = 3
GA = (42, 60, 16)
GC = (42, 90, 16)
KO = 2
O_WIN = (0.75, 0.97)
L_WIN = (0.0, 0.12)
PL = ((0, 0, 49), (0, 1, 49), (0, 2, 49), (0, 3, 49), (1, 0, 49), (1, 1, 49))
FA = (((2, 4, 3, 1, 0, 6, 5), (2, 4, 3, 1, 0, 6, 5)),
      ((2, 4, 5, 3, 1, 6, 0), (2, 4, 3, 1, 0, 6, 5)), PL)
FB = (((2, 4, 3, 1, 0, 6, 5), (2, 4, 3, 1, 0, 6, 5)),
      ((2, 4, 5, 3, 1, 6, 0), (2, 4, 3, 1, 0, 6, 5)),
      PL[:4] + ((1, 0, 35), (2, 0, 0), (1, 0, 14), (1, 1, 49)))
P_WIN = (0.5, 0.97)
OQ = (0, 2, 3, 4, 6, 1, 5)
OS0 = (2, 4, 3, 1, 0, 5, 6)
OS = (0, 1, 2, 3, 4, 5, 6)
OP = (0, 1, 2, 3, 4, 5, 6)
OW = (2, 4, 3, 0, 6, 1, 5)
PO = ((0, 2), (0, 4), (1, 2), (0, 3), (0, 0), (0, 6), (0, 1), (0, 5),
      (1, 4), (1, 3), (1, 0), (1, 6), (1, 1), (1, 5))
F_WIN = (0.02, 0.95, 0.5)
A_WIN = (0.5, 0.75)
FD = (0, 3200, 0, 3200)
B_SLOTS = (1, 53)
Q_SLOTS = (8, 50)
CT = 5
L0 = 1
LP = (0, 100, 3, 1)
S1 = 2
S2 = 1
SD = (0, 140, 120)
LAG = 2
SW = tuple(1 + 1.75 * j for j in range(9))
C_WIN = (0.02, 0.5, 0.3, 0.58)
M_WIN = (60, 1200, 2400)
RC = 8
EP = (0, 128, 224, 288, 320)
ZR = 32
PR = 112
HALO = 8
EPS = 1e-05


def _ln(x, z=None):
    if z is None:
        m = jnp.mean(x, axis=-1, keepdims=True)
    else:
        t = z
        for c in range(x.shape[-1] // 128):
            t = t + x[:, c * 128:(c + 1) * 128]
        m = jnp.sum(t, axis=-1, keepdims=True) * (1.0 / x.shape[-1])
    xc = x - m
    v = jnp.mean(xc * xc, axis=-1, keepdims=True)
    return xc * lax.rsqrt(v + EPS)


def _silu(a):
    y = 0.5 * a
    return y + y * jnp.tanh(y)


def _dot(a, b):
    return jnp.dot(a, b, preferred_element_type=F32)


def _dot_nt(a, b):
    return lax.dot_general(a, b, (((1,), (1,)), ((), ())),
                           preferred_element_type=F32)


def _pk(v):
    return pltpu.bitcast(v.astype(BF16), jnp.uint32)


def _up(v):
    return pltpu.bitcast(v, BF16)


class _Anchor:
    def __init__(self, t, zero_v):
        self.t, self.zero_v = t, zero_v

    def v(self):
        return pltpu.bitcast(
            pltpu.bitcast(self.t, jnp.uint32) & self.zero_v[0:8, :], F32)


class _Sched:
    def __init__(self, zero_v):
        self.zero_v = zero_v
        self.queue = []
        self.now = 0

    def add(self, items, t0, t1, skip=()):
        assert t0 >= self.now
        ts = [t for t in range(t0, t1)
              if not any(a <= t < b for a, b in skip)]
        self.queue += [(ts[k * len(ts) // len(items)], it)
                       for k, it in enumerate(items)]
        self.queue.sort(key=lambda e: e[0])

    def __call__(self, t, dur=None):
        dur = dur or t.shape[0]
        end = self.now + dur
        while self.queue and self.queue[0][0] < end:
            time, item = self.queue.pop(0)
            r = (time - self.now) * t.shape[0] // dur // 8 * 8
            item(_Anchor(t[r:r + 8, :128], self.zero_v))
        self.now = end
        self.last = t

    def force(self, items):
        for e in [e for e in self.queue if e[1] in items]:
            self.queue.remove(e)
            e[1](_Anchor(self.last[-8:, :128], self.zero_v))


def _rep(z, rows):
    return jnp.concatenate([z] * (rows // 8), axis=0)


def _ffn(h, wa_ref, wb_ref, sched):
    ss = []
    for n in range(wa_ref.shape[1] // 128):
        a = _dot(h, wa_ref[:, n * 128:(n + 1) * 128])
        ss.append(_silu(a))
        sched(a)
    s = jnp.concatenate(ss, axis=1).astype(BF16)
    acc = []
    for n in range(wb_ref.shape[1] // 128):
        acc.append(_dot(s, wb_ref[:, n * 128:(n + 1) * 128]))
        sched(acc[-1])
    return jnp.concatenate(acc, axis=1)


def _sa(a11, a12, a21, a22):
    return [a11 + a22, a21 + a22, a11, a22, a11 + a12, a21 - a11, a12 - a22]


def _sb(b11, b12, b21, b22):
    return [b11 + b22, b11, b12 - b22, b21 - b11, b22, b11 + b12, b21 + b22]


def _lhs7(t, u):
    h = t.shape[1] // 2
    return [v.astype(BF16)
            for v in _sa(t[:, :h], t[:, h:], u[:, :h], u[:, h:])]


_SA = ((0, 1, 3), (2, 1, 3), (0, 0, 0), (3, 0, 3), (0, 1, 1), (2, -1, 0),
       (1, -1, 3))
_SB = ((0, 1, 3), (0, 0, 0), (1, -1, 3), (2, -1, 0), (3, 0, 3), (0, 1, 1),
       (2, 1, 3))
_TG = (((0, 1), (3, 1)), ((2, 1), (3, -1)), ((1, 1), (3, 1)), ((0, 1), (2, 1)),
       ((0, -1), (1, 1)), ((3, 1),), ((0, 1),))


def _quads(x, hm):
    h = x.shape[1] // 2
    t = x[:hm]
    if x.shape[0] > 2 * hm:
        t = jnp.concatenate([t, x[2 * hm:]], axis=0)
    return t[:, :h], t[:, h:], x[hm:, :h], x[hm:, h:]


def _sax(a11, a12, a21, a22, hm):
    return [a11[:hm] + a22[:hm], a21 + a22, a11, a22, a11 + a12,
            a21[:hm] - a11[:hm], a12[:hm] - a22[:hm]]


def _acc7(acc, k, m, hm):
    for a, sg in _TG[k]:
        t = m if a in (1, 2) else m[:hm]
        if acc[a] is None:
            acc[a] = t if sg > 0 else -t
        else:
            acc[a] = acc[a] + t if sg > 0 else acc[a] - t


def _join(acc, hm):
    rest = [acc[1][hm:]] if acc[1].shape[0] > hm else []
    return (jnp.concatenate([acc[0], acc[2]], axis=0),
            jnp.concatenate([acc[1][:hm], acc[3]] + rest, axis=0))


def _pm(a, sg, b):
    return a if not sg else a + b if sg > 0 else a - b


def _ops2(load, put, tab, f, k1, z):
    def quad(a):
        return [load(a // 2 * 2 + j // 2, a % 2 * 2 + j % 2) for j in range(4)]

    a, sg, b = tab[k1]
    y = [_pm(u + _rep(z.v(), 16), sg, v) for u, v in zip(quad(a), quad(b))]
    for k2, v in enumerate(f(*y)):
        put(7 * k1 + k2, v)


def _ffn49(h49, hm, w, nfc, sched, oi, oo, plan, sb, gap, mid=None):
    src = [[n for n in range(7) if a in [e[0] for e in _TG[n]]]
           for a in range(4)]
    val = {}

    def add(key, sg, t):
        if key not in val:
            val[key] = t if sg > 0 else -t
        else:
            val[key] = _pm(val[key], sg, t)

    def collect(done, tag, k1, k2, t):
        done.add((k1, k2))
        for b, sg in _TG[k2]:
            add((tag, 'm', k1, b), sg, t)
            if all((k1, n) in done for n in src[b]):
                for a, sg1 in _TG[k1]:
                    add((tag, 'u', a, b), sg1, val[tag, 'm', k1, b])

    done = [set() for _ in range(nfc + 1)]

    pend, free = {}, [0]

    def ops(c, n, r, z):
        a, sg, a2 = _SA[n]
        rs = slice(r, r + gap[2])
        y = [_pm(val[c, 'a', a, b][rs] + _rep(z.v(), gap[2]), sg,
                 val[c, 'a', a2, b][rs]) for b in range(4)]
        for m, v in enumerate(_sa(*y)):
            sb.at[n][pl.ds(((c // KO * 7 + m) * hm + r) // 2, gap[2] // 2),
                     pl.ds(c % KO * 128, 128)] = _pk(v)

    def step_in(c, k1, k2):
        t = _dot(h49(7 * k1 + k2), w(7 * k1 + k2, c, 1))
        collect(done[c], c, k1, k2, t)
        sched(t, hm // 4)
        for a in range(4):
            for b in range(4):
                if (c, 'a', a, b) not in val and all(
                        (m, n) in done[c] for m in src[a] for n in src[b]):
                    val[c, 'a', a, b] = _silu(val[c, 'u', a, b])
        for n in oo[0]:
            if (c, n) not in pend and all(
                    (c, 'a', a, b) in val
                    for a in _SA[n][::2] for b in range(4)):
                pend[c, n] = [functools.partial(ops, c, n, r)
                              for r in range(0, hm, gap[2])]
                for e in pend[c, n]:
                    free[0] = max(free[0] + gap[0], sched.now + gap[1])
                    sched.add([e], free[0], free[0] + 1)

    def step_out(g, k1, k2):
        cs = range(g * KO, (g + 1) * KO)
        sched.force([e for c in cs for e in pend[c, k1]])
        v = _up(sb[k1, pl.ds((g * 7 + k2) * hm // 2, hm // 2), :])
        t = _dot(v, w(7 * k1 + k2, nfc + g * KO, KO))
        sched(t, hm * KO // 4)
        add(('p', k1, k2), 1, t)
        if (g + 1) * KO == nfc:
            collect(done[-1], 'o', k1, k2, val['p', k1, k2])

    todo = {(d, c): [(k1, k2) for k1 in o[0] for k2 in o[1]]
            for d, o in enumerate((oi, oo)) for c in range(nfc)}
    for d, c, n in plan:
        if d == 2:
            mid()
            continue
        for k1, k2 in todo[d, c][:n]:
            (step_out if d else step_in)(c, k1, k2)
        del todo[d, c][:n]
    return jnp.concatenate(
        [jnp.concatenate([val['o', 'u', a // 2 * 2 + b // 2, a % 2 * 2 + b % 2]
                          for b in range(4)], axis=1) for a in range(4)],
        axis=0)


def _kernel(x_hbm, w1a_hbm, w1b_hbm, wq_hbm, wk_hbm, wv_hbm, wo_hbm,
            wp1_hbm, dw_hbm, wp2_hbm, w2a_hbm, w2b_hbm,
            out_hbm,
            xin, wblk, wq, wk, wv, wo, dw,
            mq, wvo, xs, hs, ks, gs, dcs, st_mean, st_m2, bn,
            lhs49, sb, w7, w49, lhs_b, dwb, zero, zero_s,
            al_buf0, al_buf1, al_buf2,
            p_buf0, p_buf1, p_buf2, s_buf0, s_buf1, hq7,
            xsem, w1sem, w2sem, wsem, osem,
            *, B, T, D, K):
    N = B * T
    obuf = xin
    KP = KC // 2
    nkc = -(-T // KC)
    TP = nkc * KP
    NCB = D // 128
    nt = N // TM
    tpb = T // TM

    def rows(i, r0=0, n=TM):
        return pl.ds(pl.multiple_of(i * TM, 16) + r0, n)

    def col(c):
        if isinstance(c, int):
            return slice(c * 128, (c + 1) * 128)
        return pl.ds(pl.multiple_of(c * 128, 128), 128)

    na = (N - T0) // TA
    H = D // 2
    QA = TA // 4
    s_buf = (s_buf0, s_buf1)

    def arows(i, r0=0, n=TA):
        return pl.ds(pl.multiple_of(T0 + (i - 1) * TA, 16) + r0, n)

    def x_copy(i):
        rs = pl.ds(0, T0) if isinstance(i, int) and i == 0 else arows(i)
        return pltpu.make_async_copy(x_hbm.at[rs, :], xin.at[rs, :],
                                     xsem.at[i])

    nc = N // TC

    def crows(i, r0=0, n=TC):
        return pl.ds(pl.multiple_of(i * TC, 16) + r0, n)

    def o_copy(i):
        return pltpu.make_async_copy(obuf.at[crows(i), :],
                                     out_hbm.at[crows(i), :], osem.at[i])

    nfc = w49.shape[1] // (D // 4)
    P1, P2 = 4 * nfc, 4 * nfc + 2

    def w1_copies(c):
        fs = pl.ds(pl.multiple_of(c * FC, FC), FC)
        return [pltpu.make_async_copy(w1a_hbm.at[:, fs], wblk.at[c],
                                      w1sem.at[0, c]),
                pltpu.make_async_copy(w1b_hbm.at[fs, :], wblk.at[nfc + c],
                                      w1sem.at[1, c])]

    def w2_copies(c):
        fs = pl.ds(pl.multiple_of(c * FC, FC), FC)
        hs_ = pl.ds(pl.multiple_of(c // 2 * H, H), H)
        return [pltpu.make_async_copy(s, d, w2sem.at[j, c])
                for j, (s, d) in enumerate([
                    (w2a_hbm.at[:, fs], wblk.at[2 * nfc + c]),
                    (w2b_hbm.at[fs, :], wblk.at[3 * nfc + c]),
                    (wp1_hbm.at[:, pl.ds(pl.multiple_of(c * H, H), H)],
                     wblk.at[P1 + c % 2, :, hs_])])]

    assert nfc == 4
    w_pairs = [(wp2_hbm, wblk.at[P2]), (wq_hbm, wq), (wk_hbm, wk),
               (wv_hbm, wv), (wo_hbm, wo), (dw_hbm, dw)]
    w_copies = [pltpu.make_async_copy(s, d, wsem.at[j])
                for j, (s, d) in enumerate(w_pairs)]

    x_copy(0).start()
    for cp in w1_copies(0):
        cp.start()

    zero[...] = jnp.zeros(zero.shape, jnp.uint32)
    zero_s[0] = 0
    for c in range(NCB):
        gs[1, c, 0:HALO, :] = jnp.zeros((HALO, 128), F32)
        gs[nt, c, HALO + TM:, :] = jnp.zeros((HALO, 128), F32)
    for b in range(B):
        ks[:, (b * TP + T // 2) // 2:(b + 1) * TP // 2, :] = jnp.zeros(
            (7, (TP - T // 2) // 2, H), jnp.uint32)

    def zrep(z, n):
        return None if z is None else _rep(z.v(), n)

    def pair_items(first, second, rows0):
        items = []
        for r0 in rows0:
            t = []
            items += [functools.partial(first, t, r0),
                      functools.partial(second, t, r0)]
        return items

    def ln_in(src, base, quarter, rows0):
        zs = zero_s[0]

        def ln(r0, j, z):
            s_buf[j // 2][pl.ds(j % 2 * QA + r0, 16), :] = _ln(
                src[pl.ds(pl.multiple_of(base + j * quarter, 16) + r0, 16), :]
                .astype(F32), zrep(z, 16))

        def ops(r0, k1):
            def load(j, c):
                return s_buf[j // 2][pl.ds(
                    pl.multiple_of(zs + r0, 16) + j % 2 * QA, 16), col(c)]

            def put(k, v):
                lhs49.at[k // 2][pl.ds(pl.multiple_of(r0 // 2, 8), 8),
                                 col(k % 2)] = _pk(v)

            return functools.partial(_ops2, load, put, _SA, _sa, k1)

        return ([functools.partial(ln, r0, j)
                 for r0 in rows0 for j in range(4)],
                [ops(r0, k1) for r0 in rows0 for k1 in range(7)])

    def ln_out(base, rows0):
        def first(t, r0, z, off=0):
            rs = pl.ds(pl.multiple_of(base, 32) + 2 * r0 + off, 16)
            t.append(_ln(xs[rs, :], zrep(z, 16)))
            hs[rs, :] = t[-1].astype(BF16)

        def second(t, r0, z):
            first(t, r0, z, 16)
            g = base // 32 + r0 // 16
            g += g // (T // 32) * ((TP - T // 2) // 16)
            for k, v in enumerate(_lhs7(*t)):
                ks.at[k][pl.ds(pl.multiple_of(g * 8, 8), 8), :] = _pk(v)

        return pair_items(first, second, rows0)

    def prep(src, dst, r0, z=None):
        q = [src[pl.ds(r + r0, 16), c:c + H].astype(F32)
             for r in (0, H) for c in (0, H)]
        if z is not None:
            zz = jnp.concatenate([_rep(z.v(), 16)] * (H // 128), axis=1)
            q[0], q[3] = q[0] + zz, q[3] + zz
        r1 = r0 // 2 if isinstance(r0, int) else pl.multiple_of(r0 // 2, 8)
        for k, v in enumerate(_sb(*q)):
            dst.at[k][pl.ds(r1, 8), :] = _pk(v)

    Q = D // 4

    def prep2(ff, blk, n, k1):
        rpb = Q // 16

        def load(r, c):
            return wblk[blk + n // rpb, pl.ds(pl.multiple_of(
                n % rpb * 16, 16) + r * Q, 16), col(c)].astype(F32)

        def put(k, v):
            rs = pl.multiple_of(n * 8, 8)
            if ff:
                w49.at[k // 2][pl.ds(rs, 8), col(k % 2)] = _pk(v)
            else:
                dcs[pl.ds(rs + k // NCB * D, 8), col(k % NCB)] = (
                    pltpu.bitcast(v.astype(BF16), F32))

        return functools.partial(_ops2, load, put, _SB, _sb, k1)

    x_copy(0).wait()
    lhs_b[...] = _ln(xin[0:T0, :].astype(F32)).astype(BF16)
    xs[0:T0, :] = xin[0:T0, :].astype(F32)

    def first_tile(c, carry):
        for cp in w1_copies(c):
            cp.wait()

        @pl.when(c == 1)
        def _():
            x_copy(1).wait()

        @pl.when(c + 1 < nfc)
        def _():
            for cp in w1_copies(c + 1):
                cp.start()

        @pl.when(c % 2 == 0)
        def _():
            x_copy(1 + c // 2).start()

        n = -(-QA // (nfc - 1) // 16) * 16
        r0 = pl.multiple_of(jnp.clip((c - 1) * n, 0, QA - n), 16)
        assert n <= T0 // 4
        sched = _Sched(zero)
        dur = 2 * NCB * T0
        items = ln_in(xin, jnp.where(c > 0, T0, 0),
                      jnp.where(c > 0, QA, T0 // 4),
                      [r0 + r for r in range(0, n, 16)])
        sched.add(items[0], int(F_WIN[0] * dur), int(F_WIN[2] * dur))
        sched.add(items[1], int(F_WIN[2] * dur), int(F_WIN[1] * dur))
        sched.add([prep2(0, 0, (j * nfc + c) * (Q // 16) + r, k1)
                   for j in range(2) for r in range(Q // 16)
                   for k1 in range(7)],
                  int(F_WIN[0] * dur), int(F_WIN[1] * dur))
        f = _ffn(lhs_b[...], wblk.at[c], wblk.at[nfc + c], sched)
        assert not sched.queue
        xs[0:T0, :] += 0.5 * f
        return carry

    lax.fori_loop(0, nfc, first_tile, 0)
    for j in range(3, na + 1):
        x_copy(j).start()
    for c in range(nfc):
        for cp in w2_copies(c):
            cp.start()
    for cp in w_copies:
        cp.start()

    def phase_a(i, carry):
        @pl.when(i < na)
        def _():
            x_copy(i + 1).wait()

        @pl.when((i >= IW) & (i < IW + nfc))
        def _():
            for cp in w2_copies(i - IW):
                cp.wait()

        @pl.when(i == IW)
        def _():
            w_copies[0].wait()

        sched = _Sched(zero)
        dur = 49 * 2 * nfc * TA // 16
        base = jnp.maximum(T0 + (i - 2) * TA, 0)
        sched.add(ln_out(base, range(0, TA // 2, 16)),
                  int(L_WIN[0] * dur), int(L_WIN[1] * dur))
        base = T0 + jnp.minimum(i, na - 1) * TA
        items = ln_in(xin, base, QA, range(0, QA, 16))
        sched.add(items[0], int(A_WIN[0] * dur), int(A_WIN[1] * dur))
        sched.add(items[1], int(O_WIN[0] * dur), int(O_WIN[1] * dur))
        rpb = H // 16
        total = w7.shape[0] * rpb
        ipi = -(-total // (na - IW + 1))
        items = []
        for k in range(ipi):
            n = jnp.minimum(jnp.maximum(i - IW, 0) * ipi + k, total - 1)
            blk = (n // rpb + 2) % 3
            items.append(functools.partial(
                prep, wblk.at[blk + jnp.where(i >= IW, P1, 0)], w7.at[blk],
                pl.multiple_of(n % rpb * 16, 16)))
        assert ipi * (nfc - 1) <= rpb
        sched.add(items, int(P_WIN[0] * dur), int(P_WIN[1] * dur))
        total = w49.shape[1] // 8
        ipi = -(-total // (na - IW + 1))
        assert ipi <= Q // 16
        sched.add([prep2(
            1, jnp.where(i >= IW, 2 * nfc, 0),
            jnp.minimum(jnp.maximum(i - IW, 0) * ipi + k, total - 1), k1)
            for k in range(ipi) for k1 in range(7)],
            int(P_WIN[0] * dur), int(P_WIN[1] * dur))

        def h49(k):
            assert sched.now <= int(O_WIN[0] * dur) and A_WIN[1] <= O_WIN[0]
            return _up(lhs49[k // 2, :, col(k % 2)])

        f = _ffn49(
            h49, QA,
            lambda k, b, n: pltpu.bitcast(
                dcs[pl.ds(k // NCB * D + b * 64, n * 64), col(k % NCB)], BF16),
            nfc, sched, *FA, sb, GA)
        assert not sched.queue
        xs[arows(i), :] = xin[arows(i), :].astype(F32) + 0.5 * f
        return carry

    with jax.named_scope("phase_a"):
        lax.fori_loop(1, na + 1, phase_a, 0)

    for cp in w_copies[1:]:
        cp.wait()

    qk_scale = (D ** -0.5) * math.log2(math.e)

    HM = TM // 32 * 16

    def put7(dst, r0, cs, *p):
        if len(p) == 4:
            ops = enumerate(_sa(*p))
        else:
            ops = zip((1, 2, 3, 4), (p[0] + p[1], *p, p[0] + p[1]))
        for k, t in ops:
            dst[pl.ds(k * PR + r0 // 2, 8), cs] = pltpu.bitcast(
                t.astype(BF16), jnp.uint32)

    def get7(src, k, ds=pl.ds, nr=None):
        nr = nr or (TM - HM if 1 <= k <= 4 else HM)
        return pltpu.bitcast(src[ds(k * PR, nr // 2), :], BF16)

    def groups(r0):
        return (r0, HM + r0) if r0 < HM else (HM + r0,)

    def q_ops(i, r0, c, z):
        p = [hs[rows(i, r, 16), col(2 * h + c)].astype(F32)
             for r in groups(r0) for h in range(2)]
        p[0] = p[0] + _rep(z.v(), 16)
        p[-1] = p[-1] + _rep(z.v(), 16)
        put7(hq7, r0, col(c), *p)

    def q_items(i):
        return [functools.partial(q_ops, i, r0, c)
                for r0 in range(0, TM - HM, 16) for c in range(2)]

    sched = _Sched(zero)
    sched.add(ln_out(N - TA, range(0, TA // 2, 16)), *FD[:2])
    sched.add(q_items(0), *FD[2:])
    for dst in (mq, wvo):
        for u in range(2):
            t = []
            for cs in (col(u), col(u + 2)):
                t.append(_dot_nt(wq[...], wk[cs, :]) if dst is mq
                         else _dot(wv[...], wo[:, cs]))
                sched(t[-1])
            if dst is mq:
                t = [v * qk_scale for v in t]
            for k, v in enumerate(
                    _sb(t[0][:H], t[1][:H], t[0][H:], t[1][H:])):
                dst[k, :, col(u)] = _pk(v)
    assert not sched.queue
    dwf = dw[...].astype(F32)
    for k in range(K):
        dwb[k] = jnp.broadcast_to(dwf[k:k + 1, :], (8, D))

    def conv_block(p, r0, c, done, CT=CT, AT=K):
        cs = col(c)
        acc = [None]

        def item(k0, z=None):
            for k in range(k0, min(k0 + CT, K)):
                off = HALO - K // 2 + k + r0
                w = dwb[k, :, cs]
                if z is not None and k - k0 < AT:
                    w = w + z.v()
                t = gs[p + 1, c, off:off + 8, :] * w
                acc[0] = t if acc[0] is None else acc[0] + t
            if k0 + CT >= K:
                dcs[rows(p, r0, 8), cs] = acc[0]
                done(acc[0])

        return [functools.partial(item, k0) for k0 in range(0, K, CT)]

    def conv_main(p, cols=range(NCB), **kw):
        st = []

        def stats(r0, c, acc):
            if r0 == 0:
                st[:] = [acc, None, None]
                return
            shift, s1, s2 = st
            d = acc - shift
            s1 = d if s1 is None else s1 + d
            s2 = d * d if s2 is None else s2 + d * d
            st[:] = [shift, s1, s2]
            if r0 + 16 == TM:
                dm = s1 * (1.0 / (TM // 8 - 1))
                st_mean[p, :, col(c)] = shift + dm
                st_m2[p, :, col(c)] = s2 - s1 * dm

        return [it for c in cols for r0 in range(0, TM - 8, 8)
                for it in conv_block(p, r0, c,
                                     functools.partial(stats, r0, c), **kw)]

    def conv_edge(p, cols=range(NCB)):
        return [it for c in cols
                for it in conv_block(p, TM - 8, c, lambda acc: None)]


    def phase_b(i, carry):
        b = i // tpb

        sched = _Sched(zero)
        sched.add(conv_edge(jnp.maximum(i - 2, 0))
                  + conv_main(jnp.maximum(i - 1, 0), range(L0, NCB)),
                  int(B_SLOTS[0] * TM), int(B_SLOTS[1] * TM))
        sched.add(q_items(jnp.minimum(i + 1, nt - 1)),
                  int(Q_SLOTS[0] * TM), int(Q_SLOTS[1] * TM))
        acc = [None] * 4
        for k in OQ:
            t = _dot(get7(hq7, k), _up(mq[k]))
            _acc7(acc, k, t, HM)
            sched(t)
        q11, q12, q21, q22 = _quads(
            jnp.concatenate(_join(acc, HM), axis=1), HM)
        q7 = [q11[:HM] - q22[:HM], q21 - q22, q11, q22, q12 - q11,
              q21[:HM] - q11[:HM], q12[:HM] - q22[:HM]]
        q7 = [t.astype(BF16) for t in q7]

        dz = zero_s[0]
        p_buf, al_buf = (p_buf0, p_buf1, p_buf2), (al_buf0, al_buf1, al_buf2)
        s_buf = (s_buf0, s_buf1)

        def dyn(r0, n):
            return pl.ds(pl.multiple_of(dz + r0, 8), n)

        nb = KP // 128

        def chunk(j):
            return pl.ds(pl.multiple_of(b * (TP // 2), KP // 2)
                         + j * KP // 2, KP // 2)

        def combine(m, j, c):
            if len(m) == 7:
                s = [m[0] + m[3] + m[4] + m[6], m[2] + m[4],
                     m[1] + m[3], m[1] - m[0] + m[2] + m[5]]
            else:
                s = [m[0] + m[2], m[1] + m[3]]
            nv = T // 2 - j * KP - c * 128
            if nv < 128:
                lane = lax.broadcasted_iota(jnp.int32, s[0].shape, 1)
                s = [jnp.where(lane < nv, t, -jnp.inf) for t in s]
            return s

        stat = {}

        def put(w, j, r, v):
            for r0 in range(0, v.shape[0], 16):
                stat[w, j, r + r0] = v[r0:r0 + 16]

        def get(w, j, r, n=16):
            return jnp.concatenate(
                [stat[w, j, r0] for r0 in range(r, r + n, 16)], axis=0)

        def scores(j):
            m = [None] * 7
            for k in OS if j else OS0:
                m[k] = _dot_nt(
                    q7[k], _up(ks[(0, 2, 1, 4, 3, 5, 6)[k], chunk(j), :]))
                sched(m[k])
            mx = None
            for c in range(nb):
                s = combine([t[:HM, col(c)] for t in m], j, c)
                e = combine([t[HM:, col(c)] for t in m[1:5]], j, c)
                for h in range(2):
                    t = jnp.concatenate([s[h], s[2 + h], e[h]], axis=0)
                    s_buf[j % 2][:, col(h * nb + c)] = t
                    mx = t if mx is None else jnp.maximum(mx, t)
            mx = jnp.broadcast_to(jnp.max(mx, axis=-1, keepdims=True),
                                  mx.shape)
            if j:
                mx = jnp.maximum(mx, get(0, j - 1, 0, TM))
            put(0, j, 0, mx)

        part = {}

        def soft1(j, r, c0, z):
            rs = slice(r, r + 16)
            m = get(0, j, r) + _rep(z.v(), 16)
            l = functools.reduce(jnp.add, part.pop((j, r), []) + [
                jnp.exp2(s_buf[j % 2][dyn(r, 16), col(c)] - m)
                for c in range(c0, c0 + S1)])
            if c0 + S1 < 2 * nb:
                part[j, r] = [l]
                return
            l = jnp.broadcast_to(jnp.sum(l, axis=-1, keepdims=True),
                                 (16, 128))
            if j:
                l += get(1, j - 1, r) * jnp.exp2(get(0, j - 1, r) - m)
            put(1, j, r, l)
            e = (pltpu.bitcast(l, jnp.int32) >> 23) - 127
            ref = m + e.astype(F32)
            put(2, j, r, ref)
            if j:
                al_buf[j % 3][rs, :] = jnp.exp2(get(2, j - 1, r) - ref)

        def soft2(j, r0, c0, z):
            ref = [get(2, j, r) + _rep(z.v(), 16) for r in groups(r0)]
            p = [jnp.concatenate(
                [jnp.exp2(s_buf[j % 2][dyn(r, 16), col(h * nb + c)] - m)
                 for c in range(c0, c0 + S2)], axis=1)
                 for r, m in zip(groups(r0), ref) for h in range(2)]
            put7(p_buf[j % 3], r0, slice(c0 * 128, (c0 + S2) * 128), *p)

        scd = 7 * HM + 4 * (TM - 2 * HM)
        start = sched.now

        def add_soft(j):
            rbs = range(0, TM - HM, 16)
            t0, t1 = (start + int(t * scd) for t in SW[j:j + 2])
            assert t1 <= start + min(2 * j + LAG + 1, nkc + j) * scd
            assert j < 3 or t0 >= start + min(2 * j + LAG - 4,
                                              nkc + j - 2) * scd
            assert (j + 2 >= nkc
                    or t1 <= start + max(2 * j + 5 - LAG, j + 3) * scd)
            u = (t1 - t0 - sum(SD)) // (len(rbs) + 1)
            for n, r0 in enumerate(rbs):
                its = [[functools.partial(soft1, j, r, c)
                        for r in groups(r0) for c in range(0, 2 * nb, S1)],
                       [functools.partial(soft2, j, r0, c)
                        for c in range(0, nb, S2)]]
                for k, it in enumerate(its):
                    t = t0 + SD[0] + n * u + k * (u + SD[1])
                    sched.add(it, t, t + u)

        for j in range(LAG):
            scores(j)
            add_soft(j)
        acc = [None] * 4
        for j in range(nkc):
            if j + LAG < nkc:
                scores(j + LAG)
                add_soft(j + LAG)
            fresh = [j > 0] * 4
            for k in OP if j + 1 < nkc else OQ:
                w = _up(ks[(0, 2, 6, 5, 3, 4, 1)[k], chunk(j), :])
                m = _dot(get7(p_buf[j % 3], k, dyn), w)
                sched(m)
                for a, _ in _TG[k]:
                    if fresh[a]:
                        al = al_buf[j % 3][dyn(0, TM), :]
                        al = _quads(jnp.concatenate([al] * NCB, axis=1), HM)[a]
                        acc[a] = acc[a] * al[:acc[a].shape[0]]
                        fresh[a] = False
                _acc7(acc, k, m, HM)
        assert not sched.queue
        t = jnp.exp2(get(2, nkc - 1, 0, TM) - get(0, nkc - 1, 0, TM))
        t = t / get(1, nkc - 1, 0, TM)
        o = (jnp.concatenate(_join(acc, HM), axis=1)
             * jnp.concatenate([t] * NCB, axis=1))
        o7 = [t.astype(BF16) for t in _sax(*_quads(o, HM), HM)]
        acc = list(_quads(xs[rows(i), :], HM))
        acc = [acc[0][:HM], acc[1], acc[2], acc[3][:HM]]
        for k in OW:
            _acc7(acc, k, _dot(o7[k], _up(wvo[k])), HM)
        x2 = jnp.concatenate(_join(acc, HM), axis=1)
        xs[rows(i), :] = x2
        h7 = [t.astype(BF16) for t in _sax(*_quads(_ln(x2), HM), HM)]
        sched = _Sched(zero)
        acc = [[None] * 4 for _ in range(2)]
        for n, (h, k) in enumerate(PO):
            t = _dot(h7[k], _up(w7[h, k]))
            _acc7(acc[h], k, t, HM)
            sched(t)
            if any(e[0] == h for e in PO[n + 1:]):
                continue
            val, gate = _join(acc[h], HM)
            g2 = val * (0.5 + 0.5 * jnp.tanh(0.5 * gate))
            for c in (2 * h, 2 * h + 1):
                g = g2[:, col(c % 2)]
                gs[i + 1, c, HALO:HALO + TM, :] = g
                gs[i, c, HALO + TM:, :] = jnp.where(
                    i % tpb == 0, 0.0, g[:HALO])
                gs[i + 2, c, :HALO, :] = jnp.where(
                    i % tpb == tpb - 1, 0.0, g[TM - HALO:])
            if h == 0 and L0:
                rest = sum(h7[e[1]].shape[0] for e in PO[n + 1:])
                sched.add(conv_main(i, range(L0), CT=LP[2], AT=LP[3]),
                          sched.now + LP[0], sched.now + rest - LP[1])
        assert not sched.queue
        return carry

    with jax.named_scope("phase_b"):
        lax.fori_loop(0, nt, phase_b, 0)
    for item in (conv_main(nt - 1, range(L0, NCB)) + conv_edge(nt - 2)
                 + conv_edge(nt - 1)):
        item()

    ng = TM // 8 - 1
    means = st_mean[...].reshape(nt * 8, D)
    edges = jnp.concatenate([dcs[(p + 1) * TM - 8:(p + 1) * TM, :]
                             for p in range(nt)], axis=0)
    mu = jnp.sum(ng * means + edges, axis=0, keepdims=True) * (1.0 / N)
    dm = means - mu
    de = edges - mu
    var = jnp.sum(st_m2[...].reshape(nt * 8, D) + ng * (dm * dm) + de * de,
                  axis=0, keepdims=True) * (1.0 / N)
    rstd = lax.rsqrt(var + EPS)
    bn[0] = jnp.broadcast_to(mu, (8, D))
    bn[1] = jnp.broadcast_to(rstd, (8, D))

    def bn_silu(i, r0, c, z=None):
        p = []
        for r in (r0, TC // 2 + r0):
            for h in range(2):
                cs = col(2 * h + c)
                mu = bn[0, :, cs] if z is None else bn[0, :, cs] + z.v()
                y = dcs[crows(i, r, 16), cs] - _rep(mu, 16)
                p.append(_silu(y * _rep(bn[1, :, cs], 16)))
        put7(hq7, r0, col(c), *p)

    def bn_items(i):
        return [functools.partial(bn_silu, i, r0, c)
                for r0 in range(0, TC // 2, 16) for c in range(2)]

    def ln_final(i, r0=0, n=TC, z=None):
        obuf[crows(i, r0, n), :] = _ln(xs[crows(i, r0, n), :],
                                       zrep(z, n)).astype(BF16)

    for item in bn_items(0):
        item()

    QC = TC // 4

    def pw2(src, dst, sched, win):
        acc = list(_quads(xs[crows(src), :], TC // 2))
        for k in OQ:
            t = _dot(get7(hq7, k, nr=TC // 2), _up(w7[2, k]))
            _acc7(acc, k, t, TC // 2)
            sched(t)
        xs[crows(dst), :] = jnp.concatenate(_join(acc, TC // 2), axis=1)
        for items, t0, t1 in zip(
                ln_in(xs, dst * TC, QC, range(0, QC, 16)), win, win[1:]):
            sched.add(items, sched.now + t0, sched.now + t1)

    sched = _Sched(zero)
    pw2(0, 0, sched, (0, 1, 2))
    sched.force([e[1] for e in sched.queue])

    def phase_c(i, carry):
        @pl.when(i >= 2)
        def _():
            o_copy(i - 2).start()

        sched = _Sched(zero)
        dur = (7 * 8 + 49 * 2 * nfc) * TC // 16
        sched.add([functools.partial(ln_final, jnp.maximum(i - 1, 0), r, RC)
                   for r in range(0, TC, RC)],
                  int(C_WIN[0] * dur), int(C_WIN[1] * dur))
        nxt = jnp.minimum(i + 1, nc - 1)
        items = bn_items(nxt)
        sched.add(items, int(C_WIN[2] * dur), int(C_WIN[3] * dur))
        done = []

        def mid():
            sched.force(items)
            done.append(1)
            pw2(nxt, jnp.where(i + 1 < nc, i + 1, 0), sched, M_WIN)

        def h49(k):
            assert not done
            return _up(lhs49[k // 2, :QC // 2, col(k % 2)])

        f = _ffn49(h49, QC, lambda k, b, n: _up(
            w49[k // 2, b * 64:(b + n) * 64, col(k % 2)]),
            nfc, sched, *FB, sb, GC, mid)
        assert not sched.queue
        xs[crows(i), :] += 0.5 * f
        return carry

    with jax.named_scope("phase_c"):
        lax.fori_loop(0, nc, phase_c, 0)
    o_copy(nc - 2).start()
    last = []
    for k, (r0, r1) in enumerate(zip(EP[:-1], EP[1:])):
        ln_final(nc - 1, r0, r1 - r0)
        rs = crows(nc - 1, r0, r1 - r0)
        last.append(pltpu.make_async_copy(obuf.at[rs, :], out_hbm.at[rs, :],
                                          osem.at[nc - 1 + k]))
        last[-1].start()
    for i in range(nc - 1):
        o_copy(i).wait()
    for cp in last:
        cp.wait()


@jax.jit
def pallas_standalone__conformer_family_conformer__speech_kernel(
    x: jax.Array,
    w_ff1_a: jax.Array,
    w_ff1_b: jax.Array,
    w_q: jax.Array,
    w_k: jax.Array,
    w_v: jax.Array,
    w_o: jax.Array,
    w_pw1: jax.Array,
    dw: jax.Array,
    w_pw2: jax.Array,
    w_ff2_a: jax.Array,
    w_ff2_b: jax.Array,
):
    B, T, D = x.shape
    K = dw.shape[0]
    N = B * T
    weights = (w_ff1_a, w_ff1_b, w_q, w_k, w_v, w_o, w_pw1, dw, w_pw2,
               w_ff2_a, w_ff2_b)
    scratch = [pltpu.VMEM((N, D), BF16)]
    nfc = w_ff1_a.shape[1] // FC
    scratch += [pltpu.VMEM((4 * nfc + 3, D, D), BF16)]
    scratch += [pltpu.VMEM(w.shape, w.dtype)
                for w in (w_q, w_k, w_v, w_o, dw)]
    scratch += [
        pltpu.VMEM((7, D // 4, D // 2), jnp.uint32),
        pltpu.VMEM((7, D // 4, D // 2), jnp.uint32),
        pltpu.VMEM((N, D), F32),
        pltpu.VMEM((N, D), BF16),
        pltpu.VMEM((7, B * -(-T // KC) * KC // 4, D // 2), jnp.uint32),
        pltpu.VMEM((N // TM + 2, D // 128, TM + 2 * HALO, 128), F32),
        pltpu.VMEM((N, D), F32),
        pltpu.VMEM((N // TM, 8, D), F32),
        pltpu.VMEM((N // TM, 8, D), F32),
        pltpu.VMEM((2, 8, D), F32),
        pltpu.VMEM((25, TA // 8, D // 2), jnp.uint32),
        pltpu.VMEM((7, 14 * TA // 8, D // 2), jnp.uint32),
        pltpu.VMEM((3, 7, D // 4, D // 2), jnp.uint32),
        pltpu.VMEM((25, nfc * D // 4, D // 2), jnp.uint32),
        pltpu.VMEM((T0, D), BF16),
        pltpu.VMEM((K, 8, D), F32),
        pltpu.VMEM((ZR, 128), jnp.uint32),
        pltpu.SMEM((1,), jnp.int32),
        pltpu.VMEM((TM + 16, 128), F32),
        pltpu.VMEM((TM + 16, 128), F32),
        pltpu.VMEM((TM + 16, 128), F32),
        pltpu.VMEM((7 * PR, KC // 2), jnp.uint32),
        pltpu.VMEM((7 * PR, KC // 2), jnp.uint32),
        pltpu.VMEM((7 * PR, KC // 2), jnp.uint32),
        pltpu.VMEM((TM, KC), F32),
        pltpu.VMEM((TM, KC), F32),
        pltpu.VMEM((7 * PR, D // 2), jnp.uint32),
        pltpu.SemaphoreType.DMA(((N - T0) // TA + 1,)),
        pltpu.SemaphoreType.DMA((2, nfc)),
        pltpu.SemaphoreType.DMA((3, nfc)),
        pltpu.SemaphoreType.DMA((6,)),
        pltpu.SemaphoreType.DMA((N // TC + len(EP),)),
    ]
    out = pl.pallas_call(
        functools.partial(_kernel, B=B, T=T, D=D, K=K),
        out_shape=jax.ShapeDtypeStruct((N, D), x.dtype),
        in_specs=[pl.BlockSpec(memory_space=pl.ANY)] * 12,
        out_specs=pl.BlockSpec(memory_space=pl.ANY),
        scratch_shapes=scratch,
        compiler_params=pltpu.CompilerParams(
            vmem_limit_bytes=128 * 1024 * 1024),
    )(x.reshape(N, D), *weights)
    return out.reshape(B, T, D)
```

```python
import functools
import math

import jax
import jax.numpy as jnp
from jax import lax
import jax.experimental.pallas as pl
import jax.experimental.pallas.tpu as pltpu

F32 = jnp.float32
BF16 = jnp.bfloat16

TM = 400
T0 = 320
TA = 512
TC = 320
FC = 512
KC = 512
IW = 3
GA = (42, 60, 16)
GC = (42, 90, 16)
KO = 2
O_WIN = (0.785, 0.975)
L_WIN = (0.0, 0.12)
PL = ((0, 0, 49), (0, 1, 49), (0, 2, 49), (0, 3, 49), (1, 0, 49), (1, 1, 49))
FA = (((2, 4, 3, 1, 0, 6, 5), (2, 4, 3, 1, 0, 6, 5)),
      ((2, 4, 5, 3, 1, 6, 0), (2, 4, 3, 1, 0, 6, 5)), PL)
FB = (((2, 4, 3, 1, 0, 6, 5), (2, 4, 3, 1, 0, 6, 5)),
      ((2, 4, 5, 3, 1, 6, 0), (2, 4, 3, 1, 0, 6, 5)),
      PL[:4] + ((1, 0, 35), (2, 0, 0), (1, 0, 14), (1, 1, 49)))
P_WIN = (0.5, 0.97)
OQ = (0, 2, 3, 4, 6, 1, 5)
OS0 = (2, 4, 3, 1, 0, 5, 6)
OS = (0, 1, 2, 3, 4, 5, 6)
OP = (0, 1, 2, 3, 4, 5, 6)
OW = (2, 4, 3, 0, 6, 1, 5)
PO = ((0, 2), (0, 4), (1, 2), (0, 3), (0, 0), (0, 6), (0, 1), (0, 5),
      (1, 4), (1, 3), (1, 0), (1, 6), (1, 1), (1, 5))
F_WIN = (0.02, 0.97, 0.5)
A_WIN = (0.5, 0.75)
FD = (0, 3200, 0, 3200)
B_SLOTS = (1, 53)
Q_SLOTS = (8, 50)
CT = 5
L0 = 1
LP = (0, 100, 3, 1)
S1 = 2
S2 = 1
SD = (0, 140, 120)
LAG = 2
SW = tuple(1 + 1.75 * j for j in range(9))
C_WIN = (0.02, 0.51, 0.3, 0.58)
M_WIN = (55, 1200, 2270)
RC = 8
EP = (0, 128, 224, 288, 320)
ZR = 32
PR = 112
HALO = 8
EPS = 1e-05


def _ln(x, z=None):
    if z is None:
        m = jnp.mean(x, axis=-1, keepdims=True)
    else:
        t = z
        for c in range(x.shape[-1] // 128):
            t = t + x[:, c * 128:(c + 1) * 128]
        m = jnp.sum(t, axis=-1, keepdims=True) * (1.0 / x.shape[-1])
    xc = x - m
    v = jnp.mean(xc * xc, axis=-1, keepdims=True)
    return xc * lax.rsqrt(v + EPS)


def _silu(a):
    y = 0.5 * a
    return y + y * jnp.tanh(y)


def _dot(a, b):
    return jnp.dot(a, b, preferred_element_type=F32)


def _dot_nt(a, b):
    return lax.dot_general(a, b, (((1,), (1,)), ((), ())),
                           preferred_element_type=F32)


def _pk(v):
    return pltpu.bitcast(v.astype(BF16), jnp.uint32)


def _up(v):
    return pltpu.bitcast(v, BF16)


class _Anchor:
    def __init__(self, t, zero_v):
        self.t, self.zero_v = t, zero_v

    def v(self):
        return pltpu.bitcast(
            pltpu.bitcast(self.t, jnp.uint32) & self.zero_v[0:8, :], F32)


class _Sched:
    def __init__(self, zero_v):
        self.zero_v = zero_v
        self.queue = []
        self.now = 0

    def add(self, items, t0, t1, skip=()):
        assert t0 >= self.now
        ts = [t for t in range(t0, t1)
              if not any(a <= t < b for a, b in skip)]
        self.queue += [(ts[k * len(ts) // len(items)], it)
                       for k, it in enumerate(items)]
        self.queue.sort(key=lambda e: e[0])

    def __call__(self, t, dur=None):
        dur = dur or t.shape[0]
        end = self.now + dur
        while self.queue and self.queue[0][0] < end:
            time, item = self.queue.pop(0)
            r = (time - self.now) * t.shape[0] // dur // 8 * 8
            item(_Anchor(t[r:r + 8, :128], self.zero_v))
        self.now = end
        self.last = t

    def force(self, items):
        for e in [e for e in self.queue if e[1] in items]:
            self.queue.remove(e)
            e[1](_Anchor(self.last[-8:, :128], self.zero_v))


def _rep(z, rows):
    return jnp.concatenate([z] * (rows // 8), axis=0)


def _ffn(h, wa_ref, wb_ref, sched):
    ss = []
    for n in range(wa_ref.shape[1] // 128):
        a = _dot(h, wa_ref[:, n * 128:(n + 1) * 128])
        ss.append(_silu(a))
        sched(a)
    s = jnp.concatenate(ss, axis=1).astype(BF16)
    acc = []
    for n in range(wb_ref.shape[1] // 128):
        acc.append(_dot(s, wb_ref[:, n * 128:(n + 1) * 128]))
        sched(acc[-1])
    return jnp.concatenate(acc, axis=1)


def _sa(a11, a12, a21, a22):
    return [a11 + a22, a21 + a22, a11, a22, a11 + a12, a21 - a11, a12 - a22]


def _sb(b11, b12, b21, b22):
    return [b11 + b22, b11, b12 - b22, b21 - b11, b22, b11 + b12, b21 + b22]


def _lhs7(t, u):
    h = t.shape[1] // 2
    return [v.astype(BF16)
            for v in _sa(t[:, :h], t[:, h:], u[:, :h], u[:, h:])]


_SA = ((0, 1, 3), (2, 1, 3), (0, 0, 0), (3, 0, 3), (0, 1, 1), (2, -1, 0),
       (1, -1, 3))
_SB = ((0, 1, 3), (0, 0, 0), (1, -1, 3), (2, -1, 0), (3, 0, 3), (0, 1, 1),
       (2, 1, 3))
_TG = (((0, 1), (3, 1)), ((2, 1), (3, -1)), ((1, 1), (3, 1)), ((0, 1), (2, 1)),
       ((0, -1), (1, 1)), ((3, 1),), ((0, 1),))


def _quads(x, hm):
    h = x.shape[1] // 2
    t = x[:hm]
    if x.shape[0] > 2 * hm:
        t = jnp.concatenate([t, x[2 * hm:]], axis=0)
    return t[:, :h], t[:, h:], x[hm:, :h], x[hm:, h:]


def _sax(a11, a12, a21, a22, hm):
    return [a11[:hm] + a22[:hm], a21 + a22, a11, a22, a11 + a12,
            a21[:hm] - a11[:hm], a12[:hm] - a22[:hm]]


def _acc7(acc, k, m, hm):
    for a, sg in _TG[k]:
        t = m if a in (1, 2) else m[:hm]
        if acc[a] is None:
            acc[a] = t if sg > 0 else -t
        else:
            acc[a] = acc[a] + t if sg > 0 else acc[a] - t


def _join(acc, hm):
    rest = [acc[1][hm:]] if acc[1].shape[0] > hm else []
    return (jnp.concatenate([acc[0], acc[2]], axis=0),
            jnp.concatenate([acc[1][:hm], acc[3]] + rest, axis=0))


def _pm(a, sg, b):
    return a if not sg else a + b if sg > 0 else a - b


def _ops2(load, put, tab, f, k1, z):
    def quad(a):
        return [load(a // 2 * 2 + j // 2, a % 2 * 2 + j % 2) for j in range(4)]

    a, sg, b = tab[k1]
    y = [_pm(u + _rep(z.v(), 16), sg, v) for u, v in zip(quad(a), quad(b))]
    for k2, v in enumerate(f(*y)):
        put(7 * k1 + k2, v)


def _ffn49(h49, hm, w, nfc, sched, oi, oo, plan, sb, gap, mid=None):
    src = [[n for n in range(7) if a in [e[0] for e in _TG[n]]]
           for a in range(4)]
    val = {}

    def add(key, sg, t):
        if key not in val:
            val[key] = t if sg > 0 else -t
        else:
            val[key] = _pm(val[key], sg, t)

    def collect(done, tag, k1, k2, t):
        done.add((k1, k2))
        for b, sg in _TG[k2]:
            add((tag, 'm', k1, b), sg, t)
            if all((k1, n) in done for n in src[b]):
                for a, sg1 in _TG[k1]:
                    add((tag, 'u', a, b), sg1, val[tag, 'm', k1, b])

    done = [set() for _ in range(nfc + 1)]

    pend, free = {}, [0]

    def ops(c, n, r, z):
        a, sg, a2 = _SA[n]
        rs = slice(r, r + gap[2])
        y = [_pm(val[c, 'a', a, b][rs] + _rep(z.v(), gap[2]), sg,
                 val[c, 'a', a2, b][rs]) for b in range(4)]
        for m, v in enumerate(_sa(*y)):
            sb.at[n][pl.ds(((c // KO * 7 + m) * hm + r) // 2, gap[2] // 2),
                     pl.ds(c % KO * 128, 128)] = _pk(v)

    def step_in(c, k1, k2):
        t = _dot(h49(7 * k1 + k2), w(7 * k1 + k2, c, 1))
        collect(done[c], c, k1, k2, t)
        sched(t, hm // 4)
        for a in range(4):
            for b in range(4):
                if (c, 'a', a, b) not in val and all(
                        (m, n) in done[c] for m in src[a] for n in src[b]):
                    val[c, 'a', a, b] = _silu(val[c, 'u', a, b])
        for n in oo[0]:
            if (c, n) not in pend and all(
                    (c, 'a', a, b) in val
                    for a in _SA[n][::2] for b in range(4)):
                pend[c, n] = [functools.partial(ops, c, n, r)
                              for r in range(0, hm, gap[2])]
                for e in pend[c, n]:
                    free[0] = max(free[0] + gap[0], sched.now + gap[1])
                    sched.add([e], free[0], free[0] + 1)

    def step_out(g, k1, k2):
        cs = range(g * KO, (g + 1) * KO)
        sched.force([e for c in cs for e in pend[c, k1]])
        v = _up(sb[k1, pl.ds((g * 7 + k2) * hm // 2, hm // 2), :])
        t = _dot(v, w(7 * k1 + k2, nfc + g * KO, KO))
        sched(t, hm * KO // 4)
        add(('p', k1, k2), 1, t)
        if (g + 1) * KO == nfc:
            collect(done[-1], 'o', k1, k2, val['p', k1, k2])

    todo = {(d, c): [(k1, k2) for k1 in o[0] for k2 in o[1]]
            for d, o in enumerate((oi, oo)) for c in range(nfc)}
    for d, c, n in plan:
        if d == 2:
            mid()
            continue
        for k1, k2 in todo[d, c][:n]:
            (step_out if d else step_in)(c, k1, k2)
        del todo[d, c][:n]
    return jnp.concatenate(
        [jnp.concatenate([val['o', 'u', a // 2 * 2 + b // 2, a % 2 * 2 + b % 2]
                          for b in range(4)], axis=1) for a in range(4)],
        axis=0)


def _kernel(x_hbm, w1a_hbm, w1b_hbm, wq_hbm, wk_hbm, wv_hbm, wo_hbm,
            wp1_hbm, dw_hbm, wp2_hbm, w2a_hbm, w2b_hbm,
            out_hbm,
            xin, wblk, wq, wk, wv, wo, dw,
            mq, wvo, xs, hs, ks, gs, dcs, st_mean, st_m2, bn,
            lhs49, sb, w7, w49, lhs_b, dwb, zero, zero_s,
            al_buf0, al_buf1, al_buf2,
            p_buf0, p_buf1, p_buf2, s_buf0, s_buf1, hq7,
            xsem, w1sem, w2sem, wsem, osem,
            *, B, T, D, K):
    N = B * T
    obuf = xin
    KP = KC // 2
    nkc = -(-T // KC)
    TP = nkc * KP
    NCB = D // 128
    nt = N // TM
    tpb = T // TM

    def rows(i, r0=0, n=TM):
        return pl.ds(pl.multiple_of(i * TM, 16) + r0, n)

    def col(c):
        if isinstance(c, int):
            return slice(c * 128, (c + 1) * 128)
        return pl.ds(pl.multiple_of(c * 128, 128), 128)

    na = (N - T0) // TA
    H = D // 2
    QA = TA // 4
    s_buf = (s_buf0, s_buf1)

    def arows(i, r0=0, n=TA):
        return pl.ds(pl.multiple_of(T0 + (i - 1) * TA, 16) + r0, n)

    def x_copy(i):
        rs = pl.ds(0, T0) if isinstance(i, int) and i == 0 else arows(i)
        return pltpu.make_async_copy(x_hbm.at[rs, :], xin.at[rs, :],
                                     xsem.at[i])

    nc = N // TC

    def crows(i, r0=0, n=TC):
        return pl.ds(pl.multiple_of(i * TC, 16) + r0, n)

    def o_copy(i):
        return pltpu.make_async_copy(obuf.at[crows(i), :],
                                     out_hbm.at[crows(i), :], osem.at[i])

    nfc = w49.shape[1] // (D // 4)
    P1, P2 = 4 * nfc, 4 * nfc + 2

    def w1_copies(c):
        fs = pl.ds(pl.multiple_of(c * FC, FC), FC)
        return [pltpu.make_async_copy(w1a_hbm.at[:, fs], wblk.at[c],
                                      w1sem.at[0, c]),
                pltpu.make_async_copy(w1b_hbm.at[fs, :], wblk.at[nfc + c],
                                      w1sem.at[1, c])]

    def w2_copies(c):
        fs = pl.ds(pl.multiple_of(c * FC, FC), FC)
        hs_ = pl.ds(pl.multiple_of(c // 2 * H, H), H)
        return [pltpu.make_async_copy(s, d, w2sem.at[j, c])
                for j, (s, d) in enumerate([
                    (w2a_hbm.at[:, fs], wblk.at[2 * nfc + c]),
                    (w2b_hbm.at[fs, :], wblk.at[3 * nfc + c]),
                    (wp1_hbm.at[:, pl.ds(pl.multiple_of(c * H, H), H)],
                     wblk.at[P1 + c % 2, :, hs_])])]

    assert nfc == 4
    w_pairs = [(wp2_hbm, wblk.at[P2]), (wq_hbm, wq), (wk_hbm, wk),
               (wv_hbm, wv), (wo_hbm, wo), (dw_hbm, dw)]
    w_copies = [pltpu.make_async_copy(s, d, wsem.at[j])
                for j, (s, d) in enumerate(w_pairs)]

    x_copy(0).start()
    for cp in w1_copies(0):
        cp.start()

    zero[...] = jnp.zeros(zero.shape, jnp.uint32)
    zero_s[0] = 0
    for c in range(NCB):
        gs[1, c, 0:HALO, :] = jnp.zeros((HALO, 128), F32)
        gs[nt, c, HALO + TM:, :] = jnp.zeros((HALO, 128), F32)
    for b in range(B):
        ks[:, (b * TP + T // 2) // 2:(b + 1) * TP // 2, :] = jnp.zeros(
            (7, (TP - T // 2) // 2, H), jnp.uint32)

    def zrep(z, n):
        return None if z is None else _rep(z.v(), n)

    def pair_items(first, second, rows0):
        items = []
        for r0 in rows0:
            t = []
            items += [functools.partial(first, t, r0),
                      functools.partial(second, t, r0)]
        return items

    def ln_in(src, base, quarter, rows0):
        zs = zero_s[0]

        def ln(r0, j, z):
            s_buf[j // 2][pl.ds(j % 2 * QA + r0, 16), :] = _ln(
                src[pl.ds(pl.multiple_of(base + j * quarter, 16) + r0, 16), :]
                .astype(F32), zrep(z, 16))

        def ops(r0, k1):
            def load(j, c):
                return s_buf[j // 2][pl.ds(
                    pl.multiple_of(zs + r0, 16) + j % 2 * QA, 16), col(c)]

            def put(k, v):
                lhs49.at[k // 2][pl.ds(pl.multiple_of(r0 // 2, 8), 8),
                                 col(k % 2)] = _pk(v)

            return functools.partial(_ops2, load, put, _SA, _sa, k1)

        return ([functools.partial(ln, r0, j)
                 for r0 in rows0 for j in range(4)],
                [ops(r0, k1) for r0 in rows0 for k1 in range(7)])

    def ln_out(base, rows0):
        def first(t, r0, z, off=0):
            rs = pl.ds(pl.multiple_of(base, 32) + 2 * r0 + off, 16)
            t.append(_ln(xs[rs, :], zrep(z, 16)))
            hs[rs, :] = t[-1].astype(BF16)

        def second(t, r0, z):
            first(t, r0, z, 16)
            g = base // 32 + r0 // 16
            g += g // (T // 32) * ((TP - T // 2) // 16)
            for k, v in enumerate(_lhs7(*t)):
                ks.at[k][pl.ds(pl.multiple_of(g * 8, 8), 8), :] = _pk(v)

        return pair_items(first, second, rows0)

    def prep(src, dst, r0, z=None):
        q = [src[pl.ds(r + r0, 16), c:c + H].astype(F32)
             for r in (0, H) for c in (0, H)]
        if z is not None:
            zz = jnp.concatenate([_rep(z.v(), 16)] * (H // 128), axis=1)
            q[0], q[3] = q[0] + zz, q[3] + zz
        r1 = r0 // 2 if isinstance(r0, int) else pl.multiple_of(r0 // 2, 8)
        for k, v in enumerate(_sb(*q)):
            dst.at[k][pl.ds(r1, 8), :] = _pk(v)

    Q = D // 4

    def prep2(ff, blk, n, k1):
        rpb = Q // 16

        def load(r, c):
            return wblk[blk + n // rpb, pl.ds(pl.multiple_of(
                n % rpb * 16, 16) + r * Q, 16), col(c)].astype(F32)

        def put(k, v):
            rs = pl.multiple_of(n * 8, 8)
            if ff:
                w49.at[k // 2][pl.ds(rs, 8), col(k % 2)] = _pk(v)
            else:
                dcs[pl.ds(rs + k // NCB * D, 8), col(k % NCB)] = (
                    pltpu.bitcast(v.astype(BF16), F32))

        return functools.partial(_ops2, load, put, _SB, _sb, k1)

    x_copy(0).wait()
    lhs_b[...] = _ln(xin[0:T0, :].astype(F32)).astype(BF16)
    xs[0:T0, :] = xin[0:T0, :].astype(F32)

    def first_tile(c, carry):
        for cp in w1_copies(c):
            cp.wait()

        @pl.when(c == 1)
        def _():
            x_copy(1).wait()

        @pl.when(c + 1 < nfc)
        def _():
            for cp in w1_copies(c + 1):
                cp.start()

        @pl.when(c % 2 == 0)
        def _():
            x_copy(1 + c // 2).start()

        n = -(-QA // (nfc - 1) // 16) * 16
        r0 = pl.multiple_of(jnp.clip((c - 1) * n, 0, QA - n), 16)
        assert n <= T0 // 4
        sched = _Sched(zero)
        dur = 2 * NCB * T0
        items = ln_in(xin, jnp.where(c > 0, T0, 0),
                      jnp.where(c > 0, QA, T0 // 4),
                      [r0 + r for r in range(0, n, 16)])
        sched.add(items[0], int(F_WIN[0] * dur), int(F_WIN[2] * dur))
        sched.add(items[1], int(F_WIN[2] * dur), int(F_WIN[1] * dur))
        sched.add([prep2(0, 0, (j * nfc + c) * (Q // 16) + r, k1)
                   for j in range(2) for r in range(Q // 16)
                   for k1 in range(7)],
                  int(F_WIN[0] * dur), int(F_WIN[1] * dur))
        f = _ffn(lhs_b[...], wblk.at[c], wblk.at[nfc + c], sched)
        assert not sched.queue
        xs[0:T0, :] += 0.5 * f
        return carry

    lax.fori_loop(0, nfc, first_tile, 0)
    for j in range(3, na + 1):
        x_copy(j).start()
    for c in range(nfc):
        for cp in w2_copies(c):
            cp.start()
    for cp in w_copies:
        cp.start()

    def phase_a(i, carry):
        @pl.when(i < na)
        def _():
            x_copy(i + 1).wait()

        @pl.when((i >= IW) & (i < IW + nfc))
        def _():
            for cp in w2_copies(i - IW):
                cp.wait()

        @pl.when(i == IW)
        def _():
            w_copies[0].wait()

        sched = _Sched(zero)
        dur = 49 * 2 * nfc * TA // 16
        base = jnp.maximum(T0 + (i - 2) * TA, 0)
        sched.add(ln_out(base, range(0, TA // 2, 16)),
                  int(L_WIN[0] * dur), int(L_WIN[1] * dur))
        base = T0 + jnp.minimum(i, na - 1) * TA
        items = ln_in(xin, base, QA, range(0, QA, 16))
        sched.add(items[0], int(A_WIN[0] * dur), int(A_WIN[1] * dur))
        sched.add(items[1], int(O_WIN[0] * dur), int(O_WIN[1] * dur))
        rpb = H // 16
        total = w7.shape[0] * rpb
        ipi = -(-total // (na - IW + 1))
        items = []
        for k in range(ipi):
            n = jnp.minimum(jnp.maximum(i - IW, 0) * ipi + k, total - 1)
            blk = (n // rpb + 2) % 3
            items.append(functools.partial(
                prep, wblk.at[blk + jnp.where(i >= IW, P1, 0)], w7.at[blk],
                pl.multiple_of(n % rpb * 16, 16)))
        assert ipi * (nfc - 1) <= rpb
        sched.add(items, int(P_WIN[0] * dur), int(P_WIN[1] * dur))
        total = w49.shape[1] // 8
        ipi = -(-total // (na - IW + 1))
        assert ipi <= Q // 16
        sched.add([prep2(
            1, jnp.where(i >= IW, 2 * nfc, 0),
            jnp.minimum(jnp.maximum(i - IW, 0) * ipi + k, total - 1), k1)
            for k in range(ipi) for k1 in range(7)],
            int(P_WIN[0] * dur), int(P_WIN[1] * dur))

        def h49(k):
            assert sched.now <= int(O_WIN[0] * dur) and A_WIN[1] <= O_WIN[0]
            return _up(lhs49[k // 2, :, col(k % 2)])

        f = _ffn49(
            h49, QA,
            lambda k, b, n: pltpu.bitcast(
                dcs[pl.ds(k // NCB * D + b * 64, n * 64), col(k % NCB)], BF16),
            nfc, sched, *FA, sb, GA)
        assert not sched.queue
        xs[arows(i), :] = xin[arows(i), :].astype(F32) + 0.5 * f
        return carry

    with jax.named_scope("phase_a"):
        lax.fori_loop(1, na + 1, phase_a, 0)

    for cp in w_copies[1:]:
        cp.wait()

    qk_scale = (D ** -0.5) * math.log2(math.e)

    HM = TM // 32 * 16

    def put7(dst, r0, cs, *p):
        if len(p) == 4:
            ops = enumerate(_sa(*p))
        else:
            ops = zip((1, 2, 3, 4), (p[0] + p[1], *p, p[0] + p[1]))
        for k, t in ops:
            dst[pl.ds(k * PR + r0 // 2, 8), cs] = pltpu.bitcast(
                t.astype(BF16), jnp.uint32)

    def get7(src, k, ds=pl.ds, nr=None):
        nr = nr or (TM - HM if 1 <= k <= 4 else HM)
        return pltpu.bitcast(src[ds(k * PR, nr // 2), :], BF16)

    def groups(r0):
        return (r0, HM + r0) if r0 < HM else (HM + r0,)

    def q_ops(i, r0, c, z):
        p = [hs[rows(i, r, 16), col(2 * h + c)].astype(F32)
             for r in groups(r0) for h in range(2)]
        p[0] = p[0] + _rep(z.v(), 16)
        p[-1] = p[-1] + _rep(z.v(), 16)
        put7(hq7, r0, col(c), *p)

    def q_items(i):
        return [functools.partial(q_ops, i, r0, c)
                for r0 in range(0, TM - HM, 16) for c in range(2)]

    sched = _Sched(zero)
    sched.add(ln_out(N - TA, range(0, TA // 2, 16)), *FD[:2])
    sched.add(q_items(0), *FD[2:])
    for dst in (mq, wvo):
        for u in range(2):
            t = []
            for cs in (col(u), col(u + 2)):
                t.append(_dot_nt(wq[...], wk[cs, :]) if dst is mq
                         else _dot(wv[...], wo[:, cs]))
                sched(t[-1])
            if dst is mq:
                t = [v * qk_scale for v in t]
            for k, v in enumerate(
                    _sb(t[0][:H], t[1][:H], t[0][H:], t[1][H:])):
                dst[k, :, col(u)] = _pk(v)
    assert not sched.queue
    dwf = dw[...].astype(F32)
    for k in range(K):
        dwb[k] = jnp.broadcast_to(dwf[k:k + 1, :], (8, D))

    def conv_block(p, r0, c, done, CT=CT, AT=K):
        cs = col(c)
        acc = [None]

        def item(k0, z=None):
            for k in range(k0, min(k0 + CT, K)):
                off = HALO - K // 2 + k + r0
                w = dwb[k, :, cs]
                if z is not None and k - k0 < AT:
                    w = w + z.v()
                t = gs[p + 1, c, off:off + 8, :] * w
                acc[0] = t if acc[0] is None else acc[0] + t
            if k0 + CT >= K:
                dcs[rows(p, r0, 8), cs] = acc[0]
                done(acc[0])

        return [functools.partial(item, k0) for k0 in range(0, K, CT)]

    def conv_main(p, cols=range(NCB), **kw):
        st = []

        def stats(r0, c, acc):
            if r0 == 0:
                st[:] = [acc, None, None]
                return
            shift, s1, s2 = st
            d = acc - shift
            s1 = d if s1 is None else s1 + d
            s2 = d * d if s2 is None else s2 + d * d
            st[:] = [shift, s1, s2]
            if r0 + 16 == TM:
                dm = s1 * (1.0 / (TM // 8 - 1))
                st_mean[p, :, col(c)] = shift + dm
                st_m2[p, :, col(c)] = s2 - s1 * dm

        return [it for c in cols for r0 in range(0, TM - 8, 8)
                for it in conv_block(p, r0, c,
                                     functools.partial(stats, r0, c), **kw)]

    def conv_edge(p, cols=range(NCB)):
        return [it for c in cols
                for it in conv_block(p, TM - 8, c, lambda acc: None)]


    def phase_b(i, carry):
        b = i // tpb

        sched = _Sched(zero)
        sched.add(conv_edge(jnp.maximum(i - 2, 0))
                  + conv_main(jnp.maximum(i - 1, 0), range(L0, NCB)),
                  int(B_SLOTS[0] * TM), int(B_SLOTS[1] * TM))
        sched.add(q_items(jnp.minimum(i + 1, nt - 1)),
                  int(Q_SLOTS[0] * TM), int(Q_SLOTS[1] * TM))
        acc = [None] * 4
        for k in OQ:
            t = _dot(get7(hq7, k), _up(mq[k]))
            _acc7(acc, k, t, HM)
            sched(t)
        q11, q12, q21, q22 = _quads(
            jnp.concatenate(_join(acc, HM), axis=1), HM)
        q7 = [q11[:HM] - q22[:HM], q21 - q22, q11, q22, q12 - q11,
              q21[:HM] - q11[:HM], q12[:HM] - q22[:HM]]
        q7 = [t.astype(BF16) for t in q7]

        dz = zero_s[0]
        p_buf, al_buf = (p_buf0, p_buf1, p_buf2), (al_buf0, al_buf1, al_buf2)
        s_buf = (s_buf0, s_buf1)

        def dyn(r0, n):
            return pl.ds(pl.multiple_of(dz + r0, 8), n)

        nb = KP // 128

        def chunk(j):
            return pl.ds(pl.multiple_of(b * (TP // 2), KP // 2)
                         + j * KP // 2, KP // 2)

        def combine(m, j, c):
            if len(m) == 7:
                s = [m[0] + m[3] + m[4] + m[6], m[2] + m[4],
                     m[1] + m[3], m[1] - m[0] + m[2] + m[5]]
            else:
                s = [m[0] + m[2], m[1] + m[3]]
            nv = T // 2 - j * KP - c * 128
            if nv < 128:
                lane = lax.broadcasted_iota(jnp.int32, s[0].shape, 1)
                s = [jnp.where(lane < nv, t, -jnp.inf) for t in s]
            return s

        stat = {}

        def put(w, j, r, v):
            for r0 in range(0, v.shape[0], 16):
                stat[w, j, r + r0] = v[r0:r0 + 16]

        def get(w, j, r, n=16):
            return jnp.concatenate(
                [stat[w, j, r0] for r0 in range(r, r + n, 16)], axis=0)

        def scores(j):
            m = [None] * 7
            for k in OS if j else OS0:
                m[k] = _dot_nt(
                    q7[k], _up(ks[(0, 2, 1, 4, 3, 5, 6)[k], chunk(j), :]))
                sched(m[k])
            mx = None
            for c in range(nb):
                s = combine([t[:HM, col(c)] for t in m], j, c)
                e = combine([t[HM:, col(c)] for t in m[1:5]], j, c)
                for h in range(2):
                    t = jnp.concatenate([s[h], s[2 + h], e[h]], axis=0)
                    s_buf[j % 2][:, col(h * nb + c)] = t
                    mx = t if mx is None else jnp.maximum(mx, t)
            mx = jnp.broadcast_to(jnp.max(mx, axis=-1, keepdims=True),
                                  mx.shape)
            if j:
                mx = jnp.maximum(mx, get(0, j - 1, 0, TM))
            put(0, j, 0, mx)

        part = {}

        def soft1(j, r, c0, z):
            rs = slice(r, r + 16)
            m = get(0, j, r) + _rep(z.v(), 16)
            l = functools.reduce(jnp.add, part.pop((j, r), []) + [
                jnp.exp2(s_buf[j % 2][dyn(r, 16), col(c)] - m)
                for c in range(c0, c0 + S1)])
            if c0 + S1 < 2 * nb:
                part[j, r] = [l]
                return
            l = jnp.broadcast_to(jnp.sum(l, axis=-1, keepdims=True),
                                 (16, 128))
            if j:
                l += get(1, j - 1, r) * jnp.exp2(get(0, j - 1, r) - m)
            put(1, j, r, l)
            e = (pltpu.bitcast(l, jnp.int32) >> 23) - 127
            ref = m + e.astype(F32)
            put(2, j, r, ref)
            if j:
                al_buf[j % 3][rs, :] = jnp.exp2(get(2, j - 1, r) - ref)

        def soft2(j, r0, c0, z):
            ref = [get(2, j, r) + _rep(z.v(), 16) for r in groups(r0)]
            p = [jnp.concatenate(
                [jnp.exp2(s_buf[j % 2][dyn(r, 16), col(h * nb + c)] - m)
                 for c in range(c0, c0 + S2)], axis=1)
                 for r, m in zip(groups(r0), ref) for h in range(2)]
            put7(p_buf[j % 3], r0, slice(c0 * 128, (c0 + S2) * 128), *p)

        scd = 7 * HM + 4 * (TM - 2 * HM)
        start = sched.now

        def add_soft(j):
            rbs = range(0, TM - HM, 16)
            t0, t1 = (start + int(t * scd) for t in SW[j:j + 2])
            assert t1 <= start + min(2 * j + LAG + 1, nkc + j) * scd
            assert j < 3 or t0 >= start + min(2 * j + LAG - 4,
                                              nkc + j - 2) * scd
            assert (j + 2 >= nkc
                    or t1 <= start + max(2 * j + 5 - LAG, j + 3) * scd)
            u = (t1 - t0 - sum(SD)) // (len(rbs) + 1)
            for n, r0 in enumerate(rbs):
                its = [[functools.partial(soft1, j, r, c)
                        for r in groups(r0) for c in range(0, 2 * nb, S1)],
                       [functools.partial(soft2, j, r0, c)
                        for c in range(0, nb, S2)]]
                for k, it in enumerate(its):
                    t = t0 + SD[0] + n * u + k * (u + SD[1])
                    sched.add(it, t, t + u)

        for j in range(LAG):
            scores(j)
            add_soft(j)
        acc = [None] * 4
        for j in range(nkc):
            if j + LAG < nkc:
                scores(j + LAG)
                add_soft(j + LAG)
            fresh = [j > 0] * 4
            for k in OP if j + 1 < nkc else OQ:
                w = _up(ks[(0, 2, 6, 5, 3, 4, 1)[k], chunk(j), :])
                m = _dot(get7(p_buf[j % 3], k, dyn), w)
                sched(m)
                for a, _ in _TG[k]:
                    if fresh[a]:
                        al = al_buf[j % 3][dyn(0, TM), :]
                        al = _quads(jnp.concatenate([al] * NCB, axis=1), HM)[a]
                        acc[a] = acc[a] * al[:acc[a].shape[0]]
                        fresh[a] = False
                _acc7(acc, k, m, HM)
        assert not sched.queue
        t = jnp.exp2(get(2, nkc - 1, 0, TM) - get(0, nkc - 1, 0, TM))
        t = t / get(1, nkc - 1, 0, TM)
        o = (jnp.concatenate(_join(acc, HM), axis=1)
             * jnp.concatenate([t] * NCB, axis=1))
        o7 = [t.astype(BF16) for t in _sax(*_quads(o, HM), HM)]
        acc = list(_quads(xs[rows(i), :], HM))
        acc = [acc[0][:HM], acc[1], acc[2], acc[3][:HM]]
        for k in OW:
            _acc7(acc, k, _dot(o7[k], _up(wvo[k])), HM)
        x2 = jnp.concatenate(_join(acc, HM), axis=1)
        xs[rows(i), :] = x2
        h7 = [t.astype(BF16) for t in _sax(*_quads(_ln(x2), HM), HM)]
        sched = _Sched(zero)
        acc = [[None] * 4 for _ in range(2)]
        for n, (h, k) in enumerate(PO):
            t = _dot(h7[k], _up(w7[h, k]))
            _acc7(acc[h], k, t, HM)
            sched(t)
            if any(e[0] == h for e in PO[n + 1:]):
                continue
            val, gate = _join(acc[h], HM)
            g2 = val * (0.5 + 0.5 * jnp.tanh(0.5 * gate))
            for c in (2 * h, 2 * h + 1):
                g = g2[:, col(c % 2)]
                gs[i + 1, c, HALO:HALO + TM, :] = g
                gs[i, c, HALO + TM:, :] = jnp.where(
                    i % tpb == 0, 0.0, g[:HALO])
                gs[i + 2, c, :HALO, :] = jnp.where(
                    i % tpb == tpb - 1, 0.0, g[TM - HALO:])
            if h == 0 and L0:
                rest = sum(h7[e[1]].shape[0] for e in PO[n + 1:])
                sched.add(conv_main(i, range(L0), CT=LP[2], AT=LP[3]),
                          sched.now + LP[0], sched.now + rest - LP[1])
        assert not sched.queue
        return carry

    with jax.named_scope("phase_b"):
        lax.fori_loop(0, nt, phase_b, 0)
    for item in (conv_main(nt - 1, range(L0, NCB)) + conv_edge(nt - 2)
                 + conv_edge(nt - 1)):
        item()

    ng = TM // 8 - 1
    means = st_mean[...].reshape(nt * 8, D)
    edges = jnp.concatenate([dcs[(p + 1) * TM - 8:(p + 1) * TM, :]
                             for p in range(nt)], axis=0)
    mu = jnp.sum(ng * means + edges, axis=0, keepdims=True) * (1.0 / N)
    dm = means - mu
    de = edges - mu
    var = jnp.sum(st_m2[...].reshape(nt * 8, D) + ng * (dm * dm) + de * de,
                  axis=0, keepdims=True) * (1.0 / N)
    rstd = lax.rsqrt(var + EPS)
    bn[0] = jnp.broadcast_to(mu, (8, D))
    bn[1] = jnp.broadcast_to(rstd, (8, D))

    def bn_silu(i, r0, c, z=None):
        p = []
        for r in (r0, TC // 2 + r0):
            for h in range(2):
                cs = col(2 * h + c)
                mu = bn[0, :, cs] if z is None else bn[0, :, cs] + z.v()
                y = dcs[crows(i, r, 16), cs] - _rep(mu, 16)
                p.append(_silu(y * _rep(bn[1, :, cs], 16)))
        put7(hq7, r0, col(c), *p)

    def bn_items(i):
        return [functools.partial(bn_silu, i, r0, c)
                for r0 in range(0, TC // 2, 16) for c in range(2)]

    def ln_final(i, r0=0, n=TC, z=None):
        obuf[crows(i, r0, n), :] = _ln(xs[crows(i, r0, n), :],
                                       zrep(z, n)).astype(BF16)

    for item in bn_items(0):
        item()

    QC = TC // 4

    def pw2(src, dst, sched, win):
        acc = list(_quads(xs[crows(src), :], TC // 2))
        for k in OQ:
            t = _dot(get7(hq7, k, nr=TC // 2), _up(w7[2, k]))
            _acc7(acc, k, t, TC // 2)
            sched(t)
        xs[crows(dst), :] = jnp.concatenate(_join(acc, TC // 2), axis=1)
        for items, t0, t1 in zip(
                ln_in(xs, dst * TC, QC, range(0, QC, 16)), win, win[1:]):
            sched.add(items, sched.now + t0, sched.now + t1)

    sched = _Sched(zero)
    pw2(0, 0, sched, (0, 1, 2))
    sched.force([e[1] for e in sched.queue])

    def phase_c(i, carry):
        @pl.when(i >= 2)
        def _():
            o_copy(i - 2).start()

        sched = _Sched(zero)
        dur = (7 * 8 + 49 * 2 * nfc) * TC // 16
        sched.add([functools.partial(ln_final, jnp.maximum(i - 1, 0), r, RC)
                   for r in range(0, TC, RC)],
                  int(C_WIN[0] * dur), int(C_WIN[1] * dur))
        nxt = jnp.minimum(i + 1, nc - 1)
        items = bn_items(nxt)
        sched.add(items, int(C_WIN[2] * dur), int(C_WIN[3] * dur))
        done = []

        def mid():
            sched.force(items)
            done.append(1)
            pw2(nxt, jnp.where(i + 1 < nc, i + 1, 0), sched, M_WIN)

        def h49(k):
            assert not done
            return _up(lhs49[k // 2, :QC // 2, col(k % 2)])

        f = _ffn49(h49, QC, lambda k, b, n: _up(
            w49[k // 2, b * 64:(b + n) * 64, col(k % 2)]),
            nfc, sched, *FB, sb, GC, mid)
        assert not sched.queue
        xs[crows(i), :] += 0.5 * f
        return carry

    with jax.named_scope("phase_c"):
        lax.fori_loop(0, nc, phase_c, 0)
    o_copy(nc - 2).start()
    last = []
    for k, (r0, r1) in enumerate(zip(EP[:-1], EP[1:])):
        ln_final(nc - 1, r0, r1 - r0)
        rs = crows(nc - 1, r0, r1 - r0)
        last.append(pltpu.make_async_copy(obuf.at[rs, :], out_hbm.at[rs, :],
                                          osem.at[nc - 1 + k]))
        last[-1].start()
    for i in range(nc - 1):
        o_copy(i).wait()
    for cp in last:
        cp.wait()


@jax.jit
def pallas_standalone__conformer_family_conformer__speech_kernel(
    x: jax.Array,
    w_ff1_a: jax.Array,
    w_ff1_b: jax.Array,
    w_q: jax.Array,
    w_k: jax.Array,
    w_v: jax.Array,
    w_o: jax.Array,
    w_pw1: jax.Array,
    dw: jax.Array,
    w_pw2: jax.Array,
    w_ff2_a: jax.Array,
    w_ff2_b: jax.Array,
):
    B, T, D = x.shape
    K = dw.shape[0]
    N = B * T
    weights = (w_ff1_a, w_ff1_b, w_q, w_k, w_v, w_o, w_pw1, dw, w_pw2,
               w_ff2_a, w_ff2_b)
    scratch = [pltpu.VMEM((N, D), BF16)]
    nfc = w_ff1_a.shape[1] // FC
    scratch += [pltpu.VMEM((4 * nfc + 3, D, D), BF16)]
    scratch += [pltpu.VMEM(w.shape, w.dtype)
                for w in (w_q, w_k, w_v, w_o, dw)]
    scratch += [
        pltpu.VMEM((7, D // 4, D // 2), jnp.uint32),
        pltpu.VMEM((7, D // 4, D // 2), jnp.uint32),
        pltpu.VMEM((N, D), F32),
        pltpu.VMEM((N, D), BF16),
        pltpu.VMEM((7, B * -(-T // KC) * KC // 4, D // 2), jnp.uint32),
        pltpu.VMEM((N // TM + 2, D // 128, TM + 2 * HALO, 128), F32),
        pltpu.VMEM((N, D), F32),
        pltpu.VMEM((N // TM, 8, D), F32),
        pltpu.VMEM((N // TM, 8, D), F32),
        pltpu.VMEM((2, 8, D), F32),
        pltpu.VMEM((25, TA // 8, D // 2), jnp.uint32),
        pltpu.VMEM((7, 14 * TA // 8, D // 2), jnp.uint32),
        pltpu.VMEM((3, 7, D // 4, D // 2), jnp.uint32),
        pltpu.VMEM((25, nfc * D // 4, D // 2), jnp.uint32),
        pltpu.VMEM((T0, D), BF16),
        pltpu.VMEM((K, 8, D), F32),
        pltpu.VMEM((ZR, 128), jnp.uint32),
        pltpu.SMEM((1,), jnp.int32),
        pltpu.VMEM((TM + 16, 128), F32),
        pltpu.VMEM((TM + 16, 128), F32),
        pltpu.VMEM((TM + 16, 128), F32),
        pltpu.VMEM((7 * PR, KC // 2), jnp.uint32),
        pltpu.VMEM((7 * PR, KC // 2), jnp.uint32),
        pltpu.VMEM((7 * PR, KC // 2), jnp.uint32),
        pltpu.VMEM((TM, KC), F32),
        pltpu.VMEM((TM, KC), F32),
        pltpu.VMEM((7 * PR, D // 2), jnp.uint32),
        pltpu.SemaphoreType.DMA(((N - T0) // TA + 1,)),
        pltpu.SemaphoreType.DMA((2, nfc)),
        pltpu.SemaphoreType.DMA((3, nfc)),
        pltpu.SemaphoreType.DMA((6,)),
        pltpu.SemaphoreType.DMA((N // TC + len(EP),)),
    ]
    out = pl.pallas_call(
        functools.partial(_kernel, B=B, T=T, D=D, K=K),
        out_shape=jax.ShapeDtypeStruct((N, D), x.dtype),
        in_specs=[pl.BlockSpec(memory_space=pl.ANY)] * 12,
        out_specs=pl.BlockSpec(memory_space=pl.ANY),
        scratch_shapes=scratch,
        compiler_params=pltpu.CompilerParams(
            vmem_limit_bytes=128 * 1024 * 1024),
    )(x.reshape(N, D), *weights)
    return out.reshape(B, T, D)
```
